```python
import jax
import jax.numpy as jnp

def _softmax(x, axis=-1):
    return jax.nn.softmax(x, axis=axis)

def _gelu(x):
    return jax.nn.gelu(x, approximate=True)

def _silu(x):
    return jax.nn.silu(x)

def _sigmoid(x):
    return jax.nn.sigmoid(x)

def _layernorm(x, axis=-1, eps=1e-05):
    m = jnp.mean(x, axis=axis, keepdims=True)
    v = jnp.var(x, axis=axis, keepdims=True)
    return (x - m) / jnp.sqrt(v + eps)

def _scatter_add(tgt, idx, src, axis=0):
    return tgt.at[idx].add(src)

def _segment_sum(src, seg, n):
    return jax.ops.segment_sum(src, seg, n)

class _Rng:

    def __init__(self, key):
        self._k = key

    def _next(self):
        self._k, sub = jax.random.split(self._k)
        return sub

    def normal(self, shape):
        return jax.random.normal(self._next(), shape, dtype=jnp.bfloat16)

    def randint(self, lo, hi, shape):
        return jax.random.randint(self._next(), shape, lo, hi, dtype=jnp.int32)

    def uniform(self, shape, lo=0.0, hi=1.0):
        return jax.random.uniform(self._next(), shape, jnp.bfloat16, lo, hi)

    def permutation(self, n):
        return jax.random.permutation(self._next(), n)
kernel_name = 'recurrent_scan__memory_aug_recurrent_mem_tr__moe_arch_mod__prompt'

def setup_inputs():
    _rng = _Rng(jax.random.key(int.from_bytes(__import__("os").urandom(4), "little")))
    _w = lambda a: (lambda t: t.astype(jnp.bfloat16) if jnp.issubdtype(t.dtype, jnp.floating) else t)(jnp.asarray(a))

    def _A_setup():
        B, S, Dm = (1, 2048, 640)
        H, Dh = (32, 128)
        M, seg = (8, 32)
        seg = min(seg, S)
        S = S // seg * seg
        return {'x': _w((lambda *s: _rng.normal(s) * 0.05)(B, S, Dm)), 'mem0': _w((lambda *s: _rng.normal(s) * 0.05)(B, M, Dm)), 'Wq': _w((lambda *s: _rng.normal(s) * 0.05)(Dm, H, Dh) * Dm ** (-0.5)), 'Wk': _w((lambda *s: _rng.normal(s) * 0.05)(Dm, H, Dh) * Dm ** (-0.5)), 'Wv': _w((lambda *s: _rng.normal(s) * 0.05)(Dm, H, Dh) * Dm ** (-0.5)), 'Wo': _w((lambda *s: _rng.normal(s) * 0.05)(H, Dh, Dm) * (H * Dh) ** (-0.5)), 'seg_len': seg}
    _A_in = _A_setup()

    def _B_setup():
        B, S, D, F, C = (1, 2048, 640, 1728, 8)
        return {'x': _w((lambda *s: _rng.normal(s) * 0.05)(B, S, D)), 'w_r': _w((lambda *s: _rng.normal(s) * 0.05)(D)), 'w_gate': _w((lambda *s: _rng.normal(s) * 0.05)(D, F)), 'w_up': _w((lambda *s: _rng.normal(s) * 0.05)(D, F)), 'w_down': _w((lambda *s: _rng.normal(s) * 0.05)(F, D))}
    _B_in = _B_setup()
    return {'A_x': _A_in['x'], 'A_mem0': _A_in['mem0'], 'A_Wq': _A_in['Wq'], 'A_Wk': _A_in['Wk'], 'A_Wv': _A_in['Wv'], 'A_Wo': _A_in['Wo'], 'A_seg_len': _A_in['seg_len'], 'B_x': _B_in['x'], 'B_w_r': _B_in['w_r'], 'B_w_gate': _B_in['w_gate'], 'B_w_up': _B_in['w_up'], 'B_w_down': _B_in['w_down']}

def reference(A_x, A_mem0, A_Wq, A_Wk, A_Wv, A_Wo, A_seg_len, B_x, B_w_r, B_w_gate, B_w_up, B_w_down):

    def _A_ref(x, mem0, Wq, Wk, Wv, Wo, seg_len):
        B, S, Dm = x.shape
        H, Dh = (Wq.shape[1], Wq.shape[2])
        M = mem0.shape[1]
        scale = Dh ** (-0.5)
        n_seg = S // seg_len
        L = M + seg_len
        idx = jnp.arange(L)
        mask = (idx[:, None] < M) | (idx[:, None] >= idx[None, :])
        mem = mem0
        outs = []
        for s in range(n_seg):
            xs = x[:, s * seg_len:(s + 1) * seg_len, :].copy()
            h = jnp.concatenate([mem, xs], axis=1)
            q = jnp.einsum('btd,dhe->bhte', h, Wq)
            k = jnp.einsum('btd,dhe->bhte', h, Wk)
            v = jnp.einsum('btd,dhe->bhte', h, Wv)
            scores = jnp.einsum('bhqe,bhke->bhqk', q, k) * scale
            scores = jnp.where(mask[None, None], scores, -1000000000.0)
            p = _softmax(scores, axis=-1)
            o = jnp.einsum('bhqk,bhke->bhqe', p, v)
            o = jnp.einsum('bhte,hed->btd', o, Wo)
            mem = o[:, :M, :].copy()
            outs.append(o[:, M:, :])
        return jnp.concatenate(outs, axis=1)

    def _B_ref(x, w_r, w_gate, w_up, w_down):
        B, S, D = x.shape
        C = 8
        r = x @ w_r
        idx = jnp.argsort(-r, axis=-1)[:, :C]
        idx_e = jnp.repeat(idx.reshape(B, C, 1), D, axis=2)
        x_sel = jnp.take_along_axis(x, idx_e, axis=1)
        g = _silu(x_sel @ w_gate)
        u = x_sel @ w_up
        y = g * u @ w_down
        r_sel = _sigmoid(jnp.take_along_axis(r, idx, axis=1))
        y = y * r_sel.reshape(B, C, 1)
        b_off = (jnp.arange(B) * S).reshape(B, 1)
        flat_idx = (idx + b_off).reshape(B * C)
        zero = (x * 0.0).reshape(B * S, D)
        upd = _scatter_add(zero, flat_idx, y.reshape(B * C, D), axis=0)
        return x + upd.reshape(B, S, D)
    x = A_x
    xn = _layernorm(x, axis=-1)
    s = _A_ref(xn, A_mem0, A_Wq, A_Wk, A_Wv, A_Wo, A_seg_len)
    g = _silu(_B_ref(xn, B_w_r, B_w_gate, B_w_up, B_w_down))
    return x + s * g
```

```python
import functools
import math

import jax
import jax.numpy as jnp
import jax.experimental.pallas as pl
import jax.experimental.pallas.tpu as pltpu

F32 = jnp.float32
BF16 = jnp.bfloat16
U32 = jnp.uint32
I32 = jnp.int32

S = 2048
D = 640
H = 32
DH = 128
M = 8
SEG = 32
NSEG = S // SEG
L = M + SEG
FF = 1728
TOPC = 8
NT = D // 128
LIVE = SEG - 8
EPS = 1e-05
NEG = -1000000000.0
GH = 2


def _dot(a, b):
    return jax.lax.dot_general(a, b, (((1,), (0,)), ((), ())), preferred_element_type=F32)


def _dot_nt(a, b):
    return jax.lax.dot_general(a, b, (((1,), (1,)), ((), ())), preferred_element_type=F32)


def _rb(x):
    return x.astype(BF16).astype(F32)


def _sigmoid(x):
    return 1.0 / (1.0 + jnp.exp(-x))


def _kernel(x_hbm, mem0_ref, wq_hbm, wk_hbm, wv_hbm, wo_hbm, wr_ref, wg_hbm, wu_hbm, wd_hbm,
            out_hbm,
            x_v, xn_v, xb_v, raw, wp, wo_p, pre, wg_v, wu_v, wd_v, out_v, acc, o_s, sel, keys,
            sem_x, sem_w, sem_o, sem_m, sem_out):
    cp_x = pltpu.make_async_copy(x_hbm, x_v, sem_x.at[0])
    cp_x.start()
    w_hbm = [wq_hbm, wk_hbm, wv_hbm]

    def w_copy(i):
        m, c, par = i // 4, (i // 2) % 2, i % 2
        src = w_hbm[m].bitcast(U32).at[:, pl.ds(par * 16 + c * 8, 8), :]
        dst = raw.at[pl.ds(i * 2560, 2560), :].reshape(320, 8, 128)
        return pltpu.make_async_copy(src, dst, sem_w.at[i])

    for i in range(12):
        w_copy(i).start()
    mlp_copies = [pltpu.make_async_copy(s_, d_, sem_m.at[i])
                  for i, (s_, d_) in enumerate([(wg_hbm, wg_v), (wu_hbm, wu_v), (wd_hbm, wd_v)])]
    for c in mlp_copies:
        c.start()
    wo32 = wo_hbm.bitcast(U32)
    wo_copies = [pltpu.make_async_copy(wo32.at[:, pl.ds(j * 128, 128)], wo_p.at[j], sem_o.at[j])
                 for j in range(NT)]
    for c in wo_copies:
        c.start()

    cp_x.wait()
    wr5 = wr_ref[...].astype(F32)
    wr = jnp.concatenate([wr5[j:j + 1, :] for j in range(NT)], axis=1)
    LNB = 64
    lane = jax.lax.broadcasted_iota(I32, (LNB, 128), 1)
    rowi = jax.lax.broadcasted_iota(I32, (LNB, 128), 0)
    keys[...] = jnp.full((LNB, 128), jnp.iinfo(jnp.int32).min, I32)

    def ln_body(b, carry):
        r0 = pl.multiple_of(b * LNB, LNB)
        x = x_v[pl.ds(r0, LNB), :].astype(F32)
        mu = jnp.sum(x, axis=-1, keepdims=True) * (1.0 / D)
        xc = x - mu
        var = jnp.sum(xc * xc, axis=-1, keepdims=True) * (1.0 / D)
        sd = _rb(jnp.sqrt(_rb(_rb(var) + EPS)))
        xn = _rb(_rb(x - _rb(mu)) / sd)
        xn_v[pl.ds(r0, LNB), :] = xn
        xb_v[pl.ds(r0, LNB), :] = xn
        r = _rb(jnp.sum(xn * wr, axis=-1, keepdims=True))
        r = jnp.where(r == 0.0, 0.0, r)
        bits = pltpu.bitcast(jnp.broadcast_to(r, (LNB, 128)), I32) >> 16
        mono = jnp.where(bits < 0, (-32768) - bits, bits)
        mono = jnp.where(r != r, -40000, mono)
        key = mono * 4096 + (S - 1 - (r0 + rowi))
        keys[...] = jnp.where(lane == b, key, keys[...])
        return carry

    jax.lax.fori_loop(0, S // LNB, ln_body, 0)

    kv = keys[...]
    idxs = []
    for c in range(TOPC):
        mx = jnp.max(kv)
        kv = jnp.where(kv == mx, jnp.iinfo(jnp.int32).min, kv)
        idx = (S - 1) - (mx & 4095)
        idx = jnp.clip(idx, 0, S - 1)
        idxs.append(idx)
        sel[pl.ds(c, 1), :] = xn_v[pl.ds(idx, 1), :]

    def repack(ch, t, nblk):
        for gg in range(nblk):
            g = t * nblk + gg
            be = pl.multiple_of(ch * 5120 + g * 64, 64)
            bo = pl.multiple_of(ch * 5120 + 2560 + g * 64, 64)
            ev = raw.at[pl.ds(be, 64), :]
            od = raw.at[pl.ds(bo, 64), :]
            ob = pl.multiple_of(g * 8, 8)
            for p in range(8):
                a = ev[pl.ds(p, 8, stride=8), :]
                b = od[pl.ds(p, 8, stride=8), :]
                wp[ch * 16 + 2 * p, pl.ds(ob, 8), :] = (a & jnp.uint32(0xFFFF)) | (b << 16)
                wp[ch * 16 + 2 * p + 1, pl.ds(ob, 8), :] = (a >> 16) | (b & jnp.uint32(0xFFFF0000))

    xn3 = xn_v.reshape(NSEG, SEG, D)

    def pre_proj(j):
        w = pltpu.bitcast(wp[j], BF16)
        for c in range(4):
            lhs = xn3[c * 16:(c + 1) * 16, LIVE:SEG, :].reshape(128, D)
            pre[j, c * 128:(c + 1) * 128, :] = _dot(lhs, w)

    PH = 4
    NIT = 16 // PH
    w_copy(0).wait()
    w_copy(1).wait()
    jax.lax.fori_loop(0, 8, lambda t, c: (repack(0, t, 5), c)[1], 0)
    for ch in range(6):
        if ch + 1 < 6:
            w_copy(2 * ch + 2).wait()
            w_copy(2 * ch + 3).wait()

        def pro_body(t, carry, ch=ch):
            if ch + 1 < 6:
                repack(ch + 1, t, 40 // NIT)
            for u in range(PH):
                pre_proj(ch * 16 + t * PH + u)
            return carry

        jax.lax.fori_loop(0, NIT, pro_body, 0)

    for c in mlp_copies:
        c.wait()
    xs = sel[...]
    gate = _rb(_dot_nt(xs, wg_v[...]))
    up = _rb(_dot_nt(xs, wu_v[...]))
    hmid = _rb(gate * _sigmoid(gate)) * up
    y = _rb(_dot(hmid, wd_v[...]))
    r_sel = _rb(jnp.sum(xs * wr, axis=-1, keepdims=True))
    xnew = xs + _rb(y * _rb(_sigmoid(r_sel)))
    sel[...] = xnew
    for c in range(TOPC):
        xb_v[pl.ds(idxs[c], 1), :] = sel[pl.ds(c, 1), :]

    for c in wo_copies:
        c.wait()
    acc[0:M, :] = mem0_ref[...].astype(F32)
    acc[M:L, :] = jnp.zeros((SEG, D), F32)

    qi = jax.lax.broadcasted_iota(I32, (L, L), 0)
    ki = jax.lax.broadcasted_iota(I32, (L, L), 1)
    mask = (qi < M) | (qi >= ki)
    scale = DH ** (-0.5)

    def finish(sp):
        r0 = pl.multiple_of(sp * SEG, SEG)
        sa = acc[M:L, :]
        xb = xb_v[pl.ds(r0, SEG), :]
        g = xb * _sigmoid(xb)
        out_v[pl.ds(r0, SEG), :] = (x_v[pl.ds(r0, SEG), :].astype(F32) + sa * g).astype(BF16)

    def out_copy(r0, n):
        return pltpu.make_async_copy(out_v.at[pl.ds(r0, n), :], out_hbm.at[pl.ds(r0, n), :], sem_out.at[0])

    def step(s, carry):
        r0 = pl.multiple_of(s * SEG, SEG)
        p0 = pl.multiple_of(s * 8, 8)
        lhs = jnp.concatenate([acc[0:M, :], xn_v[pl.ds(r0, LIVE), :]], axis=0)
        finish(jnp.maximum(s - 1, 0))

        def proj(j):
            t = _dot(lhs, pltpu.bitcast(wp[j], BF16))
            return jnp.concatenate([t, pre[j, pl.ds(p0, 8), :]], axis=0)

        NG = H // GH
        qs, ks, vs, ps, ls = {}, {}, {}, {}, {}
        for g in range(NG + 2):
            if g < NG:
                for h in range(g * GH, (g + 1) * GH):
                    qs[h] = proj(h)
                    ks[h] = proj(H + h)
                    vs[h] = proj(2 * H + h)
            if 1 <= g <= NG:
                for h in range((g - 1) * GH, g * GH):
                    sc = _dot_nt(qs.pop(h), ks.pop(h)) * scale
                    sc = jnp.where(mask, sc, NEG)
                    e = jnp.exp(sc - jnp.max(sc, axis=-1, keepdims=True))
                    ps[h] = e
                    ls[h] = jnp.sum(e, axis=-1, keepdims=True)
            if g >= 2:
                for h in range((g - 2) * GH, (g - 1) * GH):
                    o = _dot(ps.pop(h), vs.pop(h))
                    o_s[:, h * DH:(h + 1) * DH] = o * (1.0 / ls.pop(h))
        KS = (H - 4) * DH
        for j in range(NT):
            a = _dot(o_s[:, 0:KS], pltpu.bitcast(wo_p[j, 0:KS // 2, :], BF16))
            acc[:, j * 128:(j + 1) * 128] = a
        for j in range(NT):
            a = _dot(o_s[:, KS:], pltpu.bitcast(wo_p[j, KS // 2:, :], BF16))
            acc[:, j * 128:(j + 1) * 128] += a
        return carry

    OC = 8
    for blk in range(1):
        pass

    def outer(b, carry):
        jax.lax.fori_loop(b * OC, (b + 1) * OC, step, 0)

        @pl.when(b > 0)
        def _():
            out_copy(pl.multiple_of((b - 1) * OC * SEG, OC * SEG), OC * SEG).start()
        return carry

    jax.lax.fori_loop(0, NSEG // OC, outer, 0)
    finish(NSEG - 1)
    out_copy(S - OC * SEG, OC * SEG).start()
    out_copy(0, S).wait()


@jax.jit
def pallas_recurrent_scan__memory_aug_recurrent_mem_tr__moe_arch_mod__prompt_kernel(
    A_x: jax.Array,
    A_mem0: jax.Array,
    A_Wq: jax.Array,
    A_Wk: jax.Array,
    A_Wv: jax.Array,
    A_Wo: jax.Array,
    A_seg_len: jax.Array,
    B_x: jax.Array,
    B_w_r: jax.Array,
    B_w_gate: jax.Array,
    B_w_up: jax.Array,
    B_w_down: jax.Array,
):
    del A_seg_len, B_x
    assert A_x.shape == (1, S, D) and A_Wq.shape == (D, H, DH) and A_mem0.shape == (1, M, D)
    hbm = pl.BlockSpec(memory_space=pltpu.HBM)
    vmem = pl.BlockSpec(memory_space=pltpu.VMEM)
    wview = lambda w: w.reshape(D // 2, 2 * H, DH)
    out = pl.pallas_call(
        _kernel,
        out_shape=jax.ShapeDtypeStruct((S, D), BF16),
        in_specs=[hbm, vmem, hbm, hbm, hbm, hbm, vmem, hbm, hbm, hbm],
        out_specs=hbm,
        scratch_shapes=[
            pltpu.VMEM((S, D), BF16),
            pltpu.VMEM((S, D), F32),
            pltpu.VMEM((S, D), F32),
            pltpu.VMEM((12 * 2560, 128), U32),
            pltpu.VMEM((3 * H, D // 2, 128), U32),
            pltpu.VMEM((NT, H * DH // 2, 128), U32),
            pltpu.VMEM((3 * H, NSEG * 8, DH), F32),
            pltpu.VMEM((FF, D), BF16),
            pltpu.VMEM((FF, D), BF16),
            pltpu.VMEM((FF, D), BF16),
            pltpu.VMEM((S, D), BF16),
            pltpu.VMEM((L, D), F32),
            pltpu.VMEM((L, H * DH), F32),
            pltpu.VMEM((TOPC, D), F32),
            pltpu.VMEM((64, 128), I32),
            pltpu.SemaphoreType.DMA((1,)),
            pltpu.SemaphoreType.DMA((12,)),
            pltpu.SemaphoreType.DMA((NT,)),
            pltpu.SemaphoreType.DMA((3,)),
            pltpu.SemaphoreType.DMA((1,)),
        ],
        compiler_params=pltpu.CompilerParams(vmem_limit_bytes=110 * 1024 * 1024),
    )(
        A_x.reshape(S, D),
        A_mem0.reshape(M, D),
        wview(A_Wq), wview(A_Wk), wview(A_Wv),
        A_Wo.reshape(H * DH, D),
        B_w_r.reshape(NT, 128),
        B_w_gate.T, B_w_up.T, B_w_down,
    )
    return out.reshape(1, S, D)
```

```python
import functools
import math

import jax
import jax.numpy as jnp
import jax.experimental.pallas as pl
import jax.experimental.pallas.tpu as pltpu

F32 = jnp.float32
BF16 = jnp.bfloat16
U32 = jnp.uint32
I32 = jnp.int32

S = 2048
D = 640
H = 32
DH = 128
M = 8
SEG = 32
NSEG = S // SEG
L = M + SEG
FF = 1728
TOPC = 8
NT = D // 128
LIVE = SEG - 8
EPS = 1e-05
NEG = -1000000000.0
GH = 2


def _dot(a, b):
    return jax.lax.dot_general(a, b, (((1,), (0,)), ((), ())), preferred_element_type=F32)


def _dot_nt(a, b):
    return jax.lax.dot_general(a, b, (((1,), (1,)), ((), ())), preferred_element_type=F32)


def _rb(x):
    return x.astype(BF16).astype(F32)


def _sigmoid(x):
    return 1.0 / (1.0 + jnp.exp(-x))


def _kernel(x_hbm, mem0_ref, wq_hbm, wk_hbm, wv_hbm, wo_hbm, wr_ref, wg_hbm, wu_hbm, wd_hbm,
            out_hbm,
            x_v, xn_v, xb_v, raw, wp, wo_p, pre, wg_v, wu_v, wd_v, out_v, acc, o_s, sel, keys,
            sem_in, sem_out):
    cp_x = pltpu.make_async_copy(x_hbm, x_v, sem_in.at[0])
    cp_x.start()
    w_hbm = [wq_hbm, wk_hbm, wv_hbm]

    def w_copy(i):
        m, c, par = i // 4, (i // 2) % 2, i % 2
        src = w_hbm[m].bitcast(U32).at[:, pl.ds(par * 16 + c * 8, 8), :]
        dst = raw.at[pl.ds(i * 2560, 2560), :].reshape(320, 8, 128)
        return pltpu.make_async_copy(src, dst, sem_in.at[1 + i])

    for i in range(12):
        w_copy(i).start()
    mlp_copies = [pltpu.make_async_copy(s_, d_, sem_in.at[13 + i])
                  for i, (s_, d_) in enumerate([(wg_hbm, wg_v), (wu_hbm, wu_v), (wd_hbm, wd_v)])]
    for c in mlp_copies:
        c.start()
    wo32 = wo_hbm.bitcast(U32)
    wo_copies = [pltpu.make_async_copy(wo32.at[:, pl.ds(j * 128, 128)], wo_p.at[j], sem_in.at[16 + j])
                 for j in range(NT)]
    for c in wo_copies:
        c.start()

    cp_x.wait()
    wr5 = wr_ref[...].astype(F32)
    wr = jnp.concatenate([wr5[j:j + 1, :] for j in range(NT)], axis=1)
    LNB = 64
    lane = jax.lax.broadcasted_iota(I32, (LNB, 128), 1)
    rowi = jax.lax.broadcasted_iota(I32, (LNB, 128), 0)
    keys[...] = jnp.full((LNB, 128), jnp.iinfo(jnp.int32).min, I32)

    def ln_body(b, carry):
        r0 = pl.multiple_of(b * LNB, LNB)
        x = x_v[pl.ds(r0, LNB), :].astype(F32)
        mu = jnp.sum(x, axis=-1, keepdims=True) * (1.0 / D)
        xc = x - mu
        var = jnp.sum(xc * xc, axis=-1, keepdims=True) * (1.0 / D)
        sd = _rb(jnp.sqrt(_rb(_rb(var) + EPS)))
        xn = _rb(_rb(x - _rb(mu)) / sd)
        xn_v[pl.ds(r0, LNB), :] = xn
        xb_v[pl.ds(r0, LNB), :] = xn
        r = _rb(jnp.sum(xn * wr, axis=-1, keepdims=True))
        r = jnp.where(r == 0.0, 0.0, r)
        bits = pltpu.bitcast(jnp.broadcast_to(r, (LNB, 128)), I32) >> 16
        mono = jnp.where(bits < 0, (-32768) - bits, bits)
        mono = jnp.where(r != r, -40000, mono)
        key = mono * 4096 + (S - 1 - (r0 + rowi))
        keys[...] = jnp.where(lane == b, key, keys[...])
        return carry

    jax.lax.fori_loop(0, S // LNB, ln_body, 0)

    kv = keys[...]
    idxs = []
    for c in range(TOPC):
        mx = jnp.max(kv)
        kv = jnp.where(kv == mx, jnp.iinfo(jnp.int32).min, kv)
        idx = (S - 1) - (mx & 4095)
        idx = jnp.clip(idx, 0, S - 1)
        idxs.append(idx)
        sel[pl.ds(c, 1), :] = xn_v[pl.ds(idx, 1), :]

    def repack(ch, t, nblk):
        for gg in range(nblk):
            g = t * nblk + gg
            be = pl.multiple_of(ch * 5120 + g * 64, 64)
            bo = pl.multiple_of(ch * 5120 + 2560 + g * 64, 64)
            ev = raw.at[pl.ds(be, 64), :]
            od = raw.at[pl.ds(bo, 64), :]
            ob = pl.multiple_of(g * 8, 8)
            for p in range(8):
                a = ev[pl.ds(p, 8, stride=8), :]
                b = od[pl.ds(p, 8, stride=8), :]
                wp[ch * 16 + 2 * p, pl.ds(ob, 8), :] = (a & jnp.uint32(0xFFFF)) | (b << 16)
                wp[ch * 16 + 2 * p + 1, pl.ds(ob, 8), :] = (a >> 16) | (b & jnp.uint32(0xFFFF0000))

    xn3 = xn_v.reshape(NSEG, SEG, D)

    def pre_proj(j):
        w = pltpu.bitcast(wp[j], BF16)
        for c in range(4):
            lhs = xn3[c * 16:(c + 1) * 16, LIVE:SEG, :].reshape(128, D)
            pre[j, c * 128:(c + 1) * 128, :] = _dot(lhs, w)

    PH = 4
    NIT = 16 // PH
    w_copy(0).wait()
    w_copy(1).wait()
    jax.lax.fori_loop(0, 8, lambda t, c: (repack(0, t, 5), c)[1], 0)
    for ch in range(6):
        if ch + 1 < 6:
            w_copy(2 * ch + 2).wait()
            w_copy(2 * ch + 3).wait()

        def pro_body(t, carry, ch=ch):
            if ch + 1 < 6:
                repack(ch + 1, t, 40 // NIT)
            for u in range(PH):
                pre_proj(ch * 16 + t * PH + u)
            return carry

        jax.lax.fori_loop(0, NIT, pro_body, 0)

    for c in mlp_copies:
        c.wait()
    xs = sel[...]
    gate = _rb(_dot_nt(xs, wg_v[...]))
    up = _rb(_dot_nt(xs, wu_v[...]))
    hmid = _rb(gate * _sigmoid(gate)) * up
    y = _rb(_dot(hmid, wd_v[...]))
    r_sel = _rb(jnp.sum(xs * wr, axis=-1, keepdims=True))
    xnew = xs + _rb(y * _rb(_sigmoid(r_sel)))
    sel[...] = xnew
    for c in range(TOPC):
        xb_v[pl.ds(idxs[c], 1), :] = sel[pl.ds(c, 1), :]

    for c in wo_copies:
        c.wait()
    acc[0:M, :] = mem0_ref[...].astype(F32)
    acc[M:L, :] = jnp.zeros((SEG, D), F32)

    qi = jax.lax.broadcasted_iota(I32, (L, L), 0)
    ki = jax.lax.broadcasted_iota(I32, (L, L), 1)
    mask = (qi < M) | (qi >= ki)
    scale = DH ** (-0.5)

    def finish(sp):
        r0 = pl.multiple_of(sp * SEG, SEG)
        sa = acc[M:L, :]
        xb = xb_v[pl.ds(r0, SEG), :]
        g = xb * _sigmoid(xb)
        out_v[pl.ds(r0, SEG), :] = (x_v[pl.ds(r0, SEG), :].astype(F32) + sa * g).astype(BF16)

    def out_copy(r0, n):
        return pltpu.make_async_copy(out_v.at[pl.ds(r0, n), :], out_hbm.at[pl.ds(r0, n), :], sem_out.at[0])

    def step(s, carry):
        r0 = pl.multiple_of(s * SEG, SEG)
        p0 = pl.multiple_of(s * 8, 8)
        lhs = jnp.concatenate([acc[0:M, :], xn_v[pl.ds(r0, LIVE), :]], axis=0).astype(BF16)
        finish(jnp.maximum(s - 1, 0))

        def proj(j):
            t = _dot(lhs, pltpu.bitcast(wp[j], BF16))
            return jnp.concatenate([t, pre[j, pl.ds(p0, 8), :]], axis=0)

        NG = H // GH
        qs, ks, vs, ps, os_ = {}, {}, {}, {}, {}

        def do_qkv(g):
            for h in range(g * GH, (g + 1) * GH):
                qs[h] = proj(h)
                ks[h] = proj(H + h)
                vs[h] = proj(2 * H + h)

        def do_s(g):
            for h in range(g * GH, (g + 1) * GH):
                sc = _dot_nt(qs.pop(h), ks.pop(h)) * scale
                sc = jnp.where(mask, sc, NEG)
                e = jnp.exp(sc - jnp.max(sc, axis=-1, keepdims=True))
                ps[h] = e * (1.0 / jnp.sum(e, axis=-1, keepdims=True))

        def do_pv(g):
            for h in range(g * GH, (g + 1) * GH):
                os_[h] = _dot(ps.pop(h), vs.pop(h))

        def do_o(j, h0, h1):
            o = jnp.concatenate([os_[h] for h in range(h0, h1)], axis=1)
            return _dot(o, pltpu.bitcast(wo_p[j, h0 * 64:h1 * 64, :], BF16))

        for g in range(NG):
            do_qkv(g)
            if g >= 1:
                do_s(g - 1)
            if g >= 3:
                do_pv(g - 3)
        HS = (NG - 4) * GH

        def o1(j):
            acc[:, j * 128:(j + 1) * 128] = do_o(j, 0, HS)

        o1(0)
        do_s(NG - 1)
        do_pv(NG - 3)
        o1(1)
        do_pv(NG - 2)
        o1(2)
        o1(3)
        do_pv(NG - 1)
        o1(4)
        for j in range(NT):
            acc[:, j * 128:(j + 1) * 128] += do_o(j, HS, H)
        return carry

    OC = 8
    for blk in range(1):
        pass

    def outer(b, carry):
        jax.lax.fori_loop(b * OC, (b + 1) * OC, step, 0)

        @pl.when(b > 0)
        def _():
            out_copy(pl.multiple_of((b - 1) * OC * SEG, OC * SEG), OC * SEG).start()
        return carry

    jax.lax.fori_loop(0, NSEG // OC, outer, 0)
    finish(NSEG - 1)
    out_copy(S - OC * SEG, OC * SEG).start()
    out_copy(0, S).wait()


@jax.jit
def pallas_recurrent_scan__memory_aug_recurrent_mem_tr__moe_arch_mod__prompt_kernel(
    A_x: jax.Array,
    A_mem0: jax.Array,
    A_Wq: jax.Array,
    A_Wk: jax.Array,
    A_Wv: jax.Array,
    A_Wo: jax.Array,
    A_seg_len: jax.Array,
    B_x: jax.Array,
    B_w_r: jax.Array,
    B_w_gate: jax.Array,
    B_w_up: jax.Array,
    B_w_down: jax.Array,
):
    del A_seg_len, B_x
    assert A_x.shape == (1, S, D) and A_Wq.shape == (D, H, DH) and A_mem0.shape == (1, M, D)
    hbm = pl.BlockSpec(memory_space=pltpu.HBM)
    vmem = pl.BlockSpec(memory_space=pltpu.VMEM)
    wview = lambda w: w.reshape(D // 2, 2 * H, DH)
    out = pl.pallas_call(
        _kernel,
        out_shape=jax.ShapeDtypeStruct((S, D), BF16),
        in_specs=[hbm, vmem, hbm, hbm, hbm, hbm, vmem, hbm, hbm, hbm],
        out_specs=hbm,
        scratch_shapes=[
            pltpu.VMEM((S, D), BF16),
            pltpu.VMEM((S, D), F32),
            pltpu.VMEM((S, D), F32),
            pltpu.VMEM((12 * 2560, 128), U32),
            pltpu.VMEM((3 * H, D // 2, 128), U32),
            pltpu.VMEM((NT, H * DH // 2, 128), U32),
            pltpu.VMEM((3 * H, NSEG * 8, DH), F32),
            pltpu.VMEM((FF, D), BF16),
            pltpu.VMEM((FF, D), BF16),
            pltpu.VMEM((FF, D), BF16),
            pltpu.VMEM((S, D), BF16),
            pltpu.VMEM((L, D), F32),
            pltpu.VMEM((L, H * DH), F32),
            pltpu.VMEM((TOPC, D), F32),
            pltpu.VMEM((64, 128), I32),
            pltpu.SemaphoreType.DMA((21,)),
            pltpu.SemaphoreType.DMA((1,)),
        ],
        compiler_params=pltpu.CompilerParams(vmem_limit_bytes=110 * 1024 * 1024),
    )(
        A_x.reshape(S, D),
        A_mem0.reshape(M, D),
        wview(A_Wq), wview(A_Wk), wview(A_Wv),
        A_Wo.reshape(H * DH, D),
        B_w_r.reshape(NT, 128),
        B_w_gate.T, B_w_up.T, B_w_down,
    )
    return out.reshape(1, S, D)
```

```python
import functools
import math

import jax
import jax.numpy as jnp
import jax.experimental.pallas as pl
import jax.experimental.pallas.tpu as pltpu

F32 = jnp.float32
BF16 = jnp.bfloat16
U32 = jnp.uint32
I32 = jnp.int32

S = 2048
D = 640
H = 32
DH = 128
M = 8
SEG = 32
NSEG = S // SEG
L = M + SEG
FF = 1728
TOPC = 8
NT = D // 128
LIVE = SEG - 8
EPS = 1e-05
NEG = -1000000000.0
UNROLL = 4
PH = 4
NIT = 16 // PH
GH = 2


def _dot(a, b):
    return jax.lax.dot_general(a, b, (((1,), (0,)), ((), ())), preferred_element_type=F32)


def _dot_nt(a, b):
    return jax.lax.dot_general(a, b, (((1,), (1,)), ((), ())), preferred_element_type=F32)


def _rb(x):
    return x.astype(BF16).astype(F32)


def _sigmoid(x):
    return 1.0 / (1.0 + jnp.exp(-x))


def _kernel(x_hbm, mem0_hbm, wq_hbm, wk_hbm, wv_hbm, wo_hbm, wr_hbm, wg_hbm, wu_hbm, wd_hbm,
            out_hbm,
            x_v, xa_v, x8_p, xb_v, raw, wp0, wp1, wp2, wp3, wp4, wp5, wo_p, pre, wg_v, wu_v, wd_v,
            out_v, acc, sel, yacc, keys, mem0_v, wr_v, idx_s,
            sem_in, sem_out):
    wps = [wp0, wp1, wp2, wp3, wp4, wp5]
    w_hbm = [wq_hbm, wk_hbm, wv_hbm]

    def wtile(j):
        return wps[j // 16].at[j % 16]

    PB = D // 2 // NIT
    SEM_W = 8

    def w_copy(ch, t, par):
        m, c = ch // 2, ch % 2
        d0 = t * PB
        src = w_hbm[m].bitcast(U32).at[pl.ds(d0, PB), pl.ds(par * 16 + c * 8, 8), :]
        r0 = (ch * 2 + par) * 2560 + d0 * 8
        if not isinstance(r0, int):
            r0 = pl.multiple_of(r0, 8)
        dst = raw.at[pl.ds(r0, PB * 8), :].reshape(PB, 8, 128)
        return pltpu.make_async_copy(src, dst, sem_in.at[SEM_W + ch * NIT + t])

    def w_start(ch):
        for t in range(NIT):
            for par in range(2):
                w_copy(ch, t, par).start()

    def w_wait(ch, t):
        for par in range(2):
            w_copy(ch, t, par).wait()

    cp_wr = pltpu.make_async_copy(wr_hbm, wr_v, sem_in.at[0])
    cp_x8 = pltpu.make_async_copy(x_hbm.at[:, pl.ds(LIVE, 8), :], x_v.at[:, pl.ds(LIVE, 8), :], sem_in.at[1])
    cp_xa = pltpu.make_async_copy(x_hbm.at[:, pl.ds(0, LIVE), :], x_v.at[:, pl.ds(0, LIVE), :], sem_in.at[2])
    cp_mem = pltpu.make_async_copy(mem0_hbm, mem0_v, sem_in.at[3])
    mlp_copies = [pltpu.make_async_copy(s_, d_, sem_in.at[4])
                  for s_, d_ in [(wg_hbm, wg_v), (wu_hbm, wu_v), (wd_hbm, wd_v)]]
    wo32 = wo_hbm.bitcast(U32)
    wo_copies = [pltpu.make_async_copy(wo32.at[:, pl.ds(j * 128, 128)], wo_p.at[j], sem_in.at[5])
                 for j in range(NT)]

    cp_wr.start()
    cp_x8.start()
    w_start(0)
    w_start(1)
    cp_xa.start()
    cp_mem.start()
    for ch in range(2, 6):
        w_start(ch)
    for c in mlp_copies:
        c.start()
    for c in wo_copies:
        c.start()

    IMIN = jnp.iinfo(jnp.int32).min
    xb3 = xb_v.reshape(NSEG, SEG, D)
    keys[...] = jnp.full(keys.shape, IMIN, I32)
    cp_wr.wait()
    wr5 = wr_v[...].astype(F32)
    wr = jnp.concatenate([wr5[j:j + 1, :] for j in range(NT)], axis=1)

    def layernorm(s0, nseg, t0, nrow, slot):
        n = nseg * nrow
        x = x_v[pl.ds(s0, nseg), t0:t0 + nrow, :].astype(F32).reshape(n, D)
        mu = jnp.sum(x, axis=-1, keepdims=True) * (1.0 / D)
        xc = x - mu
        var = jnp.sum(xc * xc, axis=-1, keepdims=True) * (1.0 / D)
        sd = _rb(jnp.sqrt(_rb(_rb(var) + EPS)))
        xn = _rb(_rb(x - _rb(mu)) / sd)
        xb3[pl.ds(s0, nseg), t0:t0 + nrow, :] = xn.reshape(nseg, nrow, D)
        r = _rb(jnp.sum(xn * wr, axis=-1, keepdims=True))
        r = jnp.where(r == 0.0, 0.0, r)
        bits = pltpu.bitcast(jnp.broadcast_to(r, (n, 128)), I32) >> 16
        mono = jnp.where(bits < 0, (-32768) - bits, bits)
        mono = jnp.where(r != r, -40000, mono)
        row = (jax.lax.broadcasted_iota(I32, (nseg, nrow, 128), 0) * SEG
               + jax.lax.broadcasted_iota(I32, (nseg, nrow, 128), 1)).reshape(n, 128)
        key = mono * 4096 + ((S - 1 - t0) - s0 * SEG - row)
        lane = jax.lax.broadcasted_iota(I32, (n, 128), 1)
        keys[0:n, :] = jnp.where(lane == slot, key, keys[0:n, :])
        return xn

    cp_x8.wait()

    def ln8_body(b, carry):
        xn = layernorm(b * 16, 16, LIVE, 8, b)
        x8_p[pl.ds(pl.multiple_of(b * 64, 64), 64), :] = pltpu.bitcast(xn.astype(BF16), U32)
        return carry

    jax.lax.fori_loop(0, 4, ln8_body, 0)

    def ln_rest(i):
        for u in range(2):
            s0 = i * 8 + u * 4
            xn = layernorm(s0, 4, 0, LIVE, 4 + i * 2 + u)
            xa_v[pl.ds(s0, 4), :, :] = xn.reshape(4, LIVE, D)

    def topk_round(c):
        kv = keys[...]
        mx = jnp.max(kv)
        keys[...] = jnp.where(kv == mx, IMIN, kv)
        idx = jnp.clip((S - 1) - (mx & 4095), 0, S - 1)
        idx_s[c] = idx
        sel[pl.ds(c, 1), :] = xb_v[pl.ds(idx, 1), :]

    def repack(ch, t):
        nblk = PB // 8
        for gg in range(nblk):
            g = t * nblk + gg
            be = pl.multiple_of(ch * 5120 + g * 64, 64)
            bo = pl.multiple_of(ch * 5120 + 2560 + g * 64, 64)
            ev = raw.at[pl.ds(be, 64), :]
            od = raw.at[pl.ds(bo, 64), :]
            ob = pl.multiple_of(g * 8, 8)
            for p in range(8):
                a = ev[pl.ds(p, 8, stride=8), :]
                b = od[pl.ds(p, 8, stride=8), :]
                wps[ch][2 * p, pl.ds(ob, 8), :] = (a & jnp.uint32(0xFFFF)) | (b << 16)
                wps[ch][2 * p + 1, pl.ds(ob, 8), :] = (a >> 16) | (b & jnp.uint32(0xFFFF0000))

    def pre_dot(ch, jl, c):
        w = pltpu.bitcast(wps[ch][jl], BF16)
        lhs = pltpu.bitcast(x8_p[c * 64:(c + 1) * 64, :], BF16)
        pre[ch * 16 + jl, c * 128:(c + 1) * 128, :] = _dot(lhs, w)

    def rp0_body(t, carry):
        w_wait(0, t)
        repack(0, t)
        return carry

    jax.lax.fori_loop(0, NIT, rp0_body, 0)

    FP = FF // NIT
    yacc[...] = jnp.zeros(yacc.shape, F32)
    for ch in range(6):
        if ch == 1:
            cp_xa.wait()
        if ch == 5:
            for c in mlp_copies:
                c.wait()

        def pro_body(t, carry, ch=ch):
            if ch + 1 < 6:
                w_wait(ch + 1, t)
                repack(ch + 1, t)
            if ch in (1, 2):
                ln_rest((ch - 1) * NIT + t)
            if ch == 3:
                for u in range(TOPC // NIT):
                    topk_round(t * (TOPC // NIT) + u)
            big = [(t * PH + u, c) for u in range(PH) for c in range(4)]
            if ch < 5:
                for jl, c in big:
                    pre_dot(ch, jl, c)
            else:
                f0 = pl.multiple_of(t * FP, 16)
                xs = sel[...]
                cuts = [(a_, min(a_ + 128, FP)) for a_ in range(0, FP, 128)]
                gs, us = [], []
                it = iter(big)
                for a_, b_ in cuts:
                    pre_dot(ch, *next(it))
                    gs.append(_dot_nt(xs, wg_v[pl.ds(f0 + a_, b_ - a_), :]))
                    pre_dot(ch, *next(it))
                    us.append(_dot_nt(xs, wu_v[pl.ds(f0 + a_, b_ - a_), :]))
                pre_dot(ch, *next(it))
                pre_dot(ch, *next(it))
                for (a_, b_), g_, u_ in zip(cuts, gs, us):
                    g_ = _rb(g_)
                    hm = _rb(g_ * _sigmoid(g_)) * _rb(u_)
                    pre_dot(ch, *next(it))
                    yacc[...] += _dot(hm, wd_v[pl.ds(f0 + a_, b_ - a_), :])
                for jl, c in it:
                    pre_dot(ch, jl, c)
            return carry

        jax.lax.fori_loop(0, NIT, pro_body, 0)

    xs = sel[...]
    r_sel = _rb(jnp.sum(xs * wr, axis=-1, keepdims=True))
    sel[...] = xs + _rb(_rb(yacc[...]) * _rb(_sigmoid(r_sel)))
    for c in range(TOPC):
        xb_v[pl.ds(idx_s[c], 1), :] = sel[pl.ds(c, 1), :]

    for c in wo_copies:
        c.wait()
    cp_mem.wait()
    acc[0:M, :] = mem0_v[...].astype(F32)
    acc[M:L, :] = jnp.zeros((SEG, D), F32)

    qi = jax.lax.broadcasted_iota(I32, (L, L), 0)
    ki = jax.lax.broadcasted_iota(I32, (L, L), 1)
    mask = (qi < M) | (qi >= ki)
    scale = DH ** (-0.5)

    def finish(sp):
        r0 = pl.multiple_of(sp * SEG, SEG)
        sa = acc[M:L, :]
        xb = xb_v[pl.ds(r0, SEG), :]
        g = xb * _sigmoid(xb)
        out_v[pl.ds(r0, SEG), :] = (x_v[sp].astype(F32) + sa * g).astype(BF16)

    def out_copy(r0, n):
        return pltpu.make_async_copy(out_v.at[pl.ds(r0, n), :], out_hbm.at[pl.ds(r0, n), :], sem_out.at[0])

    def step(s, carry):
        p0 = pl.multiple_of(s * 8, 8)
        lhs = jnp.concatenate([acc[0:M, :], xa_v[s]], axis=0).astype(BF16)
        finish(jnp.maximum(s - 1, 0))

        def proj(j):
            t = _dot(lhs, pltpu.bitcast(wtile(j)[...], BF16))
            return jnp.concatenate([t, pre[j, pl.ds(p0, 8), :]], axis=0)

        NG = H // GH
        qs, ks, vs, ps, os_ = {}, {}, {}, {}, {}

        def do_qkv(g):
            js = [m * H + h for h in range(g * GH, (g + 1) * GH) for m in range(3)]
            if g == 0:
                part = {}
                for kt in range(NT):
                    for j in js:
                        t = _dot(lhs[:, kt * 128:(kt + 1) * 128],
                                 pltpu.bitcast(wtile(j)[kt * 64:(kt + 1) * 64, :], BF16))
                        part[j] = t if kt == 0 else part[j] + t
                res = {j: jnp.concatenate([part[j], pre[j, pl.ds(p0, 8), :]], axis=0) for j in js}
            else:
                res = {j: proj(j) for j in js}
            for h in range(g * GH, (g + 1) * GH):
                qs[h], ks[h], vs[h] = res[h], res[H + h], res[2 * H + h]

        def do_s(g):
            for h in range(g * GH, (g + 1) * GH):
                sc = _dot_nt(qs.pop(h), ks.pop(h)) * scale
                sc = jnp.where(mask, sc, NEG)
                e = jnp.exp(sc - jnp.max(sc, axis=-1, keepdims=True))
                ps[h] = e * (1.0 / jnp.sum(e, axis=-1, keepdims=True))

        def do_pv(g):
            for h in range(g * GH, (g + 1) * GH):
                os_[h] = _dot(ps.pop(h), vs.pop(h))

        def do_o(j, h0, h1):
            o = jnp.concatenate([os_[h] for h in range(h0, h1)], axis=1)
            return _dot(o, pltpu.bitcast(wo_p[j, h0 * 64:h1 * 64, :], BF16))

        for g in range(NG):
            do_qkv(g)
            if g >= 1:
                do_s(g - 1)
            if g >= 3:
                do_pv(g - 3)
        HS = (NG - 4) * GH

        def o1(j):
            acc[:, j * 128:(j + 1) * 128] = do_o(j, 0, HS)

        o1(0)
        do_s(NG - 1)
        do_pv(NG - 3)
        o1(1)
        do_pv(NG - 2)
        o1(2)
        o1(3)
        do_pv(NG - 1)
        o1(4)
        for j in range(NT):
            acc[:, j * 128:(j + 1) * 128] += do_o(j, HS, H)
        return carry

    OC = 8

    def outer(b, carry):
        def multi(i, c):
            for u in range(UNROLL):
                step(i * UNROLL + u, c)
            return c
        jax.lax.fori_loop(b * (OC // UNROLL), (b + 1) * (OC // UNROLL), multi, 0)

        @pl.when(b > 0)
        def _():
            out_copy(pl.multiple_of((b - 1) * OC * SEG, OC * SEG), OC * SEG).start()
        return carry

    jax.lax.fori_loop(0, NSEG // OC, outer, 0)
    finish(NSEG - 1)
    out_copy(S - OC * SEG, OC * SEG).start()
    out_copy(0, S).wait()


@jax.jit
def pallas_recurrent_scan__memory_aug_recurrent_mem_tr__moe_arch_mod__prompt_kernel(
    A_x: jax.Array,
    A_mem0: jax.Array,
    A_Wq: jax.Array,
    A_Wk: jax.Array,
    A_Wv: jax.Array,
    A_Wo: jax.Array,
    A_seg_len: jax.Array,
    B_x: jax.Array,
    B_w_r: jax.Array,
    B_w_gate: jax.Array,
    B_w_up: jax.Array,
    B_w_down: jax.Array,
):
    del A_seg_len, B_x
    assert A_x.shape == (1, S, D) and A_Wq.shape == (D, H, DH) and A_mem0.shape == (1, M, D)
    hbm = pl.BlockSpec(memory_space=pltpu.HBM)
    wview = lambda w: w.reshape(D // 2, 2 * H, DH)
    out = pl.pallas_call(
        _kernel,
        out_shape=jax.ShapeDtypeStruct((S, D), BF16),
        in_specs=[hbm] * 10,
        out_specs=hbm,
        scratch_shapes=[
            pltpu.VMEM((NSEG, SEG, D), BF16),
            pltpu.VMEM((NSEG, LIVE, D), F32),
            pltpu.VMEM((NSEG * 4, D), U32),
            pltpu.VMEM((S, D), F32),
            pltpu.VMEM((12 * 2560, 128), U32),
        ] + [pltpu.VMEM((16, D // 2, 128), U32)] * 6 + [
            pltpu.VMEM((NT, H * DH // 2, 128), U32),
            pltpu.VMEM((3 * H, NSEG * 8, DH), F32),
            pltpu.VMEM((FF, D), BF16),
            pltpu.VMEM((FF, D), BF16),
            pltpu.VMEM((FF, D), BF16),
            pltpu.VMEM((S, D), BF16),
            pltpu.VMEM((L, D), F32),
            pltpu.VMEM((TOPC, D), F32),
            pltpu.VMEM((TOPC, D), F32),
            pltpu.VMEM((128, 128), I32),
            pltpu.VMEM((M, D), BF16),
            pltpu.VMEM((NT, 128), BF16),
            pltpu.SMEM((TOPC,), I32),
            pltpu.SemaphoreType.DMA((8 + 6 * NIT,)),
            pltpu.SemaphoreType.DMA((1,)),
        ],
        compiler_params=pltpu.CompilerParams(vmem_limit_bytes=110 * 1024 * 1024),
    )(
        A_x.reshape(NSEG, SEG, D),
        A_mem0.reshape(M, D),
        wview(A_Wq), wview(A_Wk), wview(A_Wv),
        A_Wo.reshape(H * DH, D),
        B_w_r.reshape(NT, 128),
        B_w_gate.T, B_w_up.T, B_w_down,
    )
    return out.reshape(1, S, D)
```

```python
import functools
import math

import jax
import jax.numpy as jnp
import jax.experimental.pallas as pl
import jax.experimental.pallas.tpu as pltpu

F32 = jnp.float32
BF16 = jnp.bfloat16
U32 = jnp.uint32
I32 = jnp.int32

S = 2048
D = 640
H = 32
DH = 128
M = 8
SEG = 32
NSEG = S // SEG
L = M + SEG
FF = 1728
TOPC = 8
NT = D // 128
LIVE = SEG - 8
EPS = 1e-05
NEG = -1000000000.0
UNROLL = 4
NPH = 24
GH = 2


def _dot(a, b):
    return jax.lax.dot_general(a, b, (((1,), (0,)), ((), ())), preferred_element_type=F32)


def _dot_nt(a, b):
    return jax.lax.dot_general(a, b, (((1,), (1,)), ((), ())), preferred_element_type=F32)


def _rb(x):
    return x.astype(BF16).astype(F32)


def _sigmoid(x):
    return 1.0 / (1.0 + jnp.exp(-x))


def _kernel(x_hbm, mem0_hbm, wq_hbm, wk_hbm, wv_hbm, wo_hbm, wr_hbm, wg_hbm, wu_hbm, wd_hbm,
            out_hbm,
            x_v, lhs_v, xa_v, xb_v, raw, w_ev, w_od, wo_p, pre, wg_v, wu_v, wd_v,
            out_v, acc, sel, yacc, keys, mem0_v, wr_v, idx_s,
            sem_in, sem_out):
    w_hbm = [wq_hbm, wk_hbm, wv_hbm]
    w_eo = [w_ev, w_od]

    def wtile(j):
        return w_eo[(j // 4) % 2].at[(j // 8) * 4 + j % 4]

    SEM_X8, SEM_XA, SEM_W = 4, 8, 16

    def w_start(k):
        for q in (2 * k, 2 * k + 1):
            src = w_hbm[q // 16].bitcast(U32).at[:, q % 16, :]
            pltpu.make_async_copy(src, raw.at[q], sem_in.at[SEM_W + k]).start()

    def w_wait(k):
        both = raw.at[pl.ds(2 * k, 2)]
        pltpu.make_async_copy(both, both, sem_in.at[SEM_W + k]).wait()

    def x8_copy(b):
        return pltpu.make_async_copy(x_hbm.at[pl.ds(b * 16, 16), pl.ds(LIVE, 8), :],
                                     x_v.at[pl.ds(b * 16, 16), pl.ds(LIVE, 8), :], sem_in.at[SEM_X8 + b])

    def xa_copy(i):
        return pltpu.make_async_copy(x_hbm.at[pl.ds(i * 8, 8), pl.ds(0, LIVE), :],
                                     x_v.at[pl.ds(i * 8, 8), pl.ds(0, LIVE), :], sem_in.at[SEM_XA + i])

    cp_wr = pltpu.make_async_copy(wr_hbm, wr_v, sem_in.at[0])
    cp_mem = pltpu.make_async_copy(mem0_hbm, mem0_v, sem_in.at[1])
    mlp_copies = [pltpu.make_async_copy(s_, d_, sem_in.at[2])
                  for s_, d_ in [(wg_hbm, wg_v), (wu_hbm, wu_v), (wd_hbm, wd_v)]]
    wo32 = wo_hbm.bitcast(U32)
    wo_copies = [pltpu.make_async_copy(wo32.at[:, pl.ds(j * 128, 128)], wo_p.at[j], sem_in.at[3])
                 for j in range(NT)]

    cp_wr.start()
    for b in range(4):
        x8_copy(b).start()
    for k in range(NPH):
        w_start(k)
        if k >= 3 and k % 2 == 1 and (k - 3) // 2 < 8:
            xa_copy((k - 3) // 2).start()
    cp_mem.start()
    for c in mlp_copies:
        c.start()
    for c in wo_copies:
        c.start()

    IMIN = jnp.iinfo(jnp.int32).min
    xb3 = xb_v.reshape(NSEG, SEG, D)
    keys[...] = jnp.full(keys.shape, IMIN, I32)
    yacc[...] = jnp.zeros(yacc.shape, F32)
    cp_wr.wait()

    def router_w():
        wr5 = wr_v[...].astype(F32)
        return jnp.concatenate([wr5[j:j + 1, :] for j in range(NT)], axis=1)

    def layernorm(s0, nseg, t0, nrow, slot, wr):
        n = nseg * nrow
        x = x_v[pl.ds(s0, nseg), t0:t0 + nrow, :].astype(F32).reshape(n, D)
        mu = jnp.sum(x, axis=-1, keepdims=True) * (1.0 / D)
        xc = x - mu
        var = jnp.sum(xc * xc, axis=-1, keepdims=True) * (1.0 / D)
        sd = _rb(jnp.sqrt(_rb(_rb(var) + EPS)))
        xn = _rb(_rb(x - _rb(mu)) / sd)
        xb3[pl.ds(s0, nseg), t0:t0 + nrow, :] = xn.reshape(nseg, nrow, D)
        r = _rb(jnp.sum(xn * wr, axis=-1, keepdims=True))
        r = jnp.where(r == 0.0, 0.0, r)
        bits = pltpu.bitcast(jnp.broadcast_to(r, (n, 128)), I32) >> 16
        mono = jnp.where(bits < 0, (-32768) - bits, bits)
        mono = jnp.where(r != r, -40000, mono)
        row = (jax.lax.broadcasted_iota(I32, (nseg, nrow, 128), 0) * SEG
               + jax.lax.broadcasted_iota(I32, (nseg, nrow, 128), 1)).reshape(n, 128)
        key = mono * 4096 + ((S - 1 - t0) - s0 * SEG - row)
        lane = jax.lax.broadcasted_iota(I32, (n, 128), 1)
        keys[0:n, :] = jnp.where(lane == slot, key, keys[0:n, :])
        return xn, key

    def ln8_body(b, carry):
        x8_copy(b).wait()
        xn, _ = layernorm(b * 16, 16, LIVE, 8, b, router_w())
        lhs_v[pl.ds(pl.multiple_of(b * 64, 64), 64), :] = pltpu.bitcast(xn.astype(BF16), U32)
        return carry

    jax.lax.fori_loop(0, 4, ln8_body, 0)

    def ln_seg(s, wr):
        xn, key = layernorm(s, 1, 0, LIVE, 4 + s, wr)
        xa_v[pl.ds(pl.multiple_of(s * LIVE, 8), LIVE), :] = xn
        return pltpu.bitcast(key, U32)

    def topk_round(c):
        kv = keys[...]
        mx = jnp.max(kv)
        keys[...] = jnp.where(kv == mx, IMIN, kv)
        idx = jnp.clip((S - 1) - (mx & 4095), 0, S - 1)
        idx_s[c] = idx
        sel[pl.ds(c, 1), :] = xb_v[pl.ds(idx, 1), :]

    def repack(k, par, slot):
        for u in range(2):
            rq = raw.at[2 * k + u]
            lo = w_eo[par].at[slot * 4 + 2 * u]
            hi = w_eo[par].at[slot * 4 + 2 * u + 1]
            for g in range(D // 16):
                a = rq[pl.ds(16 * g, 8, stride=2), :]
                b = rq[pl.ds(16 * g + 1, 8, stride=2), :]
                lo[8 * g:8 * g + 8, :] = (a & jnp.uint32(0xFFFF)) | (b << 16)
                hi[8 * g:8 * g + 8, :] = (a >> 16) | (b & jnp.uint32(0xFFFF0000))

    def phase(k, par, slot, after_dot=None, side=None):
        for u in range(4):
            for c in range(4):
                w = pltpu.bitcast(w_eo[par][slot * 4 + u], BF16)
                lhs = lhs_v[c * 64:(c + 1) * 64, :]
                if side is not None and c == 3:
                    tok = side(u)
                    n = tok.shape[0]
                    head = jnp.where(k < 0, tok, lhs[0:n, 0:128])
                    lhs = jnp.concatenate(
                        [jnp.concatenate([head, lhs[0:n, 128:]], axis=1), lhs[n:, :]], axis=0)
                pre[4 * k + u, c * 128:(c + 1) * 128, :] = _dot(pltpu.bitcast(lhs, BF16), w)
                if after_dot is not None:
                    after_dot()

    def two_phases(i, after_dot=None, side=None):
        k = 2 * i + 1
        repack(k + 1, 0, i + 1)
        phase(k, 1, i, after_dot, side)
        repack(k + 2, 1, i + 1)
        phase(k + 1, 0, i + 1, after_dot, None if side is None else (lambda u: side(4 + u)))

    w_wait(0)
    repack(0, 0, 0)
    w_wait(1)
    repack(1, 1, 0)
    phase(0, 0, 0)

    def ln_body(i, carry):
        w_wait(2 * i + 2)
        w_wait(2 * i + 3)
        xa_copy(i).wait()
        wr = router_w()
        two_phases(i, side=lambda u: ln_seg(i * 8 + u, wr))
        return carry

    jax.lax.fori_loop(0, 8, ln_body, 0)

    w_wait(18)
    w_wait(19)
    for c in range(TOPC):
        topk_round(c)
    two_phases(8)

    for c in mlp_copies:
        c.wait()
    FP = FF // 2

    def mlp_body(t, carry):
        i = 9 + t
        w_wait(2 * i + 2)
        w_wait(2 * i + 3)
        f0 = pl.multiple_of(t * FP, 16)
        xs = sel[...]
        cuts = [(a_, min(a_ + 128, FP)) for a_ in range(0, FP, 128)]
        val = {}

        def up_tile(which, n, kt):
            def run():
                a_, b_ = cuts[n]
                w = (wg_v, wu_v)[which][pl.ds(f0 + a_, b_ - a_), kt * 128:(kt + 1) * 128]
                r = _dot_nt(xs[:, kt * 128:(kt + 1) * 128], w)
                val[which, n] = r if kt == 0 else val[which, n] + r
            return run

        def down_tile(n, j):
            def run():
                a_, b_ = cuts[n]
                if j == 0:
                    g_ = _rb(val.pop((0, n)))
                    val['h', n] = _rb(g_ * _sigmoid(g_)) * _rb(val.pop((1, n)))
                r = _dot(val['h', n], wd_v[pl.ds(f0 + a_, b_ - a_), j * 128:(j + 1) * 128])
                val['y', j] = r if n == 0 else val['y', j] + r
            return run

        jobs = [up_tile(which, n, kt) for n in range(len(cuts)) for which in range(2) for kt in range(NT)]
        jobs += [down_tile(n, j) for n in range(len(cuts)) for j in range(NT)]

        def after_dot():
            for _ in range(4):
                if jobs:
                    jobs.pop(0)()

        two_phases(i, after_dot=after_dot)
        yacc[...] += jnp.concatenate([val['y', j] for j in range(NT)], axis=1)
        return carry

    jax.lax.fori_loop(0, 2, mlp_body, 0)

    cp_mem.wait()
    acc[0:M, :] = mem0_v[...].astype(F32)
    acc[M:L, :] = jnp.zeros((SEG, D), F32)
    xs = sel[...]
    r_sel = _rb(jnp.sum(xs * router_w(), axis=-1, keepdims=True))
    sel[...] = xs + _rb(_rb(yacc[...]) * _rb(_sigmoid(r_sel)))
    for c in range(TOPC):
        xb_v[pl.ds(idx_s[c], 1), :] = sel[pl.ds(c, 1), :]
    phase(NPH - 1, 1, NPH // 2 - 1)

    for c in wo_copies:
        c.wait()

    qi = jax.lax.broadcasted_iota(I32, (L, L), 0)
    ki = jax.lax.broadcasted_iota(I32, (L, L), 1)
    mask = (qi < M) | (qi >= ki)
    scale = DH ** (-0.5)

    def finish(sp):
        r0 = pl.multiple_of(sp * SEG, SEG)
        sa = acc[M:L, :]
        xb = xb_v[pl.ds(r0, SEG), :]
        g = xb * _sigmoid(xb)
        out_v[pl.ds(r0, SEG), :] = (x_v[sp].astype(F32) + sa * g).astype(BF16)

    def out_copy(r0, n):
        return pltpu.make_async_copy(out_v.at[pl.ds(r0, n), :], out_hbm.at[pl.ds(r0, n), :], sem_out.at[0])

    def step(i, u):
        s = i * UNROLL + u
        pre_i = pre.at[:, pl.ds(pl.multiple_of(i * (8 * UNROLL), 8 * UNROLL), 8 * UNROLL), :]
        xa_i = xa_v.at[pl.ds(pl.multiple_of(i * (LIVE * UNROLL), 8 * UNROLL), LIVE * UNROLL), :]
        xa = xa_i[u * LIVE:(u + 1) * LIVE, :]
        lhs = jnp.concatenate([acc[0:M, :], xa], axis=0).astype(BF16)
        finish(jnp.maximum(s - 1, 0) if u == 0 else s - 1)

        def proj(j):
            t = _dot(lhs, pltpu.bitcast(wtile(j)[...], BF16))
            return jnp.concatenate([t, pre_i[j, u * 8:(u + 1) * 8, :]], axis=0)

        NG = H // GH
        qs, ks, vs, ps, os_ = {}, {}, {}, {}, {}

        def do_qkv(g):
            js = [m * H + h for h in range(g * GH, (g + 1) * GH) for m in range(3)]
            if g == 0:
                part = {}
                for kt in range(NT):
                    for j in js:
                        t = _dot(lhs[:, kt * 128:(kt + 1) * 128],
                                 pltpu.bitcast(wtile(j)[kt * 64:(kt + 1) * 64, :], BF16))
                        part[j] = t if kt == 0 else part[j] + t
                res = {j: jnp.concatenate([part[j], pre_i[j, u * 8:(u + 1) * 8, :]], axis=0) for j in js}
            else:
                res = {j: proj(j) for j in js}
            for h in range(g * GH, (g + 1) * GH):
                qs[h], ks[h], vs[h] = res[h], res[H + h], res[2 * H + h]

        def do_s(g):
            for h in range(g * GH, (g + 1) * GH):
                sc = _dot_nt(qs.pop(h), ks.pop(h)) * scale
                sc = jnp.where(mask, sc, NEG)
                e = jnp.exp(sc - jnp.max(sc, axis=-1, keepdims=True))
                ps[h] = e * (1.0 / jnp.sum(e, axis=-1, keepdims=True))

        def do_pv(g):
            for h in range(g * GH, (g + 1) * GH):
                os_[h] = _dot(ps.pop(h), vs.pop(h))

        def do_o(j, h0, h1):
            o = jnp.concatenate([os_[h] for h in range(h0, h1)], axis=1)
            return _dot(o, pltpu.bitcast(wo_p[j, h0 * 64:h1 * 64, :], BF16))

        for g in range(NG):
            do_qkv(g)
            if g >= 1:
                do_s(g - 1)
            if g >= 3:
                do_pv(g - 3)
        HS = (NG - 4) * GH

        def o1(j):
            acc[:, j * 128:(j + 1) * 128] = do_o(j, 0, HS)

        o1(0)
        do_s(NG - 1)
        do_pv(NG - 3)
        o1(1)
        do_pv(NG - 2)
        o1(2)
        o1(3)
        do_pv(NG - 1)
        o1(4)
        for j in range(NT):
            acc[:, j * 128:(j + 1) * 128] += do_o(j, HS, H)

    def multi(i, carry):
        for u in range(UNROLL):
            step(i, u)
        r0 = pl.multiple_of(i * (UNROLL * SEG), SEG)
        out_copy(r0, (UNROLL - 1) * SEG).start()

        @pl.when(i > 0)
        def _():
            out_copy(pl.multiple_of(r0 - SEG, SEG), SEG).start()
        return carry

    jax.lax.fori_loop(0, NSEG // UNROLL, multi, 0)
    finish(NSEG - 1)
    out_copy(S - SEG, SEG).start()
    out_copy(0, S).wait()


@jax.jit
def pallas_recurrent_scan__memory_aug_recurrent_mem_tr__moe_arch_mod__prompt_kernel(
    A_x: jax.Array,
    A_mem0: jax.Array,
    A_Wq: jax.Array,
    A_Wk: jax.Array,
    A_Wv: jax.Array,
    A_Wo: jax.Array,
    A_seg_len: jax.Array,
    B_x: jax.Array,
    B_w_r: jax.Array,
    B_w_gate: jax.Array,
    B_w_up: jax.Array,
    B_w_down: jax.Array,
):
    del A_seg_len, B_x
    assert A_x.shape == (1, S, D) and A_Wq.shape == (D, H, DH) and A_mem0.shape == (1, M, D)
    hbm = pl.BlockSpec(memory_space=pltpu.HBM)
    out = pl.pallas_call(
        _kernel,
        out_shape=jax.ShapeDtypeStruct((S, D), BF16),
        in_specs=[hbm] * 10,
        out_specs=hbm,
        scratch_shapes=[
            pltpu.VMEM((NSEG, SEG, D), BF16),
            pltpu.VMEM((NSEG * 4, D), U32),
            pltpu.VMEM((NSEG * LIVE, D), F32),
            pltpu.VMEM((S, D), F32),
            pltpu.VMEM((2 * NPH, D, 128), U32),
            pltpu.VMEM((2 * NPH, D // 2, 128), U32),
            pltpu.VMEM((2 * NPH, D // 2, 128), U32),
            pltpu.VMEM((NT, H * DH // 2, 128), U32),
            pltpu.VMEM((3 * H, NSEG * 8, DH), F32),
            pltpu.VMEM((FF, D), BF16),
            pltpu.VMEM((FF, D), BF16),
            pltpu.VMEM((FF, D), BF16),
            pltpu.VMEM((S, D), BF16),
            pltpu.VMEM((L, D), F32),
            pltpu.VMEM((TOPC, D), F32),
            pltpu.VMEM((TOPC, D), F32),
            pltpu.VMEM((128, 128), I32),
            pltpu.VMEM((M, D), BF16),
            pltpu.VMEM((NT, 128), BF16),
            pltpu.SMEM((TOPC,), I32),
            pltpu.SemaphoreType.DMA((16 + NPH,)),
            pltpu.SemaphoreType.DMA((1,)),
        ],
        compiler_params=pltpu.CompilerParams(vmem_limit_bytes=110 * 1024 * 1024),
    )(
        A_x.reshape(NSEG, SEG, D),
        A_mem0.reshape(M, D),
        A_Wq, A_Wk, A_Wv,
        A_Wo.reshape(H * DH, D),
        B_w_r.reshape(NT, 128),
        B_w_gate.T, B_w_up.T, B_w_down,
    )
    return out.reshape(1, S, D)
```

```python
import functools
import math

import jax
import jax.numpy as jnp
import jax.experimental.pallas as pl
import jax.experimental.pallas.tpu as pltpu

F32 = jnp.float32
BF16 = jnp.bfloat16
U32 = jnp.uint32
I32 = jnp.int32

S = 2048
D = 640
H = 32
DH = 128
M = 8
SEG = 32
NSEG = S // SEG
L = M + SEG
FF = 1728
TOPC = 8
NT = D // 128
LIVE = SEG - 8
EPS = 1e-05
NEG = -1000000000.0
UNROLL = 4
NPH = 24
GH = 2


def _dot(a, b):
    return jax.lax.dot_general(a, b, (((1,), (0,)), ((), ())), preferred_element_type=F32)


def _dot_nt(a, b):
    return jax.lax.dot_general(a, b, (((1,), (1,)), ((), ())), preferred_element_type=F32)


def _rb(x):
    return x.astype(BF16).astype(F32)


def _sigmoid(x):
    return 1.0 / (1.0 + jnp.exp(-x))


def _kernel(x_hbm, mem0_hbm, wq_hbm, wk_hbm, wv_hbm, wo_hbm, wr_hbm, wg_hbm, wu_hbm, wd_hbm,
            out_hbm,
            x_v, lhs_v, xa_v, xb_v, raw, w_ev, w_od, wo_p, pre, wg_v, wu_v, wd_v,
            out_v, acc, sel, yacc, keys, mem0_v, wr_v, idx_s,
            sem_in, sem_out):
    w_hbm = [wq_hbm, wk_hbm, wv_hbm]
    w_eo = [w_ev, w_od]

    def wtile(j):
        return w_eo[(j // 4) % 2].at[(j // 8) * 4 + j % 4]

    SEM_X8, SEM_XA, SEM_W = 4, 8, 16

    def w_start(k):
        for q in (2 * k, 2 * k + 1):
            src = w_hbm[q // 16].bitcast(U32).at[:, q % 16, :]
            pltpu.make_async_copy(src, raw.at[q], sem_in.at[SEM_W + k]).start()

    def w_wait(k):
        both = raw.at[pl.ds(2 * k, 2)]
        pltpu.make_async_copy(both, both, sem_in.at[SEM_W + k]).wait()

    def x8_copy(b):
        return pltpu.make_async_copy(x_hbm.at[pl.ds(b * 16, 16), pl.ds(LIVE, 8), :],
                                     x_v.at[pl.ds(b * 16, 16), pl.ds(LIVE, 8), :], sem_in.at[SEM_X8 + b])

    def xa_copy(i):
        return pltpu.make_async_copy(x_hbm.at[pl.ds(i * 8, 8), pl.ds(0, LIVE), :],
                                     x_v.at[pl.ds(i * 8, 8), pl.ds(0, LIVE), :], sem_in.at[SEM_XA + i])

    cp_wr = pltpu.make_async_copy(wr_hbm, wr_v, sem_in.at[0])
    cp_mem = pltpu.make_async_copy(mem0_hbm, mem0_v, sem_in.at[1])
    mlp_copies = [pltpu.make_async_copy(s_, d_, sem_in.at[2])
                  for s_, d_ in [(wg_hbm, wg_v), (wu_hbm, wu_v), (wd_hbm, wd_v)]]
    wo32 = wo_hbm.bitcast(U32)
    wo_copies = [pltpu.make_async_copy(wo32.at[:, pl.ds(j * 128, 128)], wo_p.at[j], sem_in.at[3])
                 for j in range(NT)]

    cp_wr.start()
    for b in range(4):
        x8_copy(b).start()
    for k in range(NPH):
        w_start(k)
        if k >= 3 and k % 2 == 1 and (k - 3) // 2 < 8:
            xa_copy((k - 3) // 2).start()
    cp_mem.start()
    for c in mlp_copies:
        c.start()
    for c in wo_copies:
        c.start()

    IMIN = jnp.iinfo(jnp.int32).min
    xb3 = xb_v.reshape(NSEG, SEG, D)
    keys[...] = jnp.full(keys.shape, IMIN, I32)
    yacc[...] = jnp.zeros(yacc.shape, F32)
    cp_wr.wait()

    def router_w():
        wr5 = wr_v[...].astype(F32)
        return jnp.concatenate([wr5[j:j + 1, :] for j in range(NT)], axis=1)

    def layernorm(s0, nseg, t0, nrow, slot, wr):
        n = nseg * nrow
        x = x_v[pl.ds(s0, nseg), t0:t0 + nrow, :].astype(F32).reshape(n, D)
        mu = jnp.sum(x, axis=-1, keepdims=True) * (1.0 / D)
        xc = x - mu
        var = jnp.sum(xc * xc, axis=-1, keepdims=True) * (1.0 / D)
        sd = _rb(jnp.sqrt(_rb(_rb(var) + EPS)))
        xn = _rb(_rb(x - _rb(mu)) / sd)
        xb3[pl.ds(s0, nseg), t0:t0 + nrow, :] = xn.reshape(nseg, nrow, D)
        r = _rb(jnp.sum(xn * wr, axis=-1, keepdims=True))
        r = jnp.where(r == 0.0, 0.0, r)
        bits = pltpu.bitcast(jnp.broadcast_to(r, (n, 128)), I32) >> 16
        mono = jnp.where(bits < 0, (-32768) - bits, bits)
        mono = jnp.where(r != r, -40000, mono)
        row = (jax.lax.broadcasted_iota(I32, (nseg, nrow, 128), 0) * SEG
               + jax.lax.broadcasted_iota(I32, (nseg, nrow, 128), 1)).reshape(n, 128)
        key = mono * 4096 + ((S - 1 - t0) - s0 * SEG - row)
        lane = jax.lax.broadcasted_iota(I32, (n, 128), 1)
        keys[0:n, :] = jnp.where(lane == slot, key, keys[0:n, :])
        return xn, key

    def ln8_body(b, carry):
        x8_copy(b).wait()
        xn, _ = layernorm(b * 16, 16, LIVE, 8, b, router_w())
        lhs_v[pl.ds(pl.multiple_of(b * 64, 64), 64), :] = pltpu.bitcast(xn.astype(BF16), U32)
        return carry

    jax.lax.fori_loop(0, 4, ln8_body, 0)

    def ln_seg(s, wr):
        xn, key = layernorm(s, 1, 0, LIVE, 4 + s, wr)
        xa_v[pl.ds(pl.multiple_of(s * LIVE, 8), LIVE), :] = xn
        return pltpu.bitcast(key, U32)

    def topk_round(c):
        kv = keys[...]
        mx = jnp.max(kv)
        keys[...] = jnp.where(kv == mx, IMIN, kv)
        idx = jnp.clip((S - 1) - (mx & 4095), 0, S - 1)
        idx_s[c] = idx
        sel[pl.ds(c, 1), :] = xb_v[pl.ds(idx, 1), :]

    def repack(k, par, slot, part=None, tie=None):
        m_lo = jnp.full((8, 128), 0xFFFF, U32)
        m_hi = jnp.full((8, 128), 0xFFFF0000, U32)
        if tie is not None:
            m_lo = jnp.where(k < 0, tie, m_lo)
            m_hi = jnp.where(k < 0, tie, m_hi)
        for u in range(2):
            rq = raw.at[2 * k + u]
            lo = w_eo[par].at[slot * 4 + 2 * u]
            hi = w_eo[par].at[slot * 4 + 2 * u + 1]
            for g in range(D // 16):
                if part is not None and (u * (D // 16) + g) % part[1] != part[0]:
                    continue
                a = rq[pl.ds(16 * g, 8, stride=2), :]
                b = rq[pl.ds(16 * g + 1, 8, stride=2), :]
                lo[8 * g:8 * g + 8, :] = (a & m_lo) | (b << 16)
                hi[8 * g:8 * g + 8, :] = (a >> 16) | (b & m_hi)

    def phase(k, par, slot, after_dot=None, side=None, nxt=None, tied=False):
        for u in range(4):
            for c in range(4):
                w = pltpu.bitcast(w_eo[par][slot * 4 + u], BF16)
                lhs = lhs_v[c * 64:(c + 1) * 64, :]
                if side is not None and c == 3:
                    tok = side(u)
                    n = tok.shape[0]
                    head = jnp.where(k < 0, tok, lhs[0:n, 0:128])
                    lhs = jnp.concatenate(
                        [jnp.concatenate([head, lhs[0:n, 128:]], axis=1), lhs[n:, :]], axis=0)
                r = _dot(pltpu.bitcast(lhs, BF16), w)
                pre[4 * k + u, c * 128:(c + 1) * 128, :] = r
                if after_dot is not None:
                    after_dot()
                if nxt is not None and u < 3:
                    repack(k + 1, 1 - par, nxt, (u * 4 + c, 12),
                           pltpu.bitcast(r[0:8, :], U32) if tied else None)

    def two_phases(i, after_dot=None, side=None):
        k = 2 * i + 1
        dyn = not isinstance(i, int)
        phase(k, 1, i, after_dot, side, i + 1)
        phase(k + 1, 0, i + 1, after_dot, None if side is None else (lambda u: side(4 + u)), i + 1, dyn)

    w_wait(0)
    repack(0, 0, 0)
    w_wait(1)
    repack(1, 1, 0)
    phase(0, 0, 0)

    def ln_body(i, carry):
        w_wait(2 * i + 2)
        w_wait(2 * i + 3)
        xa_copy(i).wait()
        wr = router_w()
        two_phases(i, side=lambda u: ln_seg(i * 8 + u, wr))
        return carry

    jax.lax.fori_loop(0, 8, ln_body, 0)

    w_wait(18)
    w_wait(19)
    for c in range(TOPC):
        topk_round(c)
    two_phases(8)

    for c in mlp_copies:
        c.wait()
    FP = FF // 2

    def mlp_body(t, carry):
        i = 9 + t
        w_wait(2 * i + 2)
        w_wait(2 * i + 3)
        f0 = pl.multiple_of(t * FP, 16)
        xs = sel[...]
        cuts = [(a_, min(a_ + 128, FP)) for a_ in range(0, FP, 128)]
        val = {}

        def up_tile(which, n, kt):
            def run():
                a_, b_ = cuts[n]
                w = (wg_v, wu_v)[which][pl.ds(f0 + a_, b_ - a_), kt * 128:(kt + 1) * 128]
                r = _dot_nt(xs[:, kt * 128:(kt + 1) * 128], w)
                val[which, n] = r if kt == 0 else val[which, n] + r
            return run

        def down_tile(n, j):
            def run():
                a_, b_ = cuts[n]
                if j == 0:
                    g_ = _rb(val.pop((0, n)))
                    val['h', n] = _rb(g_ * _sigmoid(g_)) * _rb(val.pop((1, n)))
                r = _dot(val['h', n], wd_v[pl.ds(f0 + a_, b_ - a_), j * 128:(j + 1) * 128])
                val['y', j] = r if n == 0 else val['y', j] + r
            return run

        jobs = [up_tile(which, n, kt) for n in range(len(cuts)) for which in range(2) for kt in range(NT)]
        jobs += [down_tile(n, j) for n in range(len(cuts)) for j in range(NT)]

        def after_dot():
            for _ in range(4):
                if jobs:
                    jobs.pop(0)()

        two_phases(i, after_dot=after_dot)
        yacc[...] += jnp.concatenate([val['y', j] for j in range(NT)], axis=1)
        return carry

    jax.lax.fori_loop(0, 2, mlp_body, 0)

    cp_mem.wait()
    acc[0:M, :] = mem0_v[...].astype(F32)
    acc[M:L, :] = jnp.zeros((SEG, D), F32)
    xs = sel[...]
    r_sel = _rb(jnp.sum(xs * router_w(), axis=-1, keepdims=True))
    sel[...] = xs + _rb(_rb(yacc[...]) * _rb(_sigmoid(r_sel)))
    for c in range(TOPC):
        xb_v[pl.ds(idx_s[c], 1), :] = sel[pl.ds(c, 1), :]
    phase(NPH - 1, 1, NPH // 2 - 1)

    for c in wo_copies:
        c.wait()

    qi = jax.lax.broadcasted_iota(I32, (L, L), 0)
    ki = jax.lax.broadcasted_iota(I32, (L, L), 1)
    mask = (qi < M) | (qi >= ki)
    scale = DH ** (-0.5)

    def finish(sp):
        r0 = pl.multiple_of(sp * SEG, SEG)
        sa = acc[M:L, :]
        xb = xb_v[pl.ds(r0, SEG), :]
        g = xb * _sigmoid(xb)
        out_v[pl.ds(r0, SEG), :] = (x_v[sp].astype(F32) + sa * g).astype(BF16)

    def out_copy(r0, n):
        return pltpu.make_async_copy(out_v.at[pl.ds(r0, n), :], out_hbm.at[pl.ds(r0, n), :], sem_out.at[0])

    def step(i, u):
        s = i * UNROLL + u
        pre_i = pre.at[:, pl.ds(pl.multiple_of(i * (8 * UNROLL), 8 * UNROLL), 8 * UNROLL), :]
        xa_i = xa_v.at[pl.ds(pl.multiple_of(i * (LIVE * UNROLL), 8 * UNROLL), LIVE * UNROLL), :]
        xa = xa_i[u * LIVE:(u + 1) * LIVE, :]
        lhs = jnp.concatenate([acc[0:M, :], xa], axis=0).astype(BF16)
        finish(jnp.maximum(s - 1, 0) if u == 0 else s - 1)

        def proj(j):
            t = _dot(lhs, pltpu.bitcast(wtile(j)[...], BF16))
            return jnp.concatenate([t, pre_i[j, u * 8:(u + 1) * 8, :]], axis=0)

        NG = H // GH
        qs, ks, vs, ps, os_ = {}, {}, {}, {}, {}

        def do_qkv(g):
            js = [m * H + h for h in range(g * GH, (g + 1) * GH) for m in range(3)]
            if g == 0:
                part = {}
                for kt in range(NT):
                    for j in js:
                        t = _dot(lhs[:, kt * 128:(kt + 1) * 128],
                                 pltpu.bitcast(wtile(j)[kt * 64:(kt + 1) * 64, :], BF16))
                        part[j] = t if kt == 0 else part[j] + t
                res = {j: jnp.concatenate([part[j], pre_i[j, u * 8:(u + 1) * 8, :]], axis=0) for j in js}
            else:
                res = {j: proj(j) for j in js}
            for h in range(g * GH, (g + 1) * GH):
                qs[h], ks[h], vs[h] = res[h], res[H + h], res[2 * H + h]

        def do_s(g):
            for h in range(g * GH, (g + 1) * GH):
                sc = _dot_nt(qs.pop(h), ks.pop(h)) * scale
                sc = jnp.where(mask, sc, NEG)
                e = jnp.exp(sc - jnp.max(sc, axis=-1, keepdims=True))
                ps[h] = e * (1.0 / jnp.sum(e, axis=-1, keepdims=True))

        def do_pv(g):
            for h in range(g * GH, (g + 1) * GH):
                os_[h] = _dot(ps.pop(h), vs.pop(h))

        def do_o(j, h0, h1):
            o = jnp.concatenate([os_[h] for h in range(h0, h1)], axis=1)
            return _dot(o, pltpu.bitcast(wo_p[j, h0 * 64:h1 * 64, :], BF16))

        for g in range(NG):
            do_qkv(g)
            if g >= 1:
                do_s(g - 1)
            if g >= 3:
                do_pv(g - 3)
        HS = (NG - 4) * GH

        def o1(j):
            acc[:, j * 128:(j + 1) * 128] = do_o(j, 0, HS)

        o1(0)
        do_s(NG - 1)
        do_pv(NG - 3)
        o1(1)
        do_pv(NG - 2)
        o1(2)
        o1(3)
        do_pv(NG - 1)
        o1(4)
        for j in range(NT):
            acc[:, j * 128:(j + 1) * 128] += do_o(j, HS, H)

    def multi(i, carry):
        for u in range(UNROLL):
            step(i, u)
        r0 = pl.multiple_of(i * (UNROLL * SEG), SEG)
        out_copy(r0, (UNROLL - 1) * SEG).start()

        @pl.when(i > 0)
        def _():
            out_copy(pl.multiple_of(r0 - SEG, SEG), SEG).start()
        return carry

    jax.lax.fori_loop(0, NSEG // UNROLL, multi, 0)
    finish(NSEG - 1)
    out_copy(S - SEG, SEG).start()
    out_copy(0, S).wait()


@jax.jit
def pallas_recurrent_scan__memory_aug_recurrent_mem_tr__moe_arch_mod__prompt_kernel(
    A_x: jax.Array,
    A_mem0: jax.Array,
    A_Wq: jax.Array,
    A_Wk: jax.Array,
    A_Wv: jax.Array,
    A_Wo: jax.Array,
    A_seg_len: jax.Array,
    B_x: jax.Array,
    B_w_r: jax.Array,
    B_w_gate: jax.Array,
    B_w_up: jax.Array,
    B_w_down: jax.Array,
):
    del A_seg_len, B_x
    assert A_x.shape == (1, S, D) and A_Wq.shape == (D, H, DH) and A_mem0.shape == (1, M, D)
    hbm = pl.BlockSpec(memory_space=pltpu.HBM)
    out = pl.pallas_call(
        _kernel,
        out_shape=jax.ShapeDtypeStruct((S, D), BF16),
        in_specs=[hbm] * 10,
        out_specs=hbm,
        scratch_shapes=[
            pltpu.VMEM((NSEG, SEG, D), BF16),
            pltpu.VMEM((NSEG * 4, D), U32),
            pltpu.VMEM((NSEG * LIVE, D), F32),
            pltpu.VMEM((S, D), F32),
            pltpu.VMEM((2 * NPH, D, 128), U32),
            pltpu.VMEM((2 * NPH, D // 2, 128), U32),
            pltpu.VMEM((2 * NPH, D // 2, 128), U32),
            pltpu.VMEM((NT, H * DH // 2, 128), U32),
            pltpu.VMEM((3 * H, NSEG * 8, DH), F32),
            pltpu.VMEM((FF, D), BF16),
            pltpu.VMEM((FF, D), BF16),
            pltpu.VMEM((FF, D), BF16),
            pltpu.VMEM((S, D), BF16),
            pltpu.VMEM((L, D), F32),
            pltpu.VMEM((TOPC, D), F32),
            pltpu.VMEM((TOPC, D), F32),
            pltpu.VMEM((128, 128), I32),
            pltpu.VMEM((M, D), BF16),
            pltpu.VMEM((NT, 128), BF16),
            pltpu.SMEM((TOPC,), I32),
            pltpu.SemaphoreType.DMA((16 + NPH,)),
            pltpu.SemaphoreType.DMA((1,)),
        ],
        compiler_params=pltpu.CompilerParams(vmem_limit_bytes=110 * 1024 * 1024),
    )(
        A_x.reshape(NSEG, SEG, D),
        A_mem0.reshape(M, D),
        A_Wq, A_Wk, A_Wv,
        A_Wo.reshape(H * DH, D),
        B_w_r.reshape(NT, 128),
        B_w_gate.T, B_w_up.T, B_w_down,
    )
    return out.reshape(1, S, D)
```

```python
import functools
import math

import jax
import jax.numpy as jnp
import jax.experimental.pallas as pl
import jax.experimental.pallas.tpu as pltpu

F32 = jnp.float32
BF16 = jnp.bfloat16
U32 = jnp.uint32
I32 = jnp.int32

S = 2048
D = 640
H = 32
DH = 128
M = 8
SEG = 32
NSEG = S // SEG
L = M + SEG
FF = 1728
TOPC = 8
NT = D // 128
LIVE = SEG - 8
EPS = 1e-05
NEG = -1000000000.0
UNROLL = 4
TIE0 = 2
NPH = 24
GH = 2


def _dot(a, b):
    return jax.lax.dot_general(a, b, (((1,), (0,)), ((), ())), preferred_element_type=F32)


def _dot_nt(a, b):
    return jax.lax.dot_general(a, b, (((1,), (1,)), ((), ())), preferred_element_type=F32)


def _rb(x):
    return x.astype(BF16).astype(F32)


def _sigmoid(x):
    return pl.reciprocal(1.0 + jnp.exp(-x), approx=True)


def _kernel(x_hbm, mem0_hbm, wq_hbm, wk_hbm, wv_hbm, wo_hbm, wr_hbm, wg_hbm, wu_hbm, wd_hbm,
            out_hbm,
            x_v, lhs_v, xa_v, xb_v, raw, w_ev, w_od, wo_p, pre, wg_v, wu_v, wd_v,
            out_v, acc, part_v, sel, yacc, keys, mem0_v, wr_v, idx_s,
            sem_in, sem_out):
    w_hbm = [wq_hbm, wk_hbm, wv_hbm]
    w_eo = [w_ev, w_od]

    def wtile(j):
        return w_eo[(j // 4) % 2].at[(j // 8) * 4 + j % 4]

    SEM_X8, SEM_XA, SEM_W = 4, 8, 16

    def w_start(k):
        for q in (2 * k, 2 * k + 1):
            src = w_hbm[q // 16].bitcast(U32).at[:, q % 16, :]
            pltpu.make_async_copy(src, raw.at[q], sem_in.at[SEM_W + k]).start()

    def w_wait(k):
        both = raw.at[pl.ds(2 * k, 2)]
        pltpu.make_async_copy(both, both, sem_in.at[SEM_W + k]).wait()

    def x8_copy(b):
        return pltpu.make_async_copy(x_hbm.at[pl.ds(b * 16, 16), pl.ds(LIVE, 8), :],
                                     x_v.at[pl.ds(b * 16, 16), pl.ds(LIVE, 8), :], sem_in.at[SEM_X8 + b])

    def xa_copy(i):
        return pltpu.make_async_copy(x_hbm.at[pl.ds(i * 8, 8), pl.ds(0, LIVE), :],
                                     x_v.at[pl.ds(i * 8, 8), pl.ds(0, LIVE), :], sem_in.at[SEM_XA + i])

    cp_wr = pltpu.make_async_copy(wr_hbm, wr_v, sem_in.at[0])
    cp_mem = pltpu.make_async_copy(mem0_hbm, mem0_v, sem_in.at[1])
    mlp_copies = [pltpu.make_async_copy(s_, d_, sem_in.at[2])
                  for s_, d_ in [(wg_hbm, wg_v), (wu_hbm, wu_v), (wd_hbm, wd_v)]]
    wo32 = wo_hbm.bitcast(U32)
    wo_copies = [pltpu.make_async_copy(wo32.at[:, pl.ds(j * 128, 128)], wo_p.at[j], sem_in.at[3])
                 for j in range(NT)]

    cp_wr.start()
    for b in range(4):
        x8_copy(b).start()
    for k in range(NPH):
        w_start(k)
        if k >= 3 and k % 2 == 1 and (k - 3) // 2 < 8:
            xa_copy((k - 3) // 2).start()
    cp_mem.start()
    for c in mlp_copies:
        c.start()
    for c in wo_copies:
        c.start()

    IMIN = jnp.iinfo(jnp.int32).min
    xb3 = xb_v.reshape(NSEG, SEG, D)
    keys[...] = jnp.full(keys.shape, IMIN, I32)
    yacc[...] = jnp.zeros(yacc.shape, F32)
    cp_wr.wait()

    def router_w():
        wr5 = wr_v[...].astype(F32)
        return jnp.concatenate([wr5[j:j + 1, :] for j in range(NT)], axis=1)

    def layernorm(s0, nseg, t0, nrow, slot, wr):
        n = nseg * nrow
        x = x_v[pl.ds(s0, nseg), t0:t0 + nrow, :].astype(F32).reshape(n, D)
        mu = jnp.sum(x, axis=-1, keepdims=True) * (1.0 / D)
        xc = x - mu
        var = jnp.sum(xc * xc, axis=-1, keepdims=True) * (1.0 / D)
        sd = _rb(jnp.sqrt(_rb(_rb(var) + EPS)))
        xn = _rb(_rb(x - _rb(mu)) / sd)
        xb3[pl.ds(s0, nseg), t0:t0 + nrow, :] = xn.reshape(nseg, nrow, D)
        r = _rb(jnp.sum(xn * wr, axis=-1, keepdims=True))
        r = jnp.where(r == 0.0, 0.0, r)
        bits = pltpu.bitcast(jnp.broadcast_to(r, (n, 128)), I32) >> 16
        mono = jnp.where(bits < 0, (-32768) - bits, bits)
        mono = jnp.where(r != r, -40000, mono)
        row = (jax.lax.broadcasted_iota(I32, (nseg, nrow, 128), 0) * SEG
               + jax.lax.broadcasted_iota(I32, (nseg, nrow, 128), 1)).reshape(n, 128)
        key = mono * 4096 + ((S - 1 - t0) - s0 * SEG - row)
        lane = jax.lax.broadcasted_iota(I32, (n, 128), 1)
        keys[0:n, :] = jnp.where(lane == slot, key, keys[0:n, :])
        return xn, key

    def ln8_body(b, carry):
        x8_copy(b).wait()
        xn, _ = layernorm(b * 16, 16, LIVE, 8, b, router_w())
        lhs_v[pl.ds(pl.multiple_of(b * 64, 64), 64), :] = pltpu.bitcast(xn.astype(BF16), U32)
        return carry

    jax.lax.fori_loop(0, 4, ln8_body, 0)

    def ln_seg(s, wr):
        xn, key = layernorm(s, 1, 0, LIVE, 4 + s, wr)
        xa_v[pl.ds(pl.multiple_of(s * LIVE, 8), LIVE), :] = xn
        return pltpu.bitcast(key, U32)

    def topk_round(c):
        kv = keys[...]
        mx = jnp.max(kv)
        keys[...] = jnp.where(kv == mx, IMIN, kv)
        idx = jnp.clip((S - 1) - (mx & 4095), 0, S - 1)
        idx_s[c] = idx
        sel[pl.ds(c, 1), :] = xb_v[pl.ds(idx, 1), :]

    def repack(k, par, slot, part=None, tie=None):
        m_lo = jnp.full((8, 128), 0xFFFF, U32)
        m_hi = jnp.full((8, 128), 0xFFFF0000, U32)
        if tie is not None:
            m_lo = jnp.where(k < 0, tie, m_lo)
            m_hi = jnp.where(k < 0, tie, m_hi)
        for u in range(2):
            rq = raw.at[2 * k + u]
            lo = w_eo[par].at[slot * 4 + 2 * u]
            hi = w_eo[par].at[slot * 4 + 2 * u + 1]
            for g in range(D // 16):
                if part is not None and (u * (D // 16) + g) % part[1] != part[0]:
                    continue
                a = rq[pl.ds(16 * g, 8, stride=2), :]
                b = rq[pl.ds(16 * g + 1, 8, stride=2), :]
                lo[8 * g:8 * g + 8, :] = (a & m_lo) | (b << 16)
                hi[8 * g:8 * g + 8, :] = (a >> 16) | (b & m_hi)

    def phase(k, par, slot, after_dot=None, side=None, nxt=None, tied=False):
        for u in range(4):
            for c in range(4):
                w = pltpu.bitcast(w_eo[par][slot * 4 + u], BF16)
                lhs = lhs_v[c * 64:(c + 1) * 64, :]
                if side is not None and c == 3:
                    tok = side(u)
                    n = tok.shape[0]
                    head = jnp.where(k < 0, tok, lhs[0:n, 0:128])
                    lhs = jnp.concatenate(
                        [jnp.concatenate([head, lhs[0:n, 128:]], axis=1), lhs[n:, :]], axis=0)
                r = _dot(pltpu.bitcast(lhs, BF16), w)
                pre[4 * k + u, c * 128:(c + 1) * 128, :] = r
                if after_dot is not None:
                    after_dot()
                if nxt is not None and u < 3:
                    repack(k + 1, 1 - par, nxt, (u * 4 + c, 12),
                           pltpu.bitcast(r[0:8, :], U32) if tied else None)

    def two_phases(i, after_dot=None, side=None):
        k = 2 * i + 1
        dyn = not isinstance(i, int)
        phase(k, 1, i, after_dot, side, i + 1)
        phase(k + 1, 0, i + 1, after_dot, None if side is None else (lambda u: side(4 + u)), i + 1, dyn)

    w_wait(0)
    repack(0, 0, 0)
    w_wait(1)
    repack(1, 1, 0)
    phase(0, 0, 0)

    def ln_body(i, carry):
        w_wait(2 * i + 2)
        w_wait(2 * i + 3)
        xa_copy(i).wait()
        wr = router_w()
        two_phases(i, side=lambda u: ln_seg(i * 8 + u, wr))
        return carry

    jax.lax.fori_loop(0, 8, ln_body, 0)

    w_wait(18)
    w_wait(19)
    for c in range(TOPC):
        topk_round(c)
    two_phases(8)

    for c in mlp_copies:
        c.wait()
    FP = FF // 2

    def mlp_body(t, carry):
        i = 9 + t
        w_wait(2 * i + 2)
        w_wait(2 * i + 3)
        f0 = pl.multiple_of(t * FP, 16)
        xs = sel[...]
        cuts = [(a_, min(a_ + 128, FP)) for a_ in range(0, FP, 128)]
        val = {}

        def up_tile(which, n, kt):
            def run():
                a_, b_ = cuts[n]
                w = (wg_v, wu_v)[which][pl.ds(f0 + a_, b_ - a_), kt * 128:(kt + 1) * 128]
                r = _dot_nt(xs[:, kt * 128:(kt + 1) * 128], w)
                val[which, n] = r if kt == 0 else val[which, n] + r
            return run

        def down_tile(n, j):
            def run():
                a_, b_ = cuts[n]
                if j == 0:
                    g_ = _rb(val.pop((0, n)))
                    val['h', n] = _rb(g_ * _sigmoid(g_)) * _rb(val.pop((1, n)))
                r = _dot(val['h', n], wd_v[pl.ds(f0 + a_, b_ - a_), j * 128:(j + 1) * 128])
                val['y', j] = r if n == 0 else val['y', j] + r
            return run

        jobs = [up_tile(which, n, kt) for n in range(len(cuts)) for which in range(2) for kt in range(NT)]
        jobs += [down_tile(n, j) for n in range(len(cuts)) for j in range(NT)]

        def after_dot():
            for _ in range(4):
                if jobs:
                    jobs.pop(0)()

        two_phases(i, after_dot=after_dot)
        yacc[...] += jnp.concatenate([val['y', j] for j in range(NT)], axis=1)
        return carry

    jax.lax.fori_loop(0, 2, mlp_body, 0)

    cp_mem.wait()
    acc[0:M, :] = mem0_v[...].astype(F32)
    acc[M:L, :] = jnp.zeros((SEG, D), F32)
    xs = sel[...]
    r_sel = _rb(jnp.sum(xs * router_w(), axis=-1, keepdims=True))
    sel[...] = xs + _rb(_rb(yacc[...]) * _rb(_sigmoid(r_sel)))
    for c in range(TOPC):
        xb_v[pl.ds(idx_s[c], 1), :] = sel[pl.ds(c, 1), :]
    phase(NPH - 1, 1, NPH // 2 - 1)

    for c in wo_copies:
        c.wait()

    qi = jax.lax.broadcasted_iota(I32, (L, L), 0)
    ki = jax.lax.broadcasted_iota(I32, (L, L), 1)
    mask = (qi < M) | (qi >= ki)
    scale = DH ** (-0.5)

    def finish(sp, sa):
        r0 = pl.multiple_of(sp * SEG, SEG)
        xb = xb_v[pl.ds(r0, SEG), :]
        g = xb * _sigmoid(xb)
        o = x_v[sp].astype(F32) + sa * g
        out_v[pl.ds(r0, SEG), :] = o.astype(BF16)
        return o

    def out_copy(r0, n):
        return pltpu.make_async_copy(out_v.at[pl.ds(r0, n), :], out_hbm.at[pl.ds(r0, n), :], sem_out.at[0])

    def step(i, u, prev):
        s = i * UNROLL + u
        pre_i = pre.at[:, pl.ds(pl.multiple_of(i * (8 * UNROLL), 8 * UNROLL), 8 * UNROLL), :]
        xa_i = xa_v.at[pl.ds(pl.multiple_of(i * (LIVE * UNROLL), 8 * UNROLL), LIVE * UNROLL), :]
        xa = xa_i[u * LIVE:(u + 1) * LIVE, :]
        lhs = jnp.concatenate([prev[0:M, :], xa], axis=0).astype(BF16)
        fin = finish(jnp.maximum(s - 1, 0) if u == 0 else s - 1, prev[M:L, :])

        def proj(j):
            t = _dot(lhs, pltpu.bitcast(wtile(j)[...], BF16))
            if u == 0 and TIE0 <= j < TIE0 + NT:
                t = jnp.where(i < 0, fin[:, (j - TIE0) * 128:(j - TIE0 + 1) * 128], t)
            return jnp.concatenate([t, pre_i[j, u * 8:(u + 1) * 8, :]], axis=0)

        NG = H // GH
        qs, ks, vs, ps, os_ = {}, {}, {}, {}, {}

        def do_qkv(g):
            js = [m * H + h for h in range(g * GH, (g + 1) * GH) for m in range(3)]
            if g == 0:
                part = {}
                for kt in range(NT):
                    for j in js:
                        t = _dot(lhs[:, kt * 128:(kt + 1) * 128],
                                 pltpu.bitcast(wtile(j)[kt * 64:(kt + 1) * 64, :], BF16))
                        part[j] = t if kt == 0 else part[j] + t
                res = {j: jnp.concatenate([part[j], pre_i[j, u * 8:(u + 1) * 8, :]], axis=0) for j in js}
            else:
                res = {j: proj(j) for j in js}
            for h in range(g * GH, (g + 1) * GH):
                qs[h], ks[h], vs[h] = res[h], res[H + h], res[2 * H + h]

        def do_s(g):
            for h in range(g * GH, (g + 1) * GH):
                sc = _dot_nt(qs.pop(h), ks.pop(h)) * scale
                sc = jnp.where(mask, sc, NEG)
                e = jnp.exp(sc - jnp.max(sc, axis=-1, keepdims=True))
                ps[h] = e * pl.reciprocal(jnp.sum(e, axis=-1, keepdims=True), approx=True)

        def do_pv(g):
            for h in range(g * GH, (g + 1) * GH):
                os_[h] = _dot(ps.pop(h), vs.pop(h))

        def do_o(j, h0, h1):
            o = jnp.concatenate([os_[h] for h in range(h0, h1)], axis=1)
            return _dot(o, pltpu.bitcast(wo_p[j, h0 * 64:h1 * 64, :], BF16))

        for g in range(NG):
            do_qkv(g)
            if g >= 1:
                do_s(g - 1)
            if g >= 3:
                do_pv(g - 3)
        HS = (NG - 4) * GH

        def o1(j):
            part_v[:, j * 128:(j + 1) * 128] = do_o(j, 0, HS)

        o1(0)
        do_s(NG - 1)
        do_pv(NG - 3)
        o1(1)
        do_pv(NG - 2)
        o1(2)
        o1(3)
        do_pv(NG - 1)
        o1(4)
        return jnp.concatenate(
            [part_v[:, j * 128:(j + 1) * 128] + do_o(j, HS, H) for j in range(NT)], axis=1)

    def multi(i, carry):
        cur = acc[...]
        for u in range(UNROLL):
            cur = step(i, u, cur)
        acc[...] = cur
        r0 = pl.multiple_of(i * (UNROLL * SEG), SEG)
        out_copy(r0, (UNROLL - 1) * SEG).start()

        @pl.when(i > 0)
        def _():
            out_copy(pl.multiple_of(r0 - SEG, SEG), SEG).start()
        return carry

    jax.lax.fori_loop(0, NSEG // UNROLL, multi, 0)
    finish(NSEG - 1, acc[M:L, :])
    out_copy(S - SEG, SEG).start()
    out_copy(0, S).wait()


@jax.jit
def pallas_recurrent_scan__memory_aug_recurrent_mem_tr__moe_arch_mod__prompt_kernel(
    A_x: jax.Array,
    A_mem0: jax.Array,
    A_Wq: jax.Array,
    A_Wk: jax.Array,
    A_Wv: jax.Array,
    A_Wo: jax.Array,
    A_seg_len: jax.Array,
    B_x: jax.Array,
    B_w_r: jax.Array,
    B_w_gate: jax.Array,
    B_w_up: jax.Array,
    B_w_down: jax.Array,
):
    del A_seg_len, B_x
    assert A_x.shape == (1, S, D) and A_Wq.shape == (D, H, DH) and A_mem0.shape == (1, M, D)
    hbm = pl.BlockSpec(memory_space=pltpu.HBM)
    out = pl.pallas_call(
        _kernel,
        out_shape=jax.ShapeDtypeStruct((S, D), BF16),
        in_specs=[hbm] * 10,
        out_specs=hbm,
        scratch_shapes=[
            pltpu.VMEM((NSEG, SEG, D), BF16),
            pltpu.VMEM((NSEG * 4, D), U32),
            pltpu.VMEM((NSEG * LIVE, D), F32),
            pltpu.VMEM((S, D), F32),
            pltpu.VMEM((2 * NPH, D, 128), U32),
            pltpu.VMEM((2 * NPH, D // 2, 128), U32),
            pltpu.VMEM((2 * NPH, D // 2, 128), U32),
            pltpu.VMEM((NT, H * DH // 2, 128), U32),
            pltpu.VMEM((3 * H, NSEG * 8, DH), F32),
            pltpu.VMEM((FF, D), BF16),
            pltpu.VMEM((FF, D), BF16),
            pltpu.VMEM((FF, D), BF16),
            pltpu.VMEM((S, D), BF16),
            pltpu.VMEM((L, D), F32),
            pltpu.VMEM((L, D), F32),
            pltpu.VMEM((TOPC, D), F32),
            pltpu.VMEM((TOPC, D), F32),
            pltpu.VMEM((128, 128), I32),
            pltpu.VMEM((M, D), BF16),
            pltpu.VMEM((NT, 128), BF16),
            pltpu.SMEM((TOPC,), I32),
            pltpu.SemaphoreType.DMA((16 + NPH,)),
            pltpu.SemaphoreType.DMA((1,)),
        ],
        compiler_params=pltpu.CompilerParams(vmem_limit_bytes=110 * 1024 * 1024),
    )(
        A_x.reshape(NSEG, SEG, D),
        A_mem0.reshape(M, D),
        A_Wq, A_Wk, A_Wv,
        A_Wo.reshape(H * DH, D),
        B_w_r.reshape(NT, 128),
        B_w_gate.T, B_w_up.T, B_w_down,
    )
    return out.reshape(1, S, D)
```

```python
import functools
import math

import jax
import jax.numpy as jnp
import jax.experimental.pallas as pl
import jax.experimental.pallas.tpu as pltpu

F32 = jnp.float32
BF16 = jnp.bfloat16
U32 = jnp.uint32
I32 = jnp.int32

S = 2048
D = 640
H = 32
DH = 128
M = 8
SEG = 32
NSEG = S // SEG
L = M + SEG
FF = 1728
TOPC = 8
NT = D // 128
LIVE = SEG - 8
EPS = 1e-05
NEG = -1000000000.0
UNROLL = 4
NKV = 32
LOG2E = math.log2(math.e)
TIE0 = 2
NPH = 24
TA, TB, TL = 1, 4, 3
SEQ = False
HALF = False
BQ, BK, BP, BV = 1, 1, 1, 1
GH = 2


def _dot(a, b):
    return jax.lax.dot_general(a, b, (((1,), (0,)), ((), ())), preferred_element_type=F32)


def _dot_nt(a, b):
    return jax.lax.dot_general(a, b, (((1,), (1,)), ((), ())), preferred_element_type=F32)


def _rb(x):
    return x.astype(BF16).astype(F32)


def _sigmoid(x):
    return pl.reciprocal(1.0 + jnp.exp(-x), approx=True)


def _tree(f, xs):
    while len(xs) > 1:
        xs = [f(xs[n], xs[n + 1]) if n + 1 < len(xs) else xs[n] for n in range(0, len(xs), 2)]
    return xs[0]


def _kernel(x_hbm, mem0_hbm, wq_hbm, wk_hbm, wv_hbm, wo_hbm, wr_hbm, wg_hbm, wu_hbm, wd_hbm,
            out_hbm,
            x_v, lhs_v, xa_v, xb_v, raw, w_ev, w_od, wo_p, pre, wg_v, wu_v, wd_v,
            out_v, acc, part_v, kv_s, sel, yacc, keys, mem0_v, wr_v, idx_s,
            sem_in, sem_out):
    w_hbm = [wq_hbm, wk_hbm, wv_hbm]
    w_eo = [w_ev, w_od]

    def wtile(j):
        return w_eo[(j // 4) % 2].at[(j // 8) * 4 + j % 4]

    SEM_X8, SEM_XA, SEM_W = 4, 8, 16

    def w_start(k):
        for q in (2 * k, 2 * k + 1):
            src = w_hbm[q // 16].bitcast(U32).at[:, q % 16, :]
            pltpu.make_async_copy(src, raw.at[q], sem_in.at[SEM_W + k]).start()

    def w_wait(k):
        both = raw.at[pl.ds(2 * k, 2)]
        pltpu.make_async_copy(both, both, sem_in.at[SEM_W + k]).wait()

    def x8_copy(b):
        return pltpu.make_async_copy(x_hbm.at[pl.ds(b * 16, 16), pl.ds(LIVE, 8), :],
                                     x_v.at[pl.ds(b * 16, 16), pl.ds(LIVE, 8), :], sem_in.at[SEM_X8 + b])

    def xa_copy(i):
        return pltpu.make_async_copy(x_hbm.at[pl.ds(i * 8, 8), pl.ds(0, LIVE), :],
                                     x_v.at[pl.ds(i * 8, 8), pl.ds(0, LIVE), :], sem_in.at[SEM_XA + i])

    cp_wr = pltpu.make_async_copy(wr_hbm, wr_v, sem_in.at[0])
    cp_mem = pltpu.make_async_copy(mem0_hbm, mem0_v, sem_in.at[1])
    mlp_copies = [pltpu.make_async_copy(s_, d_, sem_in.at[2])
                  for s_, d_ in [(wg_hbm, wg_v), (wu_hbm, wu_v), (wd_hbm, wd_v)]]
    wo32 = wo_hbm.bitcast(U32)
    wo_copies = [pltpu.make_async_copy(wo32.at[:, pl.ds(j * 128, 128)], wo_p.at[j], sem_in.at[3])
                 for j in range(NT)]

    cp_wr.start()
    for b in range(4):
        x8_copy(b).start()
    for k in range(NPH):
        w_start(k)
        if k >= 3 and k % 2 == 1 and (k - 3) // 2 < 8:
            xa_copy((k - 3) // 2).start()
    cp_mem.start()
    for c in mlp_copies:
        c.start()
    for c in wo_copies:
        c.start()

    IMIN = jnp.iinfo(jnp.int32).min
    xb3 = xb_v.reshape(NSEG, SEG, D)
    keys[...] = jnp.full(keys.shape, IMIN, I32)
    yacc[...] = jnp.zeros(yacc.shape, F32)
    cp_wr.wait()

    def router_w():
        wr5 = wr_v[...].astype(F32)
        return jnp.concatenate([wr5[j:j + 1, :] for j in range(NT)], axis=1)

    def layernorm(s0, nseg, t0, nrow, slot, wr):
        n = nseg * nrow
        x = x_v[pl.ds(s0, nseg), t0:t0 + nrow, :].astype(F32).reshape(n, D)
        mu = jnp.sum(x, axis=-1, keepdims=True) * (1.0 / D)
        xc = x - mu
        var = jnp.sum(xc * xc, axis=-1, keepdims=True) * (1.0 / D)
        sd = _rb(jnp.sqrt(_rb(_rb(var) + EPS)))
        xn = _rb(_rb(x - _rb(mu)) / sd)
        xb3[pl.ds(s0, nseg), t0:t0 + nrow, :] = xn.reshape(nseg, nrow, D)
        r = _rb(jnp.sum(xn * wr, axis=-1, keepdims=True))
        r = jnp.where(r == 0.0, 0.0, r)
        bits = pltpu.bitcast(jnp.broadcast_to(r, (n, 128)), I32) >> 16
        mono = jnp.where(bits < 0, (-32768) - bits, bits)
        mono = jnp.where(r != r, -40000, mono)
        row = (jax.lax.broadcasted_iota(I32, (nseg, nrow, 128), 0) * SEG
               + jax.lax.broadcasted_iota(I32, (nseg, nrow, 128), 1)).reshape(n, 128)
        key = mono * 4096 + ((S - 1 - t0) - s0 * SEG - row)
        lane = jax.lax.broadcasted_iota(I32, (n, 128), 1)
        keys[0:n, :] = jnp.where(lane == slot, key, keys[0:n, :])
        return xn, key

    def ln8_body(b, carry):
        x8_copy(b).wait()
        xn, _ = layernorm(b * 16, 16, LIVE, 8, b, router_w())
        lhs_v[pl.ds(pl.multiple_of(b * 64, 64), 64), :] = pltpu.bitcast(xn.astype(BF16), U32)
        return carry

    jax.lax.fori_loop(0, 4, ln8_body, 0)

    def ln_seg(s, wr):
        xn, key = layernorm(s, 1, 0, LIVE, 4 + s, wr)
        xa_v[pl.ds(pl.multiple_of(s * LIVE, 8), LIVE), :] = xn
        return pltpu.bitcast(key, U32)

    def topk_round(c):
        kv = keys[...]
        mx = jnp.max(kv)
        keys[...] = jnp.where(kv == mx, IMIN, kv)
        idx = jnp.clip((S - 1) - (mx & 4095), 0, S - 1)
        idx_s[c] = idx
        sel[pl.ds(c, 1), :] = xb_v[pl.ds(idx, 1), :]

    def repack(k, par, slot, part=None, tie=None):
        m_lo = jnp.full((8, 128), 0xFFFF, U32)
        m_hi = jnp.full((8, 128), 0xFFFF0000, U32)
        if tie is not None:
            m_lo = jnp.where(k < 0, tie, m_lo)
            m_hi = jnp.where(k < 0, tie, m_hi)
        for u in range(2):
            rq = raw.at[2 * k + u]
            lo = w_eo[par].at[slot * 4 + 2 * u]
            hi = w_eo[par].at[slot * 4 + 2 * u + 1]
            for g in range(D // 16):
                if part is not None and (u * (D // 16) + g) % part[1] != part[0]:
                    continue
                a = rq[pl.ds(16 * g, 8, stride=2), :]
                b = rq[pl.ds(16 * g + 1, 8, stride=2), :]
                lo[8 * g:8 * g + 8, :] = (a & m_lo) | (b << 16)
                hi[8 * g:8 * g + 8, :] = (a >> 16) | (b & m_hi)

    def phase(k, par, slot, after_dot=None, side=None, nxt=None, tied=False):
        for u in range(4):
            for c in range(4):
                w = pltpu.bitcast(w_eo[par][slot * 4 + u], BF16)
                lhs = lhs_v[c * 64:(c + 1) * 64, :]
                if side is not None and c == 3:
                    tok = side(u)
                    n = tok.shape[0]
                    head = jnp.where(k < 0, tok, lhs[0:n, 0:128])
                    lhs = jnp.concatenate(
                        [jnp.concatenate([head, lhs[0:n, 128:]], axis=1), lhs[n:, :]], axis=0)
                r = _dot(pltpu.bitcast(lhs, BF16), w)
                pre[4 * k + u, c * 128:(c + 1) * 128, :] = r
                if after_dot is not None:
                    after_dot()
                if nxt is not None and u < 3:
                    repack(k + 1, 1 - par, nxt, (u * 4 + c, 12),
                           pltpu.bitcast(r[0:8, :], U32) if tied else None)

    def two_phases(i, after_dot=None, side=None):
        k = 2 * i + 1
        dyn = not isinstance(i, int)
        phase(k, 1, i, after_dot, side, i + 1)
        phase(k + 1, 0, i + 1, after_dot, None if side is None else (lambda u: side(4 + u)), i + 1, dyn)

    w_wait(0)
    repack(0, 0, 0)
    w_wait(1)
    repack(1, 1, 0)
    phase(0, 0, 0)

    def ln_body(i, carry):
        w_wait(2 * i + 2)
        w_wait(2 * i + 3)
        xa_copy(i).wait()
        wr = router_w()
        two_phases(i, side=lambda u: ln_seg(i * 8 + u, wr))
        return carry

    jax.lax.fori_loop(0, 8, ln_body, 0)

    w_wait(18)
    w_wait(19)
    for c in range(TOPC):
        topk_round(c)
    two_phases(8)

    for c in mlp_copies:
        c.wait()
    FP = FF // 2

    def mlp_body(t, carry):
        i = 9 + t
        w_wait(2 * i + 2)
        w_wait(2 * i + 3)
        f0 = pl.multiple_of(t * FP, 16)
        xs = sel[...]
        cuts = [(a_, min(a_ + 128, FP)) for a_ in range(0, FP, 128)]
        val = {}

        def up_tile(which, n, kt):
            def run():
                a_, b_ = cuts[n]
                w = (wg_v, wu_v)[which][pl.ds(f0 + a_, b_ - a_), kt * 128:(kt + 1) * 128]
                r = _dot_nt(xs[:, kt * 128:(kt + 1) * 128], w)
                val[which, n] = r if kt == 0 else val[which, n] + r
            return run

        def down_tile(n, j):
            def run():
                a_, b_ = cuts[n]
                if j == 0:
                    g_ = _rb(val.pop((0, n)))
                    val['h', n] = _rb(g_ * _sigmoid(g_)) * _rb(val.pop((1, n)))
                r = _dot(val['h', n], wd_v[pl.ds(f0 + a_, b_ - a_), j * 128:(j + 1) * 128])
                val['y', j] = r if n == 0 else val['y', j] + r
            return run

        jobs = [up_tile(which, n, kt) for n in range(len(cuts)) for which in range(2) for kt in range(NT)]
        jobs += [down_tile(n, j) for n in range(len(cuts)) for j in range(NT)]

        def after_dot():
            for _ in range(4):
                if jobs:
                    jobs.pop(0)()

        two_phases(i, after_dot=after_dot)
        yacc[...] += jnp.concatenate([val['y', j] for j in range(NT)], axis=1)
        return carry

    jax.lax.fori_loop(0, 2, mlp_body, 0)

    cp_mem.wait()
    acc[0:M, :] = mem0_v[...].astype(F32)
    acc[M:L, :] = jnp.zeros((SEG, D), F32)
    xs = sel[...]
    r_sel = _rb(jnp.sum(xs * router_w(), axis=-1, keepdims=True))
    sel[...] = xs + _rb(_rb(yacc[...]) * _rb(_sigmoid(r_sel)))
    for c in range(TOPC):
        xb_v[pl.ds(idx_s[c], 1), :] = sel[pl.ds(c, 1), :]
    phase(NPH - 1, 1, NPH // 2 - 1)

    for c in wo_copies:
        c.wait()

    qi = jax.lax.broadcasted_iota(I32, (L, L), 0)
    ki = jax.lax.broadcasted_iota(I32, (L, L), 1)
    mask = (qi < M) | (qi >= ki)
    scale = DH ** (-0.5)
    qm_i = jax.lax.broadcasted_iota(I32, (L - 8, L), 0)
    mask_m = (qm_i < M) | (qm_i + 8 >= jax.lax.broadcasted_iota(I32, (L - 8, L), 1))
    sub = jax.lax.broadcasted_iota(I32, (8, DH), 0)

    def finish(sp, sa):
        r0 = pl.multiple_of(sp * SEG, SEG)
        xb = xb_v[pl.ds(r0, SEG), :]
        g = xb * _sigmoid(xb)
        o = x_v[sp].astype(F32) + sa * g
        out_v[pl.ds(r0, SEG), :] = o.astype(BF16)
        return o

    def out_copy(r0, n):
        return pltpu.make_async_copy(out_v.at[pl.ds(r0, n), :], out_hbm.at[pl.ds(r0, n), :], sem_out.at[0])

    def step(i, u, prev):
        s = i * UNROLL + u
        pre_i = pre.at[:, pl.ds(pl.multiple_of(i * (8 * UNROLL), 8 * UNROLL), 8 * UNROLL), :]
        xa_i = xa_v.at[pl.ds(pl.multiple_of(i * (LIVE * UNROLL), 8 * UNROLL), LIVE * UNROLL), :]
        xa = xa_i[u * LIVE:(u + 1) * LIVE, :]
        lhs = jnp.concatenate([prev[0:M, :], xa], axis=0).astype(BF16)
        fin = finish(jnp.maximum(s - 1, 0) if u == 0 else s - 1, prev[M:L, :])

        def proj(j, tie=None):
            lh = lhs
            if tie is not None:
                top = pltpu.bitcast(lhs[0:16, 0:128], U32)
                top = pltpu.bitcast(jnp.where(i < 0, pltpu.bitcast(tie, U32), top), BF16)
                lh = jnp.concatenate([jnp.concatenate([top, lhs[0:16, 128:]], axis=1), lhs[16:, :]], axis=0)
            t = _dot(lh, pltpu.bitcast(wtile(j)[...], BF16))
            if u == 0 and TIE0 <= j < TIE0 + NT:
                t = jnp.where(i < 0, fin[:, (j - TIE0) * 128:(j - TIE0 + 1) * 128], t)
            return jnp.concatenate([t, pre_i[j, u * 8:(u + 1) * 8, :]], axis=0)

        NG = H // GH
        qs, ks, vs, ps, os_, ox = {}, {}, {}, {}, {}, {}

        def do_qkv(g):
            js = [m * H + h for h in range(g * GH, (g + 1) * GH) for m in range(3)]
            if g == 0:
                part = {}
                for kt in range(NT):
                    for j in js:
                        t = _dot(lhs[:, kt * 128:(kt + 1) * 128],
                                 pltpu.bitcast(wtile(j)[kt * 64:(kt + 1) * 64, :], BF16))
                        part[j] = t if kt == 0 else part[j] + t
                res = {j: jnp.concatenate([part[j], pre_i[j, u * 8:(u + 1) * 8, :]], axis=0) for j in js}
            else:
                res = {}
                for n, j in enumerate(js):
                    tie = None
                    for hh, pos in ((0, TA), (1, TB)):
                        if n == pos and g >= TL:
                            tie = ox[(g - TL) * GH + hh]
                    res[j] = proj(j, tie)
            for h in range(g * GH, (g + 1) * GH):
                qs[h], ks[h], vs[h] = res[h], res[H + h], res[2 * H + h]

        def vpu_rows(h, a, q, k, v):
            nk = 8 * a + 8
            qa = q[8 * a:8 * a + 8, :] * (scale * LOG2E)
            sj = []
            for j in range(nk):
                sc = jnp.sum(qa * kv_s[h % NKV, 0, pl.ds(j, 8, stride=0), :], axis=-1, keepdims=True)
                sc = jnp.broadcast_to(sc, (8, DH))
                if j > 8 * a:
                    sc = jnp.where(sub >= j - 8 * a, sc, NEG * LOG2E)
                sj.append(sc)
            def part(js):
                mx = _tree(jnp.maximum, [sj[j] for j in js])
                es = [jnp.exp2(sj[j] - mx) for j in js]
                red = (lambda f, xs: functools.reduce(f, xs)) if SEQ else _tree
                den = red(jnp.add, es)
                o = red(jnp.add, [e * kv_s[h % NKV, 1, pl.ds(j, 8, stride=0), :] for j, e in zip(js, es)])
                return mx, den, o
            if HALF:
                m1, d1, o1 = part(range(8))
                m2, d2, o2 = part(range(8, 16))
                mx = jnp.maximum(m1, m2)
                a1, a2 = jnp.exp2(m1 - mx), jnp.exp2(m2 - mx)
                den, o = d1 * a1 + d2 * a2, o1 * a1 + o2 * a2
            else:
                _, den, o = part(range(nk))
            return o * pl.reciprocal(den, approx=True)

        def do_s(g):
            for h in range(g * GH, (g + 1) * GH):
                q, k = qs.pop(h), ks.pop(h)
                kv_s[h % NKV, 0] = k[0:16, :]
                kv_s[h % NKV, 1] = vs[h][0:16, :]
                ox[h] = vpu_rows(h, 1, q, k, vs[h])
                qm = jnp.concatenate([q[0:8, :], q[16:, :]], axis=0)
                sc = _dot_nt(qm.astype(BF16) if BQ else qm, k.astype(BF16) if BK else k) * scale
                sc = jnp.where(mask_m, sc, NEG)
                e = jnp.exp(sc - jnp.max(sc, axis=-1, keepdims=True))
                ps[h] = e * pl.reciprocal(jnp.sum(e, axis=-1, keepdims=True), approx=True)

        def do_pv(g):
            for h in range(g * GH, (g + 1) * GH):
                v = vs.pop(h)
                if g >= NG - TL:
                    v = jnp.concatenate([jnp.where(i < 0, ox[h], v[0:8, :]), v[8:, :]], axis=0)
                p_ = ps.pop(h)
                o = _dot(p_.astype(BF16) if BP else p_, v.astype(BF16) if BV else v)
                os_[h] = jnp.concatenate([o[0:8, :], ox.pop(h), o[8:, :]], axis=0)

        def do_o(j, h0, h1):
            o = jnp.concatenate([os_[h] for h in range(h0, h1)], axis=1)
            return _dot(o, pltpu.bitcast(wo_p[j, h0 * 64:h1 * 64, :], BF16))

        for g in range(NG):
            do_qkv(g)
            if g >= 1:
                do_s(g - 1)
            if g >= 3:
                do_pv(g - 3)
        HS = (NG - 4) * GH

        def o1(j):
            part_v[:, j * 128:(j + 1) * 128] = do_o(j, 0, HS)

        o1(0)
        do_s(NG - 1)
        do_pv(NG - 3)
        o1(1)
        do_pv(NG - 2)
        o1(2)
        o1(3)
        do_pv(NG - 1)
        o1(4)
        return jnp.concatenate(
            [part_v[:, j * 128:(j + 1) * 128] + do_o(j, HS, H) for j in range(NT)], axis=1)

    def multi(i, carry):
        cur = acc[...]
        for u in range(UNROLL):
            cur = step(i, u, cur)
        acc[...] = cur
        r0 = pl.multiple_of(i * (UNROLL * SEG), SEG)
        out_copy(r0, (UNROLL - 1) * SEG).start()

        @pl.when(i > 0)
        def _():
            out_copy(pl.multiple_of(r0 - SEG, SEG), SEG).start()
        return carry

    jax.lax.fori_loop(0, NSEG // UNROLL, multi, 0)
    finish(NSEG - 1, acc[M:L, :])
    out_copy(S - SEG, SEG).start()
    out_copy(0, S).wait()


@jax.jit
def pallas_recurrent_scan__memory_aug_recurrent_mem_tr__moe_arch_mod__prompt_kernel(
    A_x: jax.Array,
    A_mem0: jax.Array,
    A_Wq: jax.Array,
    A_Wk: jax.Array,
    A_Wv: jax.Array,
    A_Wo: jax.Array,
    A_seg_len: jax.Array,
    B_x: jax.Array,
    B_w_r: jax.Array,
    B_w_gate: jax.Array,
    B_w_up: jax.Array,
    B_w_down: jax.Array,
):
    del A_seg_len, B_x
    assert A_x.shape == (1, S, D) and A_Wq.shape == (D, H, DH) and A_mem0.shape == (1, M, D)
    hbm = pl.BlockSpec(memory_space=pltpu.HBM)
    out = pl.pallas_call(
        _kernel,
        out_shape=jax.ShapeDtypeStruct((S, D), BF16),
        in_specs=[hbm] * 10,
        out_specs=hbm,
        scratch_shapes=[
            pltpu.VMEM((NSEG, SEG, D), BF16),
            pltpu.VMEM((NSEG * 4, D), U32),
            pltpu.VMEM((NSEG * LIVE, D), F32),
            pltpu.VMEM((S, D), F32),
            pltpu.VMEM((2 * NPH, D, 128), U32),
            pltpu.VMEM((2 * NPH, D // 2, 128), U32),
            pltpu.VMEM((2 * NPH, D // 2, 128), U32),
            pltpu.VMEM((NT, H * DH // 2, 128), U32),
            pltpu.VMEM((3 * H, NSEG * 8, DH), F32),
            pltpu.VMEM((FF, D), BF16),
            pltpu.VMEM((FF, D), BF16),
            pltpu.VMEM((FF, D), BF16),
            pltpu.VMEM((S, D), BF16),
            pltpu.VMEM((L, D), F32),
            pltpu.VMEM((L, D), F32),
            pltpu.VMEM((NKV, 2, 16, DH), F32),
            pltpu.VMEM((TOPC, D), F32),
            pltpu.VMEM((TOPC, D), F32),
            pltpu.VMEM((128, 128), I32),
            pltpu.VMEM((M, D), BF16),
            pltpu.VMEM((NT, 128), BF16),
            pltpu.SMEM((TOPC,), I32),
            pltpu.SemaphoreType.DMA((16 + NPH,)),
            pltpu.SemaphoreType.DMA((1,)),
        ],
        compiler_params=pltpu.CompilerParams(vmem_limit_bytes=110 * 1024 * 1024),
    )(
        A_x.reshape(NSEG, SEG, D),
        A_mem0.reshape(M, D),
        A_Wq, A_Wk, A_Wv,
        A_Wo.reshape(H * DH, D),
        B_w_r.reshape(NT, 128),
        B_w_gate.T, B_w_up.T, B_w_down,
    )
    return out.reshape(1, S, D)
```

```python
import functools
import math

import jax
import jax.numpy as jnp
import jax.experimental.pallas as pl
import jax.experimental.pallas.tpu as pltpu

F32 = jnp.float32
BF16 = jnp.bfloat16
U32 = jnp.uint32
I32 = jnp.int32

S = 2048
D = 640
H = 32
DH = 128
M = 8
SEG = 32
NSEG = S // SEG
L = M + SEG
FF = 1728
TOPC = 8
NT = D // 128
LIVE = SEG - 8
EPS = 1e-05
NEG = -1000000000.0
UNROLL = 4
NKV = 32
LOG2E = math.log2(math.e)
TIE0 = 2
NPH = 24
TA, TB, TL = 1, 4, 3
SEQ = False
HALF = False
BQ, BK, BP, BV = 1, 1, 1, 1
TP = (1, 4)
ORD = 0
LS, LP = 1, 3
PVFIRST = False
HS = 24
TAIL = ((0, 'sp'), (1, 'p'), (3, 'p'))
GH = 2


def _dot(a, b):
    return jax.lax.dot_general(a, b, (((1,), (0,)), ((), ())), preferred_element_type=F32)


def _dot_nt(a, b):
    return jax.lax.dot_general(a, b, (((1,), (1,)), ((), ())), preferred_element_type=F32)


def _rb(x):
    return x.astype(BF16).astype(F32)


def _sigmoid(x):
    return pl.reciprocal(1.0 + jnp.exp(-x), approx=True)


def _tree(f, xs):
    while len(xs) > 1:
        xs = [f(xs[n], xs[n + 1]) if n + 1 < len(xs) else xs[n] for n in range(0, len(xs), 2)]
    return xs[0]


def _kernel(x_hbm, mem0_hbm, wq_hbm, wk_hbm, wv_hbm, wo_hbm, wr_hbm, wg_hbm, wu_hbm, wd_hbm,
            out_hbm,
            x_v, lhs_v, xa_v, xb_v, raw, w_ev, w_od, wo_p, pre, wg_v, wu_v, wd_v,
            out_v, acc, part_v, kv_s, sel, yacc, keys, mem0_v, wr_v, idx_s,
            sem_in, sem_out):
    w_hbm = [wq_hbm, wk_hbm, wv_hbm]
    w_eo = [w_ev, w_od]

    def wtile(j):
        return w_eo[(j // 4) % 2].at[(j // 8) * 4 + j % 4]

    SEM_X8, SEM_XA, SEM_W = 4, 8, 16

    def w_start(k):
        for q in (2 * k, 2 * k + 1):
            src = w_hbm[q // 16].bitcast(U32).at[:, q % 16, :]
            pltpu.make_async_copy(src, raw.at[q], sem_in.at[SEM_W + k]).start()

    def w_wait(k):
        both = raw.at[pl.ds(2 * k, 2)]
        pltpu.make_async_copy(both, both, sem_in.at[SEM_W + k]).wait()

    def x8_copy(b):
        return pltpu.make_async_copy(x_hbm.at[pl.ds(b * 16, 16), pl.ds(LIVE, 8), :],
                                     x_v.at[pl.ds(b * 16, 16), pl.ds(LIVE, 8), :], sem_in.at[SEM_X8 + b])

    def xa_copy(i):
        return pltpu.make_async_copy(x_hbm.at[pl.ds(i * 8, 8), pl.ds(0, LIVE), :],
                                     x_v.at[pl.ds(i * 8, 8), pl.ds(0, LIVE), :], sem_in.at[SEM_XA + i])

    cp_wr = pltpu.make_async_copy(wr_hbm, wr_v, sem_in.at[0])
    cp_mem = pltpu.make_async_copy(mem0_hbm, mem0_v, sem_in.at[1])
    mlp_copies = [pltpu.make_async_copy(s_, d_, sem_in.at[2])
                  for s_, d_ in [(wg_hbm, wg_v), (wu_hbm, wu_v), (wd_hbm, wd_v)]]
    wo32 = wo_hbm.bitcast(U32)
    wo_copies = [pltpu.make_async_copy(wo32.at[:, pl.ds(j * 128, 128)], wo_p.at[j], sem_in.at[3])
                 for j in range(NT)]

    cp_wr.start()
    for b in range(4):
        x8_copy(b).start()
    for k in range(NPH):
        w_start(k)
        if k >= 3 and k % 2 == 1 and (k - 3) // 2 < 8:
            xa_copy((k - 3) // 2).start()
    cp_mem.start()
    for c in mlp_copies:
        c.start()
    for c in wo_copies:
        c.start()

    IMIN = jnp.iinfo(jnp.int32).min
    xb3 = xb_v.reshape(NSEG, SEG, D)
    keys[...] = jnp.full(keys.shape, IMIN, I32)
    yacc[...] = jnp.zeros(yacc.shape, F32)
    kv_s[:, :, 0:8, :] = jnp.zeros((NKV, 2, 8, DH), F32)
    cp_wr.wait()

    def router_w():
        wr5 = wr_v[...].astype(F32)
        return jnp.concatenate([wr5[j:j + 1, :] for j in range(NT)], axis=1)

    def layernorm(s0, nseg, t0, nrow, slot, wr):
        n = nseg * nrow
        x = x_v[pl.ds(s0, nseg), t0:t0 + nrow, :].astype(F32).reshape(n, D)
        mu = jnp.sum(x, axis=-1, keepdims=True) * (1.0 / D)
        xc = x - mu
        var = jnp.sum(xc * xc, axis=-1, keepdims=True) * (1.0 / D)
        sd = _rb(jnp.sqrt(_rb(_rb(var) + EPS)))
        xn = _rb(_rb(x - _rb(mu)) / sd)
        xb3[pl.ds(s0, nseg), t0:t0 + nrow, :] = xn.reshape(nseg, nrow, D)
        r = _rb(jnp.sum(xn * wr, axis=-1, keepdims=True))
        r = jnp.where(r == 0.0, 0.0, r)
        bits = pltpu.bitcast(jnp.broadcast_to(r, (n, 128)), I32) >> 16
        mono = jnp.where(bits < 0, (-32768) - bits, bits)
        mono = jnp.where(r != r, -40000, mono)
        row = (jax.lax.broadcasted_iota(I32, (nseg, nrow, 128), 0) * SEG
               + jax.lax.broadcasted_iota(I32, (nseg, nrow, 128), 1)).reshape(n, 128)
        key = mono * 4096 + ((S - 1 - t0) - s0 * SEG - row)
        lane = jax.lax.broadcasted_iota(I32, (n, 128), 1)
        keys[0:n, :] = jnp.where(lane == slot, key, keys[0:n, :])
        return xn, key

    def ln8_body(b, carry):
        x8_copy(b).wait()
        xn, _ = layernorm(b * 16, 16, LIVE, 8, b, router_w())
        lhs_v[pl.ds(pl.multiple_of(b * 64, 64), 64), :] = pltpu.bitcast(xn.astype(BF16), U32)
        return carry

    jax.lax.fori_loop(0, 4, ln8_body, 0)

    def ln_seg(s, wr):
        xn, key = layernorm(s, 1, 0, LIVE, 4 + s, wr)
        xa_v[pl.ds(pl.multiple_of(s * LIVE, 8), LIVE), :] = xn
        return pltpu.bitcast(key, U32)

    def topk_round(c):
        kv = keys[...]
        mx = jnp.max(kv)
        keys[...] = jnp.where(kv == mx, IMIN, kv)
        idx = jnp.clip((S - 1) - (mx & 4095), 0, S - 1)
        idx_s[c] = idx
        sel[pl.ds(c, 1), :] = xb_v[pl.ds(idx, 1), :]

    def repack(k, par, slot, part=None, tie=None):
        m_lo = jnp.full((8, 128), 0xFFFF, U32)
        m_hi = jnp.full((8, 128), 0xFFFF0000, U32)
        if tie is not None:
            m_lo = jnp.where(k < 0, tie, m_lo)
            m_hi = jnp.where(k < 0, tie, m_hi)
        for u in range(2):
            rq = raw.at[2 * k + u]
            lo = w_eo[par].at[slot * 4 + 2 * u]
            hi = w_eo[par].at[slot * 4 + 2 * u + 1]
            for g in range(D // 16):
                if part is not None and (u * (D // 16) + g) % part[1] != part[0]:
                    continue
                a = rq[pl.ds(16 * g, 8, stride=2), :]
                b = rq[pl.ds(16 * g + 1, 8, stride=2), :]
                lo[8 * g:8 * g + 8, :] = (a & m_lo) | (b << 16)
                hi[8 * g:8 * g + 8, :] = (a >> 16) | (b & m_hi)

    def phase(k, par, slot, after_dot=None, side=None, nxt=None, tied=False):
        for u in range(4):
            for c in range(4):
                w = pltpu.bitcast(w_eo[par][slot * 4 + u], BF16)
                lhs = lhs_v[c * 64:(c + 1) * 64, :]
                if side is not None and c == 3:
                    tok = side(u)
                    n = tok.shape[0]
                    head = jnp.where(k < 0, tok, lhs[0:n, 0:128])
                    lhs = jnp.concatenate(
                        [jnp.concatenate([head, lhs[0:n, 128:]], axis=1), lhs[n:, :]], axis=0)
                r = _dot(pltpu.bitcast(lhs, BF16), w)
                pre[4 * k + u, c * 128:(c + 1) * 128, :] = r
                if after_dot is not None:
                    after_dot()
                if nxt is not None and u < 3:
                    repack(k + 1, 1 - par, nxt, (u * 4 + c, 12),
                           pltpu.bitcast(r[0:8, :], U32) if tied else None)

    def two_phases(i, after_dot=None, side=None):
        k = 2 * i + 1
        dyn = not isinstance(i, int)
        phase(k, 1, i, after_dot, side, i + 1)
        phase(k + 1, 0, i + 1, after_dot, None if side is None else (lambda u: side(4 + u)), i + 1, dyn)

    w_wait(0)
    repack(0, 0, 0)
    w_wait(1)
    repack(1, 1, 0)
    phase(0, 0, 0)

    def ln_body(i, carry):
        w_wait(2 * i + 2)
        w_wait(2 * i + 3)
        xa_copy(i).wait()
        wr = router_w()
        two_phases(i, side=lambda u: ln_seg(i * 8 + u, wr))
        return carry

    jax.lax.fori_loop(0, 8, ln_body, 0)

    w_wait(18)
    w_wait(19)
    for c in range(TOPC):
        topk_round(c)
    two_phases(8)

    for c in mlp_copies:
        c.wait()
    FP = FF // 2

    def mlp_body(t, carry):
        i = 9 + t
        w_wait(2 * i + 2)
        w_wait(2 * i + 3)
        f0 = pl.multiple_of(t * FP, 16)
        xs = sel[...]
        cuts = [(a_, min(a_ + 128, FP)) for a_ in range(0, FP, 128)]
        val = {}

        def up_tile(which, n, kt):
            def run():
                a_, b_ = cuts[n]
                w = (wg_v, wu_v)[which][pl.ds(f0 + a_, b_ - a_), kt * 128:(kt + 1) * 128]
                r = _dot_nt(xs[:, kt * 128:(kt + 1) * 128], w)
                val[which, n] = r if kt == 0 else val[which, n] + r
            return run

        def down_tile(n, j):
            def run():
                a_, b_ = cuts[n]
                if j == 0:
                    g_ = _rb(val.pop((0, n)))
                    val['h', n] = _rb(g_ * _sigmoid(g_)) * _rb(val.pop((1, n)))
                r = _dot(val['h', n], wd_v[pl.ds(f0 + a_, b_ - a_), j * 128:(j + 1) * 128])
                val['y', j] = r if n == 0 else val['y', j] + r
            return run

        jobs = [up_tile(which, n, kt) for n in range(len(cuts)) for which in range(2) for kt in range(NT)]
        jobs += [down_tile(n, j) for n in range(len(cuts)) for j in range(NT)]

        def after_dot():
            for _ in range(4):
                if jobs:
                    jobs.pop(0)()

        two_phases(i, after_dot=after_dot)
        yacc[...] += jnp.concatenate([val['y', j] for j in range(NT)], axis=1)
        return carry

    jax.lax.fori_loop(0, 2, mlp_body, 0)

    cp_mem.wait()
    acc[0:M, :] = mem0_v[...].astype(F32)
    acc[M:L, :] = jnp.zeros((SEG, D), F32)
    xs = sel[...]
    r_sel = _rb(jnp.sum(xs * router_w(), axis=-1, keepdims=True))
    sel[...] = xs + _rb(_rb(yacc[...]) * _rb(_sigmoid(r_sel)))
    for c in range(TOPC):
        xb_v[pl.ds(idx_s[c], 1), :] = sel[pl.ds(c, 1), :]
    phase(NPH - 1, 1, NPH // 2 - 1)

    for c in wo_copies:
        c.wait()

    qi = jax.lax.broadcasted_iota(I32, (L, L), 0)
    ki = jax.lax.broadcasted_iota(I32, (L, L), 1)
    mask = (qi < M) | (qi >= ki)
    scale = DH ** (-0.5)
    qm_i = jax.lax.broadcasted_iota(I32, (L - 8, L), 0)
    mask_m = (qm_i < M) | (qm_i + 8 >= jax.lax.broadcasted_iota(I32, (L - 8, L), 1))
    sub = jax.lax.broadcasted_iota(I32, (8, DH), 0)

    def finish(sp, sa):
        r0 = pl.multiple_of(sp * SEG, SEG)
        xb = xb_v[pl.ds(r0, SEG), :]
        g = xb * _sigmoid(xb)
        o = x_v[sp].astype(F32) + sa * g
        out_v[pl.ds(r0, SEG), :] = o.astype(BF16)
        return o

    def out_copy(r0, n):
        return pltpu.make_async_copy(out_v.at[pl.ds(r0, n), :], out_hbm.at[pl.ds(r0, n), :], sem_out.at[0])

    def step(i, u, prev):
        s = i * UNROLL + u
        pre_i = pre.at[:, pl.ds(pl.multiple_of(i * (8 * UNROLL), 8 * UNROLL), 8 * UNROLL), :]
        xa_i = xa_v.at[pl.ds(pl.multiple_of(i * (LIVE * UNROLL), 8 * UNROLL), LIVE * UNROLL), :]
        xa = xa_i[u * LIVE:(u + 1) * LIVE, :]
        lhs = jnp.concatenate([prev[0:M, :], xa], axis=0).astype(BF16)
        fin = finish(jnp.maximum(s - 1, 0) if u == 0 else s - 1, prev[M:L, :])

        def proj(j, tie=None):
            lh = lhs
            if tie is not None:
                top = pltpu.bitcast(lhs[0:16, 0:128], U32)
                top = pltpu.bitcast(jnp.where(i < 0, pltpu.bitcast(tie, U32), top), BF16)
                lh = jnp.concatenate([jnp.concatenate([top, lhs[0:16, 128:]], axis=1), lhs[16:, :]], axis=0)
            t = _dot(lh, pltpu.bitcast(wtile(j)[...], BF16))
            if u == 0 and TIE0 <= j < TIE0 + NT:
                t = jnp.where(i < 0, fin[:, (j - TIE0) * 128:(j - TIE0 + 1) * 128], t)
            return jnp.concatenate([t, pre_i[j, u * 8:(u + 1) * 8, :]], axis=0)

        NG = H // GH
        qs, ks, vs, ps, os_, ox = {}, {}, {}, {}, {}, {}

        def do_qkv(g):
            if ORD == 0:
                js = [m * H + h for h in range(g * GH, (g + 1) * GH) for m in range(3)]
            elif ORD == 1:
                js = [m * H + h for m in range(3) for h in range(g * GH, (g + 1) * GH)]
            else:
                js = [m * H + h for h in range(g * GH, (g + 1) * GH) for m in (1, 0, 2)]
            if g == 0:
                js, rest = js[:6], js[6:]
                part = {}
                for kt in range(NT):
                    for j in js:
                        t = _dot(lhs[:, kt * 128:(kt + 1) * 128],
                                 pltpu.bitcast(wtile(j)[kt * 64:(kt + 1) * 64, :], BF16))
                        part[j] = t if kt == 0 else part[j] + t
                res = {j: jnp.concatenate([part[j], pre_i[j, u * 8:(u + 1) * 8, :]], axis=0) for j in js}
                for j in rest:
                    res[j] = proj(j)
            else:
                res = {}
                for n, j in enumerate(js):
                    tie = None
                    for hh, pos in enumerate(TP):
                        if n == pos and g >= TL:
                            tie = ox[(g - TL) * GH + hh]
                    res[j] = proj(j, tie)
            for h in range(g * GH, (g + 1) * GH):
                qs[h], ks[h], vs[h] = res[h], res[H + h], res[2 * H + h]

        def vpu_rows(h, q, k, v):
            def win(which, val, r):
                if r % 8 == 0:
                    return val[8 - r:16 - r, :]
                return kv_s[h % NKV, which, 16 - r:24 - r, :]

            qa = q[8:16, :] * (scale * LOG2E)
            sj = []
            for r in range(16):
                sc = jnp.sum(qa * win(0, k, r), axis=-1, keepdims=True)
                sc = jnp.broadcast_to(sc, (8, DH))
                if r > 8:
                    sc = jnp.where(sub >= r - 8, sc, -jnp.inf)
                sj.append(sc)
            mx = _tree(jnp.maximum, sj)
            es = [jnp.exp2(x - mx) for x in sj]
            den = _tree(jnp.add, es)
            o = _tree(jnp.add, [e * win(1, v, r) for r, e in enumerate(es)])
            return o * pl.reciprocal(den, approx=True)

        def do_s(g):
            for h in range(g * GH, (g + 1) * GH):
                q, k = qs.pop(h), ks.pop(h)
                kv_s[h % NKV, 0, 8:24, :] = k[0:16, :]
                kv_s[h % NKV, 1, 8:24, :] = vs[h][0:16, :]
                ox[h] = vpu_rows(h, q, k, vs[h])
                qm = jnp.concatenate([q[0:8, :], q[16:, :]], axis=0)
                sc = _dot_nt(qm.astype(BF16) if BQ else qm, k.astype(BF16) if BK else k) * scale
                sc = jnp.where(mask_m, sc, NEG)
                e = jnp.exp(sc - jnp.max(sc, axis=-1, keepdims=True))
                ps[h] = e * pl.reciprocal(jnp.sum(e, axis=-1, keepdims=True), approx=True)

        def do_pv(g):
            for h in range(g * GH, (g + 1) * GH):
                v = vs.pop(h)
                if g >= NG - TL:
                    v = jnp.concatenate([jnp.where(i < 0, ox[h], v[0:8, :]), v[8:, :]], axis=0)
                p_ = ps.pop(h)
                o = _dot(p_.astype(BF16) if BP else p_, v.astype(BF16) if BV else v)
                os_[h] = jnp.concatenate([o[0:8, :], ox.pop(h), o[8:, :]], axis=0)

        def do_o(j, h0, h1):
            o = jnp.concatenate([os_[h] for h in range(h0, h1)], axis=1)
            return _dot(o, pltpu.bitcast(wo_p[j, h0 * 64:h1 * 64, :], BF16))

        for g in range(NG):
            if PVFIRST and g >= LP:
                do_pv(g - LP)
            do_qkv(g)
            if g >= LS:
                do_s(g - LS)
            if not PVFIRST and g >= LP:
                do_pv(g - LP)
        sched = dict(TAIL)
        ns, npv = NG - LS, NG - LP
        for j in range(NT):
            part_v[:, j * 128:(j + 1) * 128] = do_o(j, 0, HS)
            for c_ in sched.get(j, ''):
                if c_ == 's':
                    do_s(ns)
                    ns += 1
                else:
                    do_pv(npv)
                    npv += 1
        assert ns == NG and npv == NG
        return jnp.concatenate(
            [part_v[:, j * 128:(j + 1) * 128] + do_o(j, HS, H) for j in range(NT)], axis=1)

    def multi(i, carry):
        cur = acc[...]
        for u in range(UNROLL):
            cur = step(i, u, cur)
        acc[...] = cur
        r0 = pl.multiple_of(i * (UNROLL * SEG), SEG)
        out_copy(r0, (UNROLL - 1) * SEG).start()

        @pl.when(i > 0)
        def _():
            out_copy(pl.multiple_of(r0 - SEG, SEG), SEG).start()
        return carry

    jax.lax.fori_loop(0, NSEG // UNROLL, multi, 0)
    finish(NSEG - 1, acc[M:L, :])
    out_copy(S - SEG, SEG).start()
    out_copy(0, S).wait()


@jax.jit
def pallas_recurrent_scan__memory_aug_recurrent_mem_tr__moe_arch_mod__prompt_kernel(
    A_x: jax.Array,
    A_mem0: jax.Array,
    A_Wq: jax.Array,
    A_Wk: jax.Array,
    A_Wv: jax.Array,
    A_Wo: jax.Array,
    A_seg_len: jax.Array,
    B_x: jax.Array,
    B_w_r: jax.Array,
    B_w_gate: jax.Array,
    B_w_up: jax.Array,
    B_w_down: jax.Array,
):
    del A_seg_len, B_x
    assert A_x.shape == (1, S, D) and A_Wq.shape == (D, H, DH) and A_mem0.shape == (1, M, D)
    hbm = pl.BlockSpec(memory_space=pltpu.HBM)
    out = pl.pallas_call(
        _kernel,
        out_shape=jax.ShapeDtypeStruct((S, D), BF16),
        in_specs=[hbm] * 10,
        out_specs=hbm,
        scratch_shapes=[
            pltpu.VMEM((NSEG, SEG, D), BF16),
            pltpu.VMEM((NSEG * 4, D), U32),
            pltpu.VMEM((NSEG * LIVE, D), F32),
            pltpu.VMEM((S, D), F32),
            pltpu.VMEM((2 * NPH, D, 128), U32),
            pltpu.VMEM((2 * NPH, D // 2, 128), U32),
            pltpu.VMEM((2 * NPH, D // 2, 128), U32),
            pltpu.VMEM((NT, H * DH // 2, 128), U32),
            pltpu.VMEM((3 * H, NSEG * 8, DH), F32),
            pltpu.VMEM((FF, D), BF16),
            pltpu.VMEM((FF, D), BF16),
            pltpu.VMEM((FF, D), BF16),
            pltpu.VMEM((S, D), BF16),
            pltpu.VMEM((L, D), F32),
            pltpu.VMEM((L, D), F32),
            pltpu.VMEM((NKV, 2, 24, DH), F32),
            pltpu.VMEM((TOPC, D), F32),
            pltpu.VMEM((TOPC, D), F32),
            pltpu.VMEM((128, 128), I32),
            pltpu.VMEM((M, D), BF16),
            pltpu.VMEM((NT, 128), BF16),
            pltpu.SMEM((TOPC,), I32),
            pltpu.SemaphoreType.DMA((16 + NPH,)),
            pltpu.SemaphoreType.DMA((1,)),
        ],
        compiler_params=pltpu.CompilerParams(vmem_limit_bytes=110 * 1024 * 1024),
    )(
        A_x.reshape(NSEG, SEG, D),
        A_mem0.reshape(M, D),
        A_Wq, A_Wk, A_Wv,
        A_Wo.reshape(H * DH, D),
        B_w_r.reshape(NT, 128),
        B_w_gate.T, B_w_up.T, B_w_down,
    )
    return out.reshape(1, S, D)
```

```python
import functools
import math

import jax
import jax.numpy as jnp
import jax.experimental.pallas as pl
import jax.experimental.pallas.tpu as pltpu

F32 = jnp.float32
BF16 = jnp.bfloat16
U32 = jnp.uint32
I32 = jnp.int32

S = 2048
D = 640
H = 32
DH = 128
M = 8
SEG = 32
NSEG = S // SEG
L = M + SEG
FF = 1728
TOPC = 8
NT = D // 128
LIVE = SEG - 8
EPS = 1e-05
NEG = -1000000000.0
UNROLL = 8
NKV = 32
LOG2E = math.log2(math.e)
TIE0 = 2
NPAIR = 3 * H // 2
KEY_NONE = -1e30
MS0, MS1 = 3, 153
TA, TB, TL = 1, 4, 3
SEQ = False
HALF = False
BQ, BK, BP, BV = 1, 1, 1, 1
TP = (1, 4)
ORD = 0
LS, LP = 1, 3
PVFIRST = False
HS = 24
TAIL = ((0, 'sp'), (1, 'p'), (3, 'p'))
GH = 2


def _dot(a, b):
    return jax.lax.dot_general(a, b, (((1,), (0,)), ((), ())), preferred_element_type=F32)


def _dot_nt(a, b):
    return jax.lax.dot_general(a, b, (((1,), (1,)), ((), ())), preferred_element_type=F32)


def _rb(x):
    return x.astype(BF16).astype(F32)


def _sigmoid(x):
    return pl.reciprocal(1.0 + jnp.exp(-x), approx=True)


def _tree(f, xs):
    while len(xs) > 1:
        xs = [f(xs[n], xs[n + 1]) if n + 1 < len(xs) else xs[n] for n in range(0, len(xs), 2)]
    return xs[0]


def _kernel(x_hbm, mem0_hbm, wq_hbm, wk_hbm, wv_hbm, wo_hbm, wr_hbm, wg_hbm, wu_hbm, wd_hbm,
            out_hbm,
            x_v, lhs_v, xa_v, xb_v, raw, w_p, wo_p, pre, wg_v, wu_v, wd_v,
            out_v, acc, part_v, kv_s, sel, upd, yacc, keys, mem0_v, wr_v, idx_s,
            sem_in, sem_out):
    w_hbm = [wq_hbm, wk_hbm, wv_hbm]

    def wtile(j):
        return w_p.at[j]

    SEM_X8, SEM_B0, SEM_LN, SEM_TK, SEM_MLP, SEM_WO = 0, 4, 7, 15, 16, 17

    def w_start(q0, n, sem):
        for q in range(q0, q0 + n):
            src = w_hbm[q // 16].bitcast(U32).at[:, q % 16, :]
            pltpu.make_async_copy(src, raw.at[q], sem_in.at[sem]).start()

    def w_wait(q0, n, sem):
        blk = raw.at[pl.ds(q0, n)]
        pltpu.make_async_copy(blk, blk, sem_in.at[sem]).wait()

    def x8_copy(b):
        return pltpu.make_async_copy(x_hbm.at[pl.ds(b * 16, 16), pl.ds(LIVE, 8), :],
                                     x_v.at[pl.ds(b * 16, 16), pl.ds(LIVE, 8), :], sem_in.at[SEM_X8 + b])

    def xa_copy(i):
        return pltpu.make_async_copy(x_hbm.at[pl.ds(i * 8, 8), pl.ds(0, LIVE), :],
                                     x_v.at[pl.ds(i * 8, 8), pl.ds(0, LIVE), :], sem_in.at[SEM_LN + i])

    cp_wr = pltpu.make_async_copy(wr_hbm, wr_v, sem_in.at[SEM_B0 + 2])
    cp_mem = pltpu.make_async_copy(mem0_hbm, mem0_v, sem_in.at[SEM_TK])
    mlp_copies = [pltpu.make_async_copy(s_, d_, sem_in.at[SEM_MLP])
                  for s_, d_ in [(wg_hbm, wg_v), (wu_hbm, wu_v), (wd_hbm, wd_v)]]
    wo32 = wo_hbm.bitcast(U32)
    wo_copies = [pltpu.make_async_copy(wo32.at[:, pl.ds(j * 128, 128)], wo_p.at[j], sem_in.at[SEM_WO])
                 for j in range(NT)]

    for b in range(4):
        x8_copy(b).start()
    w_start(0, 1, SEM_B0)
    w_start(1, 1, SEM_B0 + 1)
    w_start(2, 2, SEM_B0 + 2)
    cp_wr.start()
    for i in range(8):
        w_start(4 + 4 * i, 4, SEM_LN + i)
        xa_copy(i).start()
    w_start(36, NPAIR - 36, SEM_TK)
    cp_mem.start()
    for c in mlp_copies:
        c.start()
    for c in wo_copies:
        c.start()

    xb3 = xb_v.reshape(NSEG, SEG, D)
    keys[...] = jnp.full(keys.shape, KEY_NONE, F32)
    yacc[...] = jnp.zeros(yacc.shape, F32)
    kv_s[:, :, 0:8, :] = jnp.zeros((NKV, 2, 8, DH), F32)
    raw[NPAIR] = jnp.zeros((D, 128), U32)
    acc[M:L, :] = jnp.zeros((SEG, D), F32)

    def router_w():
        wr5 = wr_v[...].astype(F32)
        return jnp.concatenate([wr5[j:j + 1, :] for j in range(NT)], axis=1)

    def layernorm(s0, nseg, t0, nrow):
        n = nseg * nrow
        x = x_v[pl.ds(s0, nseg), t0:t0 + nrow, :].astype(F32).reshape(n, D)
        mu = jnp.sum(x, axis=-1, keepdims=True) * (1.0 / D)
        xc = x - mu
        var = jnp.sum(xc * xc, axis=-1, keepdims=True) * (1.0 / D)
        sd = _rb(jnp.sqrt(_rb(_rb(var) + EPS)))
        xn = _rb(_rb(x - _rb(mu)) / sd)
        xb3[pl.ds(s0, nseg), t0:t0 + nrow, :] = xn.reshape(nseg, nrow, D)
        return xn

    def ln8_body(b, carry):
        x8_copy(b).wait()
        xn = layernorm(b * 16, 16, LIVE, 8)
        lhs_v[pl.ds(pl.multiple_of(b * 64, 64), 64), :] = pltpu.bitcast(xn.astype(BF16), U32)
        return carry

    jax.lax.fori_loop(0, 4, ln8_body, 0)

    def ln_seg(s, wr):
        tail = xb3[s, LIVE:SEG, :]
        xn = layernorm(s, 1, 0, LIVE)
        xa_v[pl.ds(pl.multiple_of(s * LIVE, 8), LIVE), :] = xn
        r = _rb(jnp.sum(jnp.concatenate([xn, tail], axis=0) * wr, axis=-1, keepdims=True))
        r = jnp.where(r == 0.0, 0.0, r)
        bits = pltpu.bitcast(jnp.broadcast_to(r, (SEG, 128)), I32) >> 16
        mono = jnp.where(bits < 0, (-32768) - bits, bits)
        mono = jnp.where(r != r, -40000, mono)
        row = jax.lax.broadcasted_iota(I32, (SEG, 128), 0)
        key = (mono * SEG + ((SEG - 1) - row)).astype(F32)
        lane = jax.lax.broadcasted_iota(I32, (SEG, 128), 1)
        keys[...] = jnp.where(lane == s, key, keys[...])
        return pltpu.bitcast(key, U32)

    def top_rows():
        kv = keys[...]
        lane = jax.lax.broadcasted_iota(I32, (1, 128), 1).astype(F32)
        for c in range(TOPC):
            col = jnp.max(kv, axis=0, keepdims=True)
            val = jnp.floor(col * (1.0 / SEG))
            fk = val * 128.0 + (127.0 - lane)
            win = fk == jnp.max(fk, axis=1, keepdims=True)
            kv = jnp.where(win & (kv == col), KEY_NONE, kv)
            pos = lane * SEG + ((SEG - 1.0) - (col - val * SEG))
            idx = jnp.clip(jnp.max(jnp.where(win, pos, 0.0)).astype(I32), 0, S - 1)
            idx_s[c] = idx
            sel[pl.ds(c, 1), :] = xb_v[pl.ds(idx, 1), :]

    def repack(rv, wv, p, part=None, tie=None):
        m_lo = jnp.full((8, 128), 0xFFFF, U32)
        m_hi = jnp.full((8, 128), 0xFFFF0000, U32)
        if tie is not None:
            m_lo = jnp.where(tie[0], tie[1], m_lo)
            m_hi = jnp.where(tie[0], tie[1], m_hi)
        for g in range(D // 16):
            if part is not None and g % part[1] != part[0]:
                continue
            a = rv[p, pl.ds(16 * g, 8, stride=2), :]
            b = rv[p, pl.ds(16 * g + 1, 8, stride=2), :]
            wv[2 * p, 8 * g:8 * g + 8, :] = (a & m_lo) | (b << 16)
            wv[2 * p + 1, 8 * g:8 * g + 8, :] = (a >> 16) | (b & m_hi)

    def block(q0, n, never=None, side=None, jobs=None):
        rv = raw.at[pl.ds(q0, n + 1)]
        wv = w_p.at[pl.ds(2 * q0, 2 * n + 2)]
        pv = pre.at[pl.ds(2 * q0, 2 * n)]
        for u in range(2 * n):
            if u % 2 == 0 and u // 2 + 1 < n:
                repack(rv, wv, u // 2 + 1)
            for c in range(4):
                lhs = lhs_v[c * 64:(c + 1) * 64, :]
                if side is not None and c == 3:
                    tok = side(u)
                    nr = tok.shape[0]
                    head = jnp.where(never, tok, lhs[0:nr, 0:128])
                    lhs = jnp.concatenate(
                        [jnp.concatenate([head, lhs[0:nr, 128:]], axis=1), lhs[nr:, :]], axis=0)
                lhs = pltpu.bitcast(lhs, BF16)
                if jobs:
                    r = None
                    for kt in range(NT):
                        t_ = _dot(lhs[:, kt * 128:(kt + 1) * 128],
                                  pltpu.bitcast(wv[u, kt * 64:(kt + 1) * 64, :], BF16))
                        r = t_ if r is None else r + t_
                        if jobs:
                            jobs.pop(0)()
                else:
                    r = _dot(lhs, pltpu.bitcast(wv[u], BF16))
                pv[u, c * 128:(c + 1) * 128, :] = r
                n8 = (u - max(2 * n - 3, 0)) * 4 + c
                if 0 <= n8 < 8:
                    repack(rv, wv, n, (n8, 8),
                           None if never is None else (never, pltpu.bitcast(r[0:8, :], U32)))

    w_wait(0, 1, SEM_B0)
    repack(raw, w_p, 0)
    w_wait(1, 1, SEM_B0 + 1)
    block(0, 1)
    w_wait(2, 2, SEM_B0 + 2)
    cp_wr.wait()
    block(1, 2)

    def ln_body(i, carry):
        w_wait(4 + 4 * i, 4, SEM_LN + i)
        xa_copy(i).wait()
        wr = router_w()
        block(3 + 4 * i, 4, i < 0, side=lambda u: ln_seg(i * 8 + u, wr))
        return carry

    jax.lax.fori_loop(0, 8, ln_body, 0)

    w_wait(36, NPAIR - 36, SEM_TK)
    cp_mem.wait()
    acc[0:M, :] = mem0_v[...].astype(F32)
    top_rows()
    block(35, 1)

    for c in mlp_copies:
        c.wait()
    FP = FF // 3

    def mlp_body(t, carry):
        f0 = pl.multiple_of(t * FP, 16)
        xs = sel[...]
        cuts = [(a_, min(a_ + 128, FP)) for a_ in range(0, FP, 128)]
        val = {}

        def up_tile(which, n, kt):
            def run():
                a_, b_ = cuts[n]
                w = (wg_v, wu_v)[which][pl.ds(f0 + a_, b_ - a_), kt * 128:(kt + 1) * 128]
                r = _dot_nt(xs[:, kt * 128:(kt + 1) * 128], w)
                val[which, n] = r if kt == 0 else val[which, n] + r
            return run

        def down_tile(n, j):
            def run():
                a_, b_ = cuts[n]
                if j == 0:
                    g_ = _rb(val.pop((0, n)))
                    val['h', n] = _rb(g_ * _sigmoid(g_)) * _rb(val.pop((1, n)))
                r = _dot(val['h', n], wd_v[pl.ds(f0 + a_, b_ - a_), j * 128:(j + 1) * 128])
                val['y', j] = r if n == 0 else val['y', j] + r
            return run

        def skip():
            pass

        real = ([up_tile(which, n, kt) for n in range(len(cuts)) for which in range(2) for kt in range(NT)]
                + [down_tile(n, j) for n in range(len(cuts)) for j in range(NT)])
        jobs = [skip] * MS1
        for n_, job in enumerate(real):
            jobs[MS0 + (n_ * (MS1 - MS0)) // len(real)] = job
        block(36 + 4 * t, 4, t < 0, jobs=jobs)
        assert not jobs
        y = yacc[...] + jnp.concatenate([val['y', j] for j in range(NT)], axis=1)
        yacc[...] = y
        r_sel = _rb(jnp.sum(xs * router_w(), axis=-1, keepdims=True))
        upd[...] = xs + _rb(_rb(y) * _rb(_sigmoid(r_sel)))
        for c in range(TOPC):
            xb_v[pl.ds(idx_s[c], 1), :] = upd[pl.ds(c, 1), :]
        return carry

    jax.lax.fori_loop(0, 3, mlp_body, 0)

    for c in wo_copies:
        c.wait()

    qi = jax.lax.broadcasted_iota(I32, (L, L), 0)
    ki = jax.lax.broadcasted_iota(I32, (L, L), 1)
    mask = (qi < M) | (qi >= ki)
    scale = DH ** (-0.5)
    qm_i = jax.lax.broadcasted_iota(I32, (L - 8, L), 0)
    mask_m = (qm_i < M) | (qm_i + 8 >= jax.lax.broadcasted_iota(I32, (L - 8, L), 1))
    sub = jax.lax.broadcasted_iota(I32, (8, DH), 0)

    def finish(sp, sa):
        r0 = pl.multiple_of(sp * SEG, SEG)
        xb = xb_v[pl.ds(r0, SEG), :]
        g = xb * _sigmoid(xb)
        o = x_v[sp].astype(F32) + sa * g
        out_v[pl.ds(r0, SEG), :] = o.astype(BF16)
        return o

    def out_copy(r0, n):
        return pltpu.make_async_copy(out_v.at[pl.ds(r0, n), :], out_hbm.at[pl.ds(r0, n), :], sem_out.at[0])

    def step(i, u, prev):
        s = i * UNROLL + u
        pre_i = pre.at[:, pl.ds(pl.multiple_of(i * (8 * UNROLL), 8 * UNROLL), 8 * UNROLL), :]
        xa_i = xa_v.at[pl.ds(pl.multiple_of(i * (LIVE * UNROLL), 8 * UNROLL), LIVE * UNROLL), :]
        xa = xa_i[u * LIVE:(u + 1) * LIVE, :]
        lhs = jnp.concatenate([prev[0:M, :], xa], axis=0).astype(BF16)
        fin = finish(jnp.maximum(s - 1, 0) if u == 0 else s - 1, prev[M:L, :])

        def proj(j, tie=None):
            lh = lhs
            if tie is not None:
                top = pltpu.bitcast(lhs[0:16, 0:128], U32)
                top = pltpu.bitcast(jnp.where(i < 0, pltpu.bitcast(tie, U32), top), BF16)
                lh = jnp.concatenate([jnp.concatenate([top, lhs[0:16, 128:]], axis=1), lhs[16:, :]], axis=0)
            t = _dot(lh, pltpu.bitcast(wtile(j)[...], BF16))
            if u == 0 and TIE0 <= j < TIE0 + NT:
                t = jnp.where(i < 0, fin[:, (j - TIE0) * 128:(j - TIE0 + 1) * 128], t)
            return jnp.concatenate([t, pre_i[j, u * 8:(u + 1) * 8, :]], axis=0)

        NG = H // GH
        qs, ks, vs, ps, os_, ox = {}, {}, {}, {}, {}, {}

        def do_qkv(g):
            if ORD == 0:
                js = [m * H + h for h in range(g * GH, (g + 1) * GH) for m in range(3)]
            elif ORD == 1:
                js = [m * H + h for m in range(3) for h in range(g * GH, (g + 1) * GH)]
            else:
                js = [m * H + h for h in range(g * GH, (g + 1) * GH) for m in (1, 0, 2)]
            if g == 0:
                js, rest = js[:6], js[6:]
                part = {}
                for kt in range(NT):
                    for j in js:
                        t = _dot(lhs[:, kt * 128:(kt + 1) * 128],
                                 pltpu.bitcast(wtile(j)[kt * 64:(kt + 1) * 64, :], BF16))
                        part[j] = t if kt == 0 else part[j] + t
                res = {j: jnp.concatenate([part[j], pre_i[j, u * 8:(u + 1) * 8, :]], axis=0) for j in js}
                for j in rest:
                    res[j] = proj(j)
            else:
                res = {}
                for n, j in enumerate(js):
                    tie = None
                    for hh, pos in enumerate(TP):
                        if n == pos and g >= TL:
                            tie = ox[(g - TL) * GH + hh]
                    res[j] = proj(j, tie)
            for h in range(g * GH, (g + 1) * GH):
                qs[h], ks[h], vs[h] = res[h], res[H + h], res[2 * H + h]

        def vpu_rows(h, q, k, v):
            def win(which, val, r):
                if r % 8 == 0:
                    return val[8 - r:16 - r, :]
                return kv_s[h % NKV, which, 16 - r:24 - r, :]

            qa = q[8:16, :] * (scale * LOG2E)
            sj = []
            for r in range(16):
                sc = jnp.sum(qa * win(0, k, r), axis=-1, keepdims=True)
                sc = jnp.broadcast_to(sc, (8, DH))
                if r > 8:
                    sc = jnp.where(sub >= r - 8, sc, -jnp.inf)
                sj.append(sc)
            mx = _tree(jnp.maximum, sj)
            es = [jnp.exp2(x - mx) for x in sj]
            den = _tree(jnp.add, es)
            o = _tree(jnp.add, [e * win(1, v, r) for r, e in enumerate(es)])
            return o * pl.reciprocal(den, approx=True)

        def do_s(g):
            for h in range(g * GH, (g + 1) * GH):
                q, k = qs.pop(h), ks.pop(h)
                kv_s[h % NKV, 0, 8:24, :] = k[0:16, :]
                kv_s[h % NKV, 1, 8:24, :] = vs[h][0:16, :]
                ox[h] = vpu_rows(h, q, k, vs[h])
                qm = jnp.concatenate([q[0:8, :], q[16:, :]], axis=0)
                sc = _dot_nt(qm.astype(BF16) if BQ else qm, k.astype(BF16) if BK else k) * scale
                sc = jnp.where(mask_m, sc, NEG)
                e = jnp.exp(sc - jnp.max(sc, axis=-1, keepdims=True))
                ps[h] = e * pl.reciprocal(jnp.sum(e, axis=-1, keepdims=True), approx=True)

        def do_pv(g):
            for h in range(g * GH, (g + 1) * GH):
                v = vs.pop(h)
                if g >= NG - TL:
                    v = jnp.concatenate([jnp.where(i < 0, ox[h], v[0:8, :]), v[8:, :]], axis=0)
                p_ = ps.pop(h)
                o = _dot(p_.astype(BF16) if BP else p_, v.astype(BF16) if BV else v)
                os_[h] = jnp.concatenate([o[0:8, :], ox.pop(h), o[8:, :]], axis=0)

        def do_o(j, h0, h1):
            o = jnp.concatenate([os_[h] for h in range(h0, h1)], axis=1)
            return _dot(o, pltpu.bitcast(wo_p[j, h0 * 64:h1 * 64, :], BF16))

        for g in range(NG):
            if PVFIRST and g >= LP:
                do_pv(g - LP)
            do_qkv(g)
            if g >= LS:
                do_s(g - LS)
            if not PVFIRST and g >= LP:
                do_pv(g - LP)
        sched = dict(TAIL)
        ns, npv = NG - LS, NG - LP
        for j in range(NT):
            part_v[:, j * 128:(j + 1) * 128] = do_o(j, 0, HS)
            for c_ in sched.get(j, ''):
                if c_ == 's':
                    do_s(ns)
                    ns += 1
                else:
                    do_pv(npv)
                    npv += 1
        assert ns == NG and npv == NG
        return jnp.concatenate(
            [part_v[:, j * 128:(j + 1) * 128] + do_o(j, HS, H) for j in range(NT)], axis=1)

    def multi(i, carry):
        cur = acc[...]
        for u in range(UNROLL):
            cur = step(i, u, cur)
        acc[...] = cur
        r0 = pl.multiple_of(i * (UNROLL * SEG), SEG)
        out_copy(r0, (UNROLL - 1) * SEG).start()

        @pl.when(i > 0)
        def _():
            out_copy(pl.multiple_of(r0 - SEG, SEG), SEG).start()
        return carry

    jax.lax.fori_loop(0, NSEG // UNROLL, multi, 0)
    finish(NSEG - 1, acc[M:L, :])
    out_copy(S - SEG, SEG).start()
    out_copy(0, S).wait()


@jax.jit
def pallas_recurrent_scan__memory_aug_recurrent_mem_tr__moe_arch_mod__prompt_kernel(
    A_x: jax.Array,
    A_mem0: jax.Array,
    A_Wq: jax.Array,
    A_Wk: jax.Array,
    A_Wv: jax.Array,
    A_Wo: jax.Array,
    A_seg_len: jax.Array,
    B_x: jax.Array,
    B_w_r: jax.Array,
    B_w_gate: jax.Array,
    B_w_up: jax.Array,
    B_w_down: jax.Array,
):
    del A_seg_len, B_x
    assert A_x.shape == (1, S, D) and A_Wq.shape == (D, H, DH) and A_mem0.shape == (1, M, D)
    hbm = pl.BlockSpec(memory_space=pltpu.HBM)
    out = pl.pallas_call(
        _kernel,
        out_shape=jax.ShapeDtypeStruct((S, D), BF16),
        in_specs=[hbm] * 10,
        out_specs=hbm,
        scratch_shapes=[
            pltpu.VMEM((NSEG, SEG, D), BF16),
            pltpu.VMEM((NSEG * 4, D), U32),
            pltpu.VMEM((NSEG * LIVE, D), F32),
            pltpu.VMEM((S, D), F32),
            pltpu.VMEM((NPAIR + 1, D, 128), U32),
            pltpu.VMEM((2 * NPAIR + 2, D // 2, 128), U32),
            pltpu.VMEM((NT, H * DH // 2, 128), U32),
            pltpu.VMEM((3 * H, NSEG * 8, DH), F32),
            pltpu.VMEM((FF, D), BF16),
            pltpu.VMEM((FF, D), BF16),
            pltpu.VMEM((FF, D), BF16),
            pltpu.VMEM((S, D), BF16),
            pltpu.VMEM((L, D), F32),
            pltpu.VMEM((L, D), F32),
            pltpu.VMEM((NKV, 2, 24, DH), F32),
            pltpu.VMEM((TOPC, D), F32),
            pltpu.VMEM((TOPC, D), F32),
            pltpu.VMEM((TOPC, D), F32),
            pltpu.VMEM((SEG, 128), F32),
            pltpu.VMEM((M, D), BF16),
            pltpu.VMEM((NT, 128), BF16),
            pltpu.SMEM((TOPC,), I32),
            pltpu.SemaphoreType.DMA((18,)),
            pltpu.SemaphoreType.DMA((1,)),
        ],
        compiler_params=pltpu.CompilerParams(vmem_limit_bytes=110 * 1024 * 1024),
    )(
        A_x.reshape(NSEG, SEG, D),
        A_mem0.reshape(M, D),
        A_Wq, A_Wk, A_Wv,
        A_Wo.reshape(H * DH, D),
        B_w_r.reshape(NT, 128),
        B_w_gate.T, B_w_up.T, B_w_down,
    )
    return out.reshape(1, S, D)
```

```python
import math

import jax
import jax.numpy as jnp
import jax.experimental.pallas as pl
import jax.experimental.pallas.tpu as pltpu

F32 = jnp.float32
BF16 = jnp.bfloat16
U32 = jnp.uint32
I32 = jnp.int32

S = 2048
D = 640
H = 32
DH = 128
M = 8
SEG = 32
NSEG = S // SEG
L = M + SEG
FF = 1728
TOPC = 8
NT = D // 128
LIVE = SEG - 8
EPS = 1e-05
NEG = -1000000000.0
LOG2E = math.log2(math.e)
NPAIR = 3 * H // 2
KEY_NONE = -1e30

UNROLL = 8
GH = 2
LS, LP = 1, 2
TL, TP = 2, (3, 5)
HS = 24
TAIL = ((0, 'sp'), (2, 'p'))
TIE0 = 2
MS0, MS1 = 3, 153


def _dot(a, b):
    return jax.lax.dot_general(a, b, (((1,), (0,)), ((), ())), preferred_element_type=F32)


def _dot_nt(a, b):
    return jax.lax.dot_general(a, b, (((1,), (1,)), ((), ())), preferred_element_type=F32)


def _rb(x):
    return x.astype(BF16).astype(F32)


def _sigmoid(x):
    return pl.reciprocal(1.0 + jnp.exp(-x), approx=True)


def _tree(f, xs):
    while len(xs) > 1:
        xs = [f(xs[n], xs[n + 1]) if n + 1 < len(xs) else xs[n] for n in range(0, len(xs), 2)]
    return xs[0]


def _kernel(x_hbm, mem0_hbm, wq_hbm, wk_hbm, wv_hbm, wo_hbm, wr_hbm, wg_hbm, wu_hbm, wd_hbm,
            out_hbm,
            x_v, lhs_v, xa_v, xb_v, raw, w_p, wo_p, pre, wg_v, wu_v, wd_v,
            out_v, acc, part_v, kv_s, sel, upd, yacc, keys, mem0_v, wr_v, idx_s,
            sem_in, sem_out):
    w_hbm = [wq_hbm, wk_hbm, wv_hbm]

    def wtile(j):
        return w_p.at[j]

    SEM_X8, SEM_B0, SEM_LN, SEM_TK, SEM_MLP, SEM_WO = 0, 4, 7, 15, 16, 17

    def w_start(q0, n, sem):
        for q in range(q0, q0 + n):
            src = w_hbm[q // 16].bitcast(U32).at[:, q % 16, :]
            pltpu.make_async_copy(src, raw.at[q], sem_in.at[sem]).start()

    def w_wait(q0, n, sem):
        blk = raw.at[pl.ds(q0, n)]
        pltpu.make_async_copy(blk, blk, sem_in.at[sem]).wait()

    def x8_copy(b):
        return pltpu.make_async_copy(x_hbm.at[pl.ds(b * 16, 16), pl.ds(LIVE, 8), :],
                                     x_v.at[pl.ds(b * 16, 16), pl.ds(LIVE, 8), :], sem_in.at[SEM_X8 + b])

    def xa_copy(i):
        return pltpu.make_async_copy(x_hbm.at[pl.ds(i * 8, 8), pl.ds(0, LIVE), :],
                                     x_v.at[pl.ds(i * 8, 8), pl.ds(0, LIVE), :], sem_in.at[SEM_LN + i])

    cp_wr = pltpu.make_async_copy(wr_hbm, wr_v, sem_in.at[SEM_B0 + 2])
    cp_mem = pltpu.make_async_copy(mem0_hbm, mem0_v, sem_in.at[SEM_TK])
    mlp_copies = [pltpu.make_async_copy(s_, d_, sem_in.at[SEM_MLP])
                  for s_, d_ in [(wg_hbm, wg_v), (wu_hbm, wu_v), (wd_hbm, wd_v)]]
    wo32 = wo_hbm.bitcast(U32)
    wo_copies = [pltpu.make_async_copy(wo32.at[:, pl.ds(j * 128, 128)], wo_p.at[j], sem_in.at[SEM_WO])
                 for j in range(NT)]

    for b in range(4):
        x8_copy(b).start()
    w_start(0, 1, SEM_B0)
    w_start(1, 1, SEM_B0 + 1)
    w_start(2, 2, SEM_B0 + 2)
    cp_wr.start()
    for i in range(8):
        w_start(4 + 4 * i, 4, SEM_LN + i)
        xa_copy(i).start()
    w_start(36, NPAIR - 36, SEM_TK)
    cp_mem.start()
    for c in mlp_copies:
        c.start()
    for c in wo_copies:
        c.start()

    xb3 = xb_v.reshape(NSEG, SEG, D)
    keys[...] = jnp.full(keys.shape, KEY_NONE, F32)
    yacc[...] = jnp.zeros(yacc.shape, F32)
    kv_s[:, :, 0:8, :] = jnp.zeros((H, 2, 8, DH), F32)
    raw[NPAIR] = jnp.zeros((D, 128), U32)
    acc[M:L, :] = jnp.zeros((SEG, D), F32)

    def router_w():
        wr5 = wr_v[...].astype(F32)
        return jnp.concatenate([wr5[j:j + 1, :] for j in range(NT)], axis=1)

    def layernorm(s0, nseg, t0, nrow):
        n = nseg * nrow
        x = x_v[pl.ds(s0, nseg), t0:t0 + nrow, :].astype(F32).reshape(n, D)
        mu = jnp.sum(x, axis=-1, keepdims=True) * (1.0 / D)
        xc = x - mu
        var = jnp.sum(xc * xc, axis=-1, keepdims=True) * (1.0 / D)
        sd = _rb(jnp.sqrt(_rb(_rb(var) + EPS)))
        xn = _rb(_rb(x - _rb(mu)) / sd)
        xb3[pl.ds(s0, nseg), t0:t0 + nrow, :] = xn.reshape(nseg, nrow, D)
        return xn

    def ln8_body(b, carry):
        x8_copy(b).wait()
        xn = layernorm(b * 16, 16, LIVE, 8)
        lhs_v[pl.ds(pl.multiple_of(b * 64, 64), 64), :] = pltpu.bitcast(xn.astype(BF16), U32)
        return carry

    jax.lax.fori_loop(0, 4, ln8_body, 0)

    def ln_seg(s, wr):
        tail = xb3[s, LIVE:SEG, :]
        xn = layernorm(s, 1, 0, LIVE)
        xa_v[pl.ds(pl.multiple_of(s * LIVE, 8), LIVE), :] = xn
        r = _rb(jnp.sum(jnp.concatenate([xn, tail], axis=0) * wr, axis=-1, keepdims=True))
        r = jnp.where(r == 0.0, 0.0, r)
        bits = pltpu.bitcast(jnp.broadcast_to(r, (SEG, 128)), I32) >> 16
        mono = jnp.where(bits < 0, (-32768) - bits, bits)
        mono = jnp.where(r != r, -40000, mono)
        row = jax.lax.broadcasted_iota(I32, (SEG, 128), 0)
        key = (mono * SEG + ((SEG - 1) - row)).astype(F32)
        lane = jax.lax.broadcasted_iota(I32, (SEG, 128), 1)
        keys[...] = jnp.where(lane == s, key, keys[...])
        return pltpu.bitcast(key, U32)

    def top_rows():
        kv = keys[...]
        lane = jax.lax.broadcasted_iota(I32, (1, 128), 1).astype(F32)
        for c in range(TOPC):
            col = jnp.max(kv, axis=0, keepdims=True)
            val = jnp.floor(col * (1.0 / SEG))
            fk = val * 128.0 + (127.0 - lane)
            win = fk == jnp.max(fk, axis=1, keepdims=True)
            kv = jnp.where(win & (kv == col), KEY_NONE, kv)
            pos = lane * SEG + ((SEG - 1.0) - (col - val * SEG))
            idx = jnp.clip(jnp.max(jnp.where(win, pos, 0.0)).astype(I32), 0, S - 1)
            idx_s[c] = idx
            sel[pl.ds(c, 1), :] = xb_v[pl.ds(idx, 1), :]

    def repack(rv, wv, p, part=None, tie=None):
        m_lo = jnp.full((8, 128), 0xFFFF, U32)
        m_hi = jnp.full((8, 128), 0xFFFF0000, U32)
        if tie is not None:
            m_lo = jnp.where(tie[0], tie[1], m_lo)
            m_hi = jnp.where(tie[0], tie[1], m_hi)
        for g in range(D // 16):
            if part is not None and g % part[1] != part[0]:
                continue
            a = rv[p, pl.ds(16 * g, 8, stride=2), :]
            b = rv[p, pl.ds(16 * g + 1, 8, stride=2), :]
            wv[2 * p, 8 * g:8 * g + 8, :] = (a & m_lo) | (b << 16)
            wv[2 * p + 1, 8 * g:8 * g + 8, :] = (a >> 16) | (b & m_hi)

    def block(q0, n, never=None, side=None, jobs=None):
        rv = raw.at[pl.ds(q0, n + 1)]
        wv = w_p.at[pl.ds(2 * q0, 2 * n + 2)]
        pv = pre.at[pl.ds(2 * q0, 2 * n)]
        for u in range(2 * n):
            if u % 2 == 0 and u // 2 + 1 < n:
                repack(rv, wv, u // 2 + 1)
            for c in range(4):
                lhs = lhs_v[c * 64:(c + 1) * 64, :]
                if side is not None and c == 3:
                    tok = side(u)
                    nr = tok.shape[0]
                    head = jnp.where(never, tok, lhs[0:nr, 0:128])
                    lhs = jnp.concatenate(
                        [jnp.concatenate([head, lhs[0:nr, 128:]], axis=1), lhs[nr:, :]], axis=0)
                lhs = pltpu.bitcast(lhs, BF16)
                if jobs:
                    r = None
                    for kt in range(NT):
                        t_ = _dot(lhs[:, kt * 128:(kt + 1) * 128],
                                  pltpu.bitcast(wv[u, kt * 64:(kt + 1) * 64, :], BF16))
                        r = t_ if r is None else r + t_
                        if jobs:
                            jobs.pop(0)()
                else:
                    r = _dot(lhs, pltpu.bitcast(wv[u], BF16))
                pv[u, c * 128:(c + 1) * 128, :] = r
                n8 = (u - max(2 * n - 3, 0)) * 4 + c
                if 0 <= n8 < 8:
                    repack(rv, wv, n, (n8, 8),
                           None if never is None else (never, pltpu.bitcast(r[0:8, :], U32)))

    w_wait(0, 1, SEM_B0)
    repack(raw, w_p, 0)
    w_wait(1, 1, SEM_B0 + 1)
    block(0, 1)
    w_wait(2, 2, SEM_B0 + 2)
    cp_wr.wait()
    block(1, 2)

    def ln_body(i, carry):
        w_wait(4 + 4 * i, 4, SEM_LN + i)
        xa_copy(i).wait()
        wr = router_w()
        block(3 + 4 * i, 4, i < 0, side=lambda u: ln_seg(i * 8 + u, wr))
        return carry

    jax.lax.fori_loop(0, 8, ln_body, 0)

    w_wait(36, NPAIR - 36, SEM_TK)
    cp_mem.wait()
    acc[0:M, :] = mem0_v[...].astype(F32)
    top_rows()
    block(35, 1)

    for c in mlp_copies:
        c.wait()
    FP = FF // 3

    def mlp_body(t, carry):
        f0 = pl.multiple_of(t * FP, 16)
        xs = sel[...]
        cuts = [(a_, min(a_ + 128, FP)) for a_ in range(0, FP, 128)]
        val = {}

        def up_tile(which, n, kt):
            def run():
                a_, b_ = cuts[n]
                w = (wg_v, wu_v)[which][pl.ds(f0 + a_, b_ - a_), kt * 128:(kt + 1) * 128]
                r = _dot_nt(xs[:, kt * 128:(kt + 1) * 128], w)
                val[which, n] = r if kt == 0 else val[which, n] + r
            return run

        def down_tile(n, j):
            def run():
                a_, b_ = cuts[n]
                if j == 0:
                    g_ = _rb(val.pop((0, n)))
                    val['h', n] = _rb(g_ * _sigmoid(g_)) * _rb(val.pop((1, n)))
                r = _dot(val['h', n], wd_v[pl.ds(f0 + a_, b_ - a_), j * 128:(j + 1) * 128])
                val['y', j] = r if n == 0 else val['y', j] + r
            return run

        def skip():
            pass

        real = ([up_tile(which, n, kt) for n in range(len(cuts)) for which in range(2) for kt in range(NT)]
                + [down_tile(n, j) for n in range(len(cuts)) for j in range(NT)])
        jobs = [skip] * MS1
        for n_, job in enumerate(real):
            jobs[MS0 + (n_ * (MS1 - MS0)) // len(real)] = job
        block(36 + 4 * t, 4, t < 0, jobs=jobs)
        assert not jobs
        y = yacc[...] + jnp.concatenate([val['y', j] for j in range(NT)], axis=1)
        yacc[...] = y
        r_sel = _rb(jnp.sum(xs * router_w(), axis=-1, keepdims=True))
        upd[...] = xs + _rb(_rb(y) * _rb(_sigmoid(r_sel)))
        for c in range(TOPC):
            xb_v[pl.ds(jnp.clip(idx_s[c], 0, S - 1), 1), :] = upd[pl.ds(c, 1), :]
        return carry

    jax.lax.fori_loop(0, 3, mlp_body, 0)

    for c in wo_copies:
        c.wait()

    scale = DH ** (-0.5)
    qm_i = jax.lax.broadcasted_iota(I32, (L - 8, L), 0)
    mask_m = (qm_i < M) | (qm_i + 8 >= jax.lax.broadcasted_iota(I32, (L - 8, L), 1))
    sub = jax.lax.broadcasted_iota(I32, (8, DH), 0)

    def finish(sp, sa):
        r0 = pl.multiple_of(sp * SEG, SEG)
        xb = xb_v[pl.ds(r0, SEG), :]
        g = xb * _sigmoid(xb)
        o = x_v[sp].astype(F32) + sa * g
        out_v[pl.ds(r0, SEG), :] = o.astype(BF16)
        return o

    def out_copy(r0, n):
        return pltpu.make_async_copy(out_v.at[pl.ds(r0, n), :], out_hbm.at[pl.ds(r0, n), :], sem_out.at[0])

    def step(i, u, prev):
        s = i * UNROLL + u
        pre_i = pre.at[:, pl.ds(pl.multiple_of(i * (8 * UNROLL), 8 * UNROLL), 8 * UNROLL), :]
        xa_i = xa_v.at[pl.ds(pl.multiple_of(i * (LIVE * UNROLL), 8 * UNROLL), LIVE * UNROLL), :]
        xa = xa_i[u * LIVE:(u + 1) * LIVE, :]
        lhs = jnp.concatenate([prev[0:M, :], xa], axis=0).astype(BF16)
        fin = finish(jnp.maximum(s - 1, 0) if u == 0 else s - 1, prev[M:L, :])

        def proj(j, tie=None):
            lh = lhs
            if tie is not None:
                top = pltpu.bitcast(lhs[0:16, 0:128], U32)
                top = pltpu.bitcast(jnp.where(i < 0, pltpu.bitcast(tie, U32), top), BF16)
                lh = jnp.concatenate([jnp.concatenate([top, lhs[0:16, 128:]], axis=1), lhs[16:, :]], axis=0)
            t = _dot(lh, pltpu.bitcast(wtile(j)[...], BF16))
            if u == 0 and TIE0 <= j < TIE0 + NT:
                t = jnp.where(i < 0, fin[:, (j - TIE0) * 128:(j - TIE0 + 1) * 128], t)
            return jnp.concatenate([t, pre_i[j, u * 8:(u + 1) * 8, :]], axis=0)

        NG = H // GH
        qs, ks, vs, ps, os_, ox, iv, on = {}, {}, {}, {}, {}, {}, {}, {}

        def do_qkv(g):
            js = [m * H + h for h in range(g * GH, (g + 1) * GH) for m in range(3)]
            if g == 0:
                part = {}
                for kt in range(NT):
                    for j in js:
                        t = _dot(lhs[:, kt * 128:(kt + 1) * 128],
                                 pltpu.bitcast(wtile(j)[kt * 64:(kt + 1) * 64, :], BF16))
                        part[j] = t if kt == 0 else part[j] + t
                res = {j: jnp.concatenate([part[j], pre_i[j, u * 8:(u + 1) * 8, :]], axis=0) for j in js}
            else:
                res = {}
                for n, j in enumerate(js):
                    tie = None
                    for hh, pos in enumerate(TP):
                        if n == pos and g >= TL:
                            tie = ox[(g - TL) * GH + hh]
                    res[j] = proj(j, tie)
            for h in range(g * GH, (g + 1) * GH):
                qs[h], ks[h], vs[h] = res[h], res[H + h], res[2 * H + h]

        def vpu_rows(h, q, k, v):
            def win(which, val, r):
                if r % 8 == 0:
                    return val[8 - r:16 - r, :]
                return kv_s[h, which, 16 - r:24 - r, :]

            qa = q[8:16, :] * (scale * LOG2E)
            sj = []
            for r in range(16):
                sc = jnp.sum(qa * win(0, k, r), axis=-1, keepdims=True)
                sc = jnp.broadcast_to(sc, (8, DH))
                if r > 8:
                    sc = jnp.where(sub >= r - 8, sc, -jnp.inf)
                sj.append(sc)
            mx = _tree(jnp.maximum, sj)
            es = [jnp.exp2(x - mx) for x in sj]
            den = _tree(jnp.add, es)
            o = _tree(jnp.add, [e * win(1, v, r) for r, e in enumerate(es)])
            return o * pl.reciprocal(den, approx=True)

        def do_s(g):
            for h in range(g * GH, (g + 1) * GH):
                q, k = qs.pop(h), ks.pop(h)
                kv_s[h, 0, 8:24, :] = k[0:16, :]
                kv_s[h, 1, 8:24, :] = vs[h][0:16, :]
                ox[h] = vpu_rows(h, q, k, vs[h])
                qm = jnp.concatenate([q[0:8, :], q[16:, :]], axis=0)
                sc = _dot_nt(qm.astype(BF16), k.astype(BF16))
                sc = jnp.where(mask_m, sc * (scale * LOG2E), NEG * LOG2E)
                e = jnp.exp2(sc - jnp.max(sc, axis=-1, keepdims=True))
                inv = pl.reciprocal(jnp.sum(e, axis=-1, keepdims=True), approx=True)
                ps[h] = e.astype(BF16)
                iv[h] = jnp.broadcast_to(inv, (SEG, DH))

        def do_pv(g):
            for h in range(g * GH, (g + 1) * GH):
                v = vs.pop(h)
                if g >= NG - TL:
                    v = jnp.concatenate([jnp.where(i < 0, ox[h], v[0:8, :]), v[8:, :]], axis=0)
                if h >= GH:
                    v = jnp.concatenate([v[0:8, :], jnp.where(i < 0, on[h - GH], v[8:, :])], axis=0)
                on[h] = _dot(ps.pop(h), v.astype(BF16)) * iv.pop(h)
                os_[h] = jnp.concatenate([on[h][0:8, :], ox[h], on[h][8:, :]], axis=0)

        def do_o(j, h0, h1):
            o = jnp.concatenate([os_[h] for h in range(h0, h1)], axis=1)
            return _dot(o, pltpu.bitcast(wo_p[j, h0 * 64:h1 * 64, :], BF16))

        for g in range(NG):
            do_qkv(g)
            if g >= LS:
                do_s(g - LS)
            if g >= LP:
                do_pv(g - LP)
        sched = dict(TAIL)
        ns, npv = NG - LS, NG - LP
        for j in range(NT):
            part_v[:, j * 128:(j + 1) * 128] = do_o(j, 0, HS)
            for c_ in sched.get(j, ''):
                if c_ == 's':
                    do_s(ns)
                    ns += 1
                else:
                    do_pv(npv)
                    npv += 1
        assert ns == NG and npv == NG
        return jnp.concatenate(
            [part_v[:, j * 128:(j + 1) * 128] + do_o(j, HS, H) for j in range(NT)], axis=1)

    def multi(i, carry):
        cur = acc[...]
        for u in range(UNROLL):
            cur = step(i, u, cur)
        acc[...] = cur
        r0 = pl.multiple_of(i * (UNROLL * SEG), SEG)
        out_copy(r0, (UNROLL - 1) * SEG).start()

        @pl.when(i > 0)
        def _():
            out_copy(pl.multiple_of(r0 - SEG, SEG), SEG).start()
        return carry

    jax.lax.fori_loop(0, NSEG // UNROLL, multi, 0)
    finish(NSEG - 1, acc[M:L, :])
    out_copy(S - SEG, SEG).start()
    out_copy(0, S).wait()


@jax.jit
def pallas_recurrent_scan__memory_aug_recurrent_mem_tr__moe_arch_mod__prompt_kernel(
    A_x: jax.Array,
    A_mem0: jax.Array,
    A_Wq: jax.Array,
    A_Wk: jax.Array,
    A_Wv: jax.Array,
    A_Wo: jax.Array,
    A_seg_len: jax.Array,
    B_x: jax.Array,
    B_w_r: jax.Array,
    B_w_gate: jax.Array,
    B_w_up: jax.Array,
    B_w_down: jax.Array,
):
    del A_seg_len, B_x
    assert A_x.shape == (1, S, D) and A_Wq.shape == (D, H, DH) and A_mem0.shape == (1, M, D)
    hbm = pl.BlockSpec(memory_space=pltpu.HBM)
    out = pl.pallas_call(
        _kernel,
        out_shape=jax.ShapeDtypeStruct((S, D), BF16),
        in_specs=[hbm] * 10,
        out_specs=hbm,
        scratch_shapes=[
            pltpu.VMEM((NSEG, SEG, D), BF16),
            pltpu.VMEM((NSEG * 4, D), U32),
            pltpu.VMEM((NSEG * LIVE, D), F32),
            pltpu.VMEM((S, D), F32),
            pltpu.VMEM((NPAIR + 1, D, 128), U32),
            pltpu.VMEM((2 * NPAIR + 2, D // 2, 128), U32),
            pltpu.VMEM((NT, H * DH // 2, 128), U32),
            pltpu.VMEM((3 * H, NSEG * 8, DH), F32),
            pltpu.VMEM((FF, D), BF16),
            pltpu.VMEM((FF, D), BF16),
            pltpu.VMEM((FF, D), BF16),
            pltpu.VMEM((S, D), BF16),
            pltpu.VMEM((L, D), F32),
            pltpu.VMEM((L, D), F32),
            pltpu.VMEM((H, 2, 24, DH), F32),
            pltpu.VMEM((TOPC, D), F32),
            pltpu.VMEM((TOPC, D), F32),
            pltpu.VMEM((TOPC, D), F32),
            pltpu.VMEM((SEG, 128), F32),
            pltpu.VMEM((M, D), BF16),
            pltpu.VMEM((NT, 128), BF16),
            pltpu.SMEM((TOPC,), I32),
            pltpu.SemaphoreType.DMA((18,)),
            pltpu.SemaphoreType.DMA((1,)),
        ],
        compiler_params=pltpu.CompilerParams(vmem_limit_bytes=110 * 1024 * 1024),
    )(
        A_x.reshape(NSEG, SEG, D),
        A_mem0.reshape(M, D),
        A_Wq, A_Wk, A_Wv,
        A_Wo.reshape(H * DH, D),
        B_w_r.reshape(NT, 128),
        B_w_gate.T, B_w_up.T, B_w_down,
    )
    return out.reshape(1, S, D)
```

```python
import math

import jax
import jax.numpy as jnp
import jax.experimental.pallas as pl
import jax.experimental.pallas.tpu as pltpu

F32 = jnp.float32
BF16 = jnp.bfloat16
U32 = jnp.uint32
I32 = jnp.int32

S = 2048
D = 640
H = 32
DH = 128
M = 8
SEG = 32
NSEG = S // SEG
L = M + SEG
FF = 1728
TOPC = 8
NT = D // 128
LIVE = SEG - 8
EPS = 1e-05
NEG = -1000000000.0
LOG2E = math.log2(math.e)
NPAIR = 3 * H // 2
KEY_NONE = -1e30

UNROLL = 8
GH = 2
LS, LP = 1, 2
TL, TP = 2, (3, 5)
HS = 24
TAIL = ((0, 'sp'), (2, 'p'))
TIE0 = 2
MS0, MS1 = 3, 153


def _dot(a, b):
    return jax.lax.dot_general(a, b, (((1,), (0,)), ((), ())), preferred_element_type=F32)


def _dot_nt(a, b):
    return jax.lax.dot_general(a, b, (((1,), (1,)), ((), ())), preferred_element_type=F32)


def _rb(x):
    return x.astype(BF16).astype(F32)


def _sigmoid(x):
    return pl.reciprocal(1.0 + jnp.exp(-x), approx=True)


def _tree(f, xs):
    while len(xs) > 1:
        xs = [f(xs[n], xs[n + 1]) if n + 1 < len(xs) else xs[n] for n in range(0, len(xs), 2)]
    return xs[0]


def _kernel(x_hbm, mem0_hbm, wq_hbm, wk_hbm, wv_hbm, wo_hbm, wr_hbm, wg_hbm, wu_hbm, wd_hbm,
            out_hbm,
            x_v, lhs_v, xa_v, xb_v, raw, w_p, wo_p, pre, wg_v, wu_v, wd_v,
            out_v, acc, part_v, kv_s, sel, upd, yacc, keys, mem0_v, wr_v, idx_s,
            sem_in, sem_out):
    w_hbm = [wq_hbm, wk_hbm, wv_hbm]

    def wtile(j):
        return w_p.at[j]

    SEM_X8, SEM_B0, SEM_LN, SEM_TK, SEM_MLP, SEM_WO = 0, 4, 7, 15, 16, 17

    def w_start(q0, n, sem):
        for q in range(q0, q0 + n):
            src = w_hbm[q // 16].bitcast(U32).at[:, q % 16, :]
            pltpu.make_async_copy(src, raw.at[q], sem_in.at[sem]).start()

    def w_wait(q0, n, sem):
        blk = raw.at[pl.ds(q0, n)]
        pltpu.make_async_copy(blk, blk, sem_in.at[sem]).wait()

    def x8_copy(b):
        return pltpu.make_async_copy(x_hbm.at[pl.ds(b * 16, 16), pl.ds(LIVE, 8), :],
                                     x_v.at[pl.ds(b * 16, 16), pl.ds(LIVE, 8), :], sem_in.at[SEM_X8 + b])

    def xa_copy(i):
        return pltpu.make_async_copy(x_hbm.at[pl.ds(i * 8, 8), pl.ds(0, LIVE), :],
                                     x_v.at[pl.ds(i * 8, 8), pl.ds(0, LIVE), :], sem_in.at[SEM_LN + i])

    cp_wr = pltpu.make_async_copy(wr_hbm, wr_v, sem_in.at[SEM_B0 + 2])
    cp_mem = pltpu.make_async_copy(mem0_hbm, mem0_v, sem_in.at[SEM_TK])
    mlp_copies = [pltpu.make_async_copy(s_, d_, sem_in.at[SEM_MLP])
                  for s_, d_ in [(wg_hbm, wg_v), (wu_hbm, wu_v), (wd_hbm, wd_v)]]
    wo32 = wo_hbm.bitcast(U32)
    wo_copies = [pltpu.make_async_copy(wo32.at[:, pl.ds(j * 128, 128)], wo_p.at[j], sem_in.at[SEM_WO])
                 for j in range(NT)]

    for b in range(4):
        x8_copy(b).start()
    w_start(0, 1, SEM_B0)
    w_start(1, 1, SEM_B0 + 1)
    w_start(2, 2, SEM_B0 + 2)
    cp_wr.start()
    for i in range(8):
        w_start(4 + 4 * i, 4, SEM_LN + i)
        xa_copy(i).start()
    w_start(36, NPAIR - 36, SEM_TK)
    cp_mem.start()
    for c in mlp_copies:
        c.start()
    for c in wo_copies:
        c.start()

    xb3 = xb_v.reshape(NSEG, SEG, D)
    keys[...] = jnp.full(keys.shape, KEY_NONE, F32)
    yacc[...] = jnp.zeros(yacc.shape, F32)
    kv_s[:, :, 0:8, :] = jnp.zeros((H, 2, 8, DH), F32)
    raw[NPAIR] = jnp.zeros((D, 128), U32)
    acc[M:L, :] = jnp.zeros((SEG, D), F32)

    def router_w():
        wr5 = wr_v[...].astype(F32)
        return jnp.concatenate([wr5[j:j + 1, :] for j in range(NT)], axis=1)

    def layernorm(s0, nseg, t0, nrow):
        n = nseg * nrow
        x = x_v[pl.ds(s0, nseg), t0:t0 + nrow, :].astype(F32).reshape(n, D)
        mu = jnp.sum(x, axis=-1, keepdims=True) * (1.0 / D)
        xc = x - mu
        var = jnp.sum(xc * xc, axis=-1, keepdims=True) * (1.0 / D)
        sd = _rb(jnp.sqrt(_rb(_rb(var) + EPS)))
        xn = _rb(_rb(x - _rb(mu)) / sd)
        xb3[pl.ds(s0, nseg), t0:t0 + nrow, :] = xn.reshape(nseg, nrow, D)
        return xn

    def ln8_body(b, carry):
        x8_copy(b).wait()
        xn = layernorm(b * 16, 16, LIVE, 8)
        lhs_v[pl.ds(pl.multiple_of(b * 64, 64), 64), :] = pltpu.bitcast(xn.astype(BF16), U32)
        return carry

    jax.lax.fori_loop(0, 4, ln8_body, 0)

    def ln_seg(s, wr):
        tail = xb3[s, LIVE:SEG, :]
        xn = layernorm(s, 1, 0, LIVE)
        xa_v[pl.ds(pl.multiple_of(s * LIVE, 8), LIVE), :] = xn
        r = _rb(jnp.sum(jnp.concatenate([xn, tail], axis=0) * wr, axis=-1, keepdims=True))
        r = jnp.where(r == 0.0, 0.0, r)
        bits = pltpu.bitcast(jnp.broadcast_to(r, (SEG, 128)), I32) >> 16
        mono = jnp.where(bits < 0, (-32768) - bits, bits)
        mono = jnp.where(r != r, -40000, mono)
        row = jax.lax.broadcasted_iota(I32, (SEG, 128), 0)
        key = (mono * SEG + ((SEG - 1) - row)).astype(F32)
        lane = jax.lax.broadcasted_iota(I32, (SEG, 128), 1)
        keys[...] = jnp.where(lane == s, key, keys[...])
        return pltpu.bitcast(key, U32)

    def top_rows():
        kv = keys[...]
        lane = jax.lax.broadcasted_iota(I32, (1, 128), 1).astype(F32)
        for c in range(TOPC):
            col = jnp.max(kv, axis=0, keepdims=True)
            val = jnp.floor(col * (1.0 / SEG))
            fk = val * 128.0 + (127.0 - lane)
            win = fk == jnp.max(fk, axis=1, keepdims=True)
            kv = jnp.where(win & (kv == col), KEY_NONE, kv)
            pos = lane * SEG + ((SEG - 1.0) - (col - val * SEG))
            idx = jnp.clip(jnp.max(jnp.where(win, pos, 0.0)).astype(I32), 0, S - 1)
            idx_s[c] = idx
            sel[pl.ds(c, 1), :] = xb_v[pl.ds(idx, 1), :]

    def repack(rv, wv, p, part=None, tie=None):
        m_lo = jnp.full((8, 128), 0xFFFF, U32)
        m_hi = jnp.full((8, 128), 0xFFFF0000, U32)
        if tie is not None:
            m_lo = jnp.where(tie[0], tie[1], m_lo)
            m_hi = jnp.where(tie[0], tie[1], m_hi)
        for g in range(D // 16):
            if part is not None and g % part[1] != part[0]:
                continue
            a = rv[p, pl.ds(16 * g, 8, stride=2), :]
            b = rv[p, pl.ds(16 * g + 1, 8, stride=2), :]
            wv[2 * p, 8 * g:8 * g + 8, :] = (a & m_lo) | (b << 16)
            wv[2 * p + 1, 8 * g:8 * g + 8, :] = (a >> 16) | (b & m_hi)

    def block(q0, n, never=None, side=None, jobs=None):
        rv = raw.at[pl.ds(q0, n + 1)]
        wv = w_p.at[pl.ds(2 * q0, 2 * n + 2)]
        pv = pre.at[pl.ds(2 * q0, 2 * n)]
        for u in range(2 * n):
            if u % 2 == 0 and u // 2 + 1 < n:
                repack(rv, wv, u // 2 + 1)
            for c in range(4):
                lhs = lhs_v[c * 64:(c + 1) * 64, :]
                if side is not None and c == 3:
                    tok = side(u)
                    nr = tok.shape[0]
                    head = jnp.where(never, tok, lhs[0:nr, 0:128])
                    lhs = jnp.concatenate(
                        [jnp.concatenate([head, lhs[0:nr, 128:]], axis=1), lhs[nr:, :]], axis=0)
                lhs = pltpu.bitcast(lhs, BF16)
                if jobs:
                    r = None
                    for kt in range(NT):
                        t_ = _dot(lhs[:, kt * 128:(kt + 1) * 128],
                                  pltpu.bitcast(wv[u, kt * 64:(kt + 1) * 64, :], BF16))
                        r = t_ if r is None else r + t_
                        if jobs:
                            jobs.pop(0)()
                else:
                    r = _dot(lhs, pltpu.bitcast(wv[u], BF16))
                pv[u, c * 128:(c + 1) * 128, :] = r
                n8 = (u - max(2 * n - 3, 0)) * 4 + c
                if 0 <= n8 < 8:
                    repack(rv, wv, n, (n8, 8),
                           None if never is None else (never, pltpu.bitcast(r[0:8, :], U32)))

    w_wait(0, 1, SEM_B0)
    repack(raw, w_p, 0)
    w_wait(1, 1, SEM_B0 + 1)
    block(0, 1)
    w_wait(2, 2, SEM_B0 + 2)
    cp_wr.wait()
    block(1, 2)

    def ln_body(i, carry):
        w_wait(4 + 4 * i, 4, SEM_LN + i)
        xa_copy(i).wait()
        wr = router_w()
        block(3 + 4 * i, 4, i < 0, side=lambda u: ln_seg(i * 8 + u, wr))
        return carry

    jax.lax.fori_loop(0, 8, ln_body, 0)

    w_wait(36, NPAIR - 36, SEM_TK)
    cp_mem.wait()
    acc[0:M, :] = mem0_v[...].astype(F32)
    top_rows()
    block(35, 1)

    for c in mlp_copies:
        c.wait()
    FP = FF // 3

    def mlp_body(t, carry):
        f0 = pl.multiple_of(t * FP, 16)
        xs = sel[...]
        cuts = [(a_, min(a_ + 128, FP)) for a_ in range(0, FP, 128)]
        val = {}

        def up_tile(which, n, kt):
            def run():
                a_, b_ = cuts[n]
                w = (wg_v, wu_v)[which][pl.ds(f0 + a_, b_ - a_), kt * 128:(kt + 1) * 128]
                r = _dot_nt(xs[:, kt * 128:(kt + 1) * 128], w)
                val[which, n] = r if kt == 0 else val[which, n] + r
            return run

        def down_tile(n, j):
            def run():
                a_, b_ = cuts[n]
                if j == 0:
                    g_ = _rb(val.pop((0, n)))
                    val['h', n] = _rb(g_ * _sigmoid(g_)) * _rb(val.pop((1, n)))
                r = _dot(val['h', n], wd_v[pl.ds(f0 + a_, b_ - a_), j * 128:(j + 1) * 128])
                val['y', j] = r if n == 0 else val['y', j] + r
            return run

        def skip():
            pass

        real = ([up_tile(which, n, kt) for n in range(len(cuts)) for which in range(2) for kt in range(NT)]
                + [down_tile(n, j) for n in range(len(cuts)) for j in range(NT)])
        jobs = [skip] * MS1
        for n_, job in enumerate(real):
            jobs[MS0 + (n_ * (MS1 - MS0)) // len(real)] = job
        block(36 + 4 * t, 4, t < 0, jobs=jobs)
        assert not jobs
        y = yacc[...] + jnp.concatenate([val['y', j] for j in range(NT)], axis=1)
        yacc[...] = y
        r_sel = _rb(jnp.sum(xs * router_w(), axis=-1, keepdims=True))
        upd[...] = xs + _rb(_rb(y) * _rb(_sigmoid(r_sel)))
        for c in range(TOPC):
            xb_v[pl.ds(jnp.clip(idx_s[c], 0, S - 1), 1), :] = upd[pl.ds(c, 1), :]
        return carry

    jax.lax.fori_loop(0, 3, mlp_body, 0)

    for c in wo_copies:
        c.wait()

    scale = DH ** (-0.5)
    qm_i = jax.lax.broadcasted_iota(I32, (L - 8, L), 0)
    mask_m = (qm_i < M) | (qm_i + 8 >= jax.lax.broadcasted_iota(I32, (L - 8, L), 1))
    diag_ok = (jax.lax.broadcasted_iota(I32, (7, 8, DH), 1)
               > jax.lax.broadcasted_iota(I32, (7, 8, DH), 0))

    def finish(sp, sa):
        r0 = pl.multiple_of(sp * SEG, SEG)
        xb = xb_v[pl.ds(r0, SEG), :]
        g = xb * _sigmoid(xb)
        o = x_v[sp].astype(F32) + sa * g
        out_v[pl.ds(r0, SEG), :] = o.astype(BF16)
        return o

    def out_copy(r0, n):
        return pltpu.make_async_copy(out_v.at[pl.ds(r0, n), :], out_hbm.at[pl.ds(r0, n), :], sem_out.at[0])

    def step(i, u, prev):
        s = i * UNROLL + u
        pre_i = pre.at[:, pl.ds(pl.multiple_of(i * (8 * UNROLL), 8 * UNROLL), 8 * UNROLL), :]
        xa_i = xa_v.at[pl.ds(pl.multiple_of(i * (LIVE * UNROLL), 8 * UNROLL), LIVE * UNROLL), :]
        xa = xa_i[u * LIVE:(u + 1) * LIVE, :]
        lhs = jnp.concatenate([prev[0:M, :], xa], axis=0).astype(BF16)
        fin = finish(jnp.maximum(s - 1, 0) if u == 0 else s - 1, prev[M:L, :])

        def proj(j, tie=None):
            lh = lhs
            if tie is not None:
                top = pltpu.bitcast(lhs[0:16, 0:128], U32)
                top = pltpu.bitcast(jnp.where(i < 0, pltpu.bitcast(tie, U32), top), BF16)
                lh = jnp.concatenate([jnp.concatenate([top, lhs[0:16, 128:]], axis=1), lhs[16:, :]], axis=0)
            t = _dot(lh, pltpu.bitcast(wtile(j)[...], BF16))
            if u == 0 and TIE0 <= j < TIE0 + NT:
                t = jnp.where(i < 0, fin[:, (j - TIE0) * 128:(j - TIE0 + 1) * 128], t)
            return jnp.concatenate([t, pre_i[j, u * 8:(u + 1) * 8, :]], axis=0)

        NG = H // GH
        qs, ks, vs, ps, os_, ox, iv, on = {}, {}, {}, {}, {}, {}, {}, {}

        def do_qkv(g):
            js = [m * H + h for h in range(g * GH, (g + 1) * GH) for m in range(3)]
            if g == 0:
                part = {}
                for kt in range(NT):
                    for j in js:
                        t = _dot(lhs[:, kt * 128:(kt + 1) * 128],
                                 pltpu.bitcast(wtile(j)[kt * 64:(kt + 1) * 64, :], BF16))
                        part[j] = t if kt == 0 else part[j] + t
                res = {j: jnp.concatenate([part[j], pre_i[j, u * 8:(u + 1) * 8, :]], axis=0) for j in js}
            else:
                res = {}
                for n, j in enumerate(js):
                    tie = None
                    for hh, pos in enumerate(TP):
                        if n == pos and g >= TL:
                            tie = ox[(g - TL) * GH + hh]
                    res[j] = proj(j, tie)
            for h in range(g * GH, (g + 1) * GH):
                qs[h], ks[h], vs[h] = res[h], res[H + h], res[2 * H + h]

        def vpu_rows(h, q, k, v):
            def win(which, val, r):
                if r % 8 == 0:
                    return val[8 - r:16 - r, :]
                return kv_s[h, which, 16 - r:24 - r, :]

            def wins(which, val):
                return jnp.stack([win(which, val, r) for r in range(16)])

            def fold(f, x):
                while x.shape[0] > 1:
                    n = x.shape[0] // 2
                    x = f(x[:n], x[n:])
                return x[0]

            qa = q[8:16, :] * (scale * LOG2E)
            sc = jnp.sum(qa[None] * wins(0, k), axis=-1, keepdims=True)
            sc = jnp.broadcast_to(sc, (16, 8, DH))
            sc = jnp.concatenate([sc[:9], jnp.where(diag_ok, sc[9:], -jnp.inf)], axis=0)
            e = jnp.exp2(sc - fold(jnp.maximum, sc)[None])
            return fold(jnp.add, e * wins(1, v)) * pl.reciprocal(fold(jnp.add, e), approx=True)

        def do_s(g):
            for h in range(g * GH, (g + 1) * GH):
                q, k = qs.pop(h), ks.pop(h)
                kv_s[h, 0, 8:24, :] = k[0:16, :]
                kv_s[h, 1, 8:24, :] = vs[h][0:16, :]
                ox[h] = vpu_rows(h, q, k, vs[h])
                qm = jnp.concatenate([q[0:8, :], q[16:, :]], axis=0)
                sc = _dot_nt(qm.astype(BF16), k.astype(BF16))
                sc = jnp.where(mask_m, sc * (scale * LOG2E), NEG * LOG2E)
                e = jnp.exp2(sc - jnp.max(sc, axis=-1, keepdims=True))
                inv = pl.reciprocal(jnp.sum(e, axis=-1, keepdims=True), approx=True)
                ps[h] = e.astype(BF16)
                iv[h] = jnp.broadcast_to(inv, (SEG, DH))

        def do_pv(g):
            for h in range(g * GH, (g + 1) * GH):
                v = vs.pop(h)
                if g >= NG - TL:
                    v = jnp.concatenate([jnp.where(i < 0, ox[h], v[0:8, :]), v[8:, :]], axis=0)
                if h >= GH:
                    v = jnp.concatenate([v[0:8, :], jnp.where(i < 0, on[h - GH], v[8:, :])], axis=0)
                on[h] = _dot(ps.pop(h), v.astype(BF16)) * iv.pop(h)
                os_[h] = jnp.concatenate([on[h][0:8, :], ox[h], on[h][8:, :]], axis=0)

        def do_o(j, h0, h1):
            o = jnp.concatenate([os_[h] for h in range(h0, h1)], axis=1)
            return _dot(o, pltpu.bitcast(wo_p[j, h0 * 64:h1 * 64, :], BF16))

        for g in range(NG):
            do_qkv(g)
            if g >= LS:
                do_s(g - LS)
            if g >= LP:
                do_pv(g - LP)
        sched = dict(TAIL)
        ns, npv = NG - LS, NG - LP
        for j in range(NT):
            part_v[:, j * 128:(j + 1) * 128] = do_o(j, 0, HS)
            for c_ in sched.get(j, ''):
                if c_ == 's':
                    do_s(ns)
                    ns += 1
                else:
                    do_pv(npv)
                    npv += 1
        assert ns == NG and npv == NG
        return jnp.concatenate(
            [part_v[:, j * 128:(j + 1) * 128] + do_o(j, HS, H) for j in range(NT)], axis=1)

    def multi(i, carry):
        cur = acc[...]
        for u in range(UNROLL):
            cur = step(i, u, cur)
        acc[...] = cur
        r0 = pl.multiple_of(i * (UNROLL * SEG), SEG)
        out_copy(r0, (UNROLL - 1) * SEG).start()

        @pl.when(i > 0)
        def _():
            out_copy(pl.multiple_of(r0 - SEG, SEG), SEG).start()
        return carry

    jax.lax.fori_loop(0, NSEG // UNROLL, multi, 0)
    finish(NSEG - 1, acc[M:L, :])
    out_copy(S - SEG, SEG).start()
    out_copy(0, S).wait()


@jax.jit
def pallas_recurrent_scan__memory_aug_recurrent_mem_tr__moe_arch_mod__prompt_kernel(
    A_x: jax.Array,
    A_mem0: jax.Array,
    A_Wq: jax.Array,
    A_Wk: jax.Array,
    A_Wv: jax.Array,
    A_Wo: jax.Array,
    A_seg_len: jax.Array,
    B_x: jax.Array,
    B_w_r: jax.Array,
    B_w_gate: jax.Array,
    B_w_up: jax.Array,
    B_w_down: jax.Array,
):
    del A_seg_len, B_x
    assert A_x.shape == (1, S, D) and A_Wq.shape == (D, H, DH) and A_mem0.shape == (1, M, D)
    hbm = pl.BlockSpec(memory_space=pltpu.HBM)
    out = pl.pallas_call(
        _kernel,
        out_shape=jax.ShapeDtypeStruct((S, D), BF16),
        in_specs=[hbm] * 10,
        out_specs=hbm,
        scratch_shapes=[
            pltpu.VMEM((NSEG, SEG, D), BF16),
            pltpu.VMEM((NSEG * 4, D), U32),
            pltpu.VMEM((NSEG * LIVE, D), F32),
            pltpu.VMEM((S, D), F32),
            pltpu.VMEM((NPAIR + 1, D, 128), U32),
            pltpu.VMEM((2 * NPAIR + 2, D // 2, 128), U32),
            pltpu.VMEM((NT, H * DH // 2, 128), U32),
            pltpu.VMEM((3 * H, NSEG * 8, DH), F32),
            pltpu.VMEM((FF, D), BF16),
            pltpu.VMEM((FF, D), BF16),
            pltpu.VMEM((FF, D), BF16),
            pltpu.VMEM((S, D), BF16),
            pltpu.VMEM((L, D), F32),
            pltpu.VMEM((L, D), F32),
            pltpu.VMEM((H, 2, 24, DH), F32),
            pltpu.VMEM((TOPC, D), F32),
            pltpu.VMEM((TOPC, D), F32),
            pltpu.VMEM((TOPC, D), F32),
            pltpu.VMEM((SEG, 128), F32),
            pltpu.VMEM((M, D), BF16),
            pltpu.VMEM((NT, 128), BF16),
            pltpu.SMEM((TOPC,), I32),
            pltpu.SemaphoreType.DMA((18,)),
            pltpu.SemaphoreType.DMA((1,)),
        ],
        compiler_params=pltpu.CompilerParams(vmem_limit_bytes=110 * 1024 * 1024),
    )(
        A_x.reshape(NSEG, SEG, D),
        A_mem0.reshape(M, D),
        A_Wq, A_Wk, A_Wv,
        A_Wo.reshape(H * DH, D),
        B_w_r.reshape(NT, 128),
        B_w_gate.T, B_w_up.T, B_w_down,
    )
    return out.reshape(1, S, D)
```

```python
import math

import jax
import jax.numpy as jnp
import jax.experimental.pallas as pl
import jax.experimental.pallas.tpu as pltpu

F32 = jnp.float32
BF16 = jnp.bfloat16
U32 = jnp.uint32
I32 = jnp.int32

S = 2048
D = 640
H = 32
DH = 128
M = 8
SEG = 32
NSEG = S // SEG
L = M + SEG
FF = 1728
TOPC = 8
NT = D // 128
LIVE = SEG - 8
EPS = 1e-05
NEG = -1000000000.0
LOG2E = math.log2(math.e)
NPAIR = 3 * H // 2
KEY_NONE = -1e30

UNROLL = 8
GH = 2
LS, LP = 1, 2
TL, TP = 2, (3, 5)
HS = 24
TAIL = ((0, 'sp'), (2, 'p'))
TIE0 = 2
FINE = (1, 32)
LNT = (6, 10, 14, 18, 22, 25, 28, 31)
MS0, MS1 = 5, 155


def _dot(a, b):
    return jax.lax.dot_general(a, b, (((1,), (0,)), ((), ())), preferred_element_type=F32)


def _dot_nt(a, b):
    return jax.lax.dot_general(a, b, (((1,), (1,)), ((), ())), preferred_element_type=F32)


def _rb(x):
    return x.astype(BF16).astype(F32)


def _sigmoid(x):
    return pl.reciprocal(1.0 + jnp.exp(-x), approx=True)


def _tree(f, xs):
    while len(xs) > 1:
        xs = [f(xs[n], xs[n + 1]) if n + 1 < len(xs) else xs[n] for n in range(0, len(xs), 2)]
    return xs[0]


def _kernel(x_hbm, mem0_hbm, wq_hbm, wk_hbm, wv_hbm, wo_hbm, wr_hbm, wg_hbm, wu_hbm, wd_hbm,
            out_hbm,
            x_v, lhs_v, xa_v, xb_v, raw, w_p, wo_p, pre, wg_v, wu_v, wd_v,
            out_v, acc, part_v, kv_s, sel, upd, yacc, keys, mem0_v, wr_v, idx_s,
            sem_in, sem_out):
    w_hbm = [wq_hbm, wk_hbm, wv_hbm]

    def wtile(j):
        return w_p.at[j]

    SEM_X8, SEM_B0, SEM_LN, SEM_TK, SEM_MLP, SEM_WO = 0, 4, 7, 15, 16, 17

    def w_start(q0, n, sem):
        for q in range(q0, q0 + n):
            src = w_hbm[q // 16].bitcast(U32).at[:, q % 16, :]
            pltpu.make_async_copy(src, raw.at[q], sem_in.at[sem]).start()

    def w_wait(q0, n, sem):
        blk = raw.at[pl.ds(q0, n)]
        pltpu.make_async_copy(blk, blk, sem_in.at[sem]).wait()

    def x8_copy(b):
        return pltpu.make_async_copy(x_hbm.at[pl.ds(b * 16, 16), pl.ds(LIVE, 8), :],
                                     x_v.at[pl.ds(b * 16, 16), pl.ds(LIVE, 8), :], sem_in.at[SEM_X8 + b])

    def xa_copy(i):
        return pltpu.make_async_copy(x_hbm.at[pl.ds(i * 8, 8), pl.ds(0, LIVE), :],
                                     x_v.at[pl.ds(i * 8, 8), pl.ds(0, LIVE), :], sem_in.at[SEM_LN + i])

    cp_wr = pltpu.make_async_copy(wr_hbm, wr_v, sem_in.at[SEM_B0 + 2])
    cp_mem = pltpu.make_async_copy(mem0_hbm, mem0_v, sem_in.at[SEM_TK])
    mlp_copies = [pltpu.make_async_copy(s_, d_, sem_in.at[SEM_MLP])
                  for s_, d_ in [(wg_hbm, wg_v), (wu_hbm, wu_v), (wd_hbm, wd_v)]]
    wo32 = wo_hbm.bitcast(U32)
    wo_copies = [pltpu.make_async_copy(wo32.at[:, pl.ds(j * 128, 128)], wo_p.at[j], sem_in.at[SEM_WO])
                 for j in range(NT)]

    for b in range(4):
        x8_copy(b).start()
    w_start(0, 1, SEM_B0)
    w_start(1, 1, SEM_B0 + 1)
    w_start(2, 2, SEM_B0 + 2)
    cp_wr.start()
    for i in range(8):
        w_start(4 + 4 * i, 4, SEM_LN + i)
        xa_copy(i).start()
    w_start(36, NPAIR - 36, SEM_TK)
    cp_mem.start()
    for c in mlp_copies:
        c.start()
    for c in wo_copies:
        c.start()

    xb3 = xb_v.reshape(NSEG, SEG, D)
    keys[...] = jnp.full(keys.shape, KEY_NONE, F32)
    yacc[...] = jnp.zeros(yacc.shape, F32)
    kv_s[:, :, 0:8, :] = jnp.zeros((H, 2, 8, DH), F32)
    raw[NPAIR] = jnp.zeros((D, 128), U32)
    acc[M:L, :] = jnp.zeros((SEG, D), F32)

    def router_w():
        wr5 = wr_v[...].astype(F32)
        return jnp.concatenate([wr5[j:j + 1, :] for j in range(NT)], axis=1)

    def layernorm(s0, nseg, t0, nrow):
        n = nseg * nrow
        x = x_v[pl.ds(s0, nseg), t0:t0 + nrow, :].astype(F32).reshape(n, D)
        mu = jnp.sum(x, axis=-1, keepdims=True) * (1.0 / D)
        xc = x - mu
        var = jnp.sum(xc * xc, axis=-1, keepdims=True) * (1.0 / D)
        sd = _rb(jnp.sqrt(_rb(_rb(var) + EPS)))
        xn = _rb(_rb(x - _rb(mu)) / sd)
        xb3[pl.ds(s0, nseg), t0:t0 + nrow, :] = xn.reshape(nseg, nrow, D)
        return xn

    def ln8_body(b, carry):
        x8_copy(b).wait()
        xn = layernorm(b * 16, 16, LIVE, 8)
        lhs_v[pl.ds(pl.multiple_of(b * 64, 64), 64), :] = pltpu.bitcast(xn.astype(BF16), U32)
        return carry

    jax.lax.fori_loop(0, 4, ln8_body, 0)

    def ln_seg(s, wr):
        tail = xb3[s, LIVE:SEG, :]
        xn = layernorm(s, 1, 0, LIVE)
        xa_v[pl.ds(pl.multiple_of(s * LIVE, 8), LIVE), :] = xn
        r = _rb(jnp.sum(jnp.concatenate([xn, tail], axis=0) * wr, axis=-1, keepdims=True))
        r = jnp.where(r == 0.0, 0.0, r)
        bits = pltpu.bitcast(jnp.broadcast_to(r, (SEG, 128)), I32) >> 16
        mono = jnp.where(bits < 0, (-32768) - bits, bits)
        mono = jnp.where(r != r, -40000, mono)
        row = jax.lax.broadcasted_iota(I32, (SEG, 128), 0)
        key = (mono * SEG + ((SEG - 1) - row)).astype(F32)
        lane = jax.lax.broadcasted_iota(I32, (SEG, 128), 1)
        keys[...] = jnp.where(lane == s, key, keys[...])
        return pltpu.bitcast(key, U32)

    def top_rows():
        kv = keys[...]
        lane = jax.lax.broadcasted_iota(I32, (1, 128), 1).astype(F32)
        for c in range(TOPC):
            col = jnp.max(kv, axis=0, keepdims=True)
            val = jnp.floor(col * (1.0 / SEG))
            fk = val * 128.0 + (127.0 - lane)
            win = fk == jnp.max(fk, axis=1, keepdims=True)
            kv = jnp.where(win & (kv == col), KEY_NONE, kv)
            pos = lane * SEG + ((SEG - 1.0) - (col - val * SEG))
            idx = jnp.clip(jnp.max(jnp.where(win, pos, 0.0)).astype(I32), 0, S - 1)
            idx_s[c] = idx
            sel[pl.ds(c, 1), :] = xb_v[pl.ds(idx, 1), :]

    def repack(rv, wv, p, part=None, tie=None):
        m_lo = jnp.full((8, 128), 0xFFFF, U32)
        m_hi = jnp.full((8, 128), 0xFFFF0000, U32)
        if tie is not None:
            m_lo = jnp.where(tie[0], tie[1], m_lo)
            m_hi = jnp.where(tie[0], tie[1], m_hi)
        for g in range(D // 16):
            if part is not None and g % part[1] != part[0]:
                continue
            a = rv[p, pl.ds(16 * g, 8, stride=2), :]
            b = rv[p, pl.ds(16 * g + 1, 8, stride=2), :]
            wv[2 * p, 8 * g:8 * g + 8, :] = (a & m_lo) | (b << 16)
            wv[2 * p + 1, 8 * g:8 * g + 8, :] = (a >> 16) | (b & m_hi)

    def block(q0, n, never=None, side=None, jobs=None):
        rv = raw.at[pl.ds(q0, n + 1)]
        wv = w_p.at[pl.ds(2 * q0, 2 * n + 2)]
        pv = pre.at[pl.ds(2 * q0, 2 * n)]
        for u in range(2 * n):
            if u % 2 == 0 and u // 2 + 1 < n:
                repack(rv, wv, u // 2 + 1)
            for c in range(4):
                lhs = lhs_v[c * 64:(c + 1) * 64, :]
                if side is not None and 4 * u + c in LNT:
                    tok = side(LNT.index(4 * u + c))
                    nr = tok.shape[0]
                    head = jnp.where(never, tok, lhs[0:nr, 0:128])
                    lhs = jnp.concatenate(
                        [jnp.concatenate([head, lhs[0:nr, 128:]], axis=1), lhs[nr:, :]], axis=0)
                lhs = pltpu.bitcast(lhs, BF16)
                if jobs:
                    r = None
                    for kt in range(NT):
                        t_ = _dot(lhs[:, kt * 128:(kt + 1) * 128],
                                  pltpu.bitcast(wv[u, kt * 64:(kt + 1) * 64, :], BF16))
                        r = t_ if r is None else r + t_
                        if jobs:
                            jobs.pop(0)()
                elif jobs is not None and 4 * u + c >= 8 * n - FINE[0]:
                    r = jnp.concatenate([_dot(lhs[m_:m_ + FINE[1], :], pltpu.bitcast(wv[u], BF16))
                                         for m_ in range(0, 128, FINE[1])], axis=0)
                else:
                    r = _dot(lhs, pltpu.bitcast(wv[u], BF16))
                pv[u, c * 128:(c + 1) * 128, :] = r
                n8 = (u - max(2 * n - 3, 0)) * 4 + c
                if 0 <= n8 < 8:
                    repack(rv, wv, n, (n8, 8),
                           None if never is None else (never, pltpu.bitcast(r[0:8, :], U32)))

    w_wait(0, 1, SEM_B0)
    repack(raw, w_p, 0)
    w_wait(1, 1, SEM_B0 + 1)
    block(0, 1)
    w_wait(2, 2, SEM_B0 + 2)
    cp_wr.wait()
    block(1, 2)

    def ln_body(i, carry):
        w_wait(4 + 4 * i, 4, SEM_LN + i)
        xa_copy(i).wait()
        wr = router_w()
        block(3 + 4 * i, 4, i < 0, side=lambda u: ln_seg(i * 8 + u, wr))
        return carry

    jax.lax.fori_loop(0, 8, ln_body, 0)

    w_wait(36, NPAIR - 36, SEM_TK)
    cp_mem.wait()
    acc[0:M, :] = mem0_v[...].astype(F32)
    top_rows()
    block(35, 1)

    for c in mlp_copies:
        c.wait()
    FP = FF // 3

    def mlp_body(t, carry):
        f0 = pl.multiple_of(t * FP, 16)
        xs = sel[...]
        cuts = [(a_, min(a_ + 128, FP)) for a_ in range(0, FP, 128)]
        val = {}

        def up_tile(which, n, kt):
            def run():
                a_, b_ = cuts[n]
                w = (wg_v, wu_v)[which][pl.ds(f0 + a_, b_ - a_), kt * 128:(kt + 1) * 128]
                r = _dot_nt(xs[:, kt * 128:(kt + 1) * 128], w)
                val[which, n] = r if kt == 0 else val[which, n] + r
            return run

        def down_tile(n, j):
            def run():
                a_, b_ = cuts[n]
                if j == 0:
                    g_ = _rb(val.pop((0, n)))
                    val['h', n] = _rb(g_ * _sigmoid(g_)) * _rb(val.pop((1, n)))
                r = _dot(val['h', n], wd_v[pl.ds(f0 + a_, b_ - a_), j * 128:(j + 1) * 128])
                val['y', j] = r if n == 0 else val['y', j] + r
            return run

        def skip():
            pass

        real = ([up_tile(which, n, kt) for n in range(len(cuts)) for which in range(2) for kt in range(NT)]
                + [down_tile(n, j) for n in range(len(cuts)) for j in range(NT)])
        jobs = [skip] * MS1
        for n_, job in enumerate(real):
            jobs[MS0 + (n_ * (MS1 - MS0)) // len(real)] = job
        block(36 + 4 * t, 4, t < 0, jobs=jobs)
        assert not jobs
        y = yacc[...] + jnp.concatenate([val['y', j] for j in range(NT)], axis=1)
        yacc[...] = y
        r_sel = _rb(jnp.sum(xs * router_w(), axis=-1, keepdims=True))
        upd[...] = xs + _rb(_rb(y) * _rb(_sigmoid(r_sel)))
        for c in range(TOPC):
            xb_v[pl.ds(jnp.clip(idx_s[c], 0, S - 1), 1), :] = upd[pl.ds(c, 1), :]
        return carry

    jax.lax.fori_loop(0, 3, mlp_body, 0)

    for c in wo_copies:
        c.wait()

    scale = DH ** (-0.5)
    qm_i = jax.lax.broadcasted_iota(I32, (L - 8, L), 0)
    mask_m = (qm_i < M) | (qm_i + 8 >= jax.lax.broadcasted_iota(I32, (L - 8, L), 1))
    diag_ok = (jax.lax.broadcasted_iota(I32, (7, 8, DH), 1)
               > jax.lax.broadcasted_iota(I32, (7, 8, DH), 0))

    def finish(sp, sa):
        r0 = pl.multiple_of(sp * SEG, SEG)
        xb = xb_v[pl.ds(r0, SEG), :]
        g = xb * _sigmoid(xb)
        o = x_v[sp].astype(F32) + sa * g
        out_v[pl.ds(r0, SEG), :] = o.astype(BF16)
        return o

    def out_copy(r0, n):
        return pltpu.make_async_copy(out_v.at[pl.ds(r0, n), :], out_hbm.at[pl.ds(r0, n), :], sem_out.at[0])

    def step(i, u, prev):
        s = i * UNROLL + u
        pre_i = pre.at[:, pl.ds(pl.multiple_of(i * (8 * UNROLL), 8 * UNROLL), 8 * UNROLL), :]
        xa_i = xa_v.at[pl.ds(pl.multiple_of(i * (LIVE * UNROLL), 8 * UNROLL), LIVE * UNROLL), :]
        xa = xa_i[u * LIVE:(u + 1) * LIVE, :]
        lhs = jnp.concatenate([prev[0:M, :], xa], axis=0).astype(BF16)
        fin = finish(jnp.maximum(s - 1, 0) if u == 0 else s - 1, prev[M:L, :])

        def proj(j, tie=None):
            lh = lhs
            if tie is not None:
                top = pltpu.bitcast(lhs[0:16, 0:128], U32)
                top = pltpu.bitcast(jnp.where(i < 0, pltpu.bitcast(tie, U32), top), BF16)
                lh = jnp.concatenate([jnp.concatenate([top, lhs[0:16, 128:]], axis=1), lhs[16:, :]], axis=0)
            t = _dot(lh, pltpu.bitcast(wtile(j)[...], BF16))
            if u == 0 and TIE0 <= j < TIE0 + NT:
                t = jnp.where(i < 0, fin[:, (j - TIE0) * 128:(j - TIE0 + 1) * 128], t)
            return jnp.concatenate([t, pre_i[j, u * 8:(u + 1) * 8, :]], axis=0)

        NG = H // GH
        qs, ks, vs, ps, os_, ox, iv, on = {}, {}, {}, {}, {}, {}, {}, {}

        def do_qkv(g):
            js = [m * H + h for h in range(g * GH, (g + 1) * GH) for m in range(3)]
            if g == 0:
                part = {}
                for kt in range(NT):
                    for j in js:
                        t = _dot(lhs[:, kt * 128:(kt + 1) * 128],
                                 pltpu.bitcast(wtile(j)[kt * 64:(kt + 1) * 64, :], BF16))
                        part[j] = t if kt == 0 else part[j] + t
                res = {j: jnp.concatenate([part[j], pre_i[j, u * 8:(u + 1) * 8, :]], axis=0) for j in js}
            else:
                res = {}
                for n, j in enumerate(js):
                    tie = None
                    for hh, pos in enumerate(TP):
                        if n == pos and g >= TL:
                            tie = ox[(g - TL) * GH + hh]
                    res[j] = proj(j, tie)
            for h in range(g * GH, (g + 1) * GH):
                qs[h], ks[h], vs[h] = res[h], res[H + h], res[2 * H + h]

        def vpu_rows(h, q, k, v):
            def win(which, val, r):
                if r % 8 == 0:
                    return val[8 - r:16 - r, :]
                return kv_s[h, which, 16 - r:24 - r, :]

            def wins(which, val):
                return jnp.stack([win(which, val, r) for r in range(16)])

            def fold(f, x):
                while x.shape[0] > 1:
                    n = x.shape[0] // 2
                    x = f(x[:n], x[n:])
                return x[0]

            qa = q[8:16, :] * (scale * LOG2E)
            sc = jnp.sum(qa[None] * wins(0, k), axis=-1, keepdims=True)
            sc = jnp.broadcast_to(sc, (16, 8, DH))
            sc = jnp.concatenate([sc[:9], jnp.where(diag_ok, sc[9:], -jnp.inf)], axis=0)
            e = jnp.exp2(sc - fold(jnp.maximum, sc)[None])
            return fold(jnp.add, e * wins(1, v)) * pl.reciprocal(fold(jnp.add, e), approx=True)

        def do_s(g):
            for h in range(g * GH, (g + 1) * GH):
                q, k = qs.pop(h), ks.pop(h)
                kv_s[h, 0, 8:24, :] = k[0:16, :]
                kv_s[h, 1, 8:24, :] = vs[h][0:16, :]
                ox[h] = vpu_rows(h, q, k, vs[h])
                qm = jnp.concatenate([q[0:8, :], q[16:, :]], axis=0)
                sc = _dot_nt(qm.astype(BF16), k.astype(BF16))
                sc = jnp.where(mask_m, sc * (scale * LOG2E), NEG * LOG2E)
                e = jnp.exp2(sc - jnp.max(sc, axis=-1, keepdims=True))
                inv = pl.reciprocal(jnp.sum(e, axis=-1, keepdims=True), approx=True)
                ps[h] = e.astype(BF16)
                iv[h] = jnp.broadcast_to(inv, (SEG, DH))

        def do_pv(g):
            for h in range(g * GH, (g + 1) * GH):
                v = vs.pop(h)
                if g >= NG - TL:
                    v = jnp.concatenate([jnp.where(i < 0, ox[h], v[0:8, :]), v[8:, :]], axis=0)
                if h >= GH:
                    v = jnp.concatenate([v[0:8, :], jnp.where(i < 0, on[h - GH], v[8:, :])], axis=0)
                on[h] = _dot(ps.pop(h), v.astype(BF16)) * iv.pop(h)
                os_[h] = jnp.concatenate([on[h][0:8, :], ox[h], on[h][8:, :]], axis=0)

        def do_o(j, h0, h1):
            o = jnp.concatenate([os_[h] for h in range(h0, h1)], axis=1)
            return _dot(o, pltpu.bitcast(wo_p[j, h0 * 64:h1 * 64, :], BF16))

        for g in range(NG):
            do_qkv(g)
            if g >= LS:
                do_s(g - LS)
            if g >= LP:
                do_pv(g - LP)
        sched = dict(TAIL)
        ns, npv = NG - LS, NG - LP
        for j in range(NT):
            part_v[:, j * 128:(j + 1) * 128] = do_o(j, 0, HS)
            for c_ in sched.get(j, ''):
                if c_ == 's':
                    do_s(ns)
                    ns += 1
                else:
                    do_pv(npv)
                    npv += 1
        assert ns == NG and npv == NG
        return jnp.concatenate(
            [part_v[:, j * 128:(j + 1) * 128] + do_o(j, HS, H) for j in range(NT)], axis=1)

    def multi(i, carry):
        cur = acc[...]
        for u in range(UNROLL):
            cur = step(i, u, cur)
        acc[...] = cur
        r0 = pl.multiple_of(i * (UNROLL * SEG), SEG)
        out_copy(r0, (UNROLL - 1) * SEG).start()

        @pl.when(i > 0)
        def _():
            out_copy(pl.multiple_of(r0 - SEG, SEG), SEG).start()
        return carry

    jax.lax.fori_loop(0, NSEG // UNROLL, multi, 0)
    finish(NSEG - 1, acc[M:L, :])
    out_copy(S - SEG, SEG).start()
    out_copy(0, S).wait()


@jax.jit
def pallas_recurrent_scan__memory_aug_recurrent_mem_tr__moe_arch_mod__prompt_kernel(
    A_x: jax.Array,
    A_mem0: jax.Array,
    A_Wq: jax.Array,
    A_Wk: jax.Array,
    A_Wv: jax.Array,
    A_Wo: jax.Array,
    A_seg_len: jax.Array,
    B_x: jax.Array,
    B_w_r: jax.Array,
    B_w_gate: jax.Array,
    B_w_up: jax.Array,
    B_w_down: jax.Array,
):
    del A_seg_len, B_x
    assert A_x.shape == (1, S, D) and A_Wq.shape == (D, H, DH) and A_mem0.shape == (1, M, D)
    hbm = pl.BlockSpec(memory_space=pltpu.HBM)
    out = pl.pallas_call(
        _kernel,
        out_shape=jax.ShapeDtypeStruct((S, D), BF16),
        in_specs=[hbm] * 10,
        out_specs=hbm,
        scratch_shapes=[
            pltpu.VMEM((NSEG, SEG, D), BF16),
            pltpu.VMEM((NSEG * 4, D), U32),
            pltpu.VMEM((NSEG * LIVE, D), F32),
            pltpu.VMEM((S, D), F32),
            pltpu.VMEM((NPAIR + 1, D, 128), U32),
            pltpu.VMEM((2 * NPAIR + 2, D // 2, 128), U32),
            pltpu.VMEM((NT, H * DH // 2, 128), U32),
            pltpu.VMEM((3 * H, NSEG * 8, DH), F32),
            pltpu.VMEM((FF, D), BF16),
            pltpu.VMEM((FF, D), BF16),
            pltpu.VMEM((FF, D), BF16),
            pltpu.VMEM((S, D), BF16),
            pltpu.VMEM((L, D), F32),
            pltpu.VMEM((L, D), F32),
            pltpu.VMEM((H, 2, 24, DH), F32),
            pltpu.VMEM((TOPC, D), F32),
            pltpu.VMEM((TOPC, D), F32),
            pltpu.VMEM((TOPC, D), F32),
            pltpu.VMEM((SEG, 128), F32),
            pltpu.VMEM((M, D), BF16),
            pltpu.VMEM((NT, 128), BF16),
            pltpu.SMEM((TOPC,), I32),
            pltpu.SemaphoreType.DMA((18,)),
            pltpu.SemaphoreType.DMA((1,)),
        ],
        compiler_params=pltpu.CompilerParams(vmem_limit_bytes=110 * 1024 * 1024),
    )(
        A_x.reshape(NSEG, SEG, D),
        A_mem0.reshape(M, D),
        A_Wq, A_Wk, A_Wv,
        A_Wo.reshape(H * DH, D),
        B_w_r.reshape(NT, 128),
        B_w_gate.T, B_w_up.T, B_w_down,
    )
    return out.reshape(1, S, D)
```

```python
import math

import jax
import jax.numpy as jnp
import jax.experimental.pallas as pl
import jax.experimental.pallas.tpu as pltpu

F32 = jnp.float32
BF16 = jnp.bfloat16
U32 = jnp.uint32
I32 = jnp.int32

S = 2048
D = 640
H = 32
DH = 128
M = 8
SEG = 32
NSEG = S // SEG
L = M + SEG
FF = 1728
TOPC = 8
NT = D // 128
LIVE = SEG - 8
EPS = 1e-05
NEG = -1000000000.0
LOG2E = math.log2(math.e)
NPAIR = 3 * H // 2
KEY_NONE = -1e30

UNROLL = 8
GH = 2
LS, LP = 1, 2
TL, TP = 2, (3, 5)
HS = 24
TAIL = ((0, 'sp'), (2, 'p'))
TIE0 = 2
FINE = (1, 32)
LNT = (6, 10, 14, 18, 22, 25, 28, 31)
MS0, MS1 = 5, 155


def _dot(a, b):
    return jax.lax.dot_general(a, b, (((1,), (0,)), ((), ())), preferred_element_type=F32)


def _dot_nt(a, b):
    return jax.lax.dot_general(a, b, (((1,), (1,)), ((), ())), preferred_element_type=F32)


def _rb(x):
    return x.astype(BF16).astype(F32)


def _sigmoid(x):
    return pl.reciprocal(1.0 + jnp.exp(-x), approx=True)


def _tree(f, xs):
    while len(xs) > 1:
        xs = [f(xs[n], xs[n + 1]) if n + 1 < len(xs) else xs[n] for n in range(0, len(xs), 2)]
    return xs[0]


def _kernel(x_hbm, mem0_hbm, wq_hbm, wk_hbm, wv_hbm, wo_hbm, wr_hbm, wg_hbm, wu_hbm, wd_hbm,
            out_hbm,
            x_v, lhs_v, xa_v, xb_v, raw, w_p, wo_p, pre, wg_v, wu_v, wd_v,
            out_v, acc, part_v, kv_s, sel, upd, yacc, keys, mem0_v, wr_v, idx_s,
            sem_in, sem_out):
    w_hbm = [wq_hbm, wk_hbm, wv_hbm]

    def wtile(j):
        return w_p.at[j]

    SEM_X8, SEM_B0, SEM_LN, SEM_TK, SEM_MLP, SEM_WO = 0, 4, 7, 15, 16, 17

    def w_start(q0, n, sem):
        for q in range(q0, q0 + n):
            src = w_hbm[q // 16].bitcast(U32).at[:, q % 16, :]
            pltpu.make_async_copy(src, raw.at[q, pl.ds(0, D), :], sem_in.at[sem]).start()

    def w_wait(q0, n, sem):
        blk = raw.at[pl.ds(q0, n), pl.ds(0, D), :]
        pltpu.make_async_copy(blk, blk, sem_in.at[sem]).wait()

    def x8_copy(b):
        return pltpu.make_async_copy(x_hbm.at[pl.ds(b * 16, 16), pl.ds(LIVE, 8), :],
                                     x_v.at[pl.ds(b * 16, 16), pl.ds(LIVE, 8), :], sem_in.at[SEM_X8 + b])

    def xa_copy(i):
        return pltpu.make_async_copy(x_hbm.at[pl.ds(i * 8, 8), pl.ds(0, LIVE), :],
                                     x_v.at[pl.ds(i * 8, 8), pl.ds(0, LIVE), :], sem_in.at[SEM_LN + i])

    cp_wr = pltpu.make_async_copy(wr_hbm, wr_v, sem_in.at[SEM_B0 + 2])
    cp_mem = pltpu.make_async_copy(mem0_hbm, mem0_v, sem_in.at[SEM_TK])
    mlp_copies = [pltpu.make_async_copy(s_, d_, sem_in.at[SEM_MLP])
                  for s_, d_ in [(wg_hbm, wg_v), (wu_hbm, wu_v), (wd_hbm, wd_v)]]
    wo32 = wo_hbm.bitcast(U32)
    wo_copies = [pltpu.make_async_copy(wo32.at[:, pl.ds(j * 128, 128)], wo_p.at[j], sem_in.at[SEM_WO])
                 for j in range(NT)]

    for b in range(4):
        x8_copy(b).start()
    w_start(0, 1, SEM_B0)
    w_start(1, 1, SEM_B0 + 1)
    w_start(2, 2, SEM_B0 + 2)
    cp_wr.start()
    for i in range(8):
        w_start(4 + 4 * i, 4, SEM_LN + i)
        xa_copy(i).start()
    w_start(36, NPAIR - 36, SEM_TK)
    cp_mem.start()
    for c in mlp_copies:
        c.start()
    for c in wo_copies:
        c.start()

    xb3 = xb_v.reshape(NSEG, SEG, D)
    keys[...] = jnp.full(keys.shape, KEY_NONE, F32)
    yacc[...] = jnp.zeros(yacc.shape, F32)
    kv_s[:, :, 0:8, :] = jnp.zeros((H, 2, 8, DH), F32)
    raw[NPAIR, 0:D, :] = jnp.zeros((D, 128), U32)
    acc[M:L, :] = jnp.zeros((SEG, D), F32)

    def router_w():
        wr5 = wr_v[...].astype(F32)
        return jnp.concatenate([wr5[j:j + 1, :] for j in range(NT)], axis=1)

    def layernorm(s0, nseg, t0, nrow):
        n = nseg * nrow
        x = x_v[pl.ds(s0, nseg), t0:t0 + nrow, :].astype(F32).reshape(n, D)
        mu = jnp.sum(x, axis=-1, keepdims=True) * (1.0 / D)
        xc = x - mu
        var = jnp.sum(xc * xc, axis=-1, keepdims=True) * (1.0 / D)
        sd = _rb(jnp.sqrt(_rb(_rb(var) + EPS)))
        xn = _rb(_rb(x - _rb(mu)) / sd)
        xb3[pl.ds(s0, nseg), t0:t0 + nrow, :] = xn.reshape(nseg, nrow, D)
        return xn

    def ln8_body(b, carry):
        x8_copy(b).wait()
        xn = layernorm(b * 16, 16, LIVE, 8)
        lhs_v[pl.ds(pl.multiple_of(b * 64, 64), 64), :] = pltpu.bitcast(xn.astype(BF16), U32)
        return carry

    jax.lax.fori_loop(0, 4, ln8_body, 0)

    def ln_seg(s, wr):
        tail = xb3[s, LIVE:SEG, :]
        xn = layernorm(s, 1, 0, LIVE)
        xa_v[pl.ds(pl.multiple_of(s * LIVE, 8), LIVE), :] = xn
        r = _rb(jnp.sum(jnp.concatenate([xn, tail], axis=0) * wr, axis=-1, keepdims=True))
        r = jnp.where(r == 0.0, 0.0, r)
        bits = pltpu.bitcast(jnp.broadcast_to(r, (SEG, 128)), I32) >> 16
        mono = jnp.where(bits < 0, (-32768) - bits, bits)
        mono = jnp.where(r != r, -40000, mono)
        row = jax.lax.broadcasted_iota(I32, (SEG, 128), 0)
        key = (mono * SEG + ((SEG - 1) - row)).astype(F32)
        lane = jax.lax.broadcasted_iota(I32, (SEG, 128), 1)
        keys[...] = jnp.where(lane == s, key, keys[...])
        return pltpu.bitcast(key, U32)

    def top_rows():
        kv = keys[...]
        lane = jax.lax.broadcasted_iota(I32, (1, 128), 1).astype(F32)
        for c in range(TOPC):
            col = jnp.max(kv, axis=0, keepdims=True)
            val = jnp.floor(col * (1.0 / SEG))
            fk = val * 128.0 + (127.0 - lane)
            win = fk == jnp.max(fk, axis=1, keepdims=True)
            kv = jnp.where(win & (kv == col), KEY_NONE, kv)
            pos = lane * SEG + ((SEG - 1.0) - (col - val * SEG))
            idx = jnp.clip(jnp.max(jnp.where(win, pos, 0.0)).astype(I32), 0, S - 1)
            idx_s[c] = idx
            sel[pl.ds(c, 1), :] = xb_v[pl.ds(idx, 1), :]

    def repack(rv, wv, p, part=None, tie=None):
        m_lo = jnp.full((8, 128), 0xFFFF, U32)
        m_hi = jnp.full((8, 128), 0xFFFF0000, U32)
        if tie is not None:
            m_lo = jnp.where(tie[0], tie[1], m_lo)
            m_hi = jnp.where(tie[0], tie[1], m_hi)
        for g in range(D // 16):
            if part is not None and g % part[1] != part[0]:
                continue
            a = rv[p, pl.ds(16 * g, 8, stride=2), :]
            b = rv[p, pl.ds(16 * g + 1, 8, stride=2), :]
            wv[2 * p, 8 * g:8 * g + 8, :] = (a & m_lo) | (b << 16)
            wv[2 * p + 1, 8 * g:8 * g + 8, :] = (a >> 16) | (b & m_hi)

    def block(q0, n, never=None, side=None, jobs=None):
        rv = raw.at[pl.ds(q0, n + 1)]
        wv = w_p.at[pl.ds(2 * q0, 2 * n + 2)]
        pv = pre.at[pl.ds(2 * q0, 2 * n)]
        for u in range(2 * n):
            if u % 2 == 0 and u // 2 + 1 < n:
                repack(rv, wv, u // 2 + 1)
            for c in range(4):
                lhs = lhs_v[c * 64:(c + 1) * 64, :]
                if side is not None and 4 * u + c in LNT:
                    tok = side(LNT.index(4 * u + c))
                    nr = tok.shape[0]
                    head = jnp.where(never, tok, lhs[0:nr, 0:128])
                    lhs = jnp.concatenate(
                        [jnp.concatenate([head, lhs[0:nr, 128:]], axis=1), lhs[nr:, :]], axis=0)
                lhs = pltpu.bitcast(lhs, BF16)
                if jobs:
                    r = None
                    for kt in range(NT):
                        t_ = _dot(lhs[:, kt * 128:(kt + 1) * 128],
                                  pltpu.bitcast(wv[u, kt * 64:(kt + 1) * 64, :], BF16))
                        r = t_ if r is None else r + t_
                        if jobs:
                            jobs.pop(0)()
                elif jobs is not None and 4 * u + c >= 8 * n - FINE[0]:
                    r = jnp.concatenate([_dot(lhs[m_:m_ + FINE[1], :], pltpu.bitcast(wv[u], BF16))
                                         for m_ in range(0, 128, FINE[1])], axis=0)
                else:
                    r = _dot(lhs, pltpu.bitcast(wv[u], BF16))
                pv[u, c * 128:(c + 1) * 128, :] = r
                n8 = (u - max(2 * n - 3, 0)) * 4 + c
                if 0 <= n8 < 8:
                    repack(rv, wv, n, (n8, 8),
                           None if never is None else (never, pltpu.bitcast(r[0:8, :], U32)))

    w_wait(0, 1, SEM_B0)
    repack(raw, w_p, 0)
    w_wait(1, 1, SEM_B0 + 1)
    block(0, 1)
    w_wait(2, 2, SEM_B0 + 2)
    cp_wr.wait()
    block(1, 2)

    def ln_body(i, carry):
        w_wait(4 + 4 * i, 4, SEM_LN + i)
        xa_copy(i).wait()
        wr = router_w()
        block(3 + 4 * i, 4, i < 0, side=lambda u: ln_seg(i * 8 + u, wr))
        return carry

    jax.lax.fori_loop(0, 8, ln_body, 0)

    w_wait(36, NPAIR - 36, SEM_TK)
    cp_mem.wait()
    acc[0:M, :] = mem0_v[...].astype(F32)
    top_rows()
    block(35, 1)

    for c in mlp_copies:
        c.wait()
    FP = FF // 3

    def mlp_body(t, carry):
        f0 = pl.multiple_of(t * FP, 16)
        xs = sel[...]
        cuts = [(a_, min(a_ + 128, FP)) for a_ in range(0, FP, 128)]
        val = {}

        def up_tile(which, n, kt):
            def run():
                a_, b_ = cuts[n]
                w = (wg_v, wu_v)[which][pl.ds(f0 + a_, b_ - a_), kt * 128:(kt + 1) * 128]
                r = _dot_nt(xs[:, kt * 128:(kt + 1) * 128], w)
                val[which, n] = r if kt == 0 else val[which, n] + r
            return run

        def down_tile(n, j):
            def run():
                a_, b_ = cuts[n]
                if j == 0:
                    g_ = _rb(val.pop((0, n)))
                    val['h', n] = _rb(g_ * _sigmoid(g_)) * _rb(val.pop((1, n)))
                r = _dot(val['h', n], wd_v[pl.ds(f0 + a_, b_ - a_), j * 128:(j + 1) * 128])
                val['y', j] = r if n == 0 else val['y', j] + r
            return run

        def skip():
            pass

        real = ([up_tile(which, n, kt) for n in range(len(cuts)) for which in range(2) for kt in range(NT)]
                + [down_tile(n, j) for n in range(len(cuts)) for j in range(NT)])
        jobs = [skip] * MS1
        for n_, job in enumerate(real):
            jobs[MS0 + (n_ * (MS1 - MS0)) // len(real)] = job
        block(36 + 4 * t, 4, t < 0, jobs=jobs)
        assert not jobs
        y = yacc[...] + jnp.concatenate([val['y', j] for j in range(NT)], axis=1)
        yacc[...] = y
        r_sel = _rb(jnp.sum(xs * router_w(), axis=-1, keepdims=True))
        upd[...] = xs + _rb(_rb(y) * _rb(_sigmoid(r_sel)))
        for c in range(TOPC):
            xb_v[pl.ds(jnp.clip(idx_s[c], 0, S - 1), 1), :] = upd[pl.ds(c, 1), :]
        return carry

    jax.lax.fori_loop(0, 3, mlp_body, 0)

    for c in wo_copies:
        c.wait()

    scale = DH ** (-0.5)
    qm_i = jax.lax.broadcasted_iota(I32, (L - 8, L), 0)
    mask_m = (qm_i < M) | (qm_i + 8 >= jax.lax.broadcasted_iota(I32, (L - 8, L), 1))
    diag_ok = (jax.lax.broadcasted_iota(I32, (7, 8, DH), 1)
               > jax.lax.broadcasted_iota(I32, (7, 8, DH), 0))

    def finish(sp, sa):
        r0 = pl.multiple_of(sp * SEG, SEG)
        xb = xb_v[pl.ds(r0, SEG), :]
        g = xb * _sigmoid(xb)
        o = x_v[sp].astype(F32) + sa * g
        out_v[pl.ds(r0, SEG), :] = o.astype(BF16)
        return o

    def out_copy(r0, n):
        return pltpu.make_async_copy(out_v.at[pl.ds(r0, n), :], out_hbm.at[pl.ds(r0, n), :], sem_out.at[0])

    def step(i, u, prev):
        s = i * UNROLL + u
        pre_i = pre.at[:, pl.ds(pl.multiple_of(i * (8 * UNROLL), 8 * UNROLL), 8 * UNROLL), :]
        xa_i = xa_v.at[pl.ds(pl.multiple_of(i * (LIVE * UNROLL), 8 * UNROLL), LIVE * UNROLL), :]
        xa = xa_i[u * LIVE:(u + 1) * LIVE, :]
        lhs = jnp.concatenate([prev[0:M, :], xa], axis=0).astype(BF16)
        fin = finish(jnp.maximum(s - 1, 0) if u == 0 else s - 1, prev[M:L, :])

        def proj(j, tie=None):
            lh = lhs
            if tie is not None:
                top = pltpu.bitcast(lhs[0:16, 0:128], U32)
                top = pltpu.bitcast(jnp.where(i < 0, pltpu.bitcast(tie, U32), top), BF16)
                lh = jnp.concatenate([jnp.concatenate([top, lhs[0:16, 128:]], axis=1), lhs[16:, :]], axis=0)
            t = _dot(lh, pltpu.bitcast(wtile(j)[...], BF16))
            if u == 0 and TIE0 <= j < TIE0 + NT:
                t = jnp.where(i < 0, fin[:, (j - TIE0) * 128:(j - TIE0 + 1) * 128], t)
            return jnp.concatenate([t, pre_i[j, u * 8:(u + 1) * 8, :]], axis=0)

        NG = H // GH
        qs, ks, vs, ps, os_, ox, iv, on = {}, {}, {}, {}, {}, {}, {}, {}

        def do_qkv(g):
            js = [m * H + h for h in range(g * GH, (g + 1) * GH) for m in range(3)]
            if g == 0:
                part = {}
                for kt in range(NT):
                    for j in js:
                        t = _dot(lhs[:, kt * 128:(kt + 1) * 128],
                                 pltpu.bitcast(wtile(j)[kt * 64:(kt + 1) * 64, :], BF16))
                        part[j] = t if kt == 0 else part[j] + t
                res = {j: jnp.concatenate([part[j], pre_i[j, u * 8:(u + 1) * 8, :]], axis=0) for j in js}
            else:
                res = {}
                for n, j in enumerate(js):
                    tie = None
                    for hh, pos in enumerate(TP):
                        if n == pos and g >= TL:
                            tie = ox[(g - TL) * GH + hh]
                    res[j] = proj(j, tie)
            for h in range(g * GH, (g + 1) * GH):
                qs[h], ks[h], vs[h] = res[h], res[H + h], res[2 * H + h]

        def vpu_rows(h, q, k, v):
            def win(which, val, r):
                if r % 8 == 0:
                    return val[8 - r:16 - r, :]
                return kv_s[h, which, 16 - r:24 - r, :]

            def wins(which, val):
                return jnp.stack([win(which, val, r) for r in range(16)])

            def fold(f, x):
                while x.shape[0] > 1:
                    n = x.shape[0] // 2
                    x = f(x[:n], x[n:])
                return x[0]

            qa = q[8:16, :] * (scale * LOG2E)
            sc = jnp.sum(qa[None] * wins(0, k), axis=-1, keepdims=True)
            sc = jnp.broadcast_to(sc, (16, 8, DH))
            sc = jnp.concatenate([sc[:9], jnp.where(diag_ok, sc[9:], -jnp.inf)], axis=0)
            e = jnp.exp2(sc - fold(jnp.maximum, sc)[None])
            return fold(jnp.add, e * wins(1, v)) * pl.reciprocal(fold(jnp.add, e), approx=True)

        def do_s(g):
            for h in range(g * GH, (g + 1) * GH):
                q, k = qs.pop(h), ks.pop(h)
                kv_s[h, 0, 8:24, :] = k[0:16, :]
                kv_s[h, 1, 8:24, :] = vs[h][0:16, :]
                ox[h] = vpu_rows(h, q, k, vs[h])
                qm = jnp.concatenate([q[0:8, :], q[16:, :]], axis=0)
                sc = _dot_nt(qm.astype(BF16), k.astype(BF16))
                sc = jnp.where(mask_m, sc * (scale * LOG2E), NEG * LOG2E)
                e = jnp.exp2(sc - jnp.max(sc, axis=-1, keepdims=True))
                inv = pl.reciprocal(jnp.sum(e, axis=-1, keepdims=True), approx=True)
                ps[h] = e.astype(BF16)
                iv[h] = jnp.broadcast_to(inv, (SEG, DH))

        def do_pv(g):
            for h in range(g * GH, (g + 1) * GH):
                v = vs.pop(h)
                if g >= NG - TL:
                    v = jnp.concatenate([jnp.where(i < 0, ox[h], v[0:8, :]), v[8:, :]], axis=0)
                if h >= GH:
                    v = jnp.concatenate([v[0:8, :], jnp.where(i < 0, on[h - GH], v[8:, :])], axis=0)
                on[h] = _dot(ps.pop(h), v.astype(BF16)) * iv.pop(h)
                os_[h] = jnp.concatenate([on[h][0:8, :], ox[h], on[h][8:, :]], axis=0)

        def do_o(j, h0, h1):
            o = jnp.concatenate([os_[h] for h in range(h0, h1)], axis=1)
            return _dot(o, pltpu.bitcast(wo_p[j, h0 * 64:h1 * 64, :], BF16))

        for g in range(NG):
            do_qkv(g)
            if g >= LS:
                do_s(g - LS)
            if g >= LP:
                do_pv(g - LP)
        sched = dict(TAIL)
        ns, npv = NG - LS, NG - LP
        for j in range(NT):
            part_v[:, j * 128:(j + 1) * 128] = do_o(j, 0, HS)
            for c_ in sched.get(j, ''):
                if c_ == 's':
                    do_s(ns)
                    ns += 1
                else:
                    do_pv(npv)
                    npv += 1
        assert ns == NG and npv == NG
        return jnp.concatenate(
            [part_v[:, j * 128:(j + 1) * 128] + do_o(j, HS, H) for j in range(NT)], axis=1)

    def multi(i, carry):
        cur = acc[...]
        for u in range(UNROLL):
            cur = step(i, u, cur)
        acc[...] = cur
        r0 = pl.multiple_of(i * (UNROLL * SEG), SEG)
        out_copy(r0, (UNROLL - 1) * SEG).start()

        @pl.when(i > 0)
        def _():
            out_copy(pl.multiple_of(r0 - SEG, SEG), SEG).start()
        return carry

    jax.lax.fori_loop(0, NSEG // UNROLL, multi, 0)
    finish(NSEG - 1, acc[M:L, :])
    out_copy(S - SEG, SEG).start()
    out_copy(0, S).wait()


@jax.jit
def pallas_recurrent_scan__memory_aug_recurrent_mem_tr__moe_arch_mod__prompt_kernel(
    A_x: jax.Array,
    A_mem0: jax.Array,
    A_Wq: jax.Array,
    A_Wk: jax.Array,
    A_Wv: jax.Array,
    A_Wo: jax.Array,
    A_seg_len: jax.Array,
    B_x: jax.Array,
    B_w_r: jax.Array,
    B_w_gate: jax.Array,
    B_w_up: jax.Array,
    B_w_down: jax.Array,
):
    del A_seg_len, B_x
    assert A_x.shape == (1, S, D) and A_Wq.shape == (D, H, DH) and A_mem0.shape == (1, M, D)
    hbm = pl.BlockSpec(memory_space=pltpu.HBM)
    out = pl.pallas_call(
        _kernel,
        out_shape=jax.ShapeDtypeStruct((S, D), BF16),
        in_specs=[hbm] * 10,
        out_specs=hbm,
        scratch_shapes=[
            pltpu.VMEM((NSEG, SEG, D), BF16),
            pltpu.VMEM((NSEG * 4, D), U32),
            pltpu.VMEM((NSEG * LIVE, D), F32),
            pltpu.VMEM((S, D), F32),
            pltpu.VMEM((NPAIR + 1, D + 32, 128), U32),
            pltpu.VMEM((2 * NPAIR + 2, D // 2, 128), U32),
            pltpu.VMEM((NT, H * DH // 2, 128), U32),
            pltpu.VMEM((3 * H, NSEG * 8, DH), F32),
            pltpu.VMEM((FF, D), BF16),
            pltpu.VMEM((FF, D), BF16),
            pltpu.VMEM((FF, D), BF16),
            pltpu.VMEM((S, D), BF16),
            pltpu.VMEM((L, D), F32),
            pltpu.VMEM((L, D), F32),
            pltpu.VMEM((H, 2, 24, DH), F32),
            pltpu.VMEM((TOPC, D), F32),
            pltpu.VMEM((TOPC, D), F32),
            pltpu.VMEM((TOPC, D), F32),
            pltpu.VMEM((SEG, 128), F32),
            pltpu.VMEM((M, D), BF16),
            pltpu.VMEM((NT, 128), BF16),
            pltpu.SMEM((TOPC,), I32),
            pltpu.SemaphoreType.DMA((18,)),
            pltpu.SemaphoreType.DMA((1,)),
        ],
        compiler_params=pltpu.CompilerParams(vmem_limit_bytes=110 * 1024 * 1024),
    )(
        A_x.reshape(NSEG, SEG, D),
        A_mem0.reshape(M, D),
        A_Wq, A_Wk, A_Wv,
        A_Wo.reshape(H * DH, D),
        B_w_r.reshape(NT, 128),
        B_w_gate.T, B_w_up.T, B_w_down,
    )
    return out.reshape(1, S, D)
```

```python
import math

import jax
import jax.numpy as jnp
import jax.experimental.pallas as pl
import jax.experimental.pallas.tpu as pltpu

F32 = jnp.float32
BF16 = jnp.bfloat16
U32 = jnp.uint32
I32 = jnp.int32

S = 2048
D = 640
H = 32
DH = 128
M = 8
SEG = 32
NSEG = S // SEG
L = M + SEG
FF = 1728
TOPC = 8
NT = D // 128
LIVE = SEG - 8
EPS = 1e-05
NEG = -1000000000.0
LOG2E = math.log2(math.e)
NPAIR = 3 * H // 2
KEY_NONE = -1e30

UNROLL = 8
GH = 2
LS, LP = 1, 2
TL, TP = 2, (3, 5)
HS = 24
TAIL = ((0, 'sp'), (2, 'p'))
FINE = (1, 32)
TIE0 = 2
LNT = (6, 10, 14, 18, 22, 25, 28, 31)
MS0, MS1 = 5, 155


def _dot(a, b):
    return jax.lax.dot_general(a, b, (((1,), (0,)), ((), ())), preferred_element_type=F32)


def _dot_nt(a, b):
    return jax.lax.dot_general(a, b, (((1,), (1,)), ((), ())), preferred_element_type=F32)


def _rb(x):
    return x.astype(BF16).astype(F32)


def _sigmoid(x):
    return pl.reciprocal(1.0 + jnp.exp(-x), approx=True)


def _tree(f, xs):
    while len(xs) > 1:
        xs = [f(xs[n], xs[n + 1]) if n + 1 < len(xs) else xs[n] for n in range(0, len(xs), 2)]
    return xs[0]


def _kernel(x_hbm, mem0_hbm, wq_hbm, wk_hbm, wv_hbm, wo_hbm, wr_hbm, wg_hbm, wu_hbm, wd_hbm,
            out_hbm,
            x_v, lhs_v, xa_v, xb_v, raw, w_p, wo_p, pre, wg_v, wu_v, wd_v,
            out_v, acc, part_v, kv_s, sel, upd, yacc, keys, mem0_v, wr_v, idx_s,
            sem_in, sem_out):
    w_hbm = [wq_hbm, wk_hbm, wv_hbm]

    def wtile(j):
        return w_p.at[j]

    SEM_X8, SEM_B0, SEM_LN, SEM_TK, SEM_MLP, SEM_WO = 0, 4, 7, 15, 16, 17

    def w_start(q0, n, sem):
        for q in range(q0, q0 + n):
            src = w_hbm[q // 16].bitcast(U32).at[:, q % 16, :]
            pltpu.make_async_copy(src, raw.at[q, pl.ds(0, D), :], sem_in.at[sem]).start()

    def w_wait(q0, n, sem):
        blk = raw.at[pl.ds(q0, n), pl.ds(0, D), :]
        pltpu.make_async_copy(blk, blk, sem_in.at[sem]).wait()

    def x8_copy(b):
        return pltpu.make_async_copy(x_hbm.at[pl.ds(b * 16, 16), pl.ds(LIVE, 8), :],
                                     x_v.at[pl.ds(1 + b * 16, 16), pl.ds(LIVE, 8), :], sem_in.at[SEM_X8 + b])

    def xa_copy(i):
        return pltpu.make_async_copy(x_hbm.at[pl.ds(i * 8, 8), pl.ds(0, LIVE), :],
                                     x_v.at[pl.ds(1 + i * 8, 8), pl.ds(0, LIVE), :], sem_in.at[SEM_LN + i])

    cp_wr = pltpu.make_async_copy(wr_hbm, wr_v, sem_in.at[SEM_B0 + 2])
    cp_mem = pltpu.make_async_copy(mem0_hbm, mem0_v, sem_in.at[SEM_TK])
    mlp_copies = [pltpu.make_async_copy(s_, d_, sem_in.at[SEM_MLP])
                  for s_, d_ in [(wg_hbm, wg_v), (wu_hbm, wu_v), (wd_hbm, wd_v)]]
    wo32 = wo_hbm.bitcast(U32)
    wo_copies = [pltpu.make_async_copy(wo32.at[:, pl.ds(j * 128, 128)], wo_p.at[j], sem_in.at[SEM_WO])
                 for j in range(NT)]

    for b in range(4):
        x8_copy(b).start()
    w_start(0, 1, SEM_B0)
    w_start(1, 1, SEM_B0 + 1)
    w_start(2, 2, SEM_B0 + 2)
    cp_wr.start()
    for i in range(8):
        w_start(4 + 4 * i, 4, SEM_LN + i)
        xa_copy(i).start()
    w_start(36, NPAIR - 36, SEM_TK)
    cp_mem.start()
    for c in mlp_copies:
        c.start()
    for c in wo_copies:
        c.start()

    xb3 = xb_v.reshape(NSEG + 1, SEG, D)
    x_v[0] = jnp.zeros((SEG, D), BF16)
    xb3[0] = jnp.zeros((SEG, D), F32)
    keys[...] = jnp.full(keys.shape, KEY_NONE, F32)
    yacc[...] = jnp.zeros(yacc.shape, F32)
    kv_s[:, :, 0:8, :] = jnp.zeros((H, 2, 8, DH), F32)
    raw[NPAIR, 0:D, :] = jnp.zeros((D, 128), U32)
    acc[M:L, :] = jnp.zeros((SEG, D), F32)

    def router_w():
        wr5 = wr_v[...].astype(F32)
        return jnp.concatenate([wr5[j:j + 1, :] for j in range(NT)], axis=1)

    def layernorm(s0, nseg, t0, nrow):
        n = nseg * nrow
        x = x_v[pl.ds(1 + s0, nseg), t0:t0 + nrow, :].astype(F32).reshape(n, D)
        mu = jnp.sum(x, axis=-1, keepdims=True) * (1.0 / D)
        xc = x - mu
        var = jnp.sum(xc * xc, axis=-1, keepdims=True) * (1.0 / D)
        sd = _rb(jnp.sqrt(_rb(_rb(var) + EPS)))
        xn = _rb(_rb(x - _rb(mu)) / sd)
        xb3[pl.ds(1 + s0, nseg), t0:t0 + nrow, :] = xn.reshape(nseg, nrow, D)
        return xn

    def ln8_body(b, carry):
        x8_copy(b).wait()
        xn = layernorm(b * 16, 16, LIVE, 8)
        lhs_v[pl.ds(pl.multiple_of(b * 64, 64), 64), :] = pltpu.bitcast(xn.astype(BF16), U32)
        return carry

    jax.lax.fori_loop(0, 4, ln8_body, 0)

    def ln_seg(s, wr):
        tail = xb3[1 + s, LIVE:SEG, :]
        xn = layernorm(s, 1, 0, LIVE)
        xa_v[pl.ds(pl.multiple_of(s * LIVE, 8), LIVE), :] = xn
        r = _rb(jnp.sum(jnp.concatenate([xn, tail], axis=0) * wr, axis=-1, keepdims=True))
        r = jnp.where(r == 0.0, 0.0, r)
        bits = pltpu.bitcast(jnp.broadcast_to(r, (SEG, 128)), I32) >> 16
        mono = jnp.where(bits < 0, (-32768) - bits, bits)
        mono = jnp.where(r != r, -40000, mono)
        row = jax.lax.broadcasted_iota(I32, (SEG, 128), 0)
        key = (mono * SEG + ((SEG - 1) - row)).astype(F32)
        lane = jax.lax.broadcasted_iota(I32, (SEG, 128), 1)
        keys[...] = jnp.where(lane == s, key, keys[...])
        return pltpu.bitcast(key, U32)

    def top_rows():
        kv = keys[...]
        lane = jax.lax.broadcasted_iota(I32, (1, 128), 1).astype(F32)
        for c in range(TOPC):
            col = jnp.max(kv, axis=0, keepdims=True)
            val = jnp.floor(col * (1.0 / SEG))
            fk = val * 128.0 + (127.0 - lane)
            win = fk == jnp.max(fk, axis=1, keepdims=True)
            kv = jnp.where(win & (kv == col), KEY_NONE, kv)
            pos = lane * SEG + ((SEG - 1.0) - (col - val * SEG))
            idx = jnp.clip(jnp.max(jnp.where(win, pos, 0.0)).astype(I32), 0, S - 1)
            idx_s[c] = idx
            sel[pl.ds(c, 1), :] = xb_v[pl.ds(SEG + idx, 1), :]

    def repack(rv, wv, p, part=None, tie=None):
        m_lo = jnp.full((8, 128), 0xFFFF, U32)
        m_hi = jnp.full((8, 128), 0xFFFF0000, U32)
        if tie is not None:
            m_lo = jnp.where(tie[0], tie[1], m_lo)
            m_hi = jnp.where(tie[0], tie[1], m_hi)
        for g in range(D // 16):
            if part is not None and g % part[1] != part[0]:
                continue
            a = rv[p, pl.ds(16 * g, 8, stride=2), :]
            b = rv[p, pl.ds(16 * g + 1, 8, stride=2), :]
            wv[2 * p, 8 * g:8 * g + 8, :] = (a & m_lo) | (b << 16)
            wv[2 * p + 1, 8 * g:8 * g + 8, :] = (a >> 16) | (b & m_hi)

    def block(q0, n, never=None, side=None, jobs=None):
        rv = raw.at[pl.ds(q0, n + 1)]
        wv = w_p.at[pl.ds(2 * q0, 2 * n + 2)]
        pv = pre.at[pl.ds(2 * q0, 2 * n)]
        for u in range(2 * n):
            if u % 2 == 0 and u // 2 + 1 < n:
                repack(rv, wv, u // 2 + 1)
            for c in range(4):
                lhs = lhs_v[c * 64:(c + 1) * 64, :]
                if side is not None and 4 * u + c in LNT:
                    tok = side(LNT.index(4 * u + c))
                    nr = tok.shape[0]
                    head = jnp.where(never, tok, lhs[0:nr, 0:128])
                    lhs = jnp.concatenate(
                        [jnp.concatenate([head, lhs[0:nr, 128:]], axis=1), lhs[nr:, :]], axis=0)
                lhs = pltpu.bitcast(lhs, BF16)
                if jobs:
                    r = None
                    for kt in range(NT):
                        t_ = _dot(lhs[:, kt * 128:(kt + 1) * 128],
                                  pltpu.bitcast(wv[u, kt * 64:(kt + 1) * 64, :], BF16))
                        r = t_ if r is None else r + t_
                        if jobs:
                            jobs.pop(0)()
                elif jobs is not None and 4 * u + c >= 8 * n - FINE[0]:
                    r = jnp.concatenate([_dot(lhs[m_:m_ + FINE[1], :], pltpu.bitcast(wv[u], BF16))
                                         for m_ in range(0, 128, FINE[1])], axis=0)
                else:
                    r = _dot(lhs, pltpu.bitcast(wv[u], BF16))
                pv[u, c * 128:(c + 1) * 128, :] = r
                n8 = (u - max(2 * n - 3, 0)) * 4 + c
                if 0 <= n8 < 8:
                    repack(rv, wv, n, (n8, 8),
                           None if never is None else (never, pltpu.bitcast(r[0:8, :], U32)))

    w_wait(0, 1, SEM_B0)
    repack(raw, w_p, 0)
    w_wait(1, 1, SEM_B0 + 1)
    block(0, 1)
    w_wait(2, 2, SEM_B0 + 2)
    cp_wr.wait()
    block(1, 2)

    def ln_body(i, carry):
        w_wait(4 + 4 * i, 4, SEM_LN + i)
        xa_copy(i).wait()
        wr = router_w()
        block(3 + 4 * i, 4, i < 0, side=lambda u: ln_seg(i * 8 + u, wr))
        return carry

    jax.lax.fori_loop(0, 8, ln_body, 0)

    w_wait(36, NPAIR - 36, SEM_TK)
    cp_mem.wait()
    acc[0:M, :] = mem0_v[...].astype(F32)
    top_rows()
    block(35, 1)

    for c in mlp_copies:
        c.wait()
    FP = FF // 3

    def mlp_body(t, carry):
        f0 = pl.multiple_of(t * FP, 16)
        xs = sel[...]
        cuts = [(a_, min(a_ + 128, FP)) for a_ in range(0, FP, 128)]
        val = {}

        def up_tile(which, n, kt):
            def run():
                a_, b_ = cuts[n]
                w = (wg_v, wu_v)[which][pl.ds(f0 + a_, b_ - a_), kt * 128:(kt + 1) * 128]
                r = _dot_nt(xs[:, kt * 128:(kt + 1) * 128], w)
                val[which, n] = r if kt == 0 else val[which, n] + r
            return run

        def down_tile(n, j):
            def run():
                a_, b_ = cuts[n]
                if j == 0:
                    g_ = _rb(val.pop((0, n)))
                    val['h', n] = _rb(g_ * _sigmoid(g_)) * _rb(val.pop((1, n)))
                r = _dot(val['h', n], wd_v[pl.ds(f0 + a_, b_ - a_), j * 128:(j + 1) * 128])
                val['y', j] = r if n == 0 else val['y', j] + r
            return run

        def skip():
            pass

        real = ([up_tile(which, n, kt) for n in range(len(cuts)) for which in range(2) for kt in range(NT)]
                + [down_tile(n, j) for n in range(len(cuts)) for j in range(NT)])
        jobs = [skip] * MS1
        for n_, job in enumerate(real):
            jobs[MS0 + (n_ * (MS1 - MS0)) // len(real)] = job
        block(36 + 4 * t, 4, t < 0, jobs=jobs)
        assert not jobs
        y = yacc[...] + jnp.concatenate([val['y', j] for j in range(NT)], axis=1)
        yacc[...] = y
        r_sel = _rb(jnp.sum(xs * router_w(), axis=-1, keepdims=True))
        upd[...] = xs + _rb(_rb(y) * _rb(_sigmoid(r_sel)))
        for c in range(TOPC):
            xb_v[pl.ds(SEG + jnp.clip(idx_s[c], 0, S - 1), 1), :] = upd[pl.ds(c, 1), :]
        return carry

    jax.lax.fori_loop(0, 3, mlp_body, 0)

    for c in wo_copies:
        c.wait()

    scale = DH ** (-0.5)
    qm_i = jax.lax.broadcasted_iota(I32, (L - 8, L), 0)
    mask_m = (qm_i < M) | (qm_i + 8 >= jax.lax.broadcasted_iota(I32, (L - 8, L), 1))
    diag_ok = (jax.lax.broadcasted_iota(I32, (7, 8, DH), 1)
               > jax.lax.broadcasted_iota(I32, (7, 8, DH), 0))

    def finish(s0, n, u, sa):
        xb = xb3.at[pl.ds(s0, n)][u]
        o = x_v.at[pl.ds(s0, n)][u].astype(F32) + sa * (xb * _sigmoid(xb))
        out_v.at[pl.ds(s0, n)][u] = o.astype(BF16)
        return o

    def out_copy(seg, n):
        return pltpu.make_async_copy(out_v.at[pl.ds(seg + 1, n)], out_hbm.at[pl.ds(seg, n)], sem_out.at[0])

    def step(i, u, prev):
        pre_i = pre.at[:, pl.ds(pl.multiple_of(i * (8 * UNROLL), 8 * UNROLL), 8 * UNROLL), :]
        xa_i = xa_v.at[pl.ds(pl.multiple_of(i * (LIVE * UNROLL), 8 * UNROLL), LIVE * UNROLL), :]
        pre_s = pre_i.at[:, pl.ds(pl.multiple_of(u * 8, 8), 8), :]
        xa = xa_i[pl.ds(pl.multiple_of(u * LIVE, 8), LIVE), :]
        lhs = jnp.concatenate([prev[0:M, :], xa], axis=0).astype(BF16)
        fin = finish(pl.multiple_of(i * UNROLL, UNROLL), UNROLL, u, prev[M:L, :])

        @pl.when(u == UNROLL - 2)
        def _():
            out_copy(i * UNROLL, UNROLL - 2).start()

        def proj(j, tie=None):
            lh = lhs
            if tie is not None:
                top = pltpu.bitcast(lhs[0:16, 0:128], U32)
                top = pltpu.bitcast(jnp.where(i < 0, pltpu.bitcast(tie, U32), top), BF16)
                lh = jnp.concatenate([jnp.concatenate([top, lhs[0:16, 128:]], axis=1), lhs[16:, :]], axis=0)
            t = _dot(lh, pltpu.bitcast(wtile(j)[...], BF16))
            if TIE0 <= j < TIE0 + NT:
                t = jnp.where(jnp.logical_and(i < 0, u == 0),
                              fin[:, (j - TIE0) * 128:(j - TIE0 + 1) * 128], t)
            return jnp.concatenate([t, pre_s[j]], axis=0)

        NG = H // GH
        qs, ks, vs, ps, os_, ox, iv, on = {}, {}, {}, {}, {}, {}, {}, {}

        def do_qkv(g):
            js = [m * H + h for h in range(g * GH, (g + 1) * GH) for m in range(3)]
            if g == 0:
                part = {}
                for kt in range(NT):
                    for j in js:
                        t = _dot(lhs[:, kt * 128:(kt + 1) * 128],
                                 pltpu.bitcast(wtile(j)[kt * 64:(kt + 1) * 64, :], BF16))
                        part[j] = t if kt == 0 else part[j] + t
                res = {j: jnp.concatenate([part[j], pre_s[j]], axis=0) for j in js}
            else:
                res = {}
                for n, j in enumerate(js):
                    tie = None
                    for hh, pos in enumerate(TP):
                        if n == pos and g >= TL:
                            tie = ox[(g - TL) * GH + hh]
                    res[j] = proj(j, tie)
            for h in range(g * GH, (g + 1) * GH):
                qs[h], ks[h], vs[h] = res[h], res[H + h], res[2 * H + h]

        def vpu_rows(h, q, k, v):
            def win(which, val, r):
                if r % 8 == 0:
                    return val[8 - r:16 - r, :]
                return kv_s[h, which, 16 - r:24 - r, :]

            def wins(which, val):
                return jnp.stack([win(which, val, r) for r in range(16)])

            def fold(f, x):
                while x.shape[0] > 1:
                    n = x.shape[0] // 2
                    x = f(x[:n], x[n:])
                return x[0]

            qa = q[8:16, :] * (scale * LOG2E)
            sc = jnp.sum(qa[None] * wins(0, k), axis=-1, keepdims=True)
            sc = jnp.broadcast_to(sc, (16, 8, DH))
            sc = jnp.concatenate([sc[:9], jnp.where(diag_ok, sc[9:], -jnp.inf)], axis=0)
            e = jnp.exp2(sc - fold(jnp.maximum, sc)[None])
            return fold(jnp.add, e * wins(1, v)) * pl.reciprocal(fold(jnp.add, e), approx=True)

        def do_s(g):
            for h in range(g * GH, (g + 1) * GH):
                q, k = qs.pop(h), ks.pop(h)
                kv_s[h, 0, 8:24, :] = k[0:16, :]
                kv_s[h, 1, 8:24, :] = vs[h][0:16, :]
                ox[h] = vpu_rows(h, q, k, vs[h])
                qm = jnp.concatenate([q[0:8, :], q[16:, :]], axis=0)
                sc = _dot_nt(qm.astype(BF16), k.astype(BF16))
                sc = jnp.where(mask_m, sc * (scale * LOG2E), NEG * LOG2E)
                e = jnp.exp2(sc - jnp.max(sc, axis=-1, keepdims=True))
                inv = pl.reciprocal(jnp.sum(e, axis=-1, keepdims=True), approx=True)
                ps[h] = e.astype(BF16)
                iv[h] = jnp.broadcast_to(inv, (SEG, DH))

        def do_pv(g):
            for h in range(g * GH, (g + 1) * GH):
                v = vs.pop(h)
                if g >= NG - TL:
                    v = jnp.concatenate([jnp.where(i < 0, ox[h], v[0:8, :]), v[8:, :]], axis=0)
                if h >= GH:
                    v = jnp.concatenate([v[0:8, :], jnp.where(i < 0, on[h - GH], v[8:, :])], axis=0)
                on[h] = _dot(ps.pop(h), v.astype(BF16)) * iv.pop(h)
                os_[h] = jnp.concatenate([on[h][0:8, :], ox[h], on[h][8:, :]], axis=0)

        def do_o(j, h0, h1):
            o = jnp.concatenate([os_[h] for h in range(h0, h1)], axis=1)
            return _dot(o, pltpu.bitcast(wo_p[j, h0 * 64:h1 * 64, :], BF16))

        for g in range(NG):
            do_qkv(g)
            if g >= LS:
                do_s(g - LS)
            if g >= LP:
                do_pv(g - LP)
        sched = dict(TAIL)
        ns, npv = NG - LS, NG - LP
        for j in range(NT):
            part_v[:, j * 128:(j + 1) * 128] = do_o(j, 0, HS)
            for c_ in sched.get(j, ''):
                if c_ == 's':
                    do_s(ns)
                    ns += 1
                else:
                    do_pv(npv)
                    npv += 1
        assert ns == NG and npv == NG
        return jnp.concatenate(
            [part_v[:, j * 128:(j + 1) * 128] + do_o(j, HS, H) for j in range(NT)], axis=1)

    def multi(i, carry):
        acc[...] = jax.lax.fori_loop(0, UNROLL, lambda u, cur: step(i, u, cur), acc[...],
                                     unroll=True)
        out_copy(i * UNROLL + UNROLL - 2, 1).start()

        @pl.when(i > 0)
        def _():
            out_copy(jnp.maximum(i * UNROLL - 1, 0), 1).start()
        return carry

    jax.lax.fori_loop(0, NSEG // UNROLL, multi, 0)
    finish(NSEG, 1, 0, acc[M:L, :])
    out_copy(NSEG - 1, 1).start()
    out_copy(0, NSEG).wait()


@jax.jit
def pallas_recurrent_scan__memory_aug_recurrent_mem_tr__moe_arch_mod__prompt_kernel(
    A_x: jax.Array,
    A_mem0: jax.Array,
    A_Wq: jax.Array,
    A_Wk: jax.Array,
    A_Wv: jax.Array,
    A_Wo: jax.Array,
    A_seg_len: jax.Array,
    B_x: jax.Array,
    B_w_r: jax.Array,
    B_w_gate: jax.Array,
    B_w_up: jax.Array,
    B_w_down: jax.Array,
):
    del A_seg_len, B_x
    assert A_x.shape == (1, S, D) and A_Wq.shape == (D, H, DH) and A_mem0.shape == (1, M, D)
    hbm = pl.BlockSpec(memory_space=pltpu.HBM)
    out = pl.pallas_call(
        _kernel,
        out_shape=jax.ShapeDtypeStruct((NSEG, SEG, D), BF16),
        in_specs=[hbm] * 10,
        out_specs=hbm,
        scratch_shapes=[
            pltpu.VMEM((NSEG + 2, SEG, D), BF16),
            pltpu.VMEM((NSEG * 4, D), U32),
            pltpu.VMEM((NSEG * LIVE, D), F32),
            pltpu.VMEM((S + SEG, D), F32),
            pltpu.VMEM((NPAIR + 1, D + 32, 128), U32),
            pltpu.VMEM((2 * NPAIR + 2, D // 2, 128), U32),
            pltpu.VMEM((NT, H * DH // 2, 128), U32),
            pltpu.VMEM((3 * H, NSEG * 8, DH), F32),
            pltpu.VMEM((FF, D), BF16),
            pltpu.VMEM((FF, D), BF16),
            pltpu.VMEM((FF, D), BF16),
            pltpu.VMEM((NSEG + 2, SEG, D), BF16),
            pltpu.VMEM((L, D), F32),
            pltpu.VMEM((L, D), F32),
            pltpu.VMEM((H, 2, 24, DH), F32),
            pltpu.VMEM((TOPC, D), F32),
            pltpu.VMEM((TOPC, D), F32),
            pltpu.VMEM((TOPC, D), F32),
            pltpu.VMEM((SEG, 128), F32),
            pltpu.VMEM((M, D), BF16),
            pltpu.VMEM((NT, 128), BF16),
            pltpu.SMEM((TOPC,), I32),
            pltpu.SemaphoreType.DMA((18,)),
            pltpu.SemaphoreType.DMA((1,)),
        ],
        compiler_params=pltpu.CompilerParams(vmem_limit_bytes=110 * 1024 * 1024),
    )(
        A_x.reshape(NSEG, SEG, D),
        A_mem0.reshape(M, D),
        A_Wq, A_Wk, A_Wv,
        A_Wo.reshape(H * DH, D),
        B_w_r.reshape(NT, 128),
        B_w_gate.T, B_w_up.T, B_w_down,
    )
    return out.reshape(1, S, D)
```

```python
import math

import jax
import jax.numpy as jnp
import jax.experimental.pallas as pl
import jax.experimental.pallas.tpu as pltpu

F32 = jnp.float32
BF16 = jnp.bfloat16
U32 = jnp.uint32
I32 = jnp.int32

S = 2048
D = 640
H = 32
DH = 128
M = 8
SEG = 32
NSEG = S // SEG
L = M + SEG
FF = 1728
TOPC = 8
NT = D // 128
LIVE = SEG - 8
EPS = 1e-05
NEG = -1000000000.0
LOG2E = math.log2(math.e)
NPAIR = 3 * H // 2
KEY_NONE = -1e30

UNROLL = 8
GH = 2
LS, LP = 1, 2
TL, TP = 2, (3, 5)
ORD = (0, 1, 3, 4, 5, 2)
HS = 24
TAIL = ((0, 'sp'), (2, 'p'))
FINE = (1, 32)
TIE0 = 2
LNT = (6, 10, 14, 18, 22, 25, 28, 31)
MS0, MS1 = 5, 155


def _dot(a, b):
    return jax.lax.dot_general(a, b, (((1,), (0,)), ((), ())), preferred_element_type=F32)


def _dot_nt(a, b):
    return jax.lax.dot_general(a, b, (((1,), (1,)), ((), ())), preferred_element_type=F32)


def _rb(x):
    return x.astype(BF16).astype(F32)


def _sigmoid(x):
    return pl.reciprocal(1.0 + jnp.exp(-x), approx=True)


def _kernel(x_hbm, mem0_hbm, wq_hbm, wk_hbm, wv_hbm, wo_hbm, wr_hbm, wg_hbm, wu_hbm, wd_hbm,
            out_hbm,
            x_v, lhs_v, xa_v, xb_v, raw, w_p, wo_p, pre, wg_v, wu_v, wd_v,
            out_v, acc, part_v, kv_s, sel, upd, yacc, keys, mem0_v, wr_v, idx_s,
            sem_in, sem_out):
    w_hbm = [wq_hbm, wk_hbm, wv_hbm]

    def wtile(j):
        return w_p.at[j]

    SEM_X8, SEM_B0, SEM_LN, SEM_TK, SEM_MLP, SEM_WO = 0, 4, 7, 15, 16, 17

    def w_start(q0, n, sem):
        for q in range(q0, q0 + n):
            src = w_hbm[q // 16].bitcast(U32).at[:, q % 16, :]
            pltpu.make_async_copy(src, raw.at[q, pl.ds(0, D), :], sem_in.at[sem]).start()

    def w_wait(q0, n, sem):
        blk = raw.at[pl.ds(q0, n), pl.ds(0, D), :]
        pltpu.make_async_copy(blk, blk, sem_in.at[sem]).wait()

    def x8_copy(b):
        return pltpu.make_async_copy(x_hbm.at[pl.ds(b * 16, 16), pl.ds(LIVE, 8), :],
                                     x_v.at[pl.ds(1 + b * 16, 16), pl.ds(LIVE, 8), :], sem_in.at[SEM_X8 + b])

    def xa_copy(i):
        return pltpu.make_async_copy(x_hbm.at[pl.ds(i * 8, 8), pl.ds(0, LIVE), :],
                                     x_v.at[pl.ds(1 + i * 8, 8), pl.ds(0, LIVE), :], sem_in.at[SEM_LN + i])

    cp_wr = pltpu.make_async_copy(wr_hbm, wr_v, sem_in.at[SEM_B0 + 2])
    cp_mem = pltpu.make_async_copy(mem0_hbm, mem0_v, sem_in.at[SEM_TK])
    mlp_copies = [pltpu.make_async_copy(s_, d_, sem_in.at[SEM_MLP])
                  for s_, d_ in [(wg_hbm, wg_v), (wu_hbm, wu_v), (wd_hbm, wd_v)]]
    wo32 = wo_hbm.bitcast(U32)
    wo_copies = [pltpu.make_async_copy(wo32.at[:, pl.ds(j * 128, 128)], wo_p.at[j], sem_in.at[SEM_WO])
                 for j in range(NT)]

    for b in range(4):
        x8_copy(b).start()
    w_start(0, 1, SEM_B0)
    w_start(1, 1, SEM_B0 + 1)
    w_start(2, 2, SEM_B0 + 2)
    cp_wr.start()
    for i in range(8):
        w_start(4 + 4 * i, 4, SEM_LN + i)
        xa_copy(i).start()
    w_start(36, NPAIR - 36, SEM_TK)
    cp_mem.start()
    for c in mlp_copies:
        c.start()
    for c in wo_copies:
        c.start()

    xb3 = xb_v.reshape(NSEG + 1, SEG, D)
    x_v[0] = jnp.zeros((SEG, D), BF16)
    xb3[0] = jnp.zeros((SEG, D), F32)
    keys[...] = jnp.full(keys.shape, KEY_NONE, F32)
    yacc[...] = jnp.zeros(yacc.shape, F32)
    kv_s[:, :, 0:8, :] = jnp.zeros((H, 2, 8, DH), F32)
    raw[NPAIR, 0:D, :] = jnp.zeros((D, 128), U32)
    acc[M:L, :] = jnp.zeros((SEG, D), F32)

    def router_w():
        wr5 = wr_v[...].astype(F32)
        return jnp.concatenate([wr5[j:j + 1, :] for j in range(NT)], axis=1)

    def layernorm(s0, nseg, t0, nrow):
        n = nseg * nrow
        x = x_v[pl.ds(1 + s0, nseg), t0:t0 + nrow, :].astype(F32).reshape(n, D)
        mu = jnp.sum(x, axis=-1, keepdims=True) * (1.0 / D)
        xc = x - mu
        var = jnp.sum(xc * xc, axis=-1, keepdims=True) * (1.0 / D)
        sd = _rb(jnp.sqrt(_rb(_rb(var) + EPS)))
        xn = _rb(_rb(x - _rb(mu)) / sd)
        xb3[pl.ds(1 + s0, nseg), t0:t0 + nrow, :] = xn.reshape(nseg, nrow, D)
        return xn

    def ln8_body(b, carry):
        x8_copy(b).wait()
        xn = layernorm(b * 16, 16, LIVE, 8)
        lhs_v[pl.ds(pl.multiple_of(b * 64, 64), 64), :] = pltpu.bitcast(xn.astype(BF16), U32)
        return carry

    jax.lax.fori_loop(0, 4, ln8_body, 0)

    def ln_seg(s, wr):
        tail = xb3[1 + s, LIVE:SEG, :]
        xn = layernorm(s, 1, 0, LIVE)
        xa_v[pl.ds(pl.multiple_of(s * LIVE, 8), LIVE), :] = xn
        r = _rb(jnp.sum(jnp.concatenate([xn, tail], axis=0) * wr, axis=-1, keepdims=True))
        r = jnp.where(r == 0.0, 0.0, r)
        bits = pltpu.bitcast(jnp.broadcast_to(r, (SEG, 128)), I32) >> 16
        mono = jnp.where(bits < 0, (-32768) - bits, bits)
        mono = jnp.where(r != r, -40000, mono)
        row = jax.lax.broadcasted_iota(I32, (SEG, 128), 0)
        key = (mono * SEG + ((SEG - 1) - row)).astype(F32)
        lane = jax.lax.broadcasted_iota(I32, (SEG, 128), 1)
        keys[...] = jnp.where(lane == s, key, keys[...])
        return pltpu.bitcast(key, U32)

    def top_rows():
        kv = keys[...]
        lane = jax.lax.broadcasted_iota(I32, (1, 128), 1).astype(F32)
        for c in range(TOPC):
            col = jnp.max(kv, axis=0, keepdims=True)
            val = jnp.floor(col * (1.0 / SEG))
            fk = val * 128.0 + (127.0 - lane)
            win = fk == jnp.max(fk, axis=1, keepdims=True)
            kv = jnp.where(win & (kv == col), KEY_NONE, kv)
            pos = lane * SEG + ((SEG - 1.0) - (col - val * SEG))
            idx = jnp.clip(jnp.max(jnp.where(win, pos, 0.0)).astype(I32), 0, S - 1)
            idx_s[c] = idx
            sel[pl.ds(c, 1), :] = xb_v[pl.ds(SEG + idx, 1), :]

    def repack(rv, wv, p, part=None, tie=None):
        m_lo = jnp.full((8, 128), 0xFFFF, U32)
        m_hi = jnp.full((8, 128), 0xFFFF0000, U32)
        if tie is not None:
            m_lo = jnp.where(tie[0], tie[1], m_lo)
            m_hi = jnp.where(tie[0], tie[1], m_hi)
        for g in range(D // 16):
            if part is not None and g % part[1] != part[0]:
                continue
            a = rv[p, pl.ds(16 * g, 8, stride=2), :]
            b = rv[p, pl.ds(16 * g + 1, 8, stride=2), :]
            wv[2 * p, 8 * g:8 * g + 8, :] = (a & m_lo) | (b << 16)
            wv[2 * p + 1, 8 * g:8 * g + 8, :] = (a >> 16) | (b & m_hi)

    def block(q0, n, never=None, side=None, jobs=None):
        rv = raw.at[pl.ds(q0, n + 1)]
        wv = w_p.at[pl.ds(2 * q0, 2 * n + 2)]
        pv = pre.at[pl.ds(2 * q0, 2 * n)]
        for u in range(2 * n):
            if u % 2 == 0 and u // 2 + 1 < n:
                repack(rv, wv, u // 2 + 1)
            for c in range(4):
                lhs = lhs_v[c * 64:(c + 1) * 64, :]
                if side is not None and 4 * u + c in LNT:
                    tok = side(LNT.index(4 * u + c))
                    nr = tok.shape[0]
                    head = jnp.where(never, tok, lhs[0:nr, 0:128])
                    lhs = jnp.concatenate(
                        [jnp.concatenate([head, lhs[0:nr, 128:]], axis=1), lhs[nr:, :]], axis=0)
                lhs = pltpu.bitcast(lhs, BF16)
                if jobs:
                    r = None
                    for kt in range(NT):
                        t_ = _dot(lhs[:, kt * 128:(kt + 1) * 128],
                                  pltpu.bitcast(wv[u, kt * 64:(kt + 1) * 64, :], BF16))
                        r = t_ if r is None else r + t_
                        if jobs:
                            jobs.pop(0)()
                elif jobs is not None and 4 * u + c >= 8 * n - FINE[0]:
                    r = jnp.concatenate([_dot(lhs[m_:m_ + FINE[1], :], pltpu.bitcast(wv[u], BF16))
                                         for m_ in range(0, 128, FINE[1])], axis=0)
                else:
                    r = _dot(lhs, pltpu.bitcast(wv[u], BF16))
                pv[u, c * 128:(c + 1) * 128, :] = r
                n8 = (u - max(2 * n - 3, 0)) * 4 + c
                if 0 <= n8 < 8:
                    repack(rv, wv, n, (n8, 8),
                           None if never is None else (never, pltpu.bitcast(r[0:8, :], U32)))

    w_wait(0, 1, SEM_B0)
    repack(raw, w_p, 0)
    w_wait(1, 1, SEM_B0 + 1)
    block(0, 1)
    w_wait(2, 2, SEM_B0 + 2)
    cp_wr.wait()
    block(1, 2)

    def ln_body(i, carry):
        w_wait(4 + 4 * i, 4, SEM_LN + i)
        xa_copy(i).wait()
        wr = router_w()
        block(3 + 4 * i, 4, i < 0, side=lambda u: ln_seg(i * 8 + u, wr))
        return carry

    jax.lax.fori_loop(0, 8, ln_body, 0)

    w_wait(36, NPAIR - 36, SEM_TK)
    cp_mem.wait()
    acc[0:M, :] = mem0_v[...].astype(F32)
    top_rows()
    block(35, 1)

    for c in mlp_copies:
        c.wait()
    FP = FF // 3

    def mlp_body(t, carry):
        f0 = pl.multiple_of(t * FP, 16)
        xs = sel[...]
        cuts = [(a_, min(a_ + 128, FP)) for a_ in range(0, FP, 128)]
        val = {}

        def up_tile(which, n, kt):
            def run():
                a_, b_ = cuts[n]
                w = (wg_v, wu_v)[which][pl.ds(f0 + a_, b_ - a_), kt * 128:(kt + 1) * 128]
                r = _dot_nt(xs[:, kt * 128:(kt + 1) * 128], w)
                val[which, n] = r if kt == 0 else val[which, n] + r
            return run

        def down_tile(n, j):
            def run():
                a_, b_ = cuts[n]
                if j == 0:
                    g_ = _rb(val.pop((0, n)))
                    val['h', n] = _rb(g_ * _sigmoid(g_)) * _rb(val.pop((1, n)))
                r = _dot(val['h', n], wd_v[pl.ds(f0 + a_, b_ - a_), j * 128:(j + 1) * 128])
                val['y', j] = r if n == 0 else val['y', j] + r
            return run

        def skip():
            pass

        real = ([up_tile(which, n, kt) for n in range(len(cuts)) for which in range(2) for kt in range(NT)]
                + [down_tile(n, j) for n in range(len(cuts)) for j in range(NT)])
        jobs = [skip] * MS1
        for n_, job in enumerate(real):
            jobs[MS0 + (n_ * (MS1 - MS0)) // len(real)] = job
        block(36 + 4 * t, 4, t < 0, jobs=jobs)
        assert not jobs
        y = yacc[...] + jnp.concatenate([val['y', j] for j in range(NT)], axis=1)
        yacc[...] = y
        r_sel = _rb(jnp.sum(xs * router_w(), axis=-1, keepdims=True))
        upd[...] = xs + _rb(_rb(y) * _rb(_sigmoid(r_sel)))
        for c in range(TOPC):
            xb_v[pl.ds(SEG + jnp.clip(idx_s[c], 0, S - 1), 1), :] = upd[pl.ds(c, 1), :]
        return carry

    jax.lax.fori_loop(0, 3, mlp_body, 0)

    for c in wo_copies:
        c.wait()

    scale = DH ** (-0.5)
    qm_i = jax.lax.broadcasted_iota(I32, (L - 8, L), 0)
    mask_m = (qm_i < M) | (qm_i + 8 >= jax.lax.broadcasted_iota(I32, (L - 8, L), 1))
    diag_ok = (jax.lax.broadcasted_iota(I32, (7, 8, DH), 1)
               > jax.lax.broadcasted_iota(I32, (7, 8, DH), 0))

    def finish(s0, n, u, sa):
        xb = xb3.at[pl.ds(s0, n)][u]
        o = x_v.at[pl.ds(s0, n)][u].astype(F32) + sa * (xb * _sigmoid(xb))
        out_v.at[pl.ds(s0, n)][u] = o.astype(BF16)
        return o

    def out_copy(seg, n):
        return pltpu.make_async_copy(out_v.at[pl.ds(seg + 1, n)], out_hbm.at[pl.ds(seg, n)], sem_out.at[0])

    def step(i, u, prev):
        pre_i = pre.at[:, pl.ds(pl.multiple_of(i * (8 * UNROLL), 8 * UNROLL), 8 * UNROLL), :]
        xa_i = xa_v.at[pl.ds(pl.multiple_of(i * (LIVE * UNROLL), 8 * UNROLL), LIVE * UNROLL), :]
        pre_s = pre_i.at[:, pl.ds(pl.multiple_of(u * 8, 8), 8), :]
        xa = xa_i[pl.ds(pl.multiple_of(u * LIVE, 8), LIVE), :]
        lhs = jnp.concatenate([prev[0:M, :], xa], axis=0).astype(BF16)
        fin = finish(pl.multiple_of(i * UNROLL, UNROLL), UNROLL, u, prev[M:L, :])

        @pl.when(u == UNROLL - 2)
        def _():
            out_copy(i * UNROLL, UNROLL - 2).start()

        def proj(j, tie=None):
            lh = lhs
            if tie is not None:
                top = pltpu.bitcast(lhs[0:16, 0:128], U32)
                top = pltpu.bitcast(jnp.where(i < 0, pltpu.bitcast(tie, U32), top), BF16)
                lh = jnp.concatenate([jnp.concatenate([top, lhs[0:16, 128:]], axis=1), lhs[16:, :]], axis=0)
            t = _dot(lh, pltpu.bitcast(wtile(j)[...], BF16))
            if TIE0 <= j < TIE0 + NT:
                t = jnp.where(jnp.logical_and(i < 0, u == 0),
                              fin[:, (j - TIE0) * 128:(j - TIE0 + 1) * 128], t)
            return jnp.concatenate([t, pre_s[j]], axis=0)

        NG = H // GH
        qs, ks, vs, ps, os_, ox, iv, on = {}, {}, {}, {}, {}, {}, {}, {}

        def do_qkv(g):
            js = [(x % 3) * H + g * GH + x // 3 for x in ORD]
            if g == 0:
                part = {}
                for kt in range(NT):
                    for j in js:
                        t = _dot(lhs[:, kt * 128:(kt + 1) * 128],
                                 pltpu.bitcast(wtile(j)[kt * 64:(kt + 1) * 64, :], BF16))
                        part[j] = t if kt == 0 else part[j] + t
                res = {j: jnp.concatenate([part[j], pre_s[j]], axis=0) for j in js}
            else:
                res = {}
                for n, j in enumerate(js):
                    tie = None
                    for hh, pos in enumerate(TP):
                        if n == pos and g >= TL:
                            tie = ox[(g - TL) * GH + hh]
                    res[j] = proj(j, tie)
            for h in range(g * GH, (g + 1) * GH):
                qs[h], ks[h], vs[h] = res[h], res[H + h], res[2 * H + h]

        def vpu_rows(h, q, k, v):
            def win(which, val, r):
                if r % 8 == 0:
                    return val[8 - r:16 - r, :]
                return kv_s[h, which, 16 - r:24 - r, :]

            def wins(which, val):
                return jnp.stack([win(which, val, r) for r in range(16)])

            def fold(f, x):
                while x.shape[0] > 1:
                    n = x.shape[0] // 2
                    x = f(x[:n], x[n:])
                return x[0]

            qa = q[8:16, :] * (scale * LOG2E)
            sc = jnp.sum(qa[None] * wins(0, k), axis=-1, keepdims=True)
            sc = jnp.broadcast_to(sc, (16, 8, DH))
            sc = jnp.concatenate([sc[:9], jnp.where(diag_ok, sc[9:], -jnp.inf)], axis=0)
            e = jnp.exp2(sc - fold(jnp.maximum, sc)[None])
            return fold(jnp.add, e * wins(1, v)) * pl.reciprocal(fold(jnp.add, e), approx=True)

        def do_s(g):
            for h in range(g * GH, (g + 1) * GH):
                q, k = qs.pop(h), ks.pop(h)
                kv_s[h, 0, 8:24, :] = k[0:16, :]
                kv_s[h, 1, 8:24, :] = vs[h][0:16, :]
                ox[h] = vpu_rows(h, q, k, vs[h])
                qm = jnp.concatenate([q[0:8, :], q[16:, :]], axis=0)
                sc = _dot_nt(qm.astype(BF16), k.astype(BF16))
                sc = jnp.where(mask_m, sc * (scale * LOG2E), NEG * LOG2E)
                e = jnp.exp2(sc - jnp.max(sc, axis=-1, keepdims=True))
                inv = pl.reciprocal(jnp.sum(e, axis=-1, keepdims=True), approx=True)
                ps[h] = e.astype(BF16)
                iv[h] = jnp.broadcast_to(inv, (SEG, DH))

        def do_pv(g):
            for h in range(g * GH, (g + 1) * GH):
                v = vs.pop(h)
                if g >= NG - TL:
                    v = jnp.concatenate([jnp.where(i < 0, ox[h], v[0:8, :]), v[8:, :]], axis=0)
                if h >= GH:
                    v = jnp.concatenate([v[0:8, :], jnp.where(i < 0, on[h - GH], v[8:, :])], axis=0)
                on[h] = _dot(ps.pop(h), v.astype(BF16)) * iv.pop(h)
                os_[h] = jnp.concatenate([on[h][0:8, :], ox[h], on[h][8:, :]], axis=0)

        def do_o(j, h0, h1):
            o = jnp.concatenate([os_[h] for h in range(h0, h1)], axis=1)
            return _dot(o, pltpu.bitcast(wo_p[j, h0 * 64:h1 * 64, :], BF16))

        for g in range(NG):
            do_qkv(g)
            if g >= LS:
                do_s(g - LS)
            if g >= LP:
                do_pv(g - LP)
        sched = dict(TAIL)
        ns, npv = NG - LS, NG - LP
        for j in range(NT):
            part_v[:, j * 128:(j + 1) * 128] = do_o(j, 0, HS)
            for c_ in sched.get(j, ''):
                if c_ == 's':
                    do_s(ns)
                    ns += 1
                else:
                    do_pv(npv)
                    npv += 1
        assert ns == NG and npv == NG
        return jnp.concatenate(
            [part_v[:, j * 128:(j + 1) * 128] + do_o(j, HS, H) for j in range(NT)], axis=1)

    def multi(i, carry):
        acc[...] = jax.lax.fori_loop(0, UNROLL, lambda u, cur: step(i, u, cur), acc[...],
                                     unroll=True)
        out_copy(i * UNROLL + UNROLL - 2, 1).start()

        @pl.when(i > 0)
        def _():
            out_copy(jnp.maximum(i * UNROLL - 1, 0), 1).start()
        return carry

    jax.lax.fori_loop(0, NSEG // UNROLL, multi, 0)
    finish(NSEG, 1, 0, acc[M:L, :])
    out_copy(NSEG - 1, 1).start()
    out_copy(0, NSEG).wait()


@jax.jit
def pallas_recurrent_scan__memory_aug_recurrent_mem_tr__moe_arch_mod__prompt_kernel(
    A_x: jax.Array,
    A_mem0: jax.Array,
    A_Wq: jax.Array,
    A_Wk: jax.Array,
    A_Wv: jax.Array,
    A_Wo: jax.Array,
    A_seg_len: jax.Array,
    B_x: jax.Array,
    B_w_r: jax.Array,
    B_w_gate: jax.Array,
    B_w_up: jax.Array,
    B_w_down: jax.Array,
):
    del A_seg_len, B_x
    assert A_x.shape == (1, S, D) and A_Wq.shape == (D, H, DH) and A_mem0.shape == (1, M, D)
    hbm = pl.BlockSpec(memory_space=pltpu.HBM)
    out = pl.pallas_call(
        _kernel,
        out_shape=jax.ShapeDtypeStruct((NSEG, SEG, D), BF16),
        in_specs=[hbm] * 10,
        out_specs=hbm,
        scratch_shapes=[
            pltpu.VMEM((NSEG + 2, SEG, D), BF16),
            pltpu.VMEM((NSEG * 4, D), U32),
            pltpu.VMEM((NSEG * LIVE, D), F32),
            pltpu.VMEM((S + SEG, D), F32),
            pltpu.VMEM((NPAIR + 1, D + 32, 128), U32),
            pltpu.VMEM((2 * NPAIR + 2, D // 2, 128), U32),
            pltpu.VMEM((NT, H * DH // 2, 128), U32),
            pltpu.VMEM((3 * H, NSEG * 8, DH), F32),
            pltpu.VMEM((FF, D), BF16),
            pltpu.VMEM((FF, D), BF16),
            pltpu.VMEM((FF, D), BF16),
            pltpu.VMEM((NSEG + 2, SEG, D), BF16),
            pltpu.VMEM((L, D), F32),
            pltpu.VMEM((L, D), F32),
            pltpu.VMEM((H, 2, 24, DH), F32),
            pltpu.VMEM((TOPC, D), F32),
            pltpu.VMEM((TOPC, D), F32),
            pltpu.VMEM((TOPC, D), F32),
            pltpu.VMEM((SEG, 128), F32),
            pltpu.VMEM((M, D), BF16),
            pltpu.VMEM((NT, 128), BF16),
            pltpu.SMEM((TOPC,), I32),
            pltpu.SemaphoreType.DMA((18,)),
            pltpu.SemaphoreType.DMA((1,)),
        ],
        compiler_params=pltpu.CompilerParams(vmem_limit_bytes=110 * 1024 * 1024),
    )(
        A_x.reshape(NSEG, SEG, D),
        A_mem0.reshape(M, D),
        A_Wq, A_Wk, A_Wv,
        A_Wo.reshape(H * DH, D),
        B_w_r.reshape(NT, 128),
        B_w_gate.T, B_w_up.T, B_w_down,
    )
    return out.reshape(1, S, D)
```

```python
import math

import jax
import jax.numpy as jnp
import jax.experimental.pallas as pl
import jax.experimental.pallas.tpu as pltpu

F32 = jnp.float32
BF16 = jnp.bfloat16
U32 = jnp.uint32
I32 = jnp.int32

S = 2048
D = 640
H = 32
DH = 128
M = 8
SEG = 32
NSEG = S // SEG
L = M + SEG
FF = 1728
TOPC = 8
NT = D // 128
LIVE = SEG - 8
EPS = 1e-05
NEG = -1000000000.0
LOG2E = math.log2(math.e)
NPAIR = 3 * H // 2
KEY_NONE = -1e30

UNROLL = 8
GH = 2
LS, LP = 1, 2
TL, TP = 2, (3, 5)
ORD = (0, 1, 3, 4, 5, 2)
HS = 24
TAIL = ((0, 'sp'), (2, 'p'))
FINE = (1, 32)
TIE0 = 2
LNT = (7, 13, 17, 22, 26, 31, 37, 42)
LNS = (0, 2, 7, 13, 17, 22, 26, 31)
LG = 1
NCH, NPREP, JPT = 1, 3, 2
MS0, MS1 = 8, 130


def _dot(a, b):
    return jax.lax.dot_general(a, b, (((1,), (0,)), ((), ())), preferred_element_type=F32)


def _dot_nt(a, b):
    return jax.lax.dot_general(a, b, (((1,), (1,)), ((), ())), preferred_element_type=F32)


def _rb(x):
    return x.astype(BF16).astype(F32)


def _sigmoid(x):
    return pl.reciprocal(1.0 + jnp.exp(-x), approx=True)


def _kernel(x_hbm, mem0_hbm, wq_hbm, wk_hbm, wv_hbm, wo_hbm, wr_hbm, wg_hbm, wu_hbm, wd_hbm,
            out_hbm,
            x_v, lhs_v, xs_v, xa_v, xb_v, raw, w_p, wo_p, pre, wg_v, wu_v, wd_v,
            out_v, t_v, acc, part_v, kv_s, sel, upd, yacc, keys, mem0_v, wr_v, idx_s,
            sem_in, sem_out):
    w_hbm = [wq_hbm, wk_hbm, wv_hbm]

    def wtile(j):
        return w_p.at[j]

    SEM_X8, SEM_B0, SEM_LN, SEM_TK, SEM_WO, SEM_MLP = 0, 4, 7, 15, 16, 17

    def w_start(q0, n, sem):
        for q in range(q0, q0 + n):
            src = w_hbm[q // 16].bitcast(U32).at[:, q % 16, :]
            pltpu.make_async_copy(src, raw.at[q, pl.ds(0, D), :], sem_in.at[sem]).start()

    def w_wait(q0, n, sem):
        blk = raw.at[pl.ds(q0, n), pl.ds(0, D), :]
        pltpu.make_async_copy(blk, blk, sem_in.at[sem]).wait()

    def x8_copy(b):
        return pltpu.make_async_copy(x_hbm.at[pl.ds(b * 16, 16), pl.ds(LIVE, 8), :],
                                     x_v.at[pl.ds(1 + b * 16, 16), pl.ds(LIVE, 8), :], sem_in.at[SEM_X8 + b])

    def xa_copy(i):
        return pltpu.make_async_copy(x_hbm.at[pl.ds(i * 8, 8), pl.ds(0, LIVE), :],
                                     x_v.at[pl.ds(1 + i * 8, 8), pl.ds(0, LIVE), :], sem_in.at[SEM_LN + i])

    cp_wr = pltpu.make_async_copy(wr_hbm, wr_v, sem_in.at[SEM_B0 + 2])
    cp_mem = pltpu.make_async_copy(mem0_hbm, mem0_v, sem_in.at[SEM_TK])
    FP = FF // 3

    def mlp_copies(t):
        f0 = t * FP if isinstance(t, int) else pl.multiple_of(t * FP, 16)
        return [pltpu.make_async_copy(s_.at[pl.ds(f0, FP), :], d_.at[pl.ds(f0, FP), :], sem_in.at[SEM_MLP + t])
                for s_, d_ in [(wg_hbm, wg_v), (wu_hbm, wu_v), (wd_hbm, wd_v)]]

    wo32 = wo_hbm.bitcast(U32)
    wo_copies = [pltpu.make_async_copy(wo32.at[:, pl.ds(j * 128, 128)], wo_p.at[j], sem_in.at[SEM_WO])
                 for j in range(NT)]

    for b in range(4):
        x8_copy(b).start()
    w_start(0, 1, SEM_B0)
    w_start(1, 1, SEM_B0 + 1)
    w_start(2, 2, SEM_B0 + 2)
    cp_wr.start()
    for i in range(8):
        w_start(4 + 4 * i, 4, SEM_LN + i)
        xa_copy(i).start()
    w_start(36, NPAIR - 36, SEM_TK)
    cp_mem.start()
    for t in range(3):
        for c in mlp_copies(t):
            c.start()
    for c in wo_copies:
        c.start()

    xb3 = xb_v.reshape(NSEG + 1, SEG, D)
    x_v[0] = jnp.zeros((SEG, D), BF16)
    xb3[0] = jnp.zeros((SEG, D), F32)
    keys[...] = jnp.full(keys.shape, KEY_NONE, F32)
    yacc[...] = jnp.zeros(yacc.shape, F32)
    kv_s[:, :, 0:8, :] = jnp.zeros((H, 2, 8, DH), F32)
    raw[NPAIR, 0:D, :] = jnp.zeros((D, 128), U32)
    acc[M:L, :] = jnp.zeros((SEG, D), F32)

    def router_w():
        wr5 = wr_v[...].astype(F32)
        return jnp.concatenate([wr5[j:j + 1, :] for j in range(NT)], axis=1)

    def layernorm(s0, nseg, t0, nrow, gate=None):
        n = nseg * nrow
        x = x_v[pl.ds(1 + s0, nseg), t0:t0 + nrow, :].astype(F32).reshape(n, D)
        if gate is not None:
            gv = jnp.concatenate([pltpu.bitcast(gate[1], F32)] * (n // 8), axis=0)
            x = jnp.concatenate([jnp.where(gate[0], gv, x[:, 0:128]), x[:, 128:]], axis=1)
        mu = jnp.sum(x, axis=-1, keepdims=True) * (1.0 / D)
        xc = x - mu
        var = jnp.sum(xc * xc, axis=-1, keepdims=True) * (1.0 / D)
        sd = _rb(jnp.sqrt(_rb(_rb(var) + EPS)))
        xn = _rb(_rb(x - _rb(mu)) / sd)
        xb3[pl.ds(1 + s0, nseg), t0:t0 + nrow, :] = xn.reshape(nseg, nrow, D)
        return xn

    def ln8_body(b, carry):
        x8_copy(b).wait()
        xn = layernorm(b * 16, 16, LIVE, 8)
        lhs_v[pl.ds(pl.multiple_of(b * 64, 64), 64), :] = pltpu.bitcast(xn.astype(BF16), U32)
        return carry

    jax.lax.fori_loop(0, 4, ln8_body, 0)

    def ln_seg(s, wr, gate):
        tail = xb3[1 + s, LIVE:SEG, :]
        xn = layernorm(s, 1, 0, LIVE, gate)
        xa_v[pl.ds(pl.multiple_of(s * LIVE, 8), LIVE), :] = xn
        r = _rb(jnp.sum(jnp.concatenate([xn, tail], axis=0) * wr, axis=-1, keepdims=True))
        r = jnp.where(r == 0.0, 0.0, r)
        bits = pltpu.bitcast(jnp.broadcast_to(r, (SEG, 128)), I32) >> 16
        mono = jnp.where(bits < 0, (-32768) - bits, bits)
        mono = jnp.where(r != r, -40000, mono)
        row = jax.lax.broadcasted_iota(I32, (SEG, 128), 0)
        key = (mono * SEG + ((SEG - 1) - row)).astype(F32)
        lane = jax.lax.broadcasted_iota(I32, (SEG, 128), 1)
        keys[...] = jnp.where(lane == s, key, keys[...])
        return pltpu.bitcast(key, U32)

    def top_rows():
        kv = keys[...]
        lane = jax.lax.broadcasted_iota(I32, (1, 128), 1).astype(F32)
        for c in range(TOPC):
            col = jnp.max(kv, axis=0, keepdims=True)
            val = jnp.floor(col * (1.0 / SEG))
            fk = val * 128.0 + (127.0 - lane)
            win = fk == jnp.max(fk, axis=1, keepdims=True)
            kv = jnp.where(win & (kv == col), KEY_NONE, kv)
            pos = lane * SEG + ((SEG - 1.0) - (col - val * SEG))
            idx = jnp.clip(jnp.max(jnp.where(win, pos, 0.0)).astype(I32), 0, S - 1)
            idx_s[c] = idx
            sel[pl.ds(c, 1), :] = xb_v[pl.ds(SEG + idx, 1), :]

    def repack(rv, wv, p, part=None, tie=None):
        m_lo = jnp.full((8, 128), 0xFFFF, U32)
        m_hi = jnp.full((8, 128), 0xFFFF0000, U32)
        if tie is not None:
            m_lo = jnp.where(tie[0], tie[1], m_lo)
            m_hi = jnp.where(tie[0], tie[1], m_hi)
        for g in range(D // 16):
            if part is not None and g % part[1] != part[0]:
                continue
            a = rv[p, pl.ds(16 * g, 8, stride=2), :]
            b = rv[p, pl.ds(16 * g + 1, 8, stride=2), :]
            wv[2 * p, 8 * g:8 * g + 8, :] = (a & m_lo) | (b << 16)
            wv[2 * p + 1, 8 * g:8 * g + 8, :] = (a >> 16) | (b & m_hi)

    def pack(x):
        return pltpu.bitcast(x.astype(BF16), U32)

    HR = 256 // NCH

    def xsums(k, tie=None):
        c, o = divmod(k * 16, HR)
        s1 = 1 + (2 * c * HR + o) // 8
        s2 = s1 + HR // 8
        x1 = xb3[s1:s1 + 2, LIVE:SEG, 0:512].reshape(16, 512)
        x2 = xb3[s2:s2 + 2, LIVE:SEG, 0:512].reshape(16, 512)
        if tie is not None:
            x1 = jnp.where(tie[0], tie[1], x1)
            x2 = jnp.where(tie[0], tie[1], x2)
        a11, a12, a21, a22 = x1[:, :256], x1[:, 256:], x2[:, :256], x2[:, 256:]
        for n_, y in enumerate((a11 + a22, a21 + a22, a11 + a12, a21 - a11, a12 - a22)):
            xs_v[n_, 8 * k:8 * k + 8, :] = pack(y)

    def block(q0, n, never=None):
        for u in range(2 * q0, 2 * q0 + 2 * n):
            if u % 2 == 0:
                repack(raw, w_p, u // 2 + 1)
            for c in range(4):
                r = _dot(pltpu.bitcast(lhs_v[c * 64:(c + 1) * 64, :], BF16), pltpu.bitcast(w_p[u], BF16))
                pre[u, c * 128:(c + 1) * 128, :] = r
                k = 4 * (u - 2 * q0) + c
                if never is not None and k < 8:
                    tv = jnp.concatenate([r[0:16, :]] * 4, axis=1)
                    xsums(2 * k, (never, tv))
                    xsums(2 * k + 1, (never, tv))

    def sblock(q0, n, never, side=None, jobs=None):
        rv = raw.at[pl.ds(q0, n + 1)]
        wv = w_p.at[pl.ds(2 * q0, 2 * n + 2)]
        pv = pre.at[pl.ds(2 * q0, 2 * n)]
        cnt = [0]
        pend = []

        def mm(a, b, acc_=None):
            k = cnt[0]
            cnt[0] += 1
            if side is not None and k in LNS:
                pend.append(side(LNS.index(k), None if last[0] is None or not LG else (never, last[0])))
            if side is not None and k in LNT:
                tok = pend.pop(0)
                head = jnp.where(never, tok, a[0:SEG, 0:128])
                if a.shape[1] > 128:
                    head = jnp.concatenate([head, a[0:SEG, 128:]], axis=1)
                a = head if a.shape[0] == SEG else jnp.concatenate([head, a[SEG:, :]], axis=0)
            if not jobs:
                r = _dot(pltpu.bitcast(a, BF16), b)
                return r if acc_ is None else acc_ + r
            for kt in range(a.shape[1] // 128):
                r = _dot(pltpu.bitcast(a[:, kt * 128:(kt + 1) * 128], BF16), b[kt * 128:(kt + 1) * 128, :])
                acc_ = r if acc_ is None else acc_ + r
                for _ in range(JPT):
                    if jobs:
                        jobs.pop(0)()
            return acc_

        last = [None]

        def gated(x):
            return x if last[0] is None else jnp.where(never, last[0], x)

        hp = HR // 2
        tails = {}
        for p in range(n):
            def wsum(t1, t2, sub=False):
                msk = jnp.concatenate([gated(jnp.full((8, 128), 0xFFFF0000, U32))] * 32, axis=0)
                sh = jnp.concatenate([gated(jnp.full((8, 128), 16, U32))] * 32, axis=0)

                def half(k, hi):
                    r = rv[p, 256 * k:256 * k + 256, :]
                    return pltpu.bitcast(r & msk if hi else r << sh, F32)
                a_, b_ = half(*t1), half(*t2)
                return (a_ - b_ if sub else a_ + b_).astype(BF16)

            def wt(pp, j, k0, k1):
                return pltpu.bitcast(wv[2 * pp + j, 64 * k0:64 * k1, :], BF16)

            def mark(k, r):
                last[0] = pltpu.bitcast(r[0:8, :], U32)
                if k < NPREP:
                    repack(rv, wv, p + 1, (k, NPREP), (never, last[0]))

            top5, bot5 = lhs_v[0:hp, 512:640], lhs_v[hp:2 * hp, 512:640]
            m2 = mm(xs_v[1], wt(p, 0, 0, 2))
            m5 = mm(xs_v[2], wt(p, 1, 2, 4))
            s4, s3 = wsum((1, 0), (0, 0), True), wsum((0, 1), (1, 1), True)
            mark(0, m2)
            m4 = mm(lhs_v[hp:2 * hp, 256:512], s4)
            m3 = mm(lhs_v[0:hp, 0:256], s3)
            s1 = wsum((0, 0), (1, 1))
            mark(1, m4)
            c21, c12 = m2 + m4, m3 + m5
            if p in tails:
                pv[2 * p, HR:2 * HR, :] = c21 + tails[p][0]
                pv[2 * p + 1, 0:HR, :] = c12 + tails[p][1]
            m1 = mm(xs_v[0], s1)
            c11 = mm(top5, wt(p, 0, 4, 5), (m4 - m5) + m1)
            c22 = mm(bot5, wt(p, 1, 4, 5), (m3 - m2) + m1)
            s7, s6 = wsum((1, 0), (1, 1)), wsum((0, 0), (0, 1))
            mark(2, m1)
            c11 = mm(xs_v[4], s7, c11)
            pv[2 * p, 0:HR, :] = c11
            pv[2 * p + 1, HR:2 * HR, :] = mm(xs_v[3], s6, c22)
            mark(3, c11)
            if p not in tails:
                pv[2 * p, HR:2 * HR, :] = mm(bot5, wt(p, 0, 4, 5), c21)
                pv[2 * p + 1, 0:HR, :] = mm(top5, wt(p, 1, 4, 5), c12)
                if p + 1 < n:
                    t_v[0] = mm(bot5, wt(p + 1, 0, 4, 5))
                    t_v[1] = mm(top5, wt(p + 1, 1, 4, 5))
                    tails[p + 1] = (t_v[0], t_v[1])

    idx_s[0] = 0
    w_wait(0, 1, SEM_B0)
    repack(raw, w_p, 0)
    w_wait(1, 1, SEM_B0 + 1)
    block(0, 1)
    w_wait(2, 2, SEM_B0 + 2)
    cp_wr.wait()
    block(1, 2, idx_s[0] < 0)

    def ln_body(i, carry):
        w_wait(4 + 4 * i, 4, SEM_LN + i)
        xa_copy(i).wait()
        wr = router_w()
        sblock(3 + 4 * i, 4, i < 0, side=lambda u, gate: ln_seg(i * 8 + u, wr, gate))
        return carry

    jax.lax.fori_loop(0, 8, ln_body, 0)

    w_wait(36, NPAIR - 36, SEM_TK)
    cp_mem.wait()
    acc[0:M, :] = mem0_v[...].astype(F32)
    nv = idx_s[0] < 0
    top_rows()
    sblock(35, 1, nv)


    def mlp_body(t, carry):
        for c in mlp_copies(t):
            c.wait()
        f0 = pl.multiple_of(t * FP, 16)
        xs = sel[...]
        cuts = [(a_, min(a_ + 128, FP)) for a_ in range(0, FP, 128)]
        val = {}

        def up_tile(which, n, kt):
            def run():
                a_, b_ = cuts[n]
                w = (wg_v, wu_v)[which][pl.ds(f0 + a_, b_ - a_), kt * 128:(kt + 1) * 128]
                r = _dot_nt(xs[:, kt * 128:(kt + 1) * 128], w)
                val[which, n] = r if kt == 0 else val[which, n] + r
            return run

        def down_tile(n, j):
            def run():
                a_, b_ = cuts[n]
                if j == 0:
                    g_ = _rb(val.pop((0, n)))
                    val['h', n] = _rb(g_ * _sigmoid(g_)) * _rb(val.pop((1, n)))
                r = _dot(val['h', n], wd_v[pl.ds(f0 + a_, b_ - a_), j * 128:(j + 1) * 128])
                val['y', j] = r if n == 0 else val['y', j] + r
            return run

        def skip():
            pass

        real = ([up_tile(which, n, kt) for n in range(len(cuts)) for which in range(2) for kt in range(NT)]
                + [down_tile(n, j) for n in range(len(cuts)) for j in range(NT)])
        jobs = [skip] * MS1
        for n_, job in enumerate(real):
            jobs[MS0 + (n_ * (MS1 - MS0)) // len(real)] = job
        sblock(36 + 4 * t, 4, t < 0, jobs=jobs)
        assert not jobs
        y = yacc[...] + jnp.concatenate([val['y', j] for j in range(NT)], axis=1)
        yacc[...] = y
        r_sel = _rb(jnp.sum(xs * router_w(), axis=-1, keepdims=True))
        upd[...] = xs + _rb(_rb(y) * _rb(_sigmoid(r_sel)))
        for c in range(TOPC):
            xb_v[pl.ds(SEG + jnp.clip(idx_s[c], 0, S - 1), 1), :] = upd[pl.ds(c, 1), :]
        return carry

    jax.lax.fori_loop(0, 3, mlp_body, 0)

    for c in wo_copies:
        c.wait()

    scale = DH ** (-0.5)
    qm_i = jax.lax.broadcasted_iota(I32, (L - 8, L), 0)
    mask_m = (qm_i < M) | (qm_i + 8 >= jax.lax.broadcasted_iota(I32, (L - 8, L), 1))
    diag_ok = (jax.lax.broadcasted_iota(I32, (7, 8, DH), 1)
               > jax.lax.broadcasted_iota(I32, (7, 8, DH), 0))

    def finish(s0, n, u, sa):
        xb = xb3.at[pl.ds(s0, n)][u]
        o = x_v.at[pl.ds(s0, n)][u].astype(F32) + sa * (xb * _sigmoid(xb))
        out_v.at[pl.ds(s0, n)][u] = o.astype(BF16)
        return o

    def out_copy(seg, n):
        return pltpu.make_async_copy(out_v.at[pl.ds(seg + 1, n)], out_hbm.at[pl.ds(seg, n)], sem_out.at[0])

    def step(i, u, prev):
        pre_i = pre.at[:, pl.ds(pl.multiple_of(i * (8 * UNROLL), 8 * UNROLL), 8 * UNROLL), :]
        xa_i = xa_v.at[pl.ds(pl.multiple_of(i * (LIVE * UNROLL), 8 * UNROLL), LIVE * UNROLL), :]
        pre_s = pre_i.at[:, pl.ds(pl.multiple_of(u * 8, 8), 8), :]
        xa = xa_i[pl.ds(pl.multiple_of(u * LIVE, 8), LIVE), :]
        lhs = jnp.concatenate([prev[0:M, :], xa], axis=0).astype(BF16)
        fin = finish(pl.multiple_of(i * UNROLL, UNROLL), UNROLL, u, prev[M:L, :])

        @pl.when(u == UNROLL - 2)
        def _():
            out_copy(i * UNROLL, UNROLL - 2).start()

        def proj(j, tie=None):
            lh = lhs
            if tie is not None:
                top = pltpu.bitcast(lhs[0:16, 0:128], U32)
                top = pltpu.bitcast(jnp.where(i < 0, pltpu.bitcast(tie, U32), top), BF16)
                lh = jnp.concatenate([jnp.concatenate([top, lhs[0:16, 128:]], axis=1), lhs[16:, :]], axis=0)
            t = _dot(lh, pltpu.bitcast(wtile(j)[...], BF16))
            if TIE0 <= j < TIE0 + NT:
                t = jnp.where(jnp.logical_and(i < 0, u == 0),
                              fin[:, (j - TIE0) * 128:(j - TIE0 + 1) * 128], t)
            return jnp.concatenate([t, pre_s[j]], axis=0)

        NG = H // GH
        qs, ks, vs, ps, os_, ox, iv, on = {}, {}, {}, {}, {}, {}, {}, {}

        def do_qkv(g):
            js = [(x % 3) * H + g * GH + x // 3 for x in ORD]
            if g == 0:
                part = {}
                for kt in range(NT):
                    for j in js:
                        t = _dot(lhs[:, kt * 128:(kt + 1) * 128],
                                 pltpu.bitcast(wtile(j)[kt * 64:(kt + 1) * 64, :], BF16))
                        part[j] = t if kt == 0 else part[j] + t
                res = {j: jnp.concatenate([part[j], pre_s[j]], axis=0) for j in js}
            else:
                res = {}
                for n, j in enumerate(js):
                    tie = None
                    for hh, pos in enumerate(TP):
                        if n == pos and g >= TL:
                            tie = ox[(g - TL) * GH + hh]
                    res[j] = proj(j, tie)
            for h in range(g * GH, (g + 1) * GH):
                qs[h], ks[h], vs[h] = res[h], res[H + h], res[2 * H + h]

        def vpu_rows(h, q, k, v):
            def win(which, val, r):
                if r % 8 == 0:
                    return val[8 - r:16 - r, :]
                return kv_s[h, which, 16 - r:24 - r, :]

            def wins(which, val):
                return jnp.stack([win(which, val, r) for r in range(16)])

            def fold(f, x):
                while x.shape[0] > 1:
                    n = x.shape[0] // 2
                    x = f(x[:n], x[n:])
                return x[0]

            qa = q[8:16, :] * (scale * LOG2E)
            sc = jnp.sum(qa[None] * wins(0, k), axis=-1, keepdims=True)
            sc = jnp.broadcast_to(sc, (16, 8, DH))
            sc = jnp.concatenate([sc[:9], jnp.where(diag_ok, sc[9:], -jnp.inf)], axis=0)
            e = jnp.exp2(sc - fold(jnp.maximum, sc)[None])
            return fold(jnp.add, e * wins(1, v)) * pl.reciprocal(fold(jnp.add, e), approx=True)

        def do_s(g):
            for h in range(g * GH, (g + 1) * GH):
                q, k = qs.pop(h), ks.pop(h)
                kv_s[h, 0, 8:24, :] = k[0:16, :]
                kv_s[h, 1, 8:24, :] = vs[h][0:16, :]
                ox[h] = vpu_rows(h, q, k, vs[h])
                qm = jnp.concatenate([q[0:8, :], q[16:, :]], axis=0)
                sc = _dot_nt(qm.astype(BF16), k.astype(BF16))
                sc = jnp.where(mask_m, sc * (scale * LOG2E), NEG * LOG2E)
                e = jnp.exp2(sc - jnp.max(sc, axis=-1, keepdims=True))
                inv = pl.reciprocal(jnp.sum(e, axis=-1, keepdims=True), approx=True)
                ps[h] = e.astype(BF16)
                iv[h] = jnp.broadcast_to(inv, (SEG, DH))

        def do_pv(g):
            for h in range(g * GH, (g + 1) * GH):
                v = vs.pop(h)
                if g >= NG - TL:
                    v = jnp.concatenate([jnp.where(i < 0, ox[h], v[0:8, :]), v[8:, :]], axis=0)
                if h >= GH:
                    v = jnp.concatenate([v[0:8, :], jnp.where(i < 0, on[h - GH], v[8:, :])], axis=0)
                on[h] = _dot(ps.pop(h), v.astype(BF16)) * iv.pop(h)
                os_[h] = jnp.concatenate([on[h][0:8, :], ox[h], on[h][8:, :]], axis=0)

        def do_o(j, h0, h1):
            o = jnp.concatenate([os_[h] for h in range(h0, h1)], axis=1)
            return _dot(o, pltpu.bitcast(wo_p[j, h0 * 64:h1 * 64, :], BF16))

        for g in range(NG):
            do_qkv(g)
            if g >= LS:
                do_s(g - LS)
            if g >= LP:
                do_pv(g - LP)
        sched = dict(TAIL)
        ns, npv = NG - LS, NG - LP
        for j in range(NT):
            part_v[:, j * 128:(j + 1) * 128] = do_o(j, 0, HS)
            for c_ in sched.get(j, ''):
                if c_ == 's':
                    do_s(ns)
                    ns += 1
                else:
                    do_pv(npv)
                    npv += 1
        assert ns == NG and npv == NG
        return jnp.concatenate(
            [part_v[:, j * 128:(j + 1) * 128] + do_o(j, HS, H) for j in range(NT)], axis=1)

    def multi(i, carry):
        acc[...] = jax.lax.fori_loop(0, UNROLL, lambda u, cur: step(i, u, cur), acc[...],
                                     unroll=True)
        out_copy(i * UNROLL + UNROLL - 2, 1).start()

        @pl.when(i > 0)
        def _():
            out_copy(jnp.maximum(i * UNROLL - 1, 0), 1).start()
        return carry

    jax.lax.fori_loop(0, NSEG // UNROLL, multi, 0)
    finish(NSEG, 1, 0, acc[M:L, :])
    out_copy(NSEG - 1, 1).start()
    out_copy(0, NSEG).wait()


@jax.jit
def pallas_recurrent_scan__memory_aug_recurrent_mem_tr__moe_arch_mod__prompt_kernel(
    A_x: jax.Array,
    A_mem0: jax.Array,
    A_Wq: jax.Array,
    A_Wk: jax.Array,
    A_Wv: jax.Array,
    A_Wo: jax.Array,
    A_seg_len: jax.Array,
    B_x: jax.Array,
    B_w_r: jax.Array,
    B_w_gate: jax.Array,
    B_w_up: jax.Array,
    B_w_down: jax.Array,
):
    del A_seg_len, B_x
    assert A_x.shape == (1, S, D) and A_Wq.shape == (D, H, DH) and A_mem0.shape == (1, M, D)
    hbm = pl.BlockSpec(memory_space=pltpu.HBM)
    out = pl.pallas_call(
        _kernel,
        out_shape=jax.ShapeDtypeStruct((NSEG, SEG, D), BF16),
        in_specs=[hbm] * 10,
        out_specs=hbm,
        scratch_shapes=[
            pltpu.VMEM((NSEG + 2, SEG, D), BF16),
            pltpu.VMEM((NSEG * 4, D), U32),
            pltpu.VMEM((5, 128, 256), U32),
            pltpu.VMEM((NSEG * LIVE, D), F32),
            pltpu.VMEM((S + SEG, D), F32),
            pltpu.VMEM((NPAIR + 1, D + 32, 128), U32),
            pltpu.VMEM((2 * NPAIR + 2, D // 2, 128), U32),
            pltpu.VMEM((NT, H * DH // 2, 128), U32),
            pltpu.VMEM((3 * H, NSEG * 8, DH), F32),
            pltpu.VMEM((FF, D), BF16),
            pltpu.VMEM((FF, D), BF16),
            pltpu.VMEM((FF, D), BF16),
            pltpu.VMEM((NSEG + 2, SEG, D), BF16),
            pltpu.VMEM((2, 256, DH), F32),
            pltpu.VMEM((L, D), F32),
            pltpu.VMEM((L, D), F32),
            pltpu.VMEM((H, 2, 24, DH), F32),
            pltpu.VMEM((TOPC, D), F32),
            pltpu.VMEM((TOPC, D), F32),
            pltpu.VMEM((TOPC, D), F32),
            pltpu.VMEM((SEG, 128), F32),
            pltpu.VMEM((M, D), BF16),
            pltpu.VMEM((NT, 128), BF16),
            pltpu.SMEM((TOPC,), I32),
            pltpu.SemaphoreType.DMA((20,)),
            pltpu.SemaphoreType.DMA((1,)),
        ],
        compiler_params=pltpu.CompilerParams(vmem_limit_bytes=110 * 1024 * 1024),
    )(
        A_x.reshape(NSEG, SEG, D),
        A_mem0.reshape(M, D),
        A_Wq, A_Wk, A_Wv,
        A_Wo.reshape(H * DH, D),
        B_w_r.reshape(NT, 128),
        B_w_gate.T, B_w_up.T, B_w_down,
    )
    return out.reshape(1, S, D)
```

```python
import math

import jax
import jax.numpy as jnp
import jax.experimental.pallas as pl
import jax.experimental.pallas.tpu as pltpu

F32 = jnp.float32
BF16 = jnp.bfloat16
U32 = jnp.uint32
I32 = jnp.int32

S = 2048
D = 640
H = 32
DH = 128
M = 8
SEG = 32
NSEG = S // SEG
L = M + SEG
FF = 1728
TOPC = 8
NT = D // 128
LIVE = SEG - 8
EPS = 1e-05
NEG = -1000000000.0
LOG2E = math.log2(math.e)
NPAIR = 3 * H // 2
KEY_NONE = -1e30

UNROLL = 8
GH = 2
LS, LP = 1, 2
TL, TP = 2, (3, 5)
ORD = (0, 1, 3, 4, 5, 2)
HS = 24
TAIL = ((0, 'sp'), (2, 'p'))
FINE = (1, 32)
TIE0 = 2
LNT = (7, 13, 17, 22, 26, 31, 37, 42)
LNS = (0, 2, 7, 13, 17, 22, 26, 31)
LG = 1
NCH, NPREP, JPT = 1, 3, 2
JR = (4,) * 13 + (8, 8, 8, 0, 0)
NG8, GST, GREV = 8, 4, 0


def _dot(a, b):
    return jax.lax.dot_general(a, b, (((1,), (0,)), ((), ())), preferred_element_type=F32)


def _dot_nt(a, b):
    return jax.lax.dot_general(a, b, (((1,), (1,)), ((), ())), preferred_element_type=F32)


def _rb(x):
    return x.astype(BF16).astype(F32)


def _sigmoid(x):
    return pl.reciprocal(1.0 + jnp.exp(-x), approx=True)


def _kernel(x_hbm, mem0_hbm, wq_hbm, wk_hbm, wv_hbm, wo_hbm, wr_hbm, wg_hbm, wu_hbm, wd_hbm,
            out_hbm,
            x_v, lhs_v, xs_v, xa_v, xb_v, raw, w_p, wo_p, pre, wg_v, wu_v, wd_v,
            out_v, t_v, acc, part_v, kv_s, sel, upd, yacc, keys, mem0_v, wr_v, idx_s,
            sem_in, sem_out):
    w_hbm = [wq_hbm, wk_hbm, wv_hbm]

    def wtile(j):
        return w_p.at[j]

    SEM_X8, SEM_B0, SEM_LN, SEM_TK, SEM_WO, SEM_MLP = 0, 4, 7, 15, 16, 17

    def w_start(q0, n, sem):
        for q in range(q0, q0 + n):
            src = w_hbm[q // 16].bitcast(U32).at[:, q % 16, :]
            pltpu.make_async_copy(src, raw.at[q, pl.ds(0, D), :], sem_in.at[sem]).start()

    def w_wait(q0, n, sem):
        blk = raw.at[pl.ds(q0, n), pl.ds(0, D), :]
        pltpu.make_async_copy(blk, blk, sem_in.at[sem]).wait()

    def x8_copy(b):
        return pltpu.make_async_copy(x_hbm.at[pl.ds(b * 16, 16), pl.ds(LIVE, 8), :],
                                     x_v.at[pl.ds(1 + b * 16, 16), pl.ds(LIVE, 8), :], sem_in.at[SEM_X8 + b])

    def xa_copy(i):
        return pltpu.make_async_copy(x_hbm.at[pl.ds(i * 8, 8), pl.ds(0, LIVE), :],
                                     x_v.at[pl.ds(1 + i * 8, 8), pl.ds(0, LIVE), :], sem_in.at[SEM_LN + i])

    cp_wr = pltpu.make_async_copy(wr_hbm, wr_v, sem_in.at[SEM_B0 + 2])
    cp_mem = pltpu.make_async_copy(mem0_hbm, mem0_v, sem_in.at[SEM_TK])
    FP = FF // 3

    def mlp_copies(t):
        f0 = t * FP if isinstance(t, int) else pl.multiple_of(t * FP, 16)
        return [pltpu.make_async_copy(s_.at[pl.ds(f0, FP), :], d_.at[pl.ds(f0, FP), :], sem_in.at[SEM_MLP + t])
                for s_, d_ in [(wg_hbm, wg_v), (wu_hbm, wu_v), (wd_hbm, wd_v)]]

    wo_copies = [pltpu.make_async_copy(wo_hbm.bitcast(U32), wo_p, sem_in.at[SEM_WO])]

    for b in range(4):
        x8_copy(b).start()
    w_start(0, 1, SEM_B0)
    w_start(1, 1, SEM_B0 + 1)
    w_start(2, 2, SEM_B0 + 2)
    cp_wr.start()
    for i in range(8):
        w_start(4 + 4 * i, 4, SEM_LN + i)
        xa_copy(i).start()
    w_start(36, NPAIR - 36, SEM_TK)
    cp_mem.start()
    for t in range(3):
        for c in mlp_copies(t):
            c.start()
    for c in wo_copies:
        c.start()

    xb3 = xb_v.reshape(NSEG + 1, SEG, D)
    x_v[0] = jnp.zeros((SEG, D), BF16)
    xb3[0] = jnp.zeros((SEG, D), F32)
    keys[...] = jnp.full(keys.shape, KEY_NONE, F32)
    yacc[...] = jnp.zeros(yacc.shape, F32)
    kv_s[:, :, 0:8, :] = jnp.zeros((H, 2, 8, DH), F32)
    raw[NPAIR, 0:D, :] = jnp.zeros((D, 128), U32)
    acc[M:L, :] = jnp.zeros((SEG, D), F32)

    def router_w():
        wr5 = wr_v[...].astype(F32)
        return jnp.concatenate([wr5[j:j + 1, :] for j in range(NT)], axis=1)

    def layernorm(s0, nseg, t0, nrow, gate=None):
        n = nseg * nrow
        x = x_v[pl.ds(1 + s0, nseg), t0:t0 + nrow, :].astype(F32).reshape(n, D)
        if gate is not None:
            gv = jnp.concatenate([pltpu.bitcast(gate[1], F32)] * (n // 8), axis=0)
            x = jnp.concatenate([jnp.where(gate[0], gv, x[:, 0:128]), x[:, 128:]], axis=1)
        mu = jnp.sum(x, axis=-1, keepdims=True) * (1.0 / D)
        xc = x - mu
        var = jnp.sum(xc * xc, axis=-1, keepdims=True) * (1.0 / D)
        sd = _rb(jnp.sqrt(_rb(_rb(var) + EPS)))
        xn = _rb(_rb(x - _rb(mu)) / sd)
        xb3[pl.ds(1 + s0, nseg), t0:t0 + nrow, :] = xn.reshape(nseg, nrow, D)
        return xn

    def ln8_body(b, carry):
        x8_copy(b).wait()
        xn = layernorm(b * 16, 16, LIVE, 8)
        lhs_v[pl.ds(pl.multiple_of(b * 64, 64), 64), :] = pltpu.bitcast(xn.astype(BF16), U32)
        return carry

    jax.lax.fori_loop(0, 4, ln8_body, 0)

    def ln_seg(s, wr, gate):
        tail = xb3[1 + s, LIVE:SEG, :]
        xn = layernorm(s, 1, 0, LIVE, gate)
        xa_v[pl.ds(pl.multiple_of(s * LIVE, 8), LIVE), :] = xn
        r = _rb(jnp.sum(jnp.concatenate([xn, tail], axis=0) * wr, axis=-1, keepdims=True))
        r = jnp.where(r == 0.0, 0.0, r)
        bits = pltpu.bitcast(jnp.broadcast_to(r, (SEG, 128)), I32) >> 16
        mono = jnp.where(bits < 0, (-32768) - bits, bits)
        mono = jnp.where(r != r, -40000, mono)
        row = jax.lax.broadcasted_iota(I32, (SEG, 128), 0)
        key = (mono * SEG + ((SEG - 1) - row)).astype(F32)
        lane = jax.lax.broadcasted_iota(I32, (SEG, 128), 1)
        keys[...] = jnp.where(lane == s, key, keys[...])
        return pltpu.bitcast(key, U32)

    def top_rows():
        kv = keys[...]
        lane = jax.lax.broadcasted_iota(I32, (1, 128), 1).astype(F32)
        for c in range(TOPC):
            col = jnp.max(kv, axis=0, keepdims=True)
            val = jnp.floor(col * (1.0 / SEG))
            fk = val * 128.0 + (127.0 - lane)
            win = fk == jnp.max(fk, axis=1, keepdims=True)
            kv = jnp.where(win & (kv == col), KEY_NONE, kv)
            pos = lane * SEG + ((SEG - 1.0) - (col - val * SEG))
            idx = jnp.clip(jnp.max(jnp.where(win, pos, 0.0)).astype(I32), 0, S - 1)
            idx_s[c] = idx
            sel[pl.ds(c, 1), :] = xb_v[pl.ds(SEG + idx, 1), :]

    def repack(rv, wv, p, part=None, tie=None):
        m_lo = jnp.full((8, 128), 0xFFFF, U32)
        m_hi = jnp.full((8, 128), 0xFFFF0000, U32)
        if tie is not None:
            m_lo = jnp.where(tie[0], tie[1], m_lo)
            m_hi = jnp.where(tie[0], tie[1], m_hi)
        for g in range(D // 16):
            if part is not None and g % part[1] != part[0]:
                continue
            a = rv[p, pl.ds(16 * g, 8, stride=2), :]
            b = rv[p, pl.ds(16 * g + 1, 8, stride=2), :]
            wv[2 * p, 8 * g:8 * g + 8, :] = (a & m_lo) | (b << 16)
            wv[2 * p + 1, 8 * g:8 * g + 8, :] = (a >> 16) | (b & m_hi)

    def pack(x):
        return pltpu.bitcast(x.astype(BF16), U32)

    HR = 256 // NCH

    def xsums(k, tie=None):
        c, o = divmod(k * 16, HR)
        s1 = 1 + (2 * c * HR + o) // 8
        s2 = s1 + HR // 8
        x1 = xb3[s1:s1 + 2, LIVE:SEG, 0:512].reshape(16, 512)
        x2 = xb3[s2:s2 + 2, LIVE:SEG, 0:512].reshape(16, 512)
        if tie is not None:
            x1 = jnp.where(tie[0], tie[1], x1)
            x2 = jnp.where(tie[0], tie[1], x2)
        a11, a12, a21, a22 = x1[:, :256], x1[:, 256:], x2[:, :256], x2[:, 256:]
        for n_, y in enumerate((a11 + a22, a21 + a22, a11 + a12, a21 - a11, a12 - a22)):
            xs_v[n_, 8 * k:8 * k + 8, :] = pack(y)

    def block(q0, n, never=None):
        for u in range(2 * q0, 2 * q0 + 2 * n):
            if u % 2 == 0:
                repack(raw, w_p, u // 2 + 1)
            for c in range(4):
                r = _dot(pltpu.bitcast(lhs_v[c * 64:(c + 1) * 64, :], BF16), pltpu.bitcast(w_p[u], BF16))
                pre[u, c * 128:(c + 1) * 128, :] = r
                k = 4 * (u - 2 * q0) + c
                if never is not None and k < 8:
                    tv = jnp.concatenate([r[0:16, :]] * 4, axis=1)
                    xsums(2 * k, (never, tv))
                    xsums(2 * k + 1, (never, tv))

    def sblock(q0, n, never, side=None, jobs=None):
        rv = raw.at[pl.ds(q0, n + 1)]
        wv = w_p.at[pl.ds(2 * q0, 2 * n + 2)]
        pv = pre.at[pl.ds(2 * q0, 2 * n)]
        cnt = [0]
        pend = []
        tiles = [0]

        def mm(a, b, acc_=None):
            k = cnt[0]
            cnt[0] += 1
            if side is not None and k in LNS:
                pend.append(side(LNS.index(k), None if last[0] is None or not LG else (never, last[0])))
            if side is not None and k in LNT:
                tok = pend.pop(0)
                head = jnp.where(never, tok, a[0:SEG, 0:128])
                if a.shape[1] > 128:
                    head = jnp.concatenate([head, a[0:SEG, 128:]], axis=1)
                a = head if a.shape[0] == SEG else jnp.concatenate([head, a[SEG:, :]], axis=0)
            r = _dot(pltpu.bitcast(a, BF16), b)
            r = r if acc_ is None else acc_ + r
            tiles[0] += a.shape[1] // 128
            if jobs and tiles[0] % 4 == 0:
                for _ in range(JR[tiles[0] // 4 - 1]):
                    if jobs:
                        jobs.pop(0)()
            return r

        last = [None]

        def gated(x, z):
            if last[0] is None:
                return x
            r0 = 8 * ((GREV - z if GREV else z) * GST)
            return jnp.where(never, pltpu.bitcast(lastr[0][r0:r0 + 8, :], U32), x)

        lastr = [None]
        hp = HR // 2
        tails = {}
        for p in range(n):
            def wsum(t1, t2, sub=False):
                msk = jnp.concatenate([gated(jnp.full((8, 128), 0xFFFF0000, U32), z)
                                       for z in range(NG8) for _ in range(32 // NG8)], axis=0)
                sh = jnp.concatenate([gated(jnp.full((8, 128), 16, U32), z)
                                      for z in range(NG8) for _ in range(32 // NG8)], axis=0)

                def half(k, hi):
                    r = rv[p, 256 * k:256 * k + 256, :]
                    return pltpu.bitcast(r & msk if hi else r << sh, F32)
                a_, b_ = half(*t1), half(*t2)
                return (a_ - b_ if sub else a_ + b_).astype(BF16)

            def wt(pp, j, k0, k1):
                return pltpu.bitcast(wv[2 * pp + j, 64 * k0:64 * k1, :], BF16)

            def mark(k, r):
                last[0] = pltpu.bitcast(r[0:8, :], U32)
                lastr[0] = r
                if k < NPREP:
                    repack(rv, wv, p + 1, (k, NPREP), (never, last[0]))

            top5, bot5 = lhs_v[0:hp, 512:640], lhs_v[hp:2 * hp, 512:640]
            m2 = mm(xs_v[1], wt(p, 0, 0, 2))
            m5 = mm(xs_v[2], wt(p, 1, 2, 4))
            s4, s3 = wsum((1, 0), (0, 0), True), wsum((0, 1), (1, 1), True)
            mark(0, m2)
            m4 = mm(lhs_v[hp:2 * hp, 256:512], s4)
            m3 = mm(lhs_v[0:hp, 0:256], s3)
            s1 = wsum((0, 0), (1, 1))
            mark(1, m4)
            c21, c12 = m2 + m4, m3 + m5
            if p in tails:
                pv[2 * p, HR:2 * HR, :] = c21 + tails[p][0]
                pv[2 * p + 1, 0:HR, :] = c12 + tails[p][1]
            m1 = mm(xs_v[0], s1)
            c11 = mm(top5, wt(p, 0, 4, 5), (m4 - m5) + m1)
            c22 = mm(bot5, wt(p, 1, 4, 5), (m3 - m2) + m1)
            s7, s6 = wsum((1, 0), (1, 1)), wsum((0, 0), (0, 1))
            mark(2, m1)
            c11 = mm(xs_v[4], s7, c11)
            pv[2 * p, 0:HR, :] = c11
            pv[2 * p + 1, HR:2 * HR, :] = mm(xs_v[3], s6, c22)
            mark(3, c11)
            if p not in tails:
                pv[2 * p, HR:2 * HR, :] = mm(bot5, wt(p, 0, 4, 5), c21)
                pv[2 * p + 1, 0:HR, :] = mm(top5, wt(p, 1, 4, 5), c12)
                if p + 1 < n:
                    t_v[0] = mm(bot5, wt(p + 1, 0, 4, 5))
                    t_v[1] = mm(top5, wt(p + 1, 1, 4, 5))
                    tails[p + 1] = (t_v[0], t_v[1])

    idx_s[0] = 0
    w_wait(0, 1, SEM_B0)
    repack(raw, w_p, 0)
    w_wait(1, 1, SEM_B0 + 1)
    block(0, 1)
    w_wait(2, 2, SEM_B0 + 2)
    cp_wr.wait()
    block(1, 2, idx_s[0] < 0)

    def ln_body(i, carry):
        w_wait(4 + 4 * i, 4, SEM_LN + i)
        xa_copy(i).wait()
        wr = router_w()
        sblock(3 + 4 * i, 4, i < 0, side=lambda u, gate: ln_seg(i * 8 + u, wr, gate))
        return carry

    jax.lax.fori_loop(0, 8, ln_body, 0)

    w_wait(36, NPAIR - 36, SEM_TK)
    cp_mem.wait()
    acc[0:M, :] = mem0_v[...].astype(F32)
    nv = idx_s[0] < 0
    top_rows()
    sblock(35, 1, nv)


    def mlp_body(t, carry):
        for c in mlp_copies(t):
            c.wait()
        f0 = pl.multiple_of(t * FP, 16)
        xs = sel[...]
        cuts = [(a_, min(a_ + 128, FP)) for a_ in range(0, FP, 128)]
        val = {}

        def up_tile(which, n, kt):
            def run():
                a_, b_ = cuts[n]
                w = (wg_v, wu_v)[which][pl.ds(f0 + a_, b_ - a_), kt * 128:(kt + 1) * 128]
                r = _dot_nt(xs[:, kt * 128:(kt + 1) * 128], w)
                val[which, n] = r if kt == 0 else val[which, n] + r
            return run

        def down_tile(n, j):
            def run():
                a_, b_ = cuts[n]
                if j == 0:
                    g_ = _rb(val.pop((0, n)))
                    val['h', n] = _rb(g_ * _sigmoid(g_)) * _rb(val.pop((1, n)))
                r = _dot(val['h', n], wd_v[pl.ds(f0 + a_, b_ - a_), j * 128:(j + 1) * 128])
                val['y', j] = r if n == 0 else val['y', j] + r
            return run

        jobs = ([up_tile(which, n, kt) for n in range(len(cuts)) for which in range(2) for kt in range(NT)]
                + [down_tile(n, j) for n in range(len(cuts)) for j in range(NT)])
        sblock(36 + 4 * t, 4, t < 0, jobs=jobs)
        assert not jobs
        y = yacc[...] + jnp.concatenate([val['y', j] for j in range(NT)], axis=1)
        yacc[...] = y
        r_sel = _rb(jnp.sum(xs * router_w(), axis=-1, keepdims=True))
        upd[...] = xs + _rb(_rb(y) * _rb(_sigmoid(r_sel)))
        for c in range(TOPC):
            xb_v[pl.ds(SEG + jnp.clip(idx_s[c], 0, S - 1), 1), :] = upd[pl.ds(c, 1), :]
        return carry

    jax.lax.fori_loop(0, 3, mlp_body, 0)

    for c in wo_copies:
        c.wait()

    scale = DH ** (-0.5)
    qm_i = jax.lax.broadcasted_iota(I32, (L - 8, L), 0)
    mask_m = (qm_i < M) | (qm_i + 8 >= jax.lax.broadcasted_iota(I32, (L - 8, L), 1))
    diag_ok = (jax.lax.broadcasted_iota(I32, (7, 8, DH), 1)
               > jax.lax.broadcasted_iota(I32, (7, 8, DH), 0))

    def finish(s0, n, u, sa):
        xb = xb3.at[pl.ds(s0, n)][u]
        o = x_v.at[pl.ds(s0, n)][u].astype(F32) + sa * (xb * _sigmoid(xb))
        out_v.at[pl.ds(s0, n)][u] = o.astype(BF16)
        return o

    def out_copy(seg, n):
        return pltpu.make_async_copy(out_v.at[pl.ds(seg + 1, n)], out_hbm.at[pl.ds(seg, n)], sem_out.at[0])

    def step(i, u, prev):
        pre_i = pre.at[:, pl.ds(pl.multiple_of(i * (8 * UNROLL), 8 * UNROLL), 8 * UNROLL), :]
        xa_i = xa_v.at[pl.ds(pl.multiple_of(i * (LIVE * UNROLL), 8 * UNROLL), LIVE * UNROLL), :]
        pre_s = pre_i.at[:, pl.ds(pl.multiple_of(u * 8, 8), 8), :]
        xa = xa_i[pl.ds(pl.multiple_of(u * LIVE, 8), LIVE), :]
        lhs = jnp.concatenate([prev[0:M, :], xa], axis=0).astype(BF16)
        fin = finish(pl.multiple_of(i * UNROLL, UNROLL), UNROLL, u, prev[M:L, :])

        @pl.when(u == UNROLL - 2)
        def _():
            out_copy(i * UNROLL, UNROLL - 2).start()

        def proj(j, tie=None):
            lh = lhs
            if tie is not None:
                top = pltpu.bitcast(lhs[0:16, 0:128], U32)
                top = pltpu.bitcast(jnp.where(i < 0, pltpu.bitcast(tie, U32), top), BF16)
                lh = jnp.concatenate([jnp.concatenate([top, lhs[0:16, 128:]], axis=1), lhs[16:, :]], axis=0)
            t = _dot(lh, pltpu.bitcast(wtile(j)[...], BF16))
            if TIE0 <= j < TIE0 + NT:
                t = jnp.where(jnp.logical_and(i < 0, u == 0),
                              fin[:, (j - TIE0) * 128:(j - TIE0 + 1) * 128], t)
            return jnp.concatenate([t, pre_s[j]], axis=0)

        NG = H // GH
        qs, ks, vs, ps, os_, ox, iv, on = {}, {}, {}, {}, {}, {}, {}, {}

        def do_qkv(g):
            js = [(x % 3) * H + g * GH + x // 3 for x in ORD]
            if g == 0:
                part = {}
                for kt in range(NT):
                    for j in js:
                        t = _dot(lhs[:, kt * 128:(kt + 1) * 128],
                                 pltpu.bitcast(wtile(j)[kt * 64:(kt + 1) * 64, :], BF16))
                        part[j] = t if kt == 0 else part[j] + t
                res = {j: jnp.concatenate([part[j], pre_s[j]], axis=0) for j in js}
            else:
                res = {}
                for n, j in enumerate(js):
                    tie = None
                    for hh, pos in enumerate(TP):
                        if n == pos and g >= TL:
                            tie = ox[(g - TL) * GH + hh]
                    res[j] = proj(j, tie)
            for h in range(g * GH, (g + 1) * GH):
                qs[h], ks[h], vs[h] = res[h], res[H + h], res[2 * H + h]

        def vpu_rows(h, q, k, v):
            def win(which, val, r):
                if r % 8 == 0:
                    return val[8 - r:16 - r, :]
                return kv_s[h, which, 16 - r:24 - r, :]

            def wins(which, val):
                return jnp.stack([win(which, val, r) for r in range(16)])

            def fold(f, x):
                while x.shape[0] > 1:
                    n = x.shape[0] // 2
                    x = f(x[:n], x[n:])
                return x[0]

            qa = q[8:16, :] * (scale * LOG2E)
            sc = jnp.sum(qa[None] * wins(0, k), axis=-1, keepdims=True)
            sc = jnp.broadcast_to(sc, (16, 8, DH))
            sc = jnp.concatenate([sc[:9], jnp.where(diag_ok, sc[9:], -jnp.inf)], axis=0)
            e = jnp.exp2(sc - fold(jnp.maximum, sc)[None])
            return fold(jnp.add, e * wins(1, v)) * pl.reciprocal(fold(jnp.add, e), approx=True)

        def do_s(g):
            for h in range(g * GH, (g + 1) * GH):
                q, k = qs.pop(h), ks.pop(h)
                kv_s[h, 0, 8:24, :] = k[0:16, :]
                kv_s[h, 1, 8:24, :] = vs[h][0:16, :]
                ox[h] = vpu_rows(h, q, k, vs[h])
                qm = jnp.concatenate([q[0:8, :], q[16:, :]], axis=0)
                sc = _dot_nt(qm.astype(BF16), k.astype(BF16))
                sc = jnp.where(mask_m, sc * (scale * LOG2E), NEG * LOG2E)
                e = jnp.exp2(sc - jnp.max(sc, axis=-1, keepdims=True))
                inv = pl.reciprocal(jnp.sum(e, axis=-1, keepdims=True), approx=True)
                ps[h] = e.astype(BF16)
                iv[h] = jnp.broadcast_to(inv, (SEG, DH))

        def do_pv(g):
            for h in range(g * GH, (g + 1) * GH):
                v = vs.pop(h)
                if g >= NG - TL:
                    v = jnp.concatenate([jnp.where(i < 0, ox[h], v[0:8, :]), v[8:, :]], axis=0)
                if h >= GH:
                    v = jnp.concatenate([v[0:8, :], jnp.where(i < 0, on[h - GH], v[8:, :])], axis=0)
                on[h] = _dot(ps.pop(h), v.astype(BF16)) * iv.pop(h)
                os_[h] = jnp.concatenate([on[h][0:8, :], ox[h], on[h][8:, :]], axis=0)

        def do_o(j, h0, h1):
            o = jnp.concatenate([os_[h] for h in range(h0, h1)], axis=1)
            return _dot(o, pltpu.bitcast(wo_p[h0 * 64:h1 * 64, j * 128:(j + 1) * 128], BF16))

        for g in range(NG):
            do_qkv(g)
            if g >= LS:
                do_s(g - LS)
            if g >= LP:
                do_pv(g - LP)
        sched = dict(TAIL)
        ns, npv = NG - LS, NG - LP
        for j in range(NT):
            part_v[:, j * 128:(j + 1) * 128] = do_o(j, 0, HS)
            for c_ in sched.get(j, ''):
                if c_ == 's':
                    do_s(ns)
                    ns += 1
                else:
                    do_pv(npv)
                    npv += 1
        assert ns == NG and npv == NG
        return jnp.concatenate(
            [part_v[:, j * 128:(j + 1) * 128] + do_o(j, HS, H) for j in range(NT)], axis=1)

    def multi(i, carry):
        acc[...] = jax.lax.fori_loop(0, UNROLL, lambda u, cur: step(i, u, cur), acc[...],
                                     unroll=True)
        out_copy(i * UNROLL + UNROLL - 2, 1).start()

        @pl.when(i > 0)
        def _():
            out_copy(jnp.maximum(i * UNROLL - 1, 0), 1).start()
        return carry

    jax.lax.fori_loop(0, NSEG // UNROLL, multi, 0)
    finish(NSEG, 1, 0, acc[M:L, :])
    out_copy(NSEG - 1, 1).start()
    out_copy(0, NSEG).wait()


@jax.jit
def pallas_recurrent_scan__memory_aug_recurrent_mem_tr__moe_arch_mod__prompt_kernel(
    A_x: jax.Array,
    A_mem0: jax.Array,
    A_Wq: jax.Array,
    A_Wk: jax.Array,
    A_Wv: jax.Array,
    A_Wo: jax.Array,
    A_seg_len: jax.Array,
    B_x: jax.Array,
    B_w_r: jax.Array,
    B_w_gate: jax.Array,
    B_w_up: jax.Array,
    B_w_down: jax.Array,
):
    del A_seg_len, B_x
    assert A_x.shape == (1, S, D) and A_Wq.shape == (D, H, DH) and A_mem0.shape == (1, M, D)
    hbm = pl.BlockSpec(memory_space=pltpu.HBM)
    out = pl.pallas_call(
        _kernel,
        out_shape=jax.ShapeDtypeStruct((NSEG, SEG, D), BF16),
        in_specs=[hbm] * 10,
        out_specs=hbm,
        scratch_shapes=[
            pltpu.VMEM((NSEG + 2, SEG, D), BF16),
            pltpu.VMEM((NSEG * 4, D), U32),
            pltpu.VMEM((5, 128, 256), U32),
            pltpu.VMEM((NSEG * LIVE, D), F32),
            pltpu.VMEM((S + SEG, D), F32),
            pltpu.VMEM((NPAIR + 1, D + 32, 128), U32),
            pltpu.VMEM((2 * NPAIR + 2, D // 2, 128), U32),
            pltpu.VMEM((H * DH // 2, D), U32),
            pltpu.VMEM((3 * H, NSEG * 8, DH), F32),
            pltpu.VMEM((FF, D), BF16),
            pltpu.VMEM((FF, D), BF16),
            pltpu.VMEM((FF, D), BF16),
            pltpu.VMEM((NSEG + 2, SEG, D), BF16),
            pltpu.VMEM((2, 256, DH), F32),
            pltpu.VMEM((L, D), F32),
            pltpu.VMEM((L, D), F32),
            pltpu.VMEM((H, 2, 24, DH), F32),
            pltpu.VMEM((TOPC, D), F32),
            pltpu.VMEM((TOPC, D), F32),
            pltpu.VMEM((TOPC, D), F32),
            pltpu.VMEM((SEG, 128), F32),
            pltpu.VMEM((M, D), BF16),
            pltpu.VMEM((NT, 128), BF16),
            pltpu.SMEM((TOPC,), I32),
            pltpu.SemaphoreType.DMA((20,)),
            pltpu.SemaphoreType.DMA((1,)),
        ],
        compiler_params=pltpu.CompilerParams(vmem_limit_bytes=110 * 1024 * 1024),
    )(
        A_x.reshape(NSEG, SEG, D),
        A_mem0.reshape(M, D),
        A_Wq, A_Wk, A_Wv,
        A_Wo.reshape(H * DH, D),
        B_w_r.reshape(NT, 128),
        B_w_gate.T, B_w_up.T, B_w_down,
    )
    return out.reshape(1, S, D)
```

```python
import math

import jax
import jax.numpy as jnp
import jax.experimental.pallas as pl
import jax.experimental.pallas.tpu as pltpu

F32 = jnp.float32
BF16 = jnp.bfloat16
U32 = jnp.uint32
I32 = jnp.int32

S = 2048
D = 640
H = 32
DH = 128
M = 8
SEG = 32
NSEG = S // SEG
L = M + SEG
FF = 1728
TOPC = 8
NT = D // 128
LIVE = SEG - 8
EPS = 1e-05
NEG = -1000000000.0
LOG2E = math.log2(math.e)
NPAIR = 3 * H // 2
KEY_NONE = -1e30

UNROLL = 8
GH = 2
LS, LP = 1, 2
TL, TP = 2, (3, 5)
ORD = (0, 1, 3, 4, 5, 2)
HS = 24
TAIL = ((0, 'sp'), (2, 'p'))
FINE = (1, 32)
TIE0 = 2
LNT = (7, 13, 17, 22, 26, 31, 37, 42)
LNS = (0, 2, 7, 13, 17, 22, 26, 31)
LG = 1
NCH, NPREP, JPT = 1, 3, 2
JR = (4,) * 11 + (6,) + (4,) * 5 + (0,)
NG8, GST, GREV = 8, 4, 0


def _dot(a, b):
    return jax.lax.dot_general(a, b, (((1,), (0,)), ((), ())), preferred_element_type=F32)


def _dot_nt(a, b):
    return jax.lax.dot_general(a, b, (((1,), (1,)), ((), ())), preferred_element_type=F32)


def _rb(x):
    return x.astype(BF16).astype(F32)


def _sigmoid(x):
    return pl.reciprocal(1.0 + jnp.exp(-x), approx=True)


def _kernel(x_hbm, mem0_hbm, wq_hbm, wk_hbm, wv_hbm, wo_hbm, wr_hbm, wg_hbm, wu_hbm, wd_hbm,
            out_hbm,
            x_v, lhs_v, xs_v, xa_v, xb_v, raw, w_p, wo_p, pre, wg_v, wu_v, wd_v,
            out_v, t_v, acc, part_v, kv_s, sel, upd, yacc, keys, mem0_v, wr_v, idx_s,
            sem_in, sem_out):
    w_hbm = [wq_hbm, wk_hbm, wv_hbm]

    def wtile(j):
        return w_p.at[j]

    SEM_X8, SEM_B0, SEM_LN, SEM_TK, SEM_WO, SEM_MLP = 0, 4, 7, 15, 16, 17

    def w_start(q0, n, sem):
        for q in range(q0, q0 + n):
            src = w_hbm[q // 16].bitcast(U32).at[:, q % 16, :]
            pltpu.make_async_copy(src, raw.at[q, pl.ds(0, D), :], sem_in.at[sem]).start()

    def w_wait(q0, n, sem):
        blk = raw.at[pl.ds(q0, n), pl.ds(0, D), :]
        pltpu.make_async_copy(blk, blk, sem_in.at[sem]).wait()

    def x8_copy(b):
        return pltpu.make_async_copy(x_hbm.at[pl.ds(b * 16, 16), pl.ds(LIVE, 8), :],
                                     x_v.at[pl.ds(1 + b * 16, 16), pl.ds(LIVE, 8), :], sem_in.at[SEM_X8 + b])

    def xa_copy(i):
        return pltpu.make_async_copy(x_hbm.at[pl.ds(i * 8, 8), pl.ds(0, LIVE), :],
                                     x_v.at[pl.ds(1 + i * 8, 8), pl.ds(0, LIVE), :], sem_in.at[SEM_LN + i])

    cp_wr = pltpu.make_async_copy(wr_hbm, wr_v, sem_in.at[SEM_B0 + 2])
    cp_mem = pltpu.make_async_copy(mem0_hbm, mem0_v, sem_in.at[SEM_TK])
    FP = FF // 3

    def mlp_copies(t):
        f0 = t * FP if isinstance(t, int) else pl.multiple_of(t * FP, 16)
        return [pltpu.make_async_copy(s_.at[pl.ds(f0, FP), :], d_.at[pl.ds(f0, FP), :], sem_in.at[SEM_MLP + t])
                for s_, d_ in [(wg_hbm, wg_v), (wu_hbm, wu_v), (wd_hbm, wd_v)]]

    wo_copies = [pltpu.make_async_copy(wo_hbm.bitcast(U32), wo_p, sem_in.at[SEM_WO])]

    for b in range(4):
        x8_copy(b).start()
    w_start(0, 1, SEM_B0)
    w_start(1, 1, SEM_B0 + 1)
    w_start(2, 2, SEM_B0 + 2)
    cp_wr.start()
    for i in range(8):
        w_start(4 + 4 * i, 4, SEM_LN + i)
        xa_copy(i).start()
    w_start(36, NPAIR - 36, SEM_TK)
    cp_mem.start()
    for t in range(3):
        for c in mlp_copies(t):
            c.start()
    for c in wo_copies:
        c.start()

    xb3 = xb_v.reshape(NSEG + 1, SEG, D)
    x_v[0] = jnp.zeros((SEG, D), BF16)
    xb3[0] = jnp.zeros((SEG, D), F32)
    keys[...] = jnp.full(keys.shape, KEY_NONE, F32)
    yacc[...] = jnp.zeros(yacc.shape, F32)
    kv_s[:, :, 0:8, :] = jnp.zeros((H, 2, 8, DH), F32)
    raw[NPAIR, 0:D, :] = jnp.zeros((D, 128), U32)
    acc[M:L, :] = jnp.zeros((SEG, D), F32)

    def router_w():
        wr5 = wr_v[...].astype(F32)
        return jnp.concatenate([wr5[j:j + 1, :] for j in range(NT)], axis=1)

    def layernorm(s0, nseg, t0, nrow, gate=None):
        n = nseg * nrow
        x = x_v[pl.ds(1 + s0, nseg), t0:t0 + nrow, :].astype(F32).reshape(n, D)
        if gate is not None:
            gv = jnp.concatenate([pltpu.bitcast(gate[1], F32)] * (n // 8), axis=0)
            x = jnp.concatenate([jnp.where(gate[0], gv, x[:, 0:128]), x[:, 128:]], axis=1)
        mu = jnp.sum(x, axis=-1, keepdims=True) * (1.0 / D)
        xc = x - mu
        var = jnp.sum(xc * xc, axis=-1, keepdims=True) * (1.0 / D)
        sd = _rb(jnp.sqrt(_rb(_rb(var) + EPS)))
        xn = _rb(_rb(x - _rb(mu)) / sd)
        xb3[pl.ds(1 + s0, nseg), t0:t0 + nrow, :] = xn.reshape(nseg, nrow, D)
        return xn

    def ln8_body(b, carry):
        x8_copy(b).wait()
        xn = layernorm(b * 16, 16, LIVE, 8)
        lhs_v[pl.ds(pl.multiple_of(b * 64, 64), 64), :] = pltpu.bitcast(xn.astype(BF16), U32)
        return carry

    jax.lax.fori_loop(0, 4, ln8_body, 0)

    def ln_seg(s, wr, gate):
        tail = xb3[1 + s, LIVE:SEG, :]
        xn = layernorm(s, 1, 0, LIVE, gate)
        xa_v[pl.ds(pl.multiple_of(s * LIVE, 8), LIVE), :] = xn
        r = _rb(jnp.sum(jnp.concatenate([xn, tail], axis=0) * wr, axis=-1, keepdims=True))
        r = jnp.where(r == 0.0, 0.0, r)
        bits = pltpu.bitcast(jnp.broadcast_to(r, (SEG, 128)), I32) >> 16
        mono = jnp.where(bits < 0, (-32768) - bits, bits)
        mono = jnp.where(r != r, -40000, mono)
        row = jax.lax.broadcasted_iota(I32, (SEG, 128), 0)
        key = (mono * SEG + ((SEG - 1) - row)).astype(F32)
        lane = jax.lax.broadcasted_iota(I32, (SEG, 128), 1)
        keys[...] = jnp.where(lane == s, key, keys[...])
        return pltpu.bitcast(key, U32)

    def top_rows():
        kv = keys[...]
        lane = jax.lax.broadcasted_iota(I32, (1, 128), 1).astype(F32)
        for c in range(TOPC):
            col = jnp.max(kv, axis=0, keepdims=True)
            val = jnp.floor(col * (1.0 / SEG))
            fk = val * 128.0 + (127.0 - lane)
            win = fk == jnp.max(fk, axis=1, keepdims=True)
            kv = jnp.where(win & (kv == col), KEY_NONE, kv)
            pos = lane * SEG + ((SEG - 1.0) - (col - val * SEG))
            idx = jnp.clip(jnp.max(jnp.where(win, pos, 0.0)).astype(I32), 0, S - 1)
            idx_s[c] = idx
            sel[pl.ds(c, 1), :] = xb_v[pl.ds(SEG + idx, 1), :]

    def repack(rv, wv, p, part=None, tie=None):
        m_lo = jnp.full((8, 128), 0xFFFF, U32)
        m_hi = jnp.full((8, 128), 0xFFFF0000, U32)
        if tie is not None:
            m_lo = jnp.where(tie[0], tie[1], m_lo)
            m_hi = jnp.where(tie[0], tie[1], m_hi)
        for g in range(D // 16):
            if part is not None and g % part[1] != part[0]:
                continue
            a = rv[p, pl.ds(16 * g, 8, stride=2), :]
            b = rv[p, pl.ds(16 * g + 1, 8, stride=2), :]
            wv[2 * p, 8 * g:8 * g + 8, :] = (a & m_lo) | (b << 16)
            wv[2 * p + 1, 8 * g:8 * g + 8, :] = (a >> 16) | (b & m_hi)

    def pack(x):
        return pltpu.bitcast(x.astype(BF16), U32)

    HR = 256 // NCH

    def xsums(k, tie=None):
        c, o = divmod(k * 16, HR)
        s1 = 1 + (2 * c * HR + o) // 8
        s2 = s1 + HR // 8
        x1 = xb3[s1:s1 + 2, LIVE:SEG, 0:512].reshape(16, 512)
        x2 = xb3[s2:s2 + 2, LIVE:SEG, 0:512].reshape(16, 512)
        if tie is not None:
            x1 = jnp.where(tie[0], tie[1], x1)
            x2 = jnp.where(tie[0], tie[1], x2)
        a11, a12, a21, a22 = x1[:, :256], x1[:, 256:], x2[:, :256], x2[:, 256:]
        for n_, y in enumerate((a11 + a22, a21 + a22, a11 + a12, a21 - a11, a12 - a22)):
            xs_v[n_, 8 * k:8 * k + 8, :] = pack(y)

    def block(q0, n, never=None):
        for u in range(2 * q0, 2 * q0 + 2 * n):
            if u % 2 == 0:
                repack(raw, w_p, u // 2 + 1)
            for c in range(4):
                r = _dot(pltpu.bitcast(lhs_v[c * 64:(c + 1) * 64, :], BF16), pltpu.bitcast(w_p[u], BF16))
                pre[u, c * 128:(c + 1) * 128, :] = r
                k = 4 * (u - 2 * q0) + c
                if never is not None and k < 8:
                    tv = jnp.concatenate([r[0:16, :]] * 4, axis=1)
                    xsums(2 * k, (never, tv))
                    xsums(2 * k + 1, (never, tv))

    def sblock(q0, n, never, side=None, jobs=None):
        rv = raw.at[pl.ds(q0, n + 1)]
        wv = w_p.at[pl.ds(2 * q0, 2 * n + 2)]
        pv = pre.at[pl.ds(2 * q0, 2 * n)]
        cnt = [0]
        pend = []
        tiles = [0]

        def mm(a, b, acc_=None):
            k = cnt[0]
            cnt[0] += 1
            if side is not None and k in LNS:
                pend.append(side(LNS.index(k), None if last[0] is None or not LG else (never, last[0])))
            if side is not None and k in LNT:
                tok = pend.pop(0)
                head = jnp.where(never, tok, a[0:SEG, 0:128])
                if a.shape[1] > 128:
                    head = jnp.concatenate([head, a[0:SEG, 128:]], axis=1)
                a = head if a.shape[0] == SEG else jnp.concatenate([head, a[SEG:, :]], axis=0)
            r = _dot(pltpu.bitcast(a, BF16), b)
            r = r if acc_ is None else acc_ + r
            tiles[0] += a.shape[1] // 128
            if jobs and tiles[0] % 4 == 0:
                for _ in range(JR[tiles[0] // 4 - 1]):
                    if jobs:
                        jobs.pop(0)()
            return r

        last = [None]

        def gated(x, z):
            if last[0] is None:
                return x
            r0 = 8 * ((GREV - z if GREV else z) * GST)
            return jnp.where(never, pltpu.bitcast(lastr[0][r0:r0 + 8, :], U32), x)

        lastr = [None]
        hp = HR // 2
        tails = {}
        for p in range(n):
            def wsum(t1, t2, sub=False):
                msk = jnp.concatenate([gated(jnp.full((8, 128), 0xFFFF0000, U32), z)
                                       for z in range(NG8) for _ in range(32 // NG8)], axis=0)
                sh = jnp.concatenate([gated(jnp.full((8, 128), 16, U32), z)
                                      for z in range(NG8) for _ in range(32 // NG8)], axis=0)

                def half(k, hi):
                    r = rv[p, 256 * k:256 * k + 256, :]
                    return pltpu.bitcast(r & msk if hi else r << sh, F32)
                a_, b_ = half(*t1), half(*t2)
                return (a_ - b_ if sub else a_ + b_).astype(BF16)

            def wt(pp, j, k0, k1):
                return pltpu.bitcast(wv[2 * pp + j, 64 * k0:64 * k1, :], BF16)

            def mark(k, r):
                last[0] = pltpu.bitcast(r[0:8, :], U32)
                lastr[0] = r
                if k < NPREP:
                    repack(rv, wv, p + 1, (k, NPREP), (never, last[0]))

            top5, bot5 = lhs_v[0:hp, 512:640], lhs_v[hp:2 * hp, 512:640]
            m2 = mm(xs_v[1], wt(p, 0, 0, 2))
            m5 = mm(xs_v[2], wt(p, 1, 2, 4))
            s4, s3 = wsum((1, 0), (0, 0), True), wsum((0, 1), (1, 1), True)
            mark(0, m2)
            m4 = mm(lhs_v[hp:2 * hp, 256:512], s4)
            m3 = mm(lhs_v[0:hp, 0:256], s3)
            s1 = wsum((0, 0), (1, 1))
            mark(1, m4)
            c21, c12 = m2 + m4, m3 + m5
            if p in tails:
                pv[2 * p, HR:2 * HR, :] = c21 + tails[p][0]
                pv[2 * p + 1, 0:HR, :] = c12 + tails[p][1]
            m1 = mm(xs_v[0], s1)
            c11 = mm(top5, wt(p, 0, 4, 5), (m4 - m5) + m1)
            c22 = mm(bot5, wt(p, 1, 4, 5), (m3 - m2) + m1)
            s7, s6 = wsum((1, 0), (1, 1)), wsum((0, 0), (0, 1))
            mark(2, m1)
            c11 = mm(xs_v[4], s7, c11)
            pv[2 * p, 0:HR, :] = c11
            pv[2 * p + 1, HR:2 * HR, :] = mm(xs_v[3], s6, c22)
            mark(3, c11)
            if p not in tails:
                pv[2 * p, HR:2 * HR, :] = mm(bot5, wt(p, 0, 4, 5), c21)
                pv[2 * p + 1, 0:HR, :] = mm(top5, wt(p, 1, 4, 5), c12)
                if p + 1 < n:
                    t_v[0] = mm(bot5, wt(p + 1, 0, 4, 5))
                    t_v[1] = mm(top5, wt(p + 1, 1, 4, 5))
                    tails[p + 1] = (t_v[0], t_v[1])

    idx_s[0] = 0
    w_wait(0, 1, SEM_B0)
    repack(raw, w_p, 0)
    w_wait(1, 1, SEM_B0 + 1)
    block(0, 1)
    w_wait(2, 2, SEM_B0 + 2)
    cp_wr.wait()
    block(1, 2, idx_s[0] < 0)

    def ln_body(i, carry):
        w_wait(4 + 4 * i, 4, SEM_LN + i)
        xa_copy(i).wait()
        wr = router_w()
        sblock(3 + 4 * i, 4, i < 0, side=lambda u, gate: ln_seg(i * 8 + u, wr, gate))
        return carry

    jax.lax.fori_loop(0, 8, ln_body, 0)

    w_wait(36, NPAIR - 36, SEM_TK)
    cp_mem.wait()
    acc[0:M, :] = mem0_v[...].astype(F32)
    nv = idx_s[0] < 0
    top_rows()
    sblock(35, 1, nv)


    def mlp_body(t, carry):
        for c in mlp_copies(t):
            c.wait()
        f0 = pl.multiple_of(t * FP, 16)
        xs = sel[...]
        cuts = [(a_, min(a_ + 128, FP)) for a_ in range(0, FP, 128)]
        val = {}

        def up_tile(which, n, kt):
            def run():
                a_, b_ = cuts[n]
                ws = [w_[pl.ds(f0 + a_, b_ - a_), kt * 128:(kt + 1) * 128] for w_ in (wg_v, wu_v)]
                w = ws[which] if which < 2 else jnp.concatenate(ws, axis=0)
                r = _dot_nt(xs[:, kt * 128:(kt + 1) * 128], w)
                val[which, n] = r if kt == 0 else val[which, n] + r
            return run

        def down_tile(n, j, first):
            def run():
                a_, b_ = cuts[n]
                if j == 0:
                    if (2, n) in val:
                        both = val.pop((2, n))
                        val[0, n], val[1, n] = both[:, :b_ - a_], both[:, b_ - a_:]
                    g_ = _rb(val.pop((0, n)))
                    val['h', n] = _rb(g_ * _sigmoid(g_)) * _rb(val.pop((1, n)))
                r = _dot(val['h', n], wd_v[pl.ds(f0 + a_, b_ - a_), j * 128:(j + 1) * 128])
                val['y', j] = r if first else val['y', j] + r
            return run

        nc = len(cuts)
        jobs = ([up_tile(2, nc - 1, kt) for kt in range(NT)]
                + [up_tile(which, n, kt) for n in range(nc - 1) for which in range(2) for kt in range(NT)]
                + [down_tile(n, j, n == nc - 1) for n in [nc - 1] + list(range(nc - 1)) for j in range(NT)])
        sblock(36 + 4 * t, 4, t < 0, jobs=jobs)
        assert not jobs
        y = yacc[...] + jnp.concatenate([val['y', j] for j in range(NT)], axis=1)
        yacc[...] = y
        r_sel = _rb(jnp.sum(xs * router_w(), axis=-1, keepdims=True))
        upd[...] = xs + _rb(_rb(y) * _rb(_sigmoid(r_sel)))
        for c in range(TOPC):
            xb_v[pl.ds(SEG + jnp.clip(idx_s[c], 0, S - 1), 1), :] = upd[pl.ds(c, 1), :]
        return carry

    jax.lax.fori_loop(0, 3, mlp_body, 0)

    for c in wo_copies:
        c.wait()

    scale = DH ** (-0.5)
    qm_i = jax.lax.broadcasted_iota(I32, (L - 8, L), 0)
    mask_m = (qm_i < M) | (qm_i + 8 >= jax.lax.broadcasted_iota(I32, (L - 8, L), 1))
    diag_ok = (jax.lax.broadcasted_iota(I32, (7, 8, DH), 1)
               > jax.lax.broadcasted_iota(I32, (7, 8, DH), 0))

    def finish(s0, n, u, sa):
        xb = xb3.at[pl.ds(s0, n)][u]
        o = x_v.at[pl.ds(s0, n)][u].astype(F32) + sa * (xb * _sigmoid(xb))
        out_v.at[pl.ds(s0, n)][u] = o.astype(BF16)
        return o

    def out_copy(seg, n):
        return pltpu.make_async_copy(out_v.at[pl.ds(seg + 1, n)], out_hbm.at[pl.ds(seg, n)], sem_out.at[0])

    def step(i, u, prev):
        pre_i = pre.at[:, pl.ds(pl.multiple_of(i * (8 * UNROLL), 8 * UNROLL), 8 * UNROLL), :]
        xa_i = xa_v.at[pl.ds(pl.multiple_of(i * (LIVE * UNROLL), 8 * UNROLL), LIVE * UNROLL), :]
        pre_s = pre_i.at[:, pl.ds(pl.multiple_of(u * 8, 8), 8), :]
        xa = xa_i[pl.ds(pl.multiple_of(u * LIVE, 8), LIVE), :]
        lhs = jnp.concatenate([prev[0:M, :], xa], axis=0).astype(BF16)
        fin = finish(pl.multiple_of(i * UNROLL, UNROLL), UNROLL, u, prev[M:L, :])

        @pl.when(u == UNROLL - 2)
        def _():
            out_copy(i * UNROLL, UNROLL - 2).start()

        def proj(j, tie=None):
            lh = lhs
            if tie is not None:
                top = pltpu.bitcast(lhs[0:16, 0:128], U32)
                top = pltpu.bitcast(jnp.where(i < 0, pltpu.bitcast(tie, U32), top), BF16)
                lh = jnp.concatenate([jnp.concatenate([top, lhs[0:16, 128:]], axis=1), lhs[16:, :]], axis=0)
            t = _dot(lh, pltpu.bitcast(wtile(j)[...], BF16))
            if TIE0 <= j < TIE0 + NT:
                t = jnp.where(jnp.logical_and(i < 0, u == 0),
                              fin[:, (j - TIE0) * 128:(j - TIE0 + 1) * 128], t)
            return jnp.concatenate([t, pre_s[j]], axis=0)

        NG = H // GH
        qs, ks, vs, ps, os_, ox, iv, on = {}, {}, {}, {}, {}, {}, {}, {}

        def do_qkv(g):
            js = [(x % 3) * H + g * GH + x // 3 for x in ORD]
            if g == 0:
                part = {}
                for kt in range(NT):
                    for j in js:
                        t = _dot(lhs[:, kt * 128:(kt + 1) * 128],
                                 pltpu.bitcast(wtile(j)[kt * 64:(kt + 1) * 64, :], BF16))
                        part[j] = t if kt == 0 else part[j] + t
                res = {j: jnp.concatenate([part[j], pre_s[j]], axis=0) for j in js}
            else:
                res = {}
                for n, j in enumerate(js):
                    tie = None
                    for hh, pos in enumerate(TP):
                        if n == pos and g >= TL:
                            tie = ox[(g - TL) * GH + hh]
                    res[j] = proj(j, tie)
            for h in range(g * GH, (g + 1) * GH):
                qs[h], ks[h], vs[h] = res[h], res[H + h], res[2 * H + h]

        def vpu_rows(h, q, k, v):
            def win(which, val, r):
                if r % 8 == 0:
                    return val[8 - r:16 - r, :]
                return kv_s[h, which, 16 - r:24 - r, :]

            def wins(which, val):
                return jnp.stack([win(which, val, r) for r in range(16)])

            def fold(f, x):
                while x.shape[0] > 1:
                    n = x.shape[0] // 2
                    x = f(x[:n], x[n:])
                return x[0]

            qa = q[8:16, :] * (scale * LOG2E)
            sc = jnp.sum(qa[None] * wins(0, k), axis=-1, keepdims=True)
            sc = jnp.broadcast_to(sc, (16, 8, DH))
            sc = jnp.concatenate([sc[:9], jnp.where(diag_ok, sc[9:], -jnp.inf)], axis=0)
            e = jnp.exp2(sc - fold(jnp.maximum, sc)[None])
            return fold(jnp.add, e * wins(1, v)) * pl.reciprocal(fold(jnp.add, e), approx=True)

        def do_s(g):
            for h in range(g * GH, (g + 1) * GH):
                q, k = qs.pop(h), ks.pop(h)
                kv_s[h, 0, 8:24, :] = k[0:16, :]
                kv_s[h, 1, 8:24, :] = vs[h][0:16, :]
                ox[h] = vpu_rows(h, q, k, vs[h])
                qm = jnp.concatenate([q[0:8, :], q[16:, :]], axis=0)
                sc = _dot_nt(qm.astype(BF16), k.astype(BF16))
                sc = jnp.where(mask_m, sc * (scale * LOG2E), NEG * LOG2E)
                e = jnp.exp2(sc - jnp.max(sc, axis=-1, keepdims=True))
                inv = pl.reciprocal(jnp.sum(e, axis=-1, keepdims=True), approx=True)
                ps[h] = e.astype(BF16)
                iv[h] = jnp.broadcast_to(inv, (SEG, DH))

        def do_pv(g):
            for h in range(g * GH, (g + 1) * GH):
                v = vs.pop(h)
                if g >= NG - TL:
                    v = jnp.concatenate([jnp.where(i < 0, ox[h], v[0:8, :]), v[8:, :]], axis=0)
                if h >= GH:
                    v = jnp.concatenate([v[0:8, :], jnp.where(i < 0, on[h - GH], v[8:, :])], axis=0)
                on[h] = _dot(ps.pop(h), v.astype(BF16)) * iv.pop(h)
                os_[h] = jnp.concatenate([on[h][0:8, :], ox[h], on[h][8:, :]], axis=0)

        def do_o(j, h0, h1):
            o = jnp.concatenate([os_[h] for h in range(h0, h1)], axis=1)
            return _dot(o, pltpu.bitcast(wo_p[h0 * 64:h1 * 64, j * 128:(j + 1) * 128], BF16))

        for g in range(NG):
            do_qkv(g)
            if g >= LS:
                do_s(g - LS)
            if g >= LP:
                do_pv(g - LP)
        sched = dict(TAIL)
        ns, npv = NG - LS, NG - LP
        for j in range(NT):
            part_v[:, j * 128:(j + 1) * 128] = do_o(j, 0, HS)
            for c_ in sched.get(j, ''):
                if c_ == 's':
                    do_s(ns)
                    ns += 1
                else:
                    do_pv(npv)
                    npv += 1
        assert ns == NG and npv == NG
        return jnp.concatenate(
            [part_v[:, j * 128:(j + 1) * 128] + do_o(j, HS, H) for j in range(NT)], axis=1)

    def multi(i, carry):
        acc[...] = jax.lax.fori_loop(0, UNROLL, lambda u, cur: step(i, u, cur), acc[...],
                                     unroll=True)
        out_copy(i * UNROLL + UNROLL - 2, 1).start()

        @pl.when(i > 0)
        def _():
            out_copy(jnp.maximum(i * UNROLL - 1, 0), 1).start()
        return carry

    jax.lax.fori_loop(0, NSEG // UNROLL, multi, 0)
    finish(NSEG, 1, 0, acc[M:L, :])
    out_copy(NSEG - 1, 1).start()
    out_copy(0, NSEG).wait()


@jax.jit
def pallas_recurrent_scan__memory_aug_recurrent_mem_tr__moe_arch_mod__prompt_kernel(
    A_x: jax.Array,
    A_mem0: jax.Array,
    A_Wq: jax.Array,
    A_Wk: jax.Array,
    A_Wv: jax.Array,
    A_Wo: jax.Array,
    A_seg_len: jax.Array,
    B_x: jax.Array,
    B_w_r: jax.Array,
    B_w_gate: jax.Array,
    B_w_up: jax.Array,
    B_w_down: jax.Array,
):
    del A_seg_len, B_x
    assert A_x.shape == (1, S, D) and A_Wq.shape == (D, H, DH) and A_mem0.shape == (1, M, D)
    hbm = pl.BlockSpec(memory_space=pltpu.HBM)
    out = pl.pallas_call(
        _kernel,
        out_shape=jax.ShapeDtypeStruct((NSEG, SEG, D), BF16),
        in_specs=[hbm] * 10,
        out_specs=hbm,
        scratch_shapes=[
            pltpu.VMEM((NSEG + 2, SEG, D), BF16),
            pltpu.VMEM((NSEG * 4, D), U32),
            pltpu.VMEM((5, 128, 256), U32),
            pltpu.VMEM((NSEG * LIVE, D), F32),
            pltpu.VMEM((S + SEG, D), F32),
            pltpu.VMEM((NPAIR + 1, D + 32, 128), U32),
            pltpu.VMEM((2 * NPAIR + 2, D // 2, 128), U32),
            pltpu.VMEM((H * DH // 2, D), U32),
            pltpu.VMEM((3 * H, NSEG * 8, DH), F32),
            pltpu.VMEM((FF, D), BF16),
            pltpu.VMEM((FF, D), BF16),
            pltpu.VMEM((FF, D), BF16),
            pltpu.VMEM((NSEG + 2, SEG, D), BF16),
            pltpu.VMEM((2, 256, DH), F32),
            pltpu.VMEM((L, D), F32),
            pltpu.VMEM((L, D), F32),
            pltpu.VMEM((H, 2, 24, DH), F32),
            pltpu.VMEM((TOPC, D), F32),
            pltpu.VMEM((TOPC, D), F32),
            pltpu.VMEM((TOPC, D), F32),
            pltpu.VMEM((SEG, 128), F32),
            pltpu.VMEM((M, D), BF16),
            pltpu.VMEM((NT, 128), BF16),
            pltpu.SMEM((TOPC,), I32),
            pltpu.SemaphoreType.DMA((20,)),
            pltpu.SemaphoreType.DMA((1,)),
        ],
        compiler_params=pltpu.CompilerParams(vmem_limit_bytes=110 * 1024 * 1024),
    )(
        A_x.reshape(NSEG, SEG, D),
        A_mem0.reshape(M, D),
        A_Wq, A_Wk, A_Wv,
        A_Wo.reshape(H * DH, D),
        B_w_r.reshape(NT, 128),
        B_w_gate.T, B_w_up.T, B_w_down,
    )
    return out.reshape(1, S, D)
```

```python
import math

import jax
import jax.numpy as jnp
import jax.experimental.pallas as pl
import jax.experimental.pallas.tpu as pltpu

F32 = jnp.float32
BF16 = jnp.bfloat16
U32 = jnp.uint32
I32 = jnp.int32

S = 2048
D = 640
H = 32
DH = 128
M = 8
SEG = 32
NSEG = S // SEG
L = M + SEG
FF = 1728
TOPC = 8
NT = D // 128
LIVE = SEG - 8
EPS = 1e-05
NEG = -1000000000.0
LOG2E = math.log2(math.e)
NPAIR = 3 * H // 2
KEY_NONE = -1e30

UNROLL = 8
GH = 2
LS, LP = 1, 2
TL, TP = 2, (3, 5)
ORD = (0, 1, 3, 4, 2, 5)
HS = 24
TAIL = ((1, 'sp'), (3, 'p'))
TIE0 = 2
LNS = (0, 2, 7, 13, 17, 22, 26, 31)
LNT = (7, 13, 17, 22, 26, 31, 37, 42)
NPREP = 3
JR = (4,) * 11 + (6,) + (4,) * 5 + (0,)


def _dot(a, b):
    return jax.lax.dot_general(a, b, (((1,), (0,)), ((), ())), preferred_element_type=F32)


def _dot_nt(a, b):
    return jax.lax.dot_general(a, b, (((1,), (1,)), ((), ())), preferred_element_type=F32)


def _rb(x):
    return x.astype(BF16).astype(F32)


def _sigmoid(x):
    return pl.reciprocal(1.0 + jnp.exp(-x), approx=True)


def _kernel(x_hbm, mem0_hbm, wq_hbm, wk_hbm, wv_hbm, wo_hbm, wr_hbm, wg_hbm, wu_hbm, wd_hbm,
            out_hbm,
            x_v, lhs_v, xs_v, xa_v, xb_v, raw, w_p, wo_p, pre, wg_v, wu_v, wd_v,
            out_v, t_v, acc, part_v, kv_s, sel, upd, yacc, keys, mem0_v, wr_v, idx_s,
            sem_in, sem_out):
    w_hbm = [wq_hbm, wk_hbm, wv_hbm]

    def wtile(j):
        return w_p.at[j]

    SEM_X8, SEM_B0, SEM_LN, SEM_TK, SEM_WO, SEM_MLP = 0, 4, 7, 15, 16, 17

    def w_start(q0, n, sem):
        for q in range(q0, q0 + n):
            src = w_hbm[q // 16].bitcast(U32).at[:, q % 16, :]
            pltpu.make_async_copy(src, raw.at[q, pl.ds(0, D), :], sem_in.at[sem]).start()

    def w_wait(q0, n, sem):
        blk = raw.at[pl.ds(q0, n), pl.ds(0, D), :]
        pltpu.make_async_copy(blk, blk, sem_in.at[sem]).wait()

    def x8_copy(b):
        return pltpu.make_async_copy(x_hbm.at[pl.ds(b * 16, 16), pl.ds(LIVE, 8), :],
                                     x_v.at[pl.ds(1 + b * 16, 16), pl.ds(LIVE, 8), :], sem_in.at[SEM_X8 + b])

    def xa_copy(i):
        return pltpu.make_async_copy(x_hbm.at[pl.ds(i * 8, 8), pl.ds(0, LIVE), :],
                                     x_v.at[pl.ds(1 + i * 8, 8), pl.ds(0, LIVE), :], sem_in.at[SEM_LN + i])

    cp_wr = pltpu.make_async_copy(wr_hbm, wr_v, sem_in.at[SEM_B0 + 2])
    cp_mem = pltpu.make_async_copy(mem0_hbm, mem0_v, sem_in.at[SEM_TK])
    FP = FF // 3

    def mlp_copies(t):
        f0 = t * FP if isinstance(t, int) else pl.multiple_of(t * FP, 16)
        return [pltpu.make_async_copy(s_.at[pl.ds(f0, FP), :], d_.at[pl.ds(f0, FP), :], sem_in.at[SEM_MLP + t])
                for s_, d_ in [(wg_hbm, wg_v), (wu_hbm, wu_v), (wd_hbm, wd_v)]]

    wo_copies = [pltpu.make_async_copy(wo_hbm.bitcast(U32), wo_p, sem_in.at[SEM_WO])]

    for b in range(4):
        x8_copy(b).start()
    w_start(0, 1, SEM_B0)
    w_start(1, 1, SEM_B0 + 1)
    w_start(2, 2, SEM_B0 + 2)
    cp_wr.start()
    for i in range(8):
        w_start(4 + 4 * i, 4, SEM_LN + i)
        xa_copy(i).start()
    w_start(36, NPAIR - 36, SEM_TK)
    cp_mem.start()
    for t in range(3):
        for c in mlp_copies(t):
            c.start()
    for c in wo_copies:
        c.start()

    xb3 = xb_v.reshape(NSEG + 1, SEG, D)
    x_v[0] = jnp.zeros((SEG, D), BF16)
    xb3[0] = jnp.zeros((SEG, D), F32)
    keys[...] = jnp.full(keys.shape, KEY_NONE, F32)
    yacc[...] = jnp.zeros(yacc.shape, F32)
    kv_s[:, :, 0:8, :] = jnp.zeros((H, 2, 8, DH), F32)
    raw[NPAIR, 0:D, :] = jnp.zeros((D, 128), U32)
    acc[M:L, :] = jnp.zeros((SEG, D), F32)

    def router_w():
        wr5 = wr_v[...].astype(F32)
        return jnp.concatenate([wr5[j:j + 1, :] for j in range(NT)], axis=1)

    def layernorm(s0, nseg, t0, nrow, gate=None):
        n = nseg * nrow
        x = x_v[pl.ds(1 + s0, nseg), t0:t0 + nrow, :].astype(F32).reshape(n, D)
        if gate is not None:
            gv = jnp.concatenate([pltpu.bitcast(gate[1], F32)] * (n // 8), axis=0)
            x = jnp.concatenate([jnp.where(gate[0], gv, x[:, 0:128]), x[:, 128:]], axis=1)
        mu = jnp.sum(x, axis=-1, keepdims=True) * (1.0 / D)
        xc = x - mu
        var = jnp.sum(xc * xc, axis=-1, keepdims=True) * (1.0 / D)
        sd = _rb(jnp.sqrt(_rb(_rb(var) + EPS)))
        xn = _rb(_rb(x - _rb(mu)) / sd)
        xb3[pl.ds(1 + s0, nseg), t0:t0 + nrow, :] = xn.reshape(nseg, nrow, D)
        return xn

    def ln8_body(b, carry):
        x8_copy(b).wait()
        xn = layernorm(b * 16, 16, LIVE, 8)
        lhs_v[pl.ds(pl.multiple_of(b * 64, 64), 64), :] = pltpu.bitcast(xn.astype(BF16), U32)
        return carry

    jax.lax.fori_loop(0, 4, ln8_body, 0)

    def ln_seg(s, wr, gate):
        tail = xb3[1 + s, LIVE:SEG, :]
        xn = layernorm(s, 1, 0, LIVE, gate)
        xa_v[pl.ds(pl.multiple_of(s * LIVE, 8), LIVE), :] = xn
        r = _rb(jnp.sum(jnp.concatenate([xn, tail], axis=0) * wr, axis=-1, keepdims=True))
        r = jnp.where(r == 0.0, 0.0, r)
        bits = pltpu.bitcast(jnp.broadcast_to(r, (SEG, 128)), I32) >> 16
        mono = jnp.where(bits < 0, (-32768) - bits, bits)
        mono = jnp.where(r != r, -40000, mono)
        row = jax.lax.broadcasted_iota(I32, (SEG, 128), 0)
        key = (mono * SEG + ((SEG - 1) - row)).astype(F32)
        lane = jax.lax.broadcasted_iota(I32, (SEG, 128), 1)
        keys[...] = jnp.where(lane == s, key, keys[...])
        return pltpu.bitcast(key, U32)

    def top_rows():
        kv = keys[...]
        lane = jax.lax.broadcasted_iota(I32, (1, 128), 1).astype(F32)
        for c in range(TOPC):
            col = jnp.max(kv, axis=0, keepdims=True)
            val = jnp.floor(col * (1.0 / SEG))
            fk = val * 128.0 + (127.0 - lane)
            win = fk == jnp.max(fk, axis=1, keepdims=True)
            kv = jnp.where(win & (kv == col), KEY_NONE, kv)
            pos = lane * SEG + ((SEG - 1.0) - (col - val * SEG))
            idx = jnp.clip(jnp.max(jnp.where(win, pos, 0.0)).astype(I32), 0, S - 1)
            idx_s[c] = idx
            sel[pl.ds(c, 1), :] = xb_v[pl.ds(SEG + idx, 1), :]

    def repack(rv, wv, p, part=None, tie=None):
        m_lo = jnp.full((8, 128), 0xFFFF, U32)
        m_hi = jnp.full((8, 128), 0xFFFF0000, U32)
        if tie is not None:
            m_lo = jnp.where(tie[0], tie[1], m_lo)
            m_hi = jnp.where(tie[0], tie[1], m_hi)
        for g in range(D // 16):
            if part is not None and g % part[1] != part[0]:
                continue
            a = rv[p, pl.ds(16 * g, 8, stride=2), :]
            b = rv[p, pl.ds(16 * g + 1, 8, stride=2), :]
            wv[2 * p, 8 * g:8 * g + 8, :] = (a & m_lo) | (b << 16)
            wv[2 * p + 1, 8 * g:8 * g + 8, :] = (a >> 16) | (b & m_hi)

    def pack(x):
        return pltpu.bitcast(x.astype(BF16), U32)

    HR = NSEG * 4

    def xsums(k, tie):
        s1, s2 = 1 + 2 * k, 1 + 2 * k + NSEG // 2
        x1 = jnp.where(tie[0], tie[1], xb3[s1:s1 + 2, LIVE:SEG, 0:512].reshape(16, 512))
        x2 = jnp.where(tie[0], tie[1], xb3[s2:s2 + 2, LIVE:SEG, 0:512].reshape(16, 512))
        a11, a12, a21, a22 = x1[:, :256], x1[:, 256:], x2[:, :256], x2[:, 256:]
        for n_, y in enumerate((a11 + a22, a21 + a22, a11 + a12, a21 - a11, a12 - a22)):
            xs_v[n_, 8 * k:8 * k + 8, :] = pack(y)

    def block(q0, n, never=None):
        for u in range(2 * q0, 2 * q0 + 2 * n):
            if u % 2 == 0:
                repack(raw, w_p, u // 2 + 1)
            for c in range(4):
                r = _dot(pltpu.bitcast(lhs_v[c * 64:(c + 1) * 64, :], BF16), pltpu.bitcast(w_p[u], BF16))
                pre[u, c * 128:(c + 1) * 128, :] = r
                k = 4 * (u - 2 * q0) + c
                if never is not None and k < 8:
                    tv = jnp.concatenate([r[0:16, :]] * 4, axis=1)
                    xsums(2 * k, (never, tv))
                    xsums(2 * k + 1, (never, tv))

    def sblock(q0, n, never, side=None, jobs=None):
        rv = raw.at[pl.ds(q0, n + 1)]
        wv = w_p.at[pl.ds(2 * q0, 2 * n + 2)]
        pv = pre.at[pl.ds(2 * q0, 2 * n)]
        cnt = [0]
        pend = []
        tiles = [0]
        last = [None]

        def bits(r, r0):
            return pltpu.bitcast(r[r0:r0 + 8, :], U32)

        def mm(a, b, acc_=None):
            k = cnt[0]
            cnt[0] += 1
            if side is not None and k in LNS:
                pend.append(side(LNS.index(k), None if last[0] is None else (never, bits(last[0], 0))))
            if side is not None and k in LNT:
                tok = pend.pop(0)
                head = jnp.where(never, tok, a[0:SEG, 0:128])
                if a.shape[1] > 128:
                    head = jnp.concatenate([head, a[0:SEG, 128:]], axis=1)
                a = head if a.shape[0] == SEG else jnp.concatenate([head, a[SEG:, :]], axis=0)
            r = _dot(pltpu.bitcast(a, BF16), b)
            r = r if acc_ is None else acc_ + r
            tiles[0] += a.shape[1] // 128
            if jobs and tiles[0] % 4 == 0:
                for _ in range(JR[tiles[0] // 4 - 1]):
                    if jobs:
                        jobs.pop(0)()
            return r

        def gated(c):
            x = jnp.full((8, 128), c, U32)
            xs_ = [x if last[0] is None else jnp.where(never, bits(last[0], 32 * z), x) for z in range(8)]
            return jnp.concatenate([y for y in xs_ for _ in range(4)], axis=0)

        hp = HR // 2
        tails = {}
        for p in range(n):
            def wsum(t1, t2, sub=False):
                msk, sh = gated(0xFFFF0000), gated(16)

                def half(k, hi):
                    r = rv[p, 256 * k:256 * k + 256, :]
                    return pltpu.bitcast(r & msk if hi else r << sh, F32)
                a_, b_ = half(*t1), half(*t2)
                return (a_ - b_ if sub else a_ + b_).astype(BF16)

            def wt(pp, j, k0, k1):
                return pltpu.bitcast(wv[2 * pp + j, 64 * k0:64 * k1, :], BF16)

            def mark(k, r):
                last[0] = r
                if k < NPREP:
                    repack(rv, wv, p + 1, (k, NPREP), (never, bits(r, 0)))

            top5, bot5 = lhs_v[0:hp, 512:640], lhs_v[hp:2 * hp, 512:640]
            m2 = mm(xs_v[1], wt(p, 0, 0, 2))
            m5 = mm(xs_v[2], wt(p, 1, 2, 4))
            s4, s3 = wsum((1, 0), (0, 0), True), wsum((0, 1), (1, 1), True)
            mark(0, m2)
            m4 = mm(lhs_v[hp:2 * hp, 256:512], s4)
            m3 = mm(lhs_v[0:hp, 0:256], s3)
            s1 = wsum((0, 0), (1, 1))
            mark(1, m4)
            c21, c12 = m2 + m4, m3 + m5
            if p in tails:
                pv[2 * p, HR:2 * HR, :] = c21 + tails[p][0]
                pv[2 * p + 1, 0:HR, :] = c12 + tails[p][1]
            m1 = mm(xs_v[0], s1)
            c11 = mm(top5, wt(p, 0, 4, 5), (m4 - m5) + m1)
            c22 = mm(bot5, wt(p, 1, 4, 5), (m3 - m2) + m1)
            s7, s6 = wsum((1, 0), (1, 1)), wsum((0, 0), (0, 1))
            mark(2, m1)
            c11 = mm(xs_v[4], s7, c11)
            pv[2 * p, 0:HR, :] = c11
            pv[2 * p + 1, HR:2 * HR, :] = mm(xs_v[3], s6, c22)
            mark(3, c11)
            if p not in tails:
                pv[2 * p, HR:2 * HR, :] = mm(bot5, wt(p, 0, 4, 5), c21)
                pv[2 * p + 1, 0:HR, :] = mm(top5, wt(p, 1, 4, 5), c12)
                if p + 1 < n:
                    t_v[0] = mm(bot5, wt(p + 1, 0, 4, 5))
                    t_v[1] = mm(top5, wt(p + 1, 1, 4, 5))
                    tails[p + 1] = (t_v[0], t_v[1])

    idx_s[0] = 0
    w_wait(0, 1, SEM_B0)
    repack(raw, w_p, 0)
    w_wait(1, 1, SEM_B0 + 1)
    block(0, 1)
    w_wait(2, 2, SEM_B0 + 2)
    cp_wr.wait()
    block(1, 2, idx_s[0] < 0)

    def ln_body(i, carry):
        w_wait(4 + 4 * i, 4, SEM_LN + i)
        xa_copy(i).wait()
        wr = router_w()
        sblock(3 + 4 * i, 4, i < 0, side=lambda u, gate: ln_seg(i * 8 + u, wr, gate))
        return carry

    jax.lax.fori_loop(0, 8, ln_body, 0)

    w_wait(36, NPAIR - 36, SEM_TK)
    cp_mem.wait()
    acc[0:M, :] = mem0_v[...].astype(F32)
    nv = idx_s[0] < 0
    top_rows()
    sblock(35, 1, nv)

    def mlp_body(t, carry):
        for c in mlp_copies(t):
            c.wait()
        f0 = pl.multiple_of(t * FP, 16)
        xs = sel[...]
        cuts = [(a_, min(a_ + 128, FP)) for a_ in range(0, FP, 128)]
        val = {}

        def up_tile(which, n, kt):
            def run():
                a_, b_ = cuts[n]
                ws = [w_[pl.ds(f0 + a_, b_ - a_), kt * 128:(kt + 1) * 128] for w_ in (wg_v, wu_v)]
                w = ws[which] if which < 2 else jnp.concatenate(ws, axis=0)
                r = _dot_nt(xs[:, kt * 128:(kt + 1) * 128], w)
                val[which, n] = r if kt == 0 else val[which, n] + r
            return run

        def down_tile(n, j, first):
            def run():
                a_, b_ = cuts[n]
                if j == 0:
                    if (2, n) in val:
                        both = val.pop((2, n))
                        val[0, n], val[1, n] = both[:, :b_ - a_], both[:, b_ - a_:]
                    g_ = _rb(val.pop((0, n)))
                    val['h', n] = _rb(g_ * _sigmoid(g_)) * _rb(val.pop((1, n)))
                r = _dot(val['h', n], wd_v[pl.ds(f0 + a_, b_ - a_), j * 128:(j + 1) * 128])
                val['y', j] = r if first else val['y', j] + r
            return run

        nc = len(cuts)
        jobs = ([up_tile(2, nc - 1, kt) for kt in range(NT)]
                + [up_tile(which, n, kt) for n in range(nc - 1) for which in range(2) for kt in range(NT)]
                + [down_tile(n, j, n == nc - 1) for n in [nc - 1] + list(range(nc - 1)) for j in range(NT)])
        sblock(36 + 4 * t, 4, t < 0, jobs=jobs)
        assert not jobs
        y = yacc[...] + jnp.concatenate([val['y', j] for j in range(NT)], axis=1)
        yacc[...] = y
        r_sel = _rb(jnp.sum(xs * router_w(), axis=-1, keepdims=True))
        upd[...] = xs + _rb(_rb(y) * _rb(_sigmoid(r_sel)))
        for c in range(TOPC):
            xb_v[pl.ds(SEG + jnp.clip(idx_s[c], 0, S - 1), 1), :] = upd[pl.ds(c, 1), :]
        return carry

    jax.lax.fori_loop(0, 3, mlp_body, 0)

    for c in wo_copies:
        c.wait()

    scale = DH ** (-0.5)
    qm_i = jax.lax.broadcasted_iota(I32, (L - 8, L), 0)
    mask_m = (qm_i < M) | (qm_i + 8 >= jax.lax.broadcasted_iota(I32, (L - 8, L), 1))
    diag_ok = (jax.lax.broadcasted_iota(I32, (7, 8, DH), 1)
               > jax.lax.broadcasted_iota(I32, (7, 8, DH), 0))

    def finish(s0, n, u, sa):
        xb = xb3.at[pl.ds(s0, n)][u]
        o = x_v.at[pl.ds(s0, n)][u].astype(F32) + sa * (xb * _sigmoid(xb))
        out_v.at[pl.ds(s0, n)][u] = o.astype(BF16)
        return o

    def out_copy(seg, n):
        return pltpu.make_async_copy(out_v.at[pl.ds(seg + 1, n)], out_hbm.at[pl.ds(seg, n)], sem_out.at[0])

    def step(i, u, prev):
        pre_i = pre.at[:, pl.ds(pl.multiple_of(i * (8 * UNROLL), 8 * UNROLL), 8 * UNROLL), :]
        xa_i = xa_v.at[pl.ds(pl.multiple_of(i * (LIVE * UNROLL), 8 * UNROLL), LIVE * UNROLL), :]
        pre_s = pre_i.at[:, pl.ds(pl.multiple_of(u * 8, 8), 8), :]
        xa = xa_i[pl.ds(pl.multiple_of(u * LIVE, 8), LIVE), :]
        lhs = jnp.concatenate([prev[0:M, :], xa], axis=0).astype(BF16)
        fin = finish(pl.multiple_of(i * UNROLL, UNROLL), UNROLL, u, prev[M:L, :])

        @pl.when(u == UNROLL - 2)
        def _():
            out_copy(i * UNROLL, UNROLL - 2).start()

        def proj(j, tie=None):
            lh = lhs
            if tie is not None:
                top = pltpu.bitcast(lhs[0:16, 0:128], U32)
                top = pltpu.bitcast(jnp.where(i < 0, pltpu.bitcast(tie, U32), top), BF16)
                lh = jnp.concatenate([jnp.concatenate([top, lhs[0:16, 128:]], axis=1), lhs[16:, :]], axis=0)
            t = _dot(lh, pltpu.bitcast(wtile(j)[...], BF16))
            if TIE0 <= j < TIE0 + NT:
                t = jnp.where(jnp.logical_and(i < 0, u == 0),
                              fin[:, (j - TIE0) * 128:(j - TIE0 + 1) * 128], t)
            return jnp.concatenate([t, pre_s[j]], axis=0)

        NG = H // GH
        qs, ks, vs, ps, os_, ox, iv, on = {}, {}, {}, {}, {}, {}, {}, {}

        def do_qkv(g):
            js = [(x % 3) * H + g * GH + x // 3 for x in ORD]
            if g == 0:
                part = {}
                for kt in range(NT):
                    for j in js:
                        t = _dot(lhs[:, kt * 128:(kt + 1) * 128],
                                 pltpu.bitcast(wtile(j)[kt * 64:(kt + 1) * 64, :], BF16))
                        part[j] = t if kt == 0 else part[j] + t
                res = {j: jnp.concatenate([part[j], pre_s[j]], axis=0) for j in js}
            else:
                res = {}
                for n, j in enumerate(js):
                    tie = None
                    for hh, pos in enumerate(TP):
                        if n == pos and g >= TL:
                            tie = ox[(g - TL) * GH + hh]
                    res[j] = proj(j, tie)
            for h in range(g * GH, (g + 1) * GH):
                qs[h], ks[h], vs[h] = res[h], res[H + h], res[2 * H + h]

        def vpu_rows(h, q, k, v):
            def win(which, val, r):
                if r % 8 == 0:
                    return val[8 - r:16 - r, :]
                return kv_s[h, which, 16 - r:24 - r, :]

            def wins(which, val):
                return jnp.stack([win(which, val, r) for r in range(16)])

            def fold(f, x):
                while x.shape[0] > 1:
                    n = x.shape[0] // 2
                    x = f(x[:n], x[n:])
                return x[0]

            qa = q[8:16, :] * (scale * LOG2E)
            sc = jnp.sum(qa[None] * wins(0, k), axis=-1, keepdims=True)
            sc = jnp.broadcast_to(sc, (16, 8, DH))
            sc = jnp.concatenate([sc[:9], jnp.where(diag_ok, sc[9:], -jnp.inf)], axis=0)
            e = jnp.exp2(sc - fold(jnp.maximum, sc)[None])
            return fold(jnp.add, e * wins(1, v)) * pl.reciprocal(fold(jnp.add, e), approx=True)

        def do_s(g):
            for h in range(g * GH, (g + 1) * GH):
                q, k = qs.pop(h), ks.pop(h)
                kv_s[h, 0, 8:24, :] = k[0:16, :]
                kv_s[h, 1, 8:24, :] = vs[h][0:16, :]
                ox[h] = vpu_rows(h, q, k, vs[h])
                qm = jnp.concatenate([q[0:8, :], q[16:, :]], axis=0)
                sc = _dot_nt(qm.astype(BF16), k.astype(BF16))
                sc = jnp.where(mask_m, sc * (scale * LOG2E), NEG * LOG2E)
                e = jnp.exp2(sc - jnp.max(sc, axis=-1, keepdims=True))
                inv = pl.reciprocal(jnp.sum(e, axis=-1, keepdims=True), approx=True)
                ps[h] = e.astype(BF16)
                iv[h] = jnp.broadcast_to(inv, (SEG, DH))

        def do_pv(g):
            for h in range(g * GH, (g + 1) * GH):
                v = vs.pop(h)
                if g >= NG - TL:
                    v = jnp.concatenate([jnp.where(i < 0, ox[h], v[0:8, :]), v[8:, :]], axis=0)
                if h >= GH:
                    v = jnp.concatenate([v[0:8, :], jnp.where(i < 0, on[h - GH], v[8:, :])], axis=0)
                on[h] = _dot(ps.pop(h), v.astype(BF16)) * iv.pop(h)
                os_[h] = jnp.concatenate([on[h][0:8, :], ox[h], on[h][8:, :]], axis=0)

        def do_o(j, h0, h1):
            o = jnp.concatenate([os_[h] for h in range(h0, h1)], axis=1)
            return _dot(o, pltpu.bitcast(wo_p[h0 * 64:h1 * 64, j * 128:(j + 1) * 128], BF16))

        for g in range(NG):
            do_qkv(g)
            if g >= LS:
                do_s(g - LS)
            if g >= LP:
                do_pv(g - LP)
        sched = dict(TAIL)
        ns, npv = NG - LS, NG - LP
        for j in range(NT):
            part_v[:, j * 128:(j + 1) * 128] = do_o(j, 0, HS)
            for c_ in sched.get(j, ''):
                if c_ == 's':
                    do_s(ns)
                    ns += 1
                else:
                    do_pv(npv)
                    npv += 1
        assert ns == NG and npv == NG
        return jnp.concatenate(
            [part_v[:, j * 128:(j + 1) * 128] + do_o(j, HS, H) for j in range(NT)], axis=1)

    def multi(i, carry):
        acc[...] = jax.lax.fori_loop(0, UNROLL, lambda u, cur: step(i, u, cur), acc[...],
                                     unroll=True)
        out_copy(i * UNROLL + UNROLL - 2, 1).start()

        @pl.when(i > 0)
        def _():
            out_copy(jnp.maximum(i * UNROLL - 1, 0), 1).start()
        return carry

    jax.lax.fori_loop(0, NSEG // UNROLL, multi, 0)
    finish(NSEG, 1, 0, acc[M:L, :])
    out_copy(NSEG - 1, 1).start()
    out_copy(0, NSEG).wait()


@jax.jit
def pallas_recurrent_scan__memory_aug_recurrent_mem_tr__moe_arch_mod__prompt_kernel(
    A_x: jax.Array,
    A_mem0: jax.Array,
    A_Wq: jax.Array,
    A_Wk: jax.Array,
    A_Wv: jax.Array,
    A_Wo: jax.Array,
    A_seg_len: jax.Array,
    B_x: jax.Array,
    B_w_r: jax.Array,
    B_w_gate: jax.Array,
    B_w_up: jax.Array,
    B_w_down: jax.Array,
):
    del A_seg_len, B_x
    assert A_x.shape == (1, S, D) and A_Wq.shape == (D, H, DH) and A_mem0.shape == (1, M, D)
    hbm = pl.BlockSpec(memory_space=pltpu.HBM)
    out = pl.pallas_call(
        _kernel,
        out_shape=jax.ShapeDtypeStruct((NSEG, SEG, D), BF16),
        in_specs=[hbm] * 10,
        out_specs=hbm,
        scratch_shapes=[
            pltpu.VMEM((NSEG + 2, SEG, D), BF16),
            pltpu.VMEM((NSEG * 4, D), U32),
            pltpu.VMEM((5, 128, 256), U32),
            pltpu.VMEM((NSEG * LIVE, D), F32),
            pltpu.VMEM((S + SEG, D), F32),
            pltpu.VMEM((NPAIR + 1, D + 32, 128), U32),
            pltpu.VMEM((2 * NPAIR + 2, D // 2, 128), U32),
            pltpu.VMEM((H * DH // 2, D), U32),
            pltpu.VMEM((3 * H, NSEG * 8, DH), F32),
            pltpu.VMEM((FF, D), BF16),
            pltpu.VMEM((FF, D), BF16),
            pltpu.VMEM((FF, D), BF16),
            pltpu.VMEM((NSEG + 2, SEG, D), BF16),
            pltpu.VMEM((2, 256, DH), F32),
            pltpu.VMEM((L, D), F32),
            pltpu.VMEM((L, D), F32),
            pltpu.VMEM((H, 2, 24, DH), F32),
            pltpu.VMEM((TOPC, D), F32),
            pltpu.VMEM((TOPC, D), F32),
            pltpu.VMEM((TOPC, D), F32),
            pltpu.VMEM((SEG, 128), F32),
            pltpu.VMEM((M, D), BF16),
            pltpu.VMEM((NT, 128), BF16),
            pltpu.SMEM((TOPC,), I32),
            pltpu.SemaphoreType.DMA((20,)),
            pltpu.SemaphoreType.DMA((1,)),
        ],
        compiler_params=pltpu.CompilerParams(vmem_limit_bytes=110 * 1024 * 1024),
    )(
        A_x.reshape(NSEG, SEG, D),
        A_mem0.reshape(M, D),
        A_Wq, A_Wk, A_Wv,
        A_Wo.reshape(H * DH, D),
        B_w_r.reshape(NT, 128),
        B_w_gate.T, B_w_up.T, B_w_down,
    )
    return out.reshape(1, S, D)
```
